```python
import jax
import jax.numpy as jnp

def _softmax(x, axis=-1):
    return jax.nn.softmax(x, axis=axis)

def _gelu(x):
    return jax.nn.gelu(x, approximate=True)

def _silu(x):
    return jax.nn.silu(x)

def _sigmoid(x):
    return jax.nn.sigmoid(x)

def _layernorm(x, axis=-1, eps=1e-05):
    m = jnp.mean(x, axis=axis, keepdims=True)
    v = jnp.var(x, axis=axis, keepdims=True)
    return (x - m) / jnp.sqrt(v + eps)

def _scatter_add(tgt, idx, src, axis=0):
    return tgt.at[idx].add(src)

def _segment_sum(src, seg, n):
    return jax.ops.segment_sum(src, seg, n)

class _Rng:

    def __init__(self, key):
        self._k = key

    def _next(self):
        self._k, sub = jax.random.split(self._k)
        return sub

    def normal(self, shape):
        return jax.random.normal(self._next(), shape, dtype=jnp.bfloat16)

    def randint(self, lo, hi, shape):
        return jax.random.randint(self._next(), shape, lo, hi, dtype=jnp.int32)

    def uniform(self, shape, lo=0.0, hi=1.0):
        return jax.random.uniform(self._next(), shape, jnp.bfloat16, lo, hi)

    def permutation(self, n):
        return jax.random.permutation(self._next(), n)
kernel_name = 'gated_mix__memory_aug_recurrent_mem_tr__spectral_gfnet__prompt'

def setup_inputs():
    _rng = _Rng(jax.random.key(int.from_bytes(__import__("os").urandom(4), "little")))
    _w = lambda a: (lambda t: t.astype(jnp.bfloat16) if jnp.issubdtype(t.dtype, jnp.floating) else t)(jnp.asarray(a))

    def _A_setup():
        B, S, Dm = (1, 2048, 1024)
        H, Dh = (32, 128)
        M, seg = (8, 32)
        seg = min(seg, S)
        S = S // seg * seg
        return {'x': _w((lambda *s: _rng.normal(s) * 0.05)(B, S, Dm)), 'mem0': _w((lambda *s: _rng.normal(s) * 0.05)(B, M, Dm)), 'Wq': _w((lambda *s: _rng.normal(s) * 0.05)(Dm, H, Dh) * Dm ** (-0.5)), 'Wk': _w((lambda *s: _rng.normal(s) * 0.05)(Dm, H, Dh) * Dm ** (-0.5)), 'Wv': _w((lambda *s: _rng.normal(s) * 0.05)(Dm, H, Dh) * Dm ** (-0.5)), 'Wo': _w((lambda *s: _rng.normal(s) * 0.05)(H, Dh, Dm) * (H * Dh) ** (-0.5)), 'seg_len': seg}
    _A_in = _A_setup()

    def _B_setup():
        B, S, D = (1, 2048, 1024)
        Df = D // 2 + 1
        return {'x': _w((lambda *s: _rng.normal(s) * 0.05)(B, S, D)), 'w_r': _w((lambda *s: _rng.normal(s) * 0.05)(S, Df) * 0.02), 'w_i': _w((lambda *s: _rng.normal(s) * 0.05)(S, Df) * 0.02)}
    _B_in = _B_setup()
    return {'A_x': _A_in['x'], 'A_mem0': _A_in['mem0'], 'A_Wq': _A_in['Wq'], 'A_Wk': _A_in['Wk'], 'A_Wv': _A_in['Wv'], 'A_Wo': _A_in['Wo'], 'A_seg_len': _A_in['seg_len'], 'B_x': _B_in['x'], 'B_w_r': _B_in['w_r'], 'B_w_i': _B_in['w_i'], 'gate_w': _w((lambda *s: _rng.normal(s) * 0.05)(1024))}

def reference(A_x, A_mem0, A_Wq, A_Wk, A_Wv, A_Wo, A_seg_len, B_x, B_w_r, B_w_i, gate_w):

    def _A_ref(x, mem0, Wq, Wk, Wv, Wo, seg_len):
        B, S, Dm = x.shape
        H, Dh = (Wq.shape[1], Wq.shape[2])
        M = mem0.shape[1]
        scale = Dh ** (-0.5)
        n_seg = S // seg_len
        L = M + seg_len
        idx = jnp.arange(L)
        mask = (idx[:, None] < M) | (idx[:, None] >= idx[None, :])
        mem = mem0
        outs = []
        for s in range(n_seg):
            xs = x[:, s * seg_len:(s + 1) * seg_len, :].copy()
            h = jnp.concatenate([mem, xs], axis=1)
            q = jnp.einsum('btd,dhe->bhte', h, Wq)
            k = jnp.einsum('btd,dhe->bhte', h, Wk)
            v = jnp.einsum('btd,dhe->bhte', h, Wv)
            scores = jnp.einsum('bhqe,bhke->bhqk', q, k) * scale
            scores = jnp.where(mask[None, None], scores, -1000000000.0)
            p = _softmax(scores, axis=-1)
            o = jnp.einsum('bhqk,bhke->bhqe', p, v)
            o = jnp.einsum('bhte,hed->btd', o, Wo)
            mem = o[:, :M, :].copy()
            outs.append(o[:, M:, :])
        return jnp.concatenate(outs, axis=1)

    def _B_ref(x, w_r, w_i):
        B, S, D = x.shape
        X = (lambda x, axes=(-2, -1): jnp.fft.rfft2(x.astype(jnp.float32), axes=axes))(x, axes=(-2, -1))
        W = w_r + 1j * w_i
        X = X * W
        y = (lambda x, s, axes=(-2, -1): jnp.fft.irfft2(x, s=s, axes=axes).astype(jnp.bfloat16))(X, (S, D), axes=(-2, -1))
        return y
    x = A_x
    g = _sigmoid((x * gate_w).sum(-1, keepdims=True))
    a = _A_ref(x, A_mem0, A_Wq, A_Wk, A_Wv, A_Wo, A_seg_len)
    b = _B_ref(x, B_w_r, B_w_i)
    return g * a + (1 - g) * b
```

```python
import functools
import math

import numpy as np
import jax
import jax.numpy as jnp
from jax import lax
import jax.experimental.pallas as pl
import jax.experimental.pallas.tpu as pltpu

BF, F32, U32 = jnp.bfloat16, jnp.float32, jnp.uint32

S, D, H, DH, M, SEG = 2048, 1024, 32, 128, 8, 32
NSEG = S // SEG
NP = H // 2
N1, N2 = 16, 128
NG = 5
LAG1, LAG2, SPLIT = 1, 3, 26
RSQ2 = float(np.float32(math.sqrt(0.5)))


def _to_bf16_bits(a):
    u = np.ascontiguousarray(a, dtype=np.float32).view(np.uint32)
    return ((u + 0x7FFF + ((u >> 16) & 1)) >> 16).astype(np.uint32)


def _pack_rows(a):
    b = _to_bf16_bits(a)
    return (b[..., 0::2, :] | (b[..., 1::2, :] << 16)).astype(np.uint32)


def _lane_groups(blocks, roll, where, lane):
    r = [blocks[0]] + [roll(blocks[b], b) for b in range(1, 4)]
    t = []
    for c in range(4):
        m = (lane - c) & 3
        t.append(where(m == 0, r[0], where(m == 1, r[1], where(m == 2, r[2], r[3]))))
    t3 = roll(t[3], 126)
    sel = ((lane - 1) & 7) < 4
    return [t[0], where(sel, t[1], t3), t[2], where(sel, t3, t[1])]


def _bfly8(x):
    s = [x[i] + x[i + 4] for i in range(4)]
    d = [x[i] - x[i + 4] for i in range(4)]
    e, f = s[0] + s[2], s[1] + s[3]
    t1, t2 = (d[1] - d[3]) * RSQ2, (d[1] + d[3]) * RSQ2
    return [e + f, e - f, d[0] + t1, t2 + d[2], s[0] - s[2], s[1] - s[3], d[0] - t1, t2 - d[2]]


def _bfly8_t(t):
    e, f = t[0] + t[1], t[0] - t[1]
    s = [e + t[4], f + t[5], e - t[4], f - t[5]]
    t1, t2 = t[2] - t[6], t[3] + t[7]
    d = [t[2] + t[6], (t1 + t2) * RSQ2, t[3] - t[7], (t2 - t1) * RSQ2]
    return [s[i] + d[i] for i in range(4)] + [s[i] - d[i] for i in range(4)]


@functools.lru_cache(maxsize=None)
def _constants():
    lane = np.arange(128)
    k2 = np.stack(_lane_groups([128 * b + lane for b in range(4)], np.roll, np.where, lane))
    n2 = np.arange(D)
    ang = 2 * np.pi * ((k2[:, :, None] * n2[None, None, :]) % D) / D
    rows = np.stack([np.cos(ang), -np.sin(ang)], axis=1)
    assert k2[0, 0] == 0
    rows[0, 1, 0] = np.cos(np.pi * n2)
    wgt = np.full((4, 2, 128), 2.0)
    wgt[0, :, 0] = 1.0
    fwd = rows.reshape(D, D).T
    inv = (rows * wgt[..., None]).reshape(D, D) / (S * D)
    bf = np.stack(_bfly8(list(np.eye(8))))
    binv = np.kron(np.linalg.inv(bf), np.eye(128))
    gfull = binv.T @ fwd
    ifull = inv @ binv
    gd = np.stack([gfull[256 * g:256 * g + 256, 256 * g:256 * g + 256] for g in range(4)])
    gdi = np.stack([ifull[256 * g:256 * g + 256, 256 * g:256 * g + 256] for g in range(4)])
    blk = np.kron(np.eye(4), np.ones((256, 256)))
    assert np.abs(gfull * (1 - blk)).max() < 1e-6 and np.abs(ifull * (1 - blk)).max() < 1e-12

    b = np.arange(N2)
    k1 = np.arange(N1)[:, None] + N1 * np.arange(N2)[None, :]
    th = 2 * np.pi * ((k1[:, :, None] * b[None, None, :]) % S) / S
    gr, gi = np.cos(th), -np.sin(th)
    full = np.block([[gr, -gi], [gi, gr]])
    kap = np.arange(2 * N2)
    src = ((kap >> 3) & 1) * N2 + (kap >> 4) * 8 + (kap & 7)
    gs = full[:, :, src]
    hr, hi = np.swapaxes(gr, 1, 2), -np.swapaxes(gi, 1, 2)
    gsi = np.block([[hr, -hi], [hi, hr]])
    gdp = _pack_rows(np.stack([gd, gdi]))
    gsp = _pack_rows(np.stack([gs, gsi]))
    return gdp, gsp


def _cmul_const(v, k, n, sign):
    re, im = v
    k %= n
    if k == 0:
        return re, im
    if 4 * k == n:
        return (-im, re) if sign > 0 else (im, -re)
    if 8 * k == n:
        return (((re - im) * RSQ2, (re + im) * RSQ2) if sign > 0
                else ((re + im) * RSQ2, (im - re) * RSQ2))
    if 8 * k == 3 * n:
        return (((re + im) * -RSQ2, (re - im) * RSQ2) if sign > 0
                else ((im - re) * RSQ2, (re + im) * -RSQ2))
    c, s = math.cos(2 * math.pi * k / n), sign * math.sin(2 * math.pi * k / n)
    return re * c - im * s, re * s + im * c


def _fft(v, sign):
    n = len(v)
    if n == 1:
        return v
    ev, od = _fft(v[0::2], sign), _fft(v[1::2], sign)
    lo, hi = [], []
    for k in range(n // 2):
        er, ei = ev[k]
        if 4 * k == n:
            xr, xi = od[k]
            if sign > 0:
                lo.append((er - xi, ei + xr)); hi.append((er + xi, ei - xr))
            else:
                lo.append((er + xi, ei - xr)); hi.append((er - xi, ei + xr))
            continue
        tr, ti = _cmul_const(od[k], k, n, sign)
        lo.append((er + tr, ei + ti))
        hi.append((er - tr, ei - ti))
    return lo + hi


def _mask80():
    r = lax.broadcasted_iota(jnp.int32, (80, 80), 0)
    c = lax.broadcasted_iota(jnp.int32, (80, 80), 1)

    def head(i):
        return jnp.where(i < 64, i >> 5, (i - 64) >> 3)

    def pos(i):
        j = i & 31
        return jnp.where(i < 64, jnp.where(j < M, j, j + 8), M + (i & 7))

    same = head(r) == head(c)
    ok = (pos(r) < M) | (pos(c) <= pos(r))
    return same & ok, jnp.where(same, -1e9, -jnp.inf).astype(F32)


def _as_bf(u):
    return pltpu.bitcast(u, BF)


def _as_u32(b):
    return pltpu.bitcast(b, U32)


def _dot(a, b):
    return jnp.dot(a, b, preferred_element_type=F32)


def _kernel(x_hbm, mem_ref, wq_hbm, wk_hbm, wv_hbm, wo_hbm, fr_hbm, fi_hbm, gw_ref, gd_hbm, gs_hbm,
            out_hbm,
            x_v, raw, wqkv, wo, st, sto, obuf, xb, fraw, fp, gd, gs, y, u_s, p_s, out_v, sem):
    cp_x = pltpu.make_async_copy(x_hbm, x_v, sem.at[0])
    cp_gd = pltpu.make_async_copy(gd_hbm, gd, sem.at[1])
    cp_w = [pltpu.make_async_copy(w.bitcast(U32), raw.at[m], sem.at[2 + m])
            for m, w in enumerate((wq_hbm, wk_hbm, wv_hbm))]
    cp_f = [pltpu.make_async_copy(f, fraw.at[i], sem.at[5 + i]) for i, f in enumerate((fr_hbm, fi_hbm))]
    cp_gs = pltpu.make_async_copy(gs_hbm, gs, sem.at[7])
    cp_wo = [pltpu.make_async_copy(wo_hbm.bitcast(U32).at[:, pl.ds(128 * j, 128)], wo.at[j], sem.at[8 + j])
             for j in range(8)]
    for c in [cp_gd, cp_x, cp_w[0]] + cp_f + [cp_gs, cp_w[1], cp_w[2]] + cp_wo:
        c.start()

    lane = lax.broadcasted_iota(jnp.int32, (8, 128), 1)

    cp_gd.wait()
    cp_x.wait()
    RB = 128

    def f1(i, c):
        base = pl.multiple_of(i * RB, RB)
        pieces = []
        for r in range(0, RB, 16):
            xs = x_v[pl.ds(base + r, 16), :].astype(F32)
            us = _bfly8([xs[:, 128 * a:128 * a + 128] for a in range(8)])
            pieces.append(jnp.concatenate(us, axis=1).astype(BF))
        ub = jnp.concatenate(pieces, axis=0)
        lane0 = lax.broadcasted_iota(jnp.int32, (RB, 128), 1) == 0
        for g in range(4):
            yy = _dot(ub[:, 256 * g:256 * g + 256], _as_bf(gd[0, g]))
            yr, yi = yy[:, :128], yy[:, 128:]
            if g == 0:
                y[4, 0, pl.ds(base, RB), :] = jnp.where(lane0, yi, 0.0)
                y[4, 1, pl.ds(base, RB), :] = jnp.zeros((RB, 128), F32)
                yi = jnp.where(lane0, 0.0, yi)
            y[g, 0, pl.ds(base, RB), :] = yr
            y[g, 1, pl.ds(base, RB), :] = yi
        return c

    lax.fori_loop(0, S // RB, f1, 0)

    for s2 in range(NSEG // 2):
        rows = jnp.concatenate([x_v[64 * s2:64 * s2 + 16, :].astype(F32)[0:8],
                                x_v[64 * s2 + 32:64 * s2 + 48, :].astype(F32)[0:8]], axis=0)
        xb[8 * s2:8 * s2 + 8, :] = _as_u32(rows.astype(BF))

    def relayout(m, j):
        for d0 in range(0, D, 64):
            a = raw[m, pl.ds(d0 * 16 + j, 64, stride=16), :]
            lo = pltpu.bitcast(a << 16, F32).astype(BF)
            hi = pltpu.bitcast(a & jnp.uint32(0xFFFF0000), F32).astype(BF)
            wqkv[m, 2 * j, d0 // 2:d0 // 2 + 32, :] = _as_u32(lo)
            wqkv[m, 2 * j + 1, d0 // 2:d0 // 2 + 32, :] = _as_u32(hi)

    BM = 256

    def bulk(m, j):
        for c0 in range(0, 8 * NSEG, BM):
            lhs = _as_bf(xb[c0 // 2:(c0 + BM) // 2, :])
            r1 = _dot(lhs, _as_bf(wqkv[m, 2 * j])).reshape(BM // 8, 8, 128)
            r2 = _dot(lhs, _as_bf(wqkv[m, 2 * j + 1])).reshape(BM // 8, 8, 128)
            r = jnp.concatenate([r1, r2], axis=1).reshape(BM * 2, 128).astype(BF)
            st[m, j, c0:c0 + BM, :] = _as_u32(r)

    def proj_phase(m):
        cp_w[m].wait()

        def rl(j, c):
            relayout(m, j)
            return c

        lax.fori_loop(0, NP, rl, 0)

        def bk(j, c):
            bulk(m, j)
            return c

        lax.fori_loop(0, NP, bk, 0)

    proj_phase(0)

    for c in cp_f:
        c.wait()
    FB = 64

    def fprep(i, c):
        base = pl.multiple_of(i * FB, FB)
        hb = pl.multiple_of(i * (FB // 2), FB // 2)
        ln = lax.broadcasted_iota(jnp.int32, (FB // 2, 128), 1)
        for a in range(2):
            blocks = [_as_u32(fraw[a, pl.ds(base, FB), 128 * b:128 * b + 128]) for b in range(4)]
            grp = _lane_groups(blocks, lambda v, s: pltpu.roll(v, s, 1), jnp.where, ln)
            for g in range(4):
                fp[a, g, pl.ds(hb, FB // 2), :] = grp[g]
            nyq = fraw[a, pl.ds(base, FB), 512:513].astype(F32)
            fp[a, 4, pl.ds(hb, FB // 2), :] = _as_u32(jnp.broadcast_to(nyq, (FB, 128)).astype(BF))
        return c

    lax.fori_loop(0, S // FB, fprep, 0)

    cp_gs.wait()

    def s_stage(g, c):
        def fwd(i, c2):
            r = pl.multiple_of(i * 8, 8)
            v = [(y[g, 0, pl.ds(N2 * a + r, 8), :], y[g, 1, pl.ds(N2 * a + r, 8), :]) for a in range(N1)]
            v = _fft(v, -1)
            for ka in range(N1):
                u_s[ka, pl.ds(r, 8), :] = _as_u32(jnp.concatenate(v[ka], axis=0).astype(BF))
            return c2

        lax.fori_loop(0, N2 // 8, fwd, 0)

        def mid(jj, c2):
            w32 = [fp[a, g, pl.ds(jj, N2, stride=N1 // 2), :] for a in range(2)]
            xs = [_dot(_as_bf(gs[0, 2 * jj + p]), _as_bf(u_s[2 * jj + p])) for p in range(2)]
            for p in range(2):
                if p == 0:
                    wr, wi = [pltpu.bitcast(w << 16, F32) for w in w32]
                else:
                    wr, wi = [pltpu.bitcast(w & jnp.uint32(0xFFFF0000), F32) for w in w32]
                xr, xi = xs[p][:N2], xs[p][N2:]
                z = jnp.concatenate([xr * wr - xi * wi, xr * wi + xi * wr], axis=0).astype(BF)
                p_s[2 * jj + p] = _dot(_as_bf(gs[1, 2 * jj + p]), z)
            return c2

        lax.fori_loop(0, N1 // 2, mid, 0)

        def bwd(i, c2):
            r = pl.multiple_of(i * 8, 8)
            v = [(p_s[ka, pl.ds(r, 8), :], p_s[ka, pl.ds(N2 + r, 8), :]) for ka in range(N1)]
            v = _fft(v, 1)
            for a in range(N1):
                y[g, 0, pl.ds(N2 * a + r, 8), :] = v[a][0]
                y[g, 1, pl.ds(N2 * a + r, 8), :] = v[a][1]
            return c2

        lax.fori_loop(0, N2 // 8, bwd, 0)
        return c

    lax.fori_loop(0, NG, s_stage, 0)

    proj_phase(1)
    proj_phase(2)
    for c in cp_wo:
        c.wait()

    scale = DH ** -0.5

    def softmax(s, mask, fill):
        s = jnp.where(mask, s * scale, fill)
        m = jnp.max(s, axis=-1, keepdims=True)
        e = jnp.exp(s - m)
        l = jnp.sum(e, axis=-1, keepdims=True)
        return (e * (1.0 / l)).astype(BF)

    def step(a, seg, first, mask, fill):
        R = 32 if first else 48
        qkv, ps = {}, {}
        srow = pl.multiple_of(seg * 8, 8)

        def proj(j):
            res = []
            for m in range(3):
                r1 = _dot(a, _as_bf(wqkv[m, 2 * j])).astype(BF)
                r2 = _dot(a, _as_bf(wqkv[m, 2 * j + 1])).astype(BF)
                res.append(jnp.concatenate([r1, r2, _as_bf(st[m, j, pl.ds(srow, 8), :])], axis=0))
            qkv[j] = res

        def scores(j):
            s = lax.dot_general(qkv[j][0], qkv[j][1], (((1,), (1,)), ((), ())), preferred_element_type=F32)
            ps[j] = softmax(s, mask, fill)

        def pv(j):
            o = _dot(ps[j], qkv[j][2])
            for i in range(2):
                h = 2 * j + i
                if first:
                    ob = o[32 * i:32 * i + 32].astype(BF)
                    sto[h] = o[64 + 8 * i:72 + 8 * i]
                else:
                    ob = jnp.concatenate([o[32 * i:32 * i + 32], o[64 + 8 * i:72 + 8 * i], sto[h]],
                                         axis=0).astype(BF)
                obuf[h, 0:R // 2, :] = _as_u32(ob)

        def wo_part(j, h0, h1):
            og = jnp.concatenate([_as_bf(obuf[h, 0:R // 2, :]) for h in range(h0, h1)], axis=1)
            return _dot(og, _as_bf(wo[j, h0 * 64:h1 * 64, :]))

        parts = []
        for i in range(NP + 4):
            if i < NP:
                proj(i)
            else:
                parts.append(wo_part(2 * (i - NP), 0, SPLIT))
                parts.append(wo_part(2 * (i - NP) + 1, 0, SPLIT))
            if 0 <= i - LAG1 < NP:
                scores(i - LAG1)
            if 0 <= i - LAG2 < NP:
                pv(i - LAG2)
        return jnp.concatenate([wo_part(j, SPLIT, H) + parts[j] for j in range(8)], axis=1)

    def pair(t, mem):
        mask, fill = _mask80()
        base = pl.multiple_of(t * 64, 64)
        lane0 = lax.broadcasted_iota(jnp.int32, (64, 128), 1) == 0
        ts = []
        for g in range(4):
            vr = y[g, 0, pl.ds(base, 64), :]
            vi = y[g, 1, pl.ds(base, 64), :]
            if g == 0:
                vi = jnp.where(lane0, y[4, 0, pl.ds(base, 64), :], vi)
            tt = _dot(jnp.concatenate([vr, vi], axis=1).astype(BF), _as_bf(gd[1, g]))
            ts += [tt[:, :128], tt[:, 128:]]
        b = jnp.concatenate(_bfly8_t(ts), axis=1).astype(BF).astype(F32)

        xs = x_v[pl.ds(base, 64), :].astype(F32)
        gate = jax.nn.sigmoid(jnp.sum(xs * gw_ref[...].astype(F32), axis=-1, keepdims=True))
        a = jnp.concatenate([mem, xs[8:32]], axis=0).astype(BF)
        res_a = step(a, 2 * t, True, mask, fill)
        mem = res_a[0:8].astype(BF).astype(F32)
        a = jnp.concatenate([mem, xs[40:64]], axis=0).astype(BF)
        res_b = step(a, 2 * t + 1, False, mask, fill)
        mem = res_b[0:8].astype(BF).astype(F32)
        res = jnp.concatenate([res_b[40:48], res_a[8:32], res_b[32:40], res_b[8:32]], axis=0)
        out_v[pl.ds(base, 64), :] = (gate * res + (1.0 - gate) * b).astype(BF)
        pltpu.make_async_copy(out_v.at[pl.ds(base, 64), :], out_hbm.at[pl.ds(base, 64), :], sem.at[16]).start()
        return mem

    lax.fori_loop(0, S // 64, pair, mem_ref[...].astype(F32))
    pltpu.make_async_copy(out_v, out_hbm, sem.at[16]).wait()


@functools.partial(jax.jit, static_argnames=("A_seg_len",))
def pallas_gated_mix__memory_aug_recurrent_mem_tr__spectral_gfnet__prompt_kernel(
    A_x, A_mem0, A_Wq, A_Wk, A_Wv, A_Wo, A_seg_len, B_x, B_w_r, B_w_i, gate_w,
):
    assert A_x.shape == (1, S, D) and A_mem0.shape == (1, M, D) and A_Wq.shape == (D, H, DH)
    assert int(A_seg_len) == SEG
    gdp, gsp = _constants()
    any_spec = pl.BlockSpec(memory_space=pl.ANY)
    vmem_spec = pl.BlockSpec(memory_space=pltpu.VMEM)
    out = pl.pallas_call(
        _kernel,
        out_shape=jax.ShapeDtypeStruct((S, D), BF),
        in_specs=[any_spec, vmem_spec, any_spec, any_spec, any_spec, any_spec, any_spec, any_spec,
                  vmem_spec, any_spec, any_spec],
        out_specs=any_spec,
        scratch_shapes=[
            pltpu.VMEM((S, D), BF),
            pltpu.VMEM((3, D * H // 2, DH), U32),
            pltpu.VMEM((3, H, D // 2, DH), U32),
            pltpu.VMEM((8, H * DH // 2, 128), U32),
            pltpu.VMEM((3, NP, 8 * NSEG, 128), U32),
            pltpu.VMEM((H, 8, 128), F32),
            pltpu.VMEM((H, 24, 128), U32),
            pltpu.VMEM((4 * NSEG, D), U32),
            pltpu.VMEM((2, S, D // 2 + 1), BF),
            pltpu.VMEM((2, NG, S // 2, 128), U32),
            pltpu.VMEM((2, 4, 128, 256), U32),
            pltpu.VMEM((2, N1, N2, 2 * N2), U32),
            pltpu.VMEM((NG, 2, S, 128), F32),
            pltpu.VMEM((N1, N2, 128), U32),
            pltpu.VMEM((N1, 2 * N2, 128), F32),
            pltpu.VMEM((S, D), BF),
            pltpu.SemaphoreType.DMA((17,)),
        ],
        compiler_params=pltpu.CompilerParams(vmem_limit_bytes=120 * 1024 * 1024),
    )(
        A_x.reshape(S, D), A_mem0.reshape(M, D),
        A_Wq.reshape(D * H, DH), A_Wk.reshape(D * H, DH), A_Wv.reshape(D * H, DH),
        A_Wo.reshape(H * DH, D), B_w_r, B_w_i, gate_w.reshape(1, D),
        jnp.asarray(gdp), jnp.asarray(gsp),
    )
    return out.reshape(1, S, D)
```

```python
import functools
import math

import numpy as np
import jax
import jax.numpy as jnp
from jax import lax
import jax.experimental.pallas as pl
import jax.experimental.pallas.tpu as pltpu

BF, F32, U32 = jnp.bfloat16, jnp.float32, jnp.uint32

S, D, H, DH, M, SEG = 2048, 1024, 32, 128, 8, 32
NSEG = S // SEG
NP = H // 2
N1, N2 = 32, 64
PITCH = N1 + 8
CLASSES = ((0, 4), (1, 7), (2, 6), (3, 5))
NG = 5
LAG1, LAG2, SPLIT = 1, 3, 26
SEM_X, SEM_W, SEM_GD, SEM_GS, SEM_F, SEM_WO, SEM_OUT, NSEM = 0, 8, 14, 15, 16, 17, 18, 19
RSQ2 = float(np.float32(math.sqrt(0.5)))


def _to_bf16_bits(a):
    u = np.ascontiguousarray(a, dtype=np.float32).view(np.uint32)
    return ((u + 0x7FFF + ((u >> 16) & 1)) >> 16).astype(np.uint32)


def _pack_rows(a):
    b = _to_bf16_bits(a)
    return (b[..., 0::2, :] | (b[..., 1::2, :] << 16)).astype(np.uint32)


def _bfly8(x):
    s = [x[i] + x[i + 4] for i in range(4)]
    d = [x[i] - x[i + 4] for i in range(4)]
    e, f = s[0] + s[2], s[1] + s[3]
    t1, t2 = (d[1] - d[3]) * RSQ2, (d[1] + d[3]) * RSQ2
    return [e + f, e - f, d[0] + t1, t2 + d[2], s[0] - s[2], s[1] - s[3], d[0] - t1, t2 - d[2]]


def _bfly8_t(t):
    e, f = t[0] + t[1], t[0] - t[1]
    s = [e + t[4], f + t[5], e - t[4], f - t[5]]
    t1, t2 = t[2] - t[6], t[3] + t[7]
    d = [t[2] + t[6], (t1 + t2) * RSQ2, t[3] - t[7], (t2 - t1) * RSQ2]
    return [s[i] + d[i] for i in range(4)] + [s[i] - d[i] for i in range(4)]


@functools.lru_cache(maxsize=None)
def _constants():
    k2 = np.stack([np.concatenate([c + 8 * np.arange(64) for c in cls]) for cls in CLASSES])
    n2 = np.arange(D)
    ang = 2 * np.pi * ((k2[:, :, None] * n2[None, None, :]) % D) / D
    rows = np.stack([np.cos(ang), -np.sin(ang)], axis=1)
    assert k2[0, 0] == 0
    rows[0, 1, 0] = np.cos(np.pi * n2)
    wgt = np.full((4, 2, 128), 2.0)
    wgt[0, :, 0] = 1.0
    fwd = rows.reshape(D, D).T
    inv = (rows * wgt[..., None]).reshape(D, D) / (S * D)
    bf = np.stack(_bfly8(list(np.eye(8))))
    binv = np.kron(np.linalg.inv(bf), np.eye(128))
    gfull = binv.T @ fwd
    ifull = inv @ binv
    gd = np.stack([gfull[256 * g:256 * g + 256, 256 * g:256 * g + 256] for g in range(4)])
    gdi = np.stack([ifull[256 * g:256 * g + 256, 256 * g:256 * g + 256] for g in range(4)])
    blk = np.kron(np.eye(4), np.ones((256, 256)))
    assert np.abs(gfull * (1 - blk)).max() < 1e-6 and np.abs(ifull * (1 - blk)).max() < 1e-12

    b = np.arange(N2)
    k1 = np.arange(N1)[:, None] + N1 * np.arange(N2)[None, :]
    th = 2 * np.pi * ((k1[:, :, None] * b[None, None, :]) % S) / S
    gr, gi = np.cos(th), -np.sin(th)
    full = np.block([[gr, -gi], [gi, gr]])
    kap = np.arange(2 * N2)
    src = ((kap >> 3) & 1) * N2 + (kap >> 4) * 8 + (kap & 7)
    gs = full[:, :, src]
    hr, hi = np.swapaxes(gr, 1, 2), -np.swapaxes(gi, 1, 2)
    gsi = np.block([[hr, -hi], [hi, hr]])
    gdp = _pack_rows(np.stack([gd, gdi]))
    gsp = _pack_rows(np.stack([gs, gsi]))
    return gdp, gsp


def _cmul_const(v, k, n, sign):
    re, im = v
    k %= n
    if k == 0:
        return re, im
    if 4 * k == n:
        return (-im, re) if sign > 0 else (im, -re)
    if 8 * k == n:
        return (((re - im) * RSQ2, (re + im) * RSQ2) if sign > 0
                else ((re + im) * RSQ2, (im - re) * RSQ2))
    if 8 * k == 3 * n:
        return (((re + im) * -RSQ2, (re - im) * RSQ2) if sign > 0
                else ((im - re) * RSQ2, (re + im) * -RSQ2))
    c, s = math.cos(2 * math.pi * k / n), sign * math.sin(2 * math.pi * k / n)
    return re * c - im * s, re * s + im * c


def _fft(v, sign):
    n = len(v)
    if n == 1:
        return v
    ev, od = _fft(v[0::2], sign), _fft(v[1::2], sign)
    lo, hi = [], []
    for k in range(n // 2):
        er, ei = ev[k]
        if 4 * k == n:
            xr, xi = od[k]
            if sign > 0:
                lo.append((er - xi, ei + xr)); hi.append((er + xi, ei - xr))
            else:
                lo.append((er + xi, ei - xr)); hi.append((er - xi, ei + xr))
            continue
        tr, ti = _cmul_const(od[k], k, n, sign)
        lo.append((er + tr, ei + ti))
        hi.append((er - tr, ei - ti))
    return lo + hi


def _mask80():
    r = lax.broadcasted_iota(jnp.int32, (80, 80), 0)
    c = lax.broadcasted_iota(jnp.int32, (80, 80), 1)

    def head(i):
        return jnp.where(i < 64, i >> 5, (i - 64) >> 3)

    def pos(i):
        j = i & 31
        return jnp.where(i < 64, jnp.where(j < M, j, j + 8), M + (i & 7))

    same = head(r) == head(c)
    ok = (pos(r) < M) | (pos(c) <= pos(r))
    return same & ok, jnp.where(same, -1e9, -jnp.inf).astype(F32)


def _as_bf(u):
    return pltpu.bitcast(u, BF)


def _as_u32(b):
    return pltpu.bitcast(b, U32)


def _dot(a, b):
    return jnp.dot(a, b, preferred_element_type=F32)


def _kernel(x_hbm, mem_ref, wq_hbm, wk_hbm, wv_hbm, wo_hbm, fr_hbm, fi_hbm, nr_ref, ni_ref, gw_ref,
            gd_hbm, gs_hbm,
            out_hbm,
            x_v, raw, wqkv, wo, st, sto, obuf, xb, fraw, fp, gd, gs, y, u_s, out_v, sem):
    RB = 256
    raw4 = raw.reshape(6, D, 8, DH)
    w_hbm = (wq_hbm, wk_hbm, wv_hbm)

    def cp_x(i):
        rows = pl.ds(pl.multiple_of(i * RB, RB), RB)
        return pltpu.make_async_copy(x_hbm.at[rows, :], x_v.at[rows, :], sem.at[SEM_X + i])

    def cp_w(c, cs):
        return pltpu.make_async_copy(w_hbm[cs // 2].bitcast(U32).at[:, pl.ds(8 * (cs % 2), 8), :],
                                     raw4.at[c], sem.at[SEM_W + c])

    cp_gd = pltpu.make_async_copy(gd_hbm, gd, sem.at[SEM_GD])
    cp_gs = pltpu.make_async_copy(gs_hbm, gs, sem.at[SEM_GS])
    cp_f = [pltpu.make_async_copy(f.at[pl.ds(0, 512), pl.ds(128 * c, 128)].bitcast(U32), fraw.at[a, c],
                                  sem.at[SEM_F])
            for a, f in enumerate((fr_hbm, fi_hbm)) for c in range(16)]
    cp_wo = [pltpu.make_async_copy(wo_hbm.bitcast(U32).at[:, pl.ds(128 * j, 128)], wo.at[j], sem.at[SEM_WO])
             for j in range(8)]
    for c in ([cp_gd] + [cp_x(i) for i in range(S // RB)] + [cp_w(0, 0), cp_w(1, 1)] + cp_f
              + [cp_w(2, 2), cp_gs, cp_w(3, 3), cp_w(4, 4), cp_w(5, 5)] + cp_wo):
        c.start()

    cp_gd.wait()

    def f1(i, c):
        cp_x(i).wait()
        base = pl.multiple_of(i * RB, RB)
        pieces, first8 = [], []
        for r in range(0, RB, 16):
            xs = x_v[pl.ds(base + r, 16), :].astype(F32)
            if r % SEG == 0:
                first8.append(xs[0:8])
            us = _bfly8([xs[:, 128 * a:128 * a + 128] for a in range(8)])
            pieces.append(jnp.concatenate(us, axis=1).astype(BF))
        ub = jnp.concatenate(pieces, axis=0)
        xb[pl.ds(pl.multiple_of(i * (RB // 8), RB // 8), RB // 8), :] = _as_u32(
            jnp.concatenate(first8, axis=0).astype(BF))
        lane0 = lax.broadcasted_iota(jnp.int32, (RB, 128), 1) == 0
        for g in range(4):
            yy = _dot(ub[:, 256 * g:256 * g + 256], _as_bf(gd[0, g]))
            yr, yi = yy[:, :128], yy[:, 128:]
            if g == 0:
                y[4, 0, pl.ds(base, RB), :] = jnp.where(lane0, yi, 0.0)
                y[4, 1, pl.ds(base, RB), :] = jnp.zeros((RB, 128), F32)
                yi = jnp.where(lane0, 0.0, yi)
            y[g, 0, pl.ds(base, RB), :] = yr
            y[g, 1, pl.ds(base, RB), :] = yi
        return c

    lax.fori_loop(0, S // RB, f1, 0)

    NCH = N2 // 8

    def s_fwd(i, c):
        g = i // NCH
        r = pl.multiple_of((i % NCH) * 8, 8)
        v = [(y[g, 0, pl.ds(N2 * a + r, 8), :], y[g, 1, pl.ds(N2 * a + r, 8), :]) for a in range(N1)]
        v = _fft(v, -1)
        for ka in range(N1):
            u_s[g, ka, pl.ds(r, 8), :] = _as_u32(jnp.concatenate(v[ka], axis=0).astype(BF))
        return c

    lax.fori_loop(0, NG * NCH, s_fwd, 0)

    def bulk_dots(item):
        c, jj = item // 8, item % 8
        ws = [[], []]
        for d0 in range(0, D, 64):
            a = raw[c, pl.ds(d0 * 8 + jj, 64, stride=8), :]
            ws[0].append(pltpu.bitcast(a << 16, F32).astype(BF))
            ws[1].append(pltpu.bitcast(a & jnp.uint32(0xFFFF0000), F32).astype(BF))
        ws = [jnp.concatenate(w, axis=0) for w in ws]
        res = []

        def run(p):
            wqkv[2 * item + p] = _as_u32(ws[p])
            res.append(_dot(_as_bf(xb[...]), ws[p]).reshape(NSEG, 8, 128))
            if p == 1:
                st[item] = _as_u32(jnp.concatenate(res, axis=1).reshape(16 * NSEG, 128).astype(BF))

        return [functools.partial(run, 0), functools.partial(run, 1)]

    def fprep(blk):
        ev, od = [], []
        for r in range(4):
            wr = fraw[0, blk, pl.ds(r, 64, stride=4), :]
            wi = fraw[1, blk, pl.ds(r, 64, stride=4), :]
            ev.append((wr & jnp.uint32(0xFFFF)) | (wi << 16))
            od.append((wr >> 16) | (wi & jnp.uint32(0xFFFF0000)))
        cls = lambda k: (od if k % 2 else ev)[k // 2]
        cols = pl.ds(pl.multiple_of(blk * 128, 128), 128)
        nr = pltpu.bitcast(nr_ref[:, cols].astype(F32)[0:1], U32)
        ni = pltpu.bitcast(ni_ref[:, cols].astype(F32)[0:1], U32)
        blocks = [jnp.concatenate([cls(ca), cls(cb)], axis=0) for ca, cb in CLASSES]
        blocks.append(jnp.broadcast_to((nr >> 16) | ni, (128, 128)))
        for g, blkv in enumerate(blocks):
            t = pltpu.bitcast(pltpu.bitcast(blkv, F32).T, U32)
            for q in range(128 // N1):
                row = pl.multiple_of((blk * (128 // N1) + q) * PITCH, 8)
                fp[g, pl.ds(row, N1), :] = t[q * N1:(q + 1) * N1]

    def s_mid(g, kas):
        zs = []
        for ka in kas:
            xx = _dot(_as_bf(gs[0, ka]), _as_bf(u_s[g, ka]))
            w32 = fp[g, pl.ds(ka, N2, stride=PITCH), :]
            wr = pltpu.bitcast(w32 << 16, F32)
            wi = pltpu.bitcast(w32 & jnp.uint32(0xFFFF0000), F32)
            xr, xi = xx[:N2], xx[N2:]
            zs.append(jnp.concatenate([xr * wr - xi * wi, xr * wi + xi * wr], axis=0).astype(BF))

        def finish():
            for ka, z in zip(kas, zs):
                pp = _dot(_as_bf(gs[1, ka]), z)
                y[g, 0, N2 * ka:N2 * ka + N2, :] = pp[:N2]
                y[g, 1, N2 * ka:N2 * ka + N2, :] = pp[N2:]

        return finish

    def s_bwd(g):
        for r in range(0, N2, 8):
            v = [(y[g, 0, N2 * a + r:N2 * a + r + 8, :], y[g, 1, N2 * a + r:N2 * a + r + 8, :])
                 for a in range(N1)]
            v = _fft(v, 1)
            for a in range(N1):
                y[g, 0, N2 * a + r:N2 * a + r + 8, :] = v[a][0]
                y[g, 1, N2 * a + r:N2 * a + r + 8, :] = v[a][1]

    def bulk_loop(n0, n1, kind):
        def body(n, c):
            @pl.when(n % 4 == 0)
            def _():
                cp_w(n // 4, 0).wait()

            dots = bulk_dots(2 * n) + bulk_dots(2 * n + 1)
            k = n - n0
            for q, dot in enumerate(dots):
                if kind == "mid":
                    fin = s_mid(k, range(q * N1 // 4, (q + 1) * N1 // 4))
                dot()
                if kind == "mid":
                    fin()
            if kind == "fprep":
                fprep(2 * k)
                fprep(2 * k + 1)
            if kind == "bwd":
                s_bwd(k)
            return c

        lax.fori_loop(n0, n1, body, 0)

    bulk_loop(0, 6, "plain")
    pltpu.make_async_copy(fraw, fraw, sem.at[SEM_F]).wait()
    bulk_loop(6, 14, "fprep")
    cp_gs.wait()
    bulk_loop(14, 19, "mid")
    bulk_loop(19, 24, "bwd")
    pltpu.make_async_copy(wo, wo, sem.at[SEM_WO]).wait()

    scale = DH ** -0.5

    def softmax(s, mask, fill):
        s = jnp.where(mask, s * scale, fill)
        m = jnp.max(s, axis=-1, keepdims=True)
        e = jnp.exp(s - m)
        l = jnp.sum(e, axis=-1, keepdims=True)
        return (e * (1.0 / l)).astype(BF)

    def step(a, seg, first, mask, fill):
        R = 32 if first else 48
        qkv, ps = {}, {}
        srow = pl.multiple_of(seg * 8, 8)

        def proj(j):
            res = []
            for m in range(3):
                r1 = _dot(a, _as_bf(wqkv[H * m + 2 * j])).astype(BF)
                r2 = _dot(a, _as_bf(wqkv[H * m + 2 * j + 1])).astype(BF)
                res.append(jnp.concatenate([r1, r2, _as_bf(st[NP * m + j, pl.ds(srow, 8), :])], axis=0))
            qkv[j] = res

        def scores(j):
            s = lax.dot_general(qkv[j][0], qkv[j][1], (((1,), (1,)), ((), ())), preferred_element_type=F32)
            ps[j] = softmax(s, mask, fill)

        def pv(j):
            o = _dot(ps[j], qkv[j][2])
            for i in range(2):
                h = 2 * j + i
                if first:
                    ob = o[32 * i:32 * i + 32].astype(BF)
                    sto[h] = o[64 + 8 * i:72 + 8 * i]
                else:
                    ob = jnp.concatenate([o[32 * i:32 * i + 32], o[64 + 8 * i:72 + 8 * i], sto[h]],
                                         axis=0).astype(BF)
                obuf[h, 0:R // 2, :] = _as_u32(ob)

        def wo_part(j, h0, h1):
            og = jnp.concatenate([_as_bf(obuf[h, 0:R // 2, :]) for h in range(h0, h1)], axis=1)
            return _dot(og, _as_bf(wo[j, h0 * 64:h1 * 64, :]))

        parts = []
        for i in range(NP + 4):
            if i < NP:
                proj(i)
            else:
                parts.append(wo_part(2 * (i - NP), 0, SPLIT))
                parts.append(wo_part(2 * (i - NP) + 1, 0, SPLIT))
            if 0 <= i - LAG1 < NP:
                scores(i - LAG1)
            if 0 <= i - LAG2 < NP:
                pv(i - LAG2)
        return jnp.concatenate([wo_part(j, SPLIT, H) + parts[j] for j in range(8)], axis=1)

    def pair(t, mem):
        mask, fill = _mask80()
        base = pl.multiple_of(t * 64, 64)
        lane0 = lax.broadcasted_iota(jnp.int32, (64, 128), 1) == 0
        ts = []
        for g in range(4):
            vr = y[g, 0, pl.ds(base, 64), :]
            vi = y[g, 1, pl.ds(base, 64), :]
            if g == 0:
                vi = jnp.where(lane0, y[4, 0, pl.ds(base, 64), :], vi)
            tt = _dot(jnp.concatenate([vr, vi], axis=1).astype(BF), _as_bf(gd[1, g]))
            ts += [tt[:, :128], tt[:, 128:]]
        b = jnp.concatenate(_bfly8_t(ts), axis=1).astype(BF).astype(F32)

        xs = x_v[pl.ds(base, 64), :].astype(F32)
        gate = jax.nn.sigmoid(jnp.sum(xs * gw_ref[...].astype(F32), axis=-1, keepdims=True))
        a = jnp.concatenate([mem, xs[8:32]], axis=0).astype(BF)
        res_a = step(a, 2 * t, True, mask, fill)
        mem = res_a[0:8].astype(BF).astype(F32)
        a = jnp.concatenate([mem, xs[40:64]], axis=0).astype(BF)
        res_b = step(a, 2 * t + 1, False, mask, fill)
        mem = res_b[0:8].astype(BF).astype(F32)
        res = jnp.concatenate([res_b[40:48], res_a[8:32], res_b[32:40], res_b[8:32]], axis=0)
        out_v[pl.ds(base, 64), :] = (gate * res + (1.0 - gate) * b).astype(BF)
        pltpu.make_async_copy(out_v.at[pl.ds(base, 64), :], out_hbm.at[pl.ds(base, 64), :], sem.at[SEM_OUT]).start()
        return mem

    lax.fori_loop(0, S // 64, pair, mem_ref[...].astype(F32))
    pltpu.make_async_copy(out_v, out_hbm, sem.at[SEM_OUT]).wait()


@functools.partial(jax.jit, static_argnames=("A_seg_len",))
def pallas_gated_mix__memory_aug_recurrent_mem_tr__spectral_gfnet__prompt_kernel(
    A_x, A_mem0, A_Wq, A_Wk, A_Wv, A_Wo, A_seg_len, B_x, B_w_r, B_w_i, gate_w,
):
    assert A_x.shape == (1, S, D) and A_mem0.shape == (1, M, D) and A_Wq.shape == (D, H, DH)
    assert int(A_seg_len) == SEG
    gdp, gsp = _constants()
    any_spec = pl.BlockSpec(memory_space=pl.ANY)
    vmem_spec = pl.BlockSpec(memory_space=pltpu.VMEM)
    nyq_spec = pl.BlockSpec((16, S), lambda i: (D // 32, 0))
    fr_t, fi_t = B_w_r.T, B_w_i.T
    out = pl.pallas_call(
        _kernel,
        out_shape=jax.ShapeDtypeStruct((S, D), BF),
        grid=(1,),
        in_specs=[any_spec, vmem_spec, any_spec, any_spec, any_spec, any_spec, any_spec, any_spec,
                  nyq_spec, nyq_spec, vmem_spec, any_spec, any_spec],
        out_specs=any_spec,
        scratch_shapes=[
            pltpu.VMEM((S, D), BF),
            pltpu.VMEM((6, D * 8, DH), U32),
            pltpu.VMEM((3 * H, D // 2, DH), U32),
            pltpu.VMEM((8, H * DH // 2, 128), U32),
            pltpu.VMEM((3 * NP, 8 * NSEG, 128), U32),
            pltpu.VMEM((H, 8, 128), F32),
            pltpu.VMEM((H, 24, 128), U32),
            pltpu.VMEM((4 * NSEG, D), U32),
            pltpu.VMEM((2, 16, 256, 128), U32),
            pltpu.VMEM((NG, N2 * PITCH, 128), U32),
            pltpu.VMEM((2, 4, 128, 256), U32),
            pltpu.VMEM((2, N1, N2, 2 * N2), U32),
            pltpu.VMEM((NG, 2, S, 128), F32),
            pltpu.VMEM((NG, N1, N2, 128), U32),
            pltpu.VMEM((S, D), BF),
            pltpu.SemaphoreType.DMA((NSEM,)),
        ],
        compiler_params=pltpu.CompilerParams(vmem_limit_bytes=120 * 1024 * 1024),
    )(
        A_x.reshape(S, D), A_mem0.reshape(M, D), A_Wq, A_Wk, A_Wv,
        A_Wo.reshape(H * DH, D), fr_t, fi_t, fr_t, fi_t, gate_w.reshape(1, D),
        jnp.asarray(gdp), jnp.asarray(gsp),
    )
    return out.reshape(1, S, D)
```

```python
import functools
import math

import numpy as np
import jax
import jax.numpy as jnp
from jax import lax
import jax.experimental.pallas as pl
import jax.experimental.pallas.tpu as pltpu

BF, F32, U32 = jnp.bfloat16, jnp.float32, jnp.uint32

S, D, H, DH, M, SEG = 2048, 1024, 32, 128, 8, 32
NSEG = S // SEG
NP = H // 2
N1, N2 = 32, 64
PITCH = N1 + 8
CLASSES = ((0, 4), (1, 7), (2, 6), (3, 5))
NG = 5
LAG1, LAG2, SPLIT = 1, 3, 26
NQ = 4
IPI = 4
(SEM_W, SEM_GD, SEM_GS, SEM_F, SEM_NYQ, SEM_WO, SEM_MEM, SEM_GW, SEM_OUT, SEM_X) = 0, 6, 7, 8, 9, 10, 11, 12, 13, 14
SEM_W0 = SEM_X + NQ
NSEM = SEM_W0 + NQ
RSQ2 = float(np.float32(math.sqrt(0.5)))


def _to_bf16_bits(a):
    u = np.ascontiguousarray(a, dtype=np.float32).view(np.uint32)
    return ((u + 0x7FFF + ((u >> 16) & 1)) >> 16).astype(np.uint32)


def _pack_rows(a):
    b = _to_bf16_bits(a)
    return (b[..., 0::2, :] | (b[..., 1::2, :] << 16)).astype(np.uint32)


def _bfly8(x):
    s = [x[i] + x[i + 4] for i in range(4)]
    d = [x[i] - x[i + 4] for i in range(4)]
    e, f = s[0] + s[2], s[1] + s[3]
    t1, t2 = (d[1] - d[3]) * RSQ2, (d[1] + d[3]) * RSQ2
    return [e + f, e - f, d[0] + t1, t2 + d[2], s[0] - s[2], s[1] - s[3], d[0] - t1, t2 - d[2]]


def _bfly8_t(t):
    e, f = t[0] + t[1], t[0] - t[1]
    s = [e + t[4], f + t[5], e - t[4], f - t[5]]
    t1, t2 = t[2] - t[6], t[3] + t[7]
    d = [t[2] + t[6], (t1 + t2) * RSQ2, t[3] - t[7], (t2 - t1) * RSQ2]
    return [s[i] + d[i] for i in range(4)] + [s[i] - d[i] for i in range(4)]


@functools.lru_cache(maxsize=None)
def _constants():
    k2 = np.stack([np.concatenate([c + 8 * np.arange(64) for c in cls]) for cls in CLASSES])
    n2 = np.arange(D)
    ang = 2 * np.pi * ((k2[:, :, None] * n2[None, None, :]) % D) / D
    rows = np.stack([np.cos(ang), -np.sin(ang)], axis=1)
    assert k2[0, 0] == 0
    rows[0, 1, 0] = np.cos(np.pi * n2)
    wgt = np.full((4, 2, 128), 2.0)
    wgt[0, :, 0] = 1.0
    fwd = rows.reshape(D, D).T
    inv = (rows * wgt[..., None]).reshape(D, D) / (S * D)
    bf = np.stack(_bfly8(list(np.eye(8))))
    binv = np.kron(np.linalg.inv(bf), np.eye(128))
    gfull = binv.T @ fwd
    ifull = inv @ binv
    gd = np.stack([gfull[256 * g:256 * g + 256, 256 * g:256 * g + 256] for g in range(4)])
    gdi = np.stack([ifull[256 * g:256 * g + 256, 256 * g:256 * g + 256] for g in range(4)])
    blk = np.kron(np.eye(4), np.ones((256, 256)))
    assert np.abs(gfull * (1 - blk)).max() < 1e-6 and np.abs(ifull * (1 - blk)).max() < 1e-12

    b = np.arange(N2)
    k1 = np.arange(N1)[:, None] + N1 * np.arange(N2)[None, :]
    th = 2 * np.pi * ((k1[:, :, None] * b[None, None, :]) % S) / S
    gr, gi = np.cos(th), -np.sin(th)
    full = np.block([[gr, -gi], [gi, gr]])
    kap = np.arange(2 * N2)
    src = ((kap >> 3) & 1) * N2 + (kap >> 4) * 8 + (kap & 7)
    gs = full[:, :, src]
    hr, hi = np.swapaxes(gr, 1, 2), -np.swapaxes(gi, 1, 2)
    gsi = np.block([[hr, -hi], [hi, hr]])
    gdp = _pack_rows(np.stack([gd, gdi]))
    gsp = _pack_rows(np.stack([gs, gsi]))
    return gdp, gsp


def _cmul_const(v, k, n, sign):
    re, im = v
    k %= n
    if k == 0:
        return re, im
    if 4 * k == n:
        return (-im, re) if sign > 0 else (im, -re)
    if 8 * k == n:
        return (((re - im) * RSQ2, (re + im) * RSQ2) if sign > 0
                else ((re + im) * RSQ2, (im - re) * RSQ2))
    if 8 * k == 3 * n:
        return (((re + im) * -RSQ2, (re - im) * RSQ2) if sign > 0
                else ((im - re) * RSQ2, (re + im) * -RSQ2))
    c, s = math.cos(2 * math.pi * k / n), sign * math.sin(2 * math.pi * k / n)
    return re * c - im * s, re * s + im * c


def _fft(v, sign):
    n = len(v)
    if n == 1:
        return v
    ev, od = _fft(v[0::2], sign), _fft(v[1::2], sign)
    lo, hi = [], []
    for k in range(n // 2):
        er, ei = ev[k]
        if 4 * k == n:
            xr, xi = od[k]
            if sign > 0:
                lo.append((er - xi, ei + xr)); hi.append((er + xi, ei - xr))
            else:
                lo.append((er + xi, ei - xr)); hi.append((er - xi, ei + xr))
            continue
        tr, ti = _cmul_const(od[k], k, n, sign)
        lo.append((er + tr, ei + ti))
        hi.append((er - tr, ei - ti))
    return lo + hi


def _mask80():
    r = lax.broadcasted_iota(jnp.int32, (80, 80), 0)
    c = lax.broadcasted_iota(jnp.int32, (80, 80), 1)

    def head(i):
        return jnp.where(i < 64, i >> 5, (i - 64) >> 3)

    def pos(i):
        j = i & 31
        return jnp.where(i < 64, jnp.where(j < M, j, j + 8), M + (i & 7))

    same = head(r) == head(c)
    ok = (pos(r) < M) | (pos(c) <= pos(r))
    return same & ok, jnp.where(same, -1e9, -jnp.inf).astype(F32)


def _as_bf(u):
    return pltpu.bitcast(u, BF)


def _as_u32(b):
    return pltpu.bitcast(b, U32)


def _dot(a, b):
    return jnp.dot(a, b, preferred_element_type=F32)


def _kernel(x_hbm, mem_hbm, wq_hbm, wk_hbm, wv_hbm, wo_hbm, fr_hbm, fi_hbm, gw_hbm, gd_hbm, gs_hbm,
            out_hbm,
            x_v, raw, wqkv, wo, st, sto, obuf, xb, fraw, fp, gd, gs, y, out_v, mem_ref, gw_ref, nyq,
            sem):
    KQ = D // NQ
    raw4 = raw.reshape(6, D, 8, DH)
    w_hbm = (wq_hbm, wk_hbm, wv_hbm)

    def w_src(c):
        return w_hbm[c // 2].bitcast(U32).at[:, pl.ds(8 * (c % 2), 8), :]

    def wait(dst, k):
        pltpu.make_async_copy(dst, dst, sem.at[k]).wait()

    def x_dst(q):
        return x_v.at[:, pl.ds(pl.multiple_of(q * KQ, KQ), KQ)]

    def w0_dst(q):
        return raw4.at[0, pl.ds(pl.multiple_of(q * KQ, KQ), KQ)]

    copies = []
    for q in range(NQ):
        copies.append((x_hbm.at[:, pl.ds(q * KQ, KQ)], x_dst(q), SEM_X + q))
        copies.append((w_src(0).at[pl.ds(q * KQ, KQ)], w0_dst(q), SEM_W0 + q))
    copies += [(gd_hbm, gd, SEM_GD), (w_src(1), raw4.at[1], SEM_W + 1)]
    copies += [(f.at[pl.ds(0, 512), pl.ds(128 * c, 128)].bitcast(U32), fraw.at[a, c], SEM_F)
               for a, f in enumerate((fr_hbm, fi_hbm)) for c in range(16)]
    copies += [(f.at[pl.ds(D // 2, 1), :], nyq.at[a], SEM_NYQ) for a, f in enumerate((fr_hbm, fi_hbm))]
    copies += [(w_src(2), raw4.at[2], SEM_W + 2), (gs_hbm, gs, SEM_GS)]
    copies += [(w_src(c), raw4.at[c], SEM_W + c) for c in (3, 4, 5)]
    copies += [(wo_hbm.bitcast(U32).at[:, pl.ds(128 * j, 128)], wo.at[j], SEM_WO) for j in range(8)]
    copies += [(mem_hbm, mem_ref, SEM_MEM), (gw_hbm, gw_ref, SEM_GW)]
    for src, dst, k in copies:
        pltpu.make_async_copy(src, dst, sem.at[k]).start()

    def relayout(c, jj, d_lo, nd):
        ws = [[], []]
        for d0 in range(0, nd, 64):
            a = raw[c, pl.ds((d_lo + d0) * 8 + jj, 64, stride=8), :]
            ws[0].append(pltpu.bitcast(a << 16, F32).astype(BF))
            ws[1].append(pltpu.bitcast(a & jnp.uint32(0xFFFF0000), F32).astype(BF))
        return [jnp.concatenate(w, axis=0) for w in ws]

    def store_st(item, res):
        res = [r.reshape(NSEG, 8, 128) for r in res]
        st[item] = _as_u32(jnp.concatenate(res, axis=1).reshape(16 * NSEG, 128).astype(BF))

    def acc(h):
        return y.at[h // 8, (h // 4) % 2, pl.ds(512 * (h % 4), 512), :]

    for h in range(16):
        acc(h)[...] = jnp.zeros((512, 128), F32)

    def k_slice(q, last):
        wait(x_dst(q), SEM_X + q)
        d_lo = pl.multiple_of(q * KQ, KQ)
        cols = pl.ds(d_lo, KQ)
        for s2 in range(NSEG // 2):
            rows = jnp.concatenate([x_v[64 * s2:64 * s2 + 16, cols].astype(F32)[0:8],
                                    x_v[64 * s2 + 32:64 * s2 + 48, cols].astype(F32)[0:8]], axis=0)
            xb[8 * s2:8 * s2 + 8, cols] = _as_u32(rows.astype(BF))
        wait(w0_dst(q), SEM_W0 + q)
        for jj in range(8):
            ws = relayout(0, jj, d_lo, KQ)
            res = []
            for p in range(2):
                wqkv[2 * jj + p, pl.ds(pl.multiple_of(q * (KQ // 2), KQ // 2), KQ // 2), :] = _as_u32(ws[p])
                r = _dot(_as_bf(xb[:, cols]), ws[p]) + acc(2 * jj + p)[...]
                if last:
                    res.append(r)
                else:
                    acc(2 * jj + p)[...] = r
            if last:
                store_st(jj, res)

    def k_body(q, c):
        k_slice(q, False)
        return c

    with jax.named_scope("p0"):
        lax.fori_loop(0, NQ - 1, k_body, 0)
        k_slice(NQ - 1, True)

    wait(gd, SEM_GD)
    RB, HB, QS = 128, 64, S // 4

    def f1(i, c):
        base = pl.multiple_of(i * RB, RB)
        lane0 = lax.broadcasted_iota(jnp.int32, (4 * HB, 128), 1) == 0
        for h0 in range(0, RB, HB):
            pieces = []
            for a1 in range(4):
                for r in range(h0, h0 + HB, 16):
                    xs = x_v[pl.ds(base + (QS * a1 + r), 16), :].astype(F32)
                    us = _bfly8([xs[:, 128 * a:128 * a + 128] for a in range(8)])
                    pieces.append(jnp.concatenate(us, axis=1).astype(BF))
            ub = jnp.concatenate(pieces, axis=0)

            def put(g, yr, yi):
                v = _fft([(yr[HB * a1:HB * a1 + HB], yi[HB * a1:HB * a1 + HB]) for a1 in range(4)], -1)
                for k1 in range(4):
                    rows = pl.ds(base + (QS * k1 + h0), HB)
                    y[g, 0, rows, :] = v[k1][0]
                    y[g, 1, rows, :] = v[k1][1]

            for g in range(4):
                yy = _dot(ub[:, 256 * g:256 * g + 256], _as_bf(gd[0, g]))
                yr, yi = yy[:, :128], yy[:, 128:]
                if g == 0:
                    put(4, jnp.where(lane0, yi, 0.0), jnp.zeros((4 * HB, 128), F32))
                    yi = jnp.where(lane0, 0.0, yi)
                put(g, yr, yi)
        return c

    with jax.named_scope("f1"):
        lax.fori_loop(0, QS // RB, f1, 0)

    def fprep(blk):
        ev, od = [], []
        for r in range(4):
            wr = fraw[0, blk, pl.ds(r, 64, stride=4), :]
            wi = fraw[1, blk, pl.ds(r, 64, stride=4), :]
            ev.append((wr & jnp.uint32(0xFFFF)) | (wi << 16))
            od.append((wr >> 16) | (wi & jnp.uint32(0xFFFF0000)))
        cls = lambda k: (od if k % 2 else ev)[k // 2]
        cols = pl.ds(pl.multiple_of(blk * 128, 128), 128)
        nr = pltpu.bitcast(nyq[0, :, cols].astype(F32), U32)
        ni = pltpu.bitcast(nyq[1, :, cols].astype(F32), U32)
        blocks = [jnp.concatenate([cls(ca), cls(cb)], axis=0) for ca, cb in CLASSES]
        blocks.append(jnp.broadcast_to((nr >> 16) | ni, (128, 128)))
        for g, blkv in enumerate(blocks):
            t = pltpu.bitcast(pltpu.bitcast(blkv, F32).T, U32)
            for q in range(128 // N1):
                row = pl.multiple_of((blk * (128 // N1) + q) * PITCH, 8)
                fp[g, pl.ds(row, N1), :] = t[q * N1:(q + 1) * N1]

    def s_mid(g, k1):
        def rows(a0, r):
            return slice(QS * k1 + N2 * a0 + r, QS * k1 + N2 * a0 + r + 8)

        us = [[] for _ in range(8)]
        for r in range(0, N2, 8):
            v = [_cmul_const((y[g, 0, rows(a0, r), :], y[g, 1, rows(a0, r), :]), a0 * k1, N1, -1)
                 for a0 in range(8)]
            v = _fft(v, -1)
            for k0 in range(8):
                us[k0].append(jnp.concatenate(v[k0], axis=0).astype(BF))
        zs = []
        for k0 in range(8):
            ka = k1 + 4 * k0
            xx = _dot(_as_bf(gs[0, ka]), jnp.concatenate(us[k0], axis=0))
            w32 = fp[g, pl.ds(ka, N2, stride=PITCH), :]
            wr = pltpu.bitcast(w32 << 16, F32)
            wi = pltpu.bitcast(w32 & jnp.uint32(0xFFFF0000), F32)
            xr, xi = xx[:N2], xx[N2:]
            zs.append(jnp.concatenate([xr * wr - xi * wi, xr * wi + xi * wr], axis=0).astype(BF))

        def finish():
            ps = [_dot(_as_bf(gs[1, k1 + 4 * k0]), zs[k0]) for k0 in range(8)]
            for r in range(0, N2, 8):
                v = _fft([(pp[r:r + 8], pp[N2 + r:N2 + r + 8]) for pp in ps], 1)
                for a0 in range(8):
                    vr, vi = _cmul_const(v[a0], a0 * k1, N1, 1)
                    y[g, 0, rows(a0, r), :] = vr
                    y[g, 1, rows(a0, r), :] = vi

        return finish

    def bulk_loop(n0, n1, kind):
        def body(n, c):
            ch = (n * IPI) // 8

            @pl.when((n * IPI) % 8 == 0)
            def _():
                wait(raw4.at[ch], SEM_W + ch)

            fin = None
            for i in range(IPI):
                item = n * IPI + i
                ws = relayout(ch, item % 8, 0, D)
                res = []
                for p in range(2):
                    q = 2 * i + p
                    wqkv[2 * item + p] = _as_u32(ws[p])
                    res.append(_dot(_as_bf(xb[...]), ws[p]))
                    if kind == "mid":
                        if fin is not None:
                            fin()
                        fin = s_mid(n - n0, q) if q < 4 else None
                    if kind == "fprep":
                        fprep(8 * (n - n0) + q)
                store_st(item, res)
            return c

        with jax.named_scope("bulk_" + kind):
            lax.fori_loop(n0, n1, body, 0)

    bulk_loop(2, 5, "plain")
    wait(fraw, SEM_F)
    wait(nyq, SEM_NYQ)
    bulk_loop(5, 7, "fprep")
    wait(gs, SEM_GS)
    bulk_loop(7, 12, "mid")
    wait(wo, SEM_WO)
    wait(mem_ref, SEM_MEM)
    wait(gw_ref, SEM_GW)

    scale = DH ** -0.5

    def softmax(s, mask, fill):
        s = jnp.where(mask, s * scale, fill)
        m = jnp.max(s, axis=-1, keepdims=True)
        e = jnp.exp(s - m)
        l = jnp.sum(e, axis=-1, keepdims=True)
        return (e * (1.0 / l)).astype(BF)

    def step(a, seg, first, mask, fill):
        R = 32 if first else 48
        qkv, ps = {}, {}
        srow = pl.multiple_of(seg * 8, 8)

        def proj(j):
            res = []
            for m in range(3):
                r1 = _dot(a, _as_bf(wqkv[H * m + 2 * j])).astype(BF)
                r2 = _dot(a, _as_bf(wqkv[H * m + 2 * j + 1])).astype(BF)
                res.append(jnp.concatenate([r1, r2, _as_bf(st[NP * m + j, pl.ds(srow, 8), :])], axis=0))
            qkv[j] = res

        def scores(j):
            s = lax.dot_general(qkv[j][0], qkv[j][1], (((1,), (1,)), ((), ())), preferred_element_type=F32)
            ps[j] = softmax(s, mask, fill)

        def pv(j):
            o = _dot(ps[j], qkv[j][2])
            for i in range(2):
                h = 2 * j + i
                if first:
                    ob = o[32 * i:32 * i + 32].astype(BF)
                    sto[h] = o[64 + 8 * i:72 + 8 * i]
                else:
                    ob = jnp.concatenate([o[32 * i:32 * i + 32], o[64 + 8 * i:72 + 8 * i], sto[h]],
                                         axis=0).astype(BF)
                obuf[h, 0:R // 2, :] = _as_u32(ob)

        def wo_part(j, h0, h1):
            og = jnp.concatenate([_as_bf(obuf[h, 0:R // 2, :]) for h in range(h0, h1)], axis=1)
            return _dot(og, _as_bf(wo[j, h0 * 64:h1 * 64, :]))

        parts = []
        for i in range(NP + 4):
            if i < NP:
                proj(i)
            else:
                parts.append(wo_part(2 * (i - NP), 0, SPLIT))
                parts.append(wo_part(2 * (i - NP) + 1, 0, SPLIT))
            if 0 <= i - LAG1 < NP:
                scores(i - LAG1)
            if 0 <= i - LAG2 < NP:
                pv(i - LAG2)
        return jnp.concatenate([wo_part(j, SPLIT, H) + parts[j] for j in range(8)], axis=1)

    def pair(t, mem):
        mask, fill = _mask80()
        base = pl.multiple_of(t * 64, 64)
        lane0 = lax.broadcasted_iota(jnp.int32, (64, 128), 1) == 0
        a1 = t // 8
        off = pl.multiple_of((t % 8) * 64, 64)
        s2 = (1 - 2 * (a1 & 1)).astype(F32)
        sg = (1 - (a1 & 2)).astype(F32)
        cc, ss = sg * (1 - (a1 & 1)).astype(F32), sg * (a1 & 1).astype(F32)

        def radix4(g, need_im=True):
            q = [[y[g, c, pl.ds(off + QS * k1, 64), :] for c in range(2)] for k1 in range(4)]
            br, bi = q[1][0] + s2 * q[3][0], q[1][1] + s2 * q[3][1]
            vr = q[0][0] + s2 * q[2][0] + (cc * br - ss * bi)
            vi = q[0][1] + s2 * q[2][1] + (cc * bi + ss * br) if need_im else None
            return vr, vi

        ts = []
        for g in range(4):
            vr, vi = radix4(g)
            if g == 0:
                vi = jnp.where(lane0, radix4(4, False)[0], vi)
            tt = _dot(jnp.concatenate([vr, vi], axis=1).astype(BF), _as_bf(gd[1, g]))
            ts += [tt[:, :128], tt[:, 128:]]
        b = jnp.concatenate(_bfly8_t(ts), axis=1).astype(BF).astype(F32)

        xs = x_v[pl.ds(base, 64), :].astype(F32)
        gate = jax.nn.sigmoid(jnp.sum(xs * gw_ref[...].astype(F32), axis=-1, keepdims=True))
        a = jnp.concatenate([mem, xs[8:32]], axis=0).astype(BF)
        res_a = step(a, 2 * t, True, mask, fill)
        mem = res_a[0:8].astype(BF).astype(F32)
        a = jnp.concatenate([mem, xs[40:64]], axis=0).astype(BF)
        res_b = step(a, 2 * t + 1, False, mask, fill)
        mem = res_b[0:8].astype(BF).astype(F32)
        res = jnp.concatenate([res_b[40:48], res_a[8:32], res_b[32:40], res_b[8:32]], axis=0)
        out_v[pl.ds(base, 64), :] = (gate * res + (1.0 - gate) * b).astype(BF)
        pltpu.make_async_copy(out_v.at[pl.ds(base, 64), :], out_hbm.at[pl.ds(base, 64), :], sem.at[SEM_OUT]).start()
        return mem

    with jax.named_scope("chain"):
        lax.fori_loop(0, S // 64, pair, mem_ref[...].astype(F32), unroll=1)
    pltpu.make_async_copy(out_v, out_hbm, sem.at[SEM_OUT]).wait()


@functools.partial(jax.jit, static_argnames=("A_seg_len",))
def pallas_gated_mix__memory_aug_recurrent_mem_tr__spectral_gfnet__prompt_kernel(
    A_x, A_mem0, A_Wq, A_Wk, A_Wv, A_Wo, A_seg_len, B_x, B_w_r, B_w_i, gate_w,
):
    assert A_x.shape == (1, S, D) and A_mem0.shape == (1, M, D) and A_Wq.shape == (D, H, DH)
    assert int(A_seg_len) == SEG
    gdp, gsp = _constants()
    any_spec = pl.BlockSpec(memory_space=pl.ANY)
    out = pl.pallas_call(
        _kernel,
        out_shape=jax.ShapeDtypeStruct((S, D), BF),
        in_specs=[any_spec] * 11,
        out_specs=any_spec,
        scratch_shapes=[
            pltpu.VMEM((S, D), BF),
            pltpu.VMEM((6, D * 8, DH), U32),
            pltpu.VMEM((3 * H, D // 2, DH), U32),
            pltpu.VMEM((8, H * DH // 2, 128), U32),
            pltpu.VMEM((3 * NP, 8 * NSEG, 128), U32),
            pltpu.VMEM((H, 8, 128), F32),
            pltpu.VMEM((H, 24, 128), U32),
            pltpu.VMEM((4 * NSEG, D), U32),
            pltpu.VMEM((2, 16, 256, 128), U32),
            pltpu.VMEM((NG, N2 * PITCH, 128), U32),
            pltpu.VMEM((2, 4, 128, 256), U32),
            pltpu.VMEM((2, N1, N2, 2 * N2), U32),
            pltpu.VMEM((NG, 2, S, 128), F32),
            pltpu.VMEM((S, D), BF),
            pltpu.VMEM((M, D), BF),
            pltpu.VMEM((1, D), BF),
            pltpu.VMEM((2, 1, S), BF),
            pltpu.SemaphoreType.DMA((NSEM,)),
        ],
        compiler_params=pltpu.CompilerParams(vmem_limit_bytes=120 * 1024 * 1024),
    )(
        A_x.reshape(S, D), A_mem0.reshape(M, D), A_Wq, A_Wk, A_Wv,
        A_Wo.reshape(H * DH, D), B_w_r.T, B_w_i.T, gate_w.reshape(1, D),
        jnp.asarray(gdp), jnp.asarray(gsp),
    )
    return out.reshape(1, S, D)
```

```python
import functools
import math

import numpy as np
import jax
import jax.numpy as jnp
from jax import lax
import jax.experimental.pallas as pl
import jax.experimental.pallas.tpu as pltpu

BF, F32, U32 = jnp.bfloat16, jnp.float32, jnp.uint32

S, D, H, DH, M, SEG = 2048, 1024, 32, 128, 8, 32
NSEG = S // SEG
NP = H // 2
N1, N2 = 32, 64
QS = S // 4
PITCH = N1 + 8
CLASSES = ((0, 8, 4, 12), (1, 15, 9, 7), (2, 14, 10, 6), (3, 13, 11, 5))
LAG1, LAG2, SPLIT = 1, 3, 26
NQ = 4
(SEM_W, SEM_GF, SEM_GI, SEM_SM, SEM_GS, SEM_F, SEM_NYQ, SEM_WO, SEM_MEM, SEM_GW, SEM_OUT,
 SEM_X) = 0, 6, 7, 8, 9, 10, 12, 13, 14, 15, 16, 17
SEM_W0 = SEM_X + NQ
NSEM = SEM_W0 + NQ
RSQ2 = float(np.float32(math.sqrt(0.5)))


def _bfly8(x):
    s = [x[i] + x[i + 4] for i in range(4)]
    d = [x[i] - x[i + 4] for i in range(4)]
    e, f = s[0] + s[2], s[1] + s[3]
    t1, t2 = (d[1] - d[3]) * RSQ2, (d[1] + d[3]) * RSQ2
    return [e + f, e - f, d[0] + t1, t2 + d[2], s[0] - s[2], s[1] - s[3], d[0] - t1, t2 - d[2]]


def _bfly8_t(t):
    e, f = t[0] + t[1], t[0] - t[1]
    s = [e + t[4], f + t[5], e - t[4], f - t[5]]
    t1, t2 = t[2] - t[6], t[3] + t[7]
    d = [t[2] + t[6], (t1 + t2) * RSQ2, t[3] - t[7], (t2 - t1) * RSQ2]
    return [s[i] + d[i] for i in range(4)] + [s[i] - d[i] for i in range(4)]


def _half_pre(vr, vi, lo, roll, where):
    ri = roll(vi)
    return where(lo, vr, ri), where(lo, ri, vr)


def _half_post(g, tp, tm, lo, roll, where):
    if g == 0:
        return tp, tm
    c = float(np.float32(math.cos(math.pi * g / 8)))
    s = float(np.float32(math.sin(math.pi * g / 8)))
    p, r = tp + tm, tp - tm
    rm = roll(where(lo, r, p))
    return where(lo, p, c * rm + s * r), where(lo, rm, c * r - s * rm)


def _cmul_const(v, k, n, sign):
    re, im = v
    k %= n
    if k == 0:
        return re, im
    if 4 * k == n:
        return (-im, re) if sign > 0 else (im, -re)
    if 8 * k == n:
        return (((re - im) * RSQ2, (re + im) * RSQ2) if sign > 0
                else ((re + im) * RSQ2, (im - re) * RSQ2))
    if 8 * k == 3 * n:
        return (((re + im) * -RSQ2, (re - im) * RSQ2) if sign > 0
                else ((im - re) * RSQ2, (re + im) * -RSQ2))
    c, s = math.cos(2 * math.pi * k / n), sign * math.sin(2 * math.pi * k / n)
    return re * c - im * s, re * s + im * c


def _fft(v, sign):
    n = len(v)
    if n == 1:
        return v
    ev, od = _fft(v[0::2], sign), _fft(v[1::2], sign)
    lo, hi = [], []
    for k in range(n // 2):
        er, ei = ev[k]
        if 4 * k == n:
            xr, xi = od[k]
            if sign > 0:
                lo.append((er - xi, ei + xr)); hi.append((er + xi, ei - xr))
            else:
                lo.append((er + xi, ei - xr)); hi.append((er - xi, ei + xr))
            continue
        tr, ti = _cmul_const(od[k], k, n, sign)
        lo.append((er + tr, ei + ti))
        hi.append((er - tr, ei - ti))
    return lo + hi


def _pack_rows(a):
    u = np.ascontiguousarray(a, dtype=np.float32).view(np.uint32)
    b = ((u + 0x7FFF + ((u >> 16) & 1)) >> 16).astype(np.uint32)
    return (b[..., 0::2, :] | (b[..., 1::2, :] << 16)).astype(np.uint32)


def _diag_blocks(full, n, tol):
    k = full.shape[0] // n
    blk = np.kron(np.eye(k), np.ones((n, n)))
    assert np.abs(full * (1 - blk)).max() < tol
    return np.stack([full[n * g:n * g + n, n * g:n * g + n] for g in range(k)])


def _cplx(re, im):
    return np.block([[re, im], [-im, re]])


@functools.lru_cache(maxsize=None)
def _constants():
    k2 = np.stack([np.concatenate([c + 16 * np.arange(32) for c in cls]) for cls in CLASSES])
    n2 = np.arange(D)
    ang = 2 * np.pi * ((k2[:, :, None] * n2[None, None, :]) % D) / D
    rows = np.stack([np.cos(ang), -np.sin(ang)], axis=1)
    wgt = np.where(k2 == 0, 1.0, 2.0)[:, None, :, None]
    fwd = rows.reshape(D, D).T
    inv = (rows * wgt).reshape(D, D) / (S * D)
    bf = np.stack(_bfly8(list(np.eye(8))))
    binv = np.kron(np.linalg.inv(bf), np.eye(128))
    gd = _diag_blocks(binv.T @ fwd, 256, 1e-6)
    gdi = _diag_blocks(inv @ binv, 256, 1e-12)
    eye, lo = np.eye(256), np.arange(128) < 64
    roll = lambda v: np.roll(v, 64, axis=1)
    pre = np.concatenate(_half_pre(eye[:, :128], eye[:, 128:], lo, roll, np.where), axis=1)
    gi = []
    for g in range(4):
        post = np.concatenate(_half_post(g, eye[:, :128], eye[:, 128:], lo, roll, np.where), axis=1)
        gi.append(_diag_blocks(np.linalg.inv(pre) @ gdi[g] @ np.linalg.inv(post), 128, 1e-12))
    gi = np.concatenate(gi)

    b = np.arange(N2)
    k1 = np.arange(N1)[:, None] + N1 * np.arange(N2)[None, :]
    th = 2 * np.pi * ((k1[:, :, None] * b[None, None, :]) % S) / S
    gr, gim = np.cos(th), -np.sin(th)
    full = np.block([[gr, -gim], [gim, gr]])
    kap = np.arange(2 * N2)
    src = ((kap >> 3) & 1) * N2 + (kap >> 4) * 8 + (kap & 7)
    gs = full[:, :, src]
    hr, hi = np.swapaxes(gr, 1, 2), -np.swapaxes(gim, 1, 2)
    gsi = np.block([[hr, -hi], [hi, hr]])

    lane = np.arange(128)
    kb = 8 * (lane % 16) + lane // 16
    t128 = 2 * np.pi * ((lane[:, None] * kb[None, :]) % 128) / 128
    nyf = _cplx(np.cos(t128), -np.sin(t128))
    nyi = _cplx(np.cos(t128).T, np.sin(t128).T)
    i16 = np.arange(16)
    t16 = 2 * np.pi * ((i16[:, None] * i16[None, :]) % 16) / 16
    tw = 2 * np.pi * (i16[:, None] * lane[None, :]) / S
    sm = np.zeros((80, 128), np.float32)
    sm[0:16], sm[16:32] = np.cos(tw), np.sin(tw)
    sm[32:48, :16], sm[48:64, :16] = np.cos(t16), -np.sin(t16)
    sm[64:80, :16], sm[64:80, 16:32] = np.cos(t16), -np.sin(t16)

    gfp = _pack_rows(np.concatenate([gd, nyf[None], nyi[None]]))
    return gfp, _pack_rows(gi), sm, _pack_rows(np.stack([gs, gsi]))


def _mask80():
    r = lax.broadcasted_iota(jnp.int32, (80, 80), 0)
    c = lax.broadcasted_iota(jnp.int32, (80, 80), 1)

    def head(i):
        return jnp.where(i < 64, i >> 5, (i - 64) >> 3)

    def pos(i):
        j = i & 31
        return jnp.where(i < 64, jnp.where(j < M, j, j + 8), M + (i & 7))

    same = head(r) == head(c)
    ok = (pos(r) < M) | (pos(c) <= pos(r))
    return same & ok, jnp.where(same, -1e9, -jnp.inf).astype(F32)


def _as_bf(u):
    return pltpu.bitcast(u, BF)


def _as_u32(b):
    return pltpu.bitcast(b, U32)


def _lo_f32(u):
    return pltpu.bitcast(u << 16, F32)


def _hi_f32(u):
    return pltpu.bitcast(u & jnp.uint32(0xFFFF0000), F32)


def _dot(a, b):
    return jnp.dot(a, b, preferred_element_type=F32)


def _dot_nt(a, b):
    return lax.dot_general(a, b, (((1,), (1,)), ((), ())), preferred_element_type=F32)


def _transpose_u32(u):
    return pltpu.bitcast(pltpu.bitcast(u, F32).T, U32)


def _lanes(rows):
    return lax.broadcasted_iota(jnp.int32, (rows, 128), 1)


def _kernel(x_hbm, mem_hbm, wq_hbm, wk_hbm, wv_hbm, wo_hbm, fr_hbm, fi_hbm, gw_hbm,
            gf_hbm, gi_hbm, sm_hbm, gs_hbm,
            out_hbm,
            x_v, raw, wqkv, wo, st, sto, obuf, xb, fraw, fp, gf, gi, sm, gs, y, out_v, mem_ref, gw_ref,
            nyq, xa, ct, a_s, qkv_s, ra_s, sem):
    KQ = D // NQ
    raw4 = raw.reshape(6, D, 8, DH)
    w_hbm = (wq_hbm, wk_hbm, wv_hbm)
    f_hbm = (fr_hbm, fi_hbm)

    def w_src(c):
        return w_hbm[c // 2].bitcast(U32).at[:, pl.ds(8 * (c % 2), 8), :]

    def wait(dst, k):
        pltpu.make_async_copy(dst, dst, sem.at[k]).wait()

    def x_dst(q):
        return x_v.at[:, pl.ds(pl.multiple_of(q * KQ, KQ), KQ)]

    def w0_dst(q):
        return raw4.at[0, pl.ds(pl.multiple_of(q * KQ, KQ), KQ)]

    def f_copies(h):
        return [(f_hbm[a].at[pl.ds(0, D // 2), pl.ds(128 * (8 * h + c), 128)].bitcast(U32),
                 fraw.at[h, a, c], SEM_F + h) for a in range(2) for c in range(8)]

    copies = []
    for q in range(NQ):
        copies.append((x_hbm.at[:, pl.ds(q * KQ, KQ)], x_dst(q), SEM_X + q))
        copies.append((w_src(0).at[pl.ds(q * KQ, KQ)], w0_dst(q), SEM_W0 + q))
    copies += [(gf_hbm, gf, SEM_GF), (sm_hbm, sm, SEM_SM)]
    copies += [(f_hbm[a].at[pl.ds(D // 2, 1), :], nyq.at[a], SEM_NYQ) for a in range(2)]
    copies += f_copies(0) + [(w_src(1), raw4.at[1], SEM_W + 1)] + f_copies(1) + [(gs_hbm, gs, SEM_GS)]
    copies += [(w_src(c), raw4.at[c], SEM_W + c) for c in (2, 3, 4, 5)]
    copies += [(wo_hbm.bitcast(U32).at[:, pl.ds(128 * j, 128)], wo.at[j], SEM_WO) for j in range(8)]
    copies += [(gi_hbm, gi, SEM_GI), (mem_hbm, mem_ref, SEM_MEM), (gw_hbm, gw_ref, SEM_GW)]
    for src, dst, k in copies:
        pltpu.make_async_copy(src, dst, sem.at[k]).start()

    def relayout(c, jj, d_lo, nd):
        ws = [[], []]
        for d0 in range(0, nd, 64):
            a = raw[c, pl.ds((d_lo + d0) * 8 + jj, 64, stride=8), :]
            ws[0].append(_lo_f32(a).astype(BF))
            ws[1].append(_hi_f32(a).astype(BF))
        return [jnp.concatenate(w, axis=0) for w in ws]

    def store_st(item, res):
        res = [r.reshape(NSEG, 8, 128) for r in res]
        st[item] = _as_u32(jnp.concatenate(res, axis=1).reshape(16 * NSEG, 128).astype(BF))

    def acc(h):
        return y.at[h // 8, (h // 4) % 2, pl.ds(512 * (h % 4), 512), :]

    for h in range(16):
        acc(h)[...] = jnp.zeros((512, 128), F32)

    def k_slice(q, last):
        wait(x_dst(q), SEM_X + q)
        d_lo = pl.multiple_of(q * KQ, KQ)
        cols = pl.ds(d_lo, KQ)
        for s2 in range(NSEG // 2):
            rows = jnp.concatenate([x_v[64 * s2:64 * s2 + 16, cols].astype(F32)[0:8],
                                    x_v[64 * s2 + 32:64 * s2 + 48, cols].astype(F32)[0:8]], axis=0)
            xb[8 * s2:8 * s2 + 8, cols] = _as_u32(rows.astype(BF))
        wait(w0_dst(q), SEM_W0 + q)
        for jj in range(8):
            ws = relayout(0, jj, d_lo, KQ)
            res = []
            for p in range(2):
                wqkv[2 * jj + p, pl.ds(pl.multiple_of(q * (KQ // 2), KQ // 2), KQ // 2), :] = _as_u32(ws[p])
                r = _dot(_as_bf(xb[:, cols]), ws[p]) + acc(2 * jj + p)[...]
                if last:
                    res.append(r)
                else:
                    acc(2 * jj + p)[...] = r
            if last:
                store_st(jj, res)

    def k_body(q, c):
        k_slice(q, False)
        return c

    with jax.named_scope("p0"):
        lax.fori_loop(0, NQ - 1, k_body, 0)
        k_slice(NQ - 1, True)

    wait(gf, SEM_GF)
    RB, HB = 128, 64

    def f1(i, c):
        base = pl.multiple_of(i * RB, RB)
        alt = (1 - 2 * (_lanes(16) & 1)).astype(F32).astype(BF)
        u0 = [[] for _ in range(4)]
        for h0 in range(0, RB, HB):
            pieces = []
            for a1 in range(4):
                for r in range(h0, h0 + HB, 16):
                    xs = x_v[pl.ds(base + (QS * a1 + r), 16), :].astype(F32)
                    us = _bfly8([xs[:, 128 * a:128 * a + 128] for a in range(8)])
                    pieces.append(jnp.concatenate(us, axis=1).astype(BF))
                    u0[a1].append(pieces[-1][:, :128])
            ub = jnp.concatenate(pieces, axis=0)
            if h0 + HB == RB:
                for a1 in range(4):
                    xa[pl.ds(4 * a1 + i, 1), :] = _dot_nt(alt, jnp.concatenate(u0[a1], axis=0))[0:1]
            for g in range(4):
                yy = _dot(ub[:, 256 * g:256 * g + 256], _as_bf(gf[g]))
                v = _fft([(yy[HB * a1:HB * a1 + HB, :128], yy[HB * a1:HB * a1 + HB, 128:])
                          for a1 in range(4)], -1)
                for k1 in range(4):
                    rows = pl.ds(base + (QS * k1 + h0), HB)
                    y[g, 0, rows, :] = v[k1][0]
                    y[g, 1, rows, :] = v[k1][1]
        return c

    with jax.named_scope("f1"):
        lax.fori_loop(0, QS // RB, f1, 0)

    def fprep(h, c):
        ev, od = [], []
        for r in range(8):
            wr = fraw[h, 0, c, pl.ds(r, 32, stride=8), :]
            wi = fraw[h, 1, c, pl.ds(r, 32, stride=8), :]
            ev.append((wr & jnp.uint32(0xFFFF)) | (wi << 16))
            od.append((wr >> 16) | (wi & jnp.uint32(0xFFFF0000)))
        for g, cls in enumerate(CLASSES):
            t = _transpose_u32(jnp.concatenate([(od if k % 2 else ev)[k // 2] for k in cls], axis=0))
            for q in range(128 // N1):
                row = pl.multiple_of(((8 * h + c) * (128 // N1) + q) * PITCH, 8)
                fp[g, pl.ds(row, N1), :] = t[q * N1:(q + 1) * N1]

    def nyquist():
        twc, tws = sm[0:16], sm[16:32]
        u = _dot(sm[32:64, 0:16].astype(BF), xa[...].astype(BF))
        ur, ui = u[0:16], u[16:32]
        u = jnp.concatenate([ur * twc + ui * tws, ui * twc - ur * tws], axis=1).astype(BF)
        yield
        xx = _dot(u, _as_bf(gf[4]))
        xr, xi = xx[:, :128], xx[:, 128:]
        w = (pltpu.bitcast(nyq[0].astype(F32), U32) >> 16) | pltpu.bitcast(nyq[1].astype(F32), U32)
        w = jnp.concatenate([w[:, 128 * a:128 * a + 128] for a in range(16)], axis=0)
        wt = _transpose_u32(jnp.concatenate([w] * 8, axis=0))
        blk = _lanes(16) >> 4
        wm = wt[0:16]
        for j in range(1, 8):
            wm = jnp.where(blk == j, wt[16 * j:16 * j + 16], wm)
        wr, wi = _lo_f32(wm), _hi_f32(wm)
        z = jnp.concatenate([xr * wr - xi * wi, xr * wi + xi * wr], axis=1).astype(BF)
        yield
        pp = _dot(z, _as_bf(gf[5]))
        pr, pi = pp[:, :128], pp[:, 128:]
        pp = jnp.concatenate([pr * twc - pi * tws, pi * twc + pr * tws], axis=0).astype(BF)
        yield
        cc = _dot(sm[64:80, 0:32].astype(BF), pp) * (1.0 / (S * D))
        ct[...] = jnp.concatenate([cc, jnp.zeros((112, 128), F32)], axis=0).T
        yield

    def s_mid(g, k1):
        def rows(a0, r):
            return slice(QS * k1 + N2 * a0 + r, QS * k1 + N2 * a0 + r + 8)

        us = [[] for _ in range(8)]
        for r in range(0, N2, 8):
            v = [_cmul_const((y[g, 0, rows(a0, r), :], y[g, 1, rows(a0, r), :]), a0 * k1, N1, -1)
                 for a0 in range(8)]
            v = _fft(v, -1)
            for k0 in range(8):
                us[k0].append(jnp.concatenate(v[k0], axis=0).astype(BF))
        zs = []
        for k0 in range(8):
            ka = k1 + 4 * k0
            xx = _dot(_as_bf(gs[0, ka]), jnp.concatenate(us[k0], axis=0))
            w32 = fp[g, pl.ds(ka, N2, stride=PITCH), :]
            wr, wi = _lo_f32(w32), _hi_f32(w32)
            xr, xi = xx[:N2], xx[N2:]
            zs.append(jnp.concatenate([xr * wr - xi * wi, xr * wi + xi * wr], axis=0).astype(BF))
        yield
        ps = [_dot(_as_bf(gs[1, k1 + 4 * k0]), zs[k0]) for k0 in range(8)]
        for r in range(0, N2, 8):
            v = _fft([(pp[r:r + 8], pp[N2 + r:N2 + r + 8]) for pp in ps], 1)
            for a0 in range(8):
                vr, vi = _cmul_const(v[a0], a0 * k1, N1, 1)
                y[g, 0, rows(a0, r), :] = vr
                y[g, 1, rows(a0, r), :] = vi
        yield

    def bulk(ch, jj0, n, after_dot):
        for i in range(n):
            jj = jj0 + i
            item = 8 * ch + jj
            ws = relayout(ch, jj, 0, D)
            res = []
            for p in range(2):
                wqkv[2 * item + p] = _as_u32(ws[p])
                res.append(_dot(_as_bf(xb[...]), ws[p]))
                after_dot(2 * i + p)
            store_st(item, res)

    def loop_a(h, c):
        wait(fraw.at[h], SEM_F + h)
        ny = nyquist()

        def after_dot(q):
            if q < 4:
                next(ny)
            fprep(h, q)

        bulk(1, 4 * h, 4, after_dot)
        return c

    def loop_b(g, c):
        wait(raw4.at[g + 2], SEM_W + 2 + g)
        units = [s_mid(g, k1) for k1 in range(4)]

        def after_dot(q):
            if q % 2 == 0:
                next(units[q // 4])

        bulk(g + 2, 0, 8, after_dot)
        return c

    wait(sm, SEM_SM)
    wait(nyq, SEM_NYQ)
    wait(raw4.at[1], SEM_W + 1)
    with jax.named_scope("loop_a"):
        lax.fori_loop(0, 2, loop_a, 0)
    wait(gs, SEM_GS)
    with jax.named_scope("loop_b"):
        lax.fori_loop(0, 4, loop_b, 0)
    wait(wo, SEM_WO)
    wait(gi, SEM_GI)
    wait(mem_ref, SEM_MEM)
    wait(gw_ref, SEM_GW)

    scale = DH ** -0.5

    def softmax(s, mask, fill):
        s = jnp.where(mask, s * scale, fill)
        m = jnp.max(s, axis=-1, keepdims=True)
        e = jnp.exp(s - m)
        l = jnp.sum(e, axis=-1, keepdims=True)
        return (e * (1.0 / l)).astype(BF)

    def lhs_rows(mem, seg):
        xs = x_v[pl.ds(pl.multiple_of(seg * SEG, SEG), SEG), :].astype(F32)
        return jnp.concatenate([mem, xs[8:SEG]], axis=0).astype(BF)

    def proj2(a, m, j):
        return jnp.concatenate([_dot(a, _as_bf(wqkv[H * m + 2 * j + p])).astype(BF) for p in range(2)], axis=0)

    def step(a, seg, first, mask, fill):
        R = 32 if first else 48
        qkv, ps = {}, {}
        srow = pl.multiple_of(seg * 8, 8)

        def proj(j):
            qkv[j] = [jnp.concatenate([_as_bf(qkv_s[m]) if (first and j == 0) else proj2(a, m, j),
                                       _as_bf(st[NP * m + j, pl.ds(srow, 8), :])], axis=0)
                      for m in range(3)]

        def scores(j):
            ps[j] = softmax(_dot_nt(qkv[j][0], qkv[j][1]), mask, fill)

        def pv(j):
            o = _dot(ps[j], qkv[j][2])
            for i in range(2):
                h = 2 * j + i
                if first:
                    ob = o[32 * i:32 * i + 32].astype(BF)
                    sto[h] = o[64 + 8 * i:72 + 8 * i]
                else:
                    ob = jnp.concatenate([o[32 * i:32 * i + 32], o[64 + 8 * i:72 + 8 * i], sto[h]],
                                         axis=0).astype(BF)
                obuf[h, 0:R // 2, :] = _as_u32(ob)

        def wo_part(j, h0, h1):
            og = jnp.concatenate([_as_bf(obuf[h, 0:R // 2, :]) for h in range(h0, h1)], axis=1)
            return _dot(og, _as_bf(wo[j, h0 * 64:h1 * 64, :]))

        parts = []
        for i in range(NP + 4):
            if i < NP:
                proj(i)
            else:
                parts.append(wo_part(2 * (i - NP), 0, SPLIT))
                parts.append(wo_part(2 * (i - NP) + 1, 0, SPLIT))
            if 0 <= i - LAG1 < NP:
                scores(i - LAG1)
            if 0 <= i - LAG2 < NP:
                pv(i - LAG2)
        return jnp.concatenate([wo_part(j, SPLIT, H) + parts[j] for j in range(8)], axis=1)

    def start_pair(mem, t):
        a = lhs_rows(mem, 2 * t)
        a_s[...] = _as_u32(a)
        for m in range(3):
            qkv_s[m] = _as_u32(proj2(a, m, 0))

    def pair(t, c):
        mask, fill = _mask80()
        base = pl.multiple_of(t * 64, 64)
        lane = _lanes(64)
        lo = lane < 64
        roll = lambda v: pltpu.roll(v, 64, 1)
        a1 = t // 8
        off = pl.multiple_of((t % 8) * 64, 64)
        s2 = (1 - 2 * (a1 & 1)).astype(F32)
        sg = (1 - (a1 & 2)).astype(F32)
        cc, ss = sg * (1 - (a1 & 1)).astype(F32), sg * (a1 & 1).astype(F32)

        def irfft_group(g):
            q = [[y[g, e, pl.ds(off + QS * k1, 64), :] for e in range(2)] for k1 in range(4)]
            br, bi = q[1][0] + s2 * q[3][0], q[1][1] + s2 * q[3][1]
            vr = q[0][0] + s2 * q[2][0] + (cc * br - ss * bi)
            vi = q[0][1] + s2 * q[2][1] + (cc * bi + ss * br)
            tin = _half_pre(vr, vi, lo, roll, jnp.where)
            tp, tm = [_dot(tin[e].astype(BF), _as_bf(gi[2 * g + e])) for e in range(2)]
            return list(_half_post(g, tp, tm, lo, roll, jnp.where))

        res_a = step(_as_bf(a_s[...]), 2 * t, True, mask, fill)
        ts = irfft_group(0) + irfft_group(1)
        ra_s[...] = res_a[8:32]
        a = lhs_rows(res_a[0:8].astype(BF).astype(F32), 2 * t + 1)
        res_b = step(a, 2 * t + 1, False, mask, fill)
        ts += irfft_group(2) + irfft_group(3)
        start_pair(res_b[0:8].astype(BF).astype(F32), jnp.minimum(t + 1, S // 64 - 1))

        nyc = jnp.sum(jnp.where(lane == t // 2, ct[pl.ds(pl.multiple_of((t % 2) * 64, 64), 64), :], 0.0),
                      axis=-1, keepdims=True)
        ts[0] = ts[0] + nyc * (1 - 2 * (lane & 1)).astype(F32)
        b = jnp.concatenate(_bfly8_t(ts), axis=1).astype(BF).astype(F32)
        xs = x_v[pl.ds(base, 64), :].astype(F32)
        gate = jax.nn.sigmoid(jnp.sum(xs * gw_ref[...].astype(F32), axis=-1, keepdims=True))
        res = jnp.concatenate([res_b[40:48], ra_s[...], res_b[32:40], res_b[8:32]], axis=0)
        out_v[pl.ds(base, 64), :] = (gate * res + (1.0 - gate) * b).astype(BF)
        pltpu.make_async_copy(out_v.at[pl.ds(base, 64), :], out_hbm.at[pl.ds(base, 64), :],
                              sem.at[SEM_OUT]).start()
        return c

    with jax.named_scope("chain"):
        start_pair(mem_ref[...].astype(F32), 0)
        lax.fori_loop(0, S // 64, pair, 0)
    pltpu.make_async_copy(out_v, out_hbm, sem.at[SEM_OUT]).wait()


@functools.partial(jax.jit, static_argnames=("A_seg_len",))
def pallas_gated_mix__memory_aug_recurrent_mem_tr__spectral_gfnet__prompt_kernel(
    A_x, A_mem0, A_Wq, A_Wk, A_Wv, A_Wo, A_seg_len, B_x, B_w_r, B_w_i, gate_w,
):
    assert A_x.shape == (1, S, D) and A_mem0.shape == (1, M, D) and A_Wq.shape == (D, H, DH)
    assert int(A_seg_len) == SEG
    consts = [jnp.asarray(c) for c in _constants()]
    any_spec = pl.BlockSpec(memory_space=pl.ANY)
    out = pl.pallas_call(
        _kernel,
        out_shape=jax.ShapeDtypeStruct((S, D), BF),
        in_specs=[any_spec] * 13,
        out_specs=any_spec,
        scratch_shapes=[
            pltpu.VMEM((S, D), BF),
            pltpu.VMEM((6, D * 8, DH), U32),
            pltpu.VMEM((3 * H, D // 2, DH), U32),
            pltpu.VMEM((8, H * DH // 2, 128), U32),
            pltpu.VMEM((3 * NP, 8 * NSEG, 128), U32),
            pltpu.VMEM((H, 8, 128), F32),
            pltpu.VMEM((H, 24, 128), U32),
            pltpu.VMEM((4 * NSEG, D), U32),
            pltpu.VMEM((2, 2, 8, 256, 128), U32),
            pltpu.VMEM((4, N2 * PITCH, 128), U32),
            pltpu.VMEM((6, 128, 256), U32),
            pltpu.VMEM((8, 64, 128), U32),
            pltpu.VMEM((80, 128), F32),
            pltpu.VMEM((2, N1, N2, 2 * N2), U32),
            pltpu.VMEM((4, 2, S, 128), F32),
            pltpu.VMEM((S, D), BF),
            pltpu.VMEM((M, D), BF),
            pltpu.VMEM((1, D), BF),
            pltpu.VMEM((2, 1, S), BF),
            pltpu.VMEM((16, 128), F32),
            pltpu.VMEM((128, 128), F32),
            pltpu.VMEM((16, D), U32),
            pltpu.VMEM((3, 32, 128), U32),
            pltpu.VMEM((24, D), F32),
            pltpu.SemaphoreType.DMA((NSEM,)),
        ],
        compiler_params=pltpu.CompilerParams(vmem_limit_bytes=120 * 1024 * 1024),
    )(
        A_x.reshape(S, D), A_mem0.reshape(M, D), A_Wq, A_Wk, A_Wv,
        A_Wo.reshape(H * DH, D), B_w_r.T, B_w_i.T, gate_w.reshape(1, D), *consts,
    )
    return out.reshape(1, S, D)
```

```python
import functools
import math
import os

import numpy as np
import jax
import jax.numpy as jnp
from jax import lax
import jax.experimental.pallas as pl
import jax.experimental.pallas.tpu as pltpu

BF, F32, U32 = jnp.bfloat16, jnp.float32, jnp.uint32

S, D, H, DH, M, SEG = 2048, 1024, 32, 128, 8, 32
NSEG = S // SEG
NP = H // 2
N1, N2 = 32, 64
QS = S // 4
PITCH = N1 + 8
CLASSES = ((0, 8, 4, 12), (1, 15, 9, 7), (2, 14, 10, 6), (3, 13, 11, 5))
_E = lambda k, d: int(os.environ.get(k, d))
LAG1, LAG2, SPLIT = _E("LAG1", 1), _E("LAG2", 2), _E("SPLIT", 28)
HOOK_AT = _E("HOOK_AT", 17)
ONLY = os.environ.get("ONLY", "")
KSPLIT = _E("KSPLIT", 1)
NOSPEC = _E("NOSPEC", 0)
STAGE = os.environ.get("STAGE", "")
ORDER = os.environ.get("ORDER", "vqskp")
DMAPOS = _E("DMAPOS", 0)
NQ = 4
(SEM_W, SEM_GF, SEM_GI, SEM_SM, SEM_GS, SEM_F, SEM_NYQ, SEM_WO, SEM_MEM, SEM_GW, SEM_OUT,
 SEM_X) = 0, 6, 7, 8, 9, 10, 12, 13, 14, 15, 16, 17
SEM_W0 = SEM_X + NQ
NSEM = SEM_W0 + NQ
RSQ2 = float(np.float32(math.sqrt(0.5)))


def _bfly8(x):
    s = [x[i] + x[i + 4] for i in range(4)]
    d = [x[i] - x[i + 4] for i in range(4)]
    e, f = s[0] + s[2], s[1] + s[3]
    t1, t2 = (d[1] - d[3]) * RSQ2, (d[1] + d[3]) * RSQ2
    return [e + f, e - f, d[0] + t1, t2 + d[2], s[0] - s[2], s[1] - s[3], d[0] - t1, t2 - d[2]]


def _bfly8_t(t):
    e, f = t[0] + t[1], t[0] - t[1]
    s = [e + t[4], f + t[5], e - t[4], f - t[5]]
    t1, t2 = t[2] - t[6], t[3] + t[7]
    d = [t[2] + t[6], (t1 + t2) * RSQ2, t[3] - t[7], (t2 - t1) * RSQ2]
    return [s[i] + d[i] for i in range(4)] + [s[i] - d[i] for i in range(4)]


def _half_pre(vr, vi, lo, roll, where):
    ri = roll(vi)
    return where(lo, vr, ri), where(lo, ri, vr)


def _half_post(g, tp, tm, lo, roll, where):
    if g == 0:
        return tp, tm
    c = float(np.float32(math.cos(math.pi * g / 8)))
    s = float(np.float32(math.sin(math.pi * g / 8)))
    p, r = tp + tm, tp - tm
    rm = roll(where(lo, r, p))
    return where(lo, p, c * rm + s * r), where(lo, rm, c * r - s * rm)


def _cmul_const(v, k, n, sign):
    re, im = v
    k %= n
    if k == 0:
        return re, im
    if 4 * k == n:
        return (-im, re) if sign > 0 else (im, -re)
    if 8 * k == n:
        return (((re - im) * RSQ2, (re + im) * RSQ2) if sign > 0
                else ((re + im) * RSQ2, (im - re) * RSQ2))
    if 8 * k == 3 * n:
        return (((re + im) * -RSQ2, (re - im) * RSQ2) if sign > 0
                else ((im - re) * RSQ2, (re + im) * -RSQ2))
    c, s = math.cos(2 * math.pi * k / n), sign * math.sin(2 * math.pi * k / n)
    return re * c - im * s, re * s + im * c


def _fft(v, sign):
    n = len(v)
    if n == 1:
        return v
    ev, od = _fft(v[0::2], sign), _fft(v[1::2], sign)
    lo, hi = [], []
    for k in range(n // 2):
        er, ei = ev[k]
        if 4 * k == n:
            xr, xi = od[k]
            if sign > 0:
                lo.append((er - xi, ei + xr)); hi.append((er + xi, ei - xr))
            else:
                lo.append((er + xi, ei - xr)); hi.append((er - xi, ei + xr))
            continue
        tr, ti = _cmul_const(od[k], k, n, sign)
        lo.append((er + tr, ei + ti))
        hi.append((er - tr, ei - ti))
    return lo + hi


def _pack_rows(a):
    u = np.ascontiguousarray(a, dtype=np.float32).view(np.uint32)
    b = ((u + 0x7FFF + ((u >> 16) & 1)) >> 16).astype(np.uint32)
    return (b[..., 0::2, :] | (b[..., 1::2, :] << 16)).astype(np.uint32)


def _diag_blocks(full, n, tol):
    k = full.shape[0] // n
    blk = np.kron(np.eye(k), np.ones((n, n)))
    assert np.abs(full * (1 - blk)).max() < tol
    return np.stack([full[n * g:n * g + n, n * g:n * g + n] for g in range(k)])


def _cplx(re, im):
    return np.block([[re, im], [-im, re]])


@functools.lru_cache(maxsize=None)
def _constants():
    k2 = np.stack([np.concatenate([c + 16 * np.arange(32) for c in cls]) for cls in CLASSES])
    n2 = np.arange(D)
    ang = 2 * np.pi * ((k2[:, :, None] * n2[None, None, :]) % D) / D
    rows = np.stack([np.cos(ang), -np.sin(ang)], axis=1)
    wgt = np.where(k2 == 0, 1.0, 2.0)[:, None, :, None]
    fwd = rows.reshape(D, D).T
    inv = (rows * wgt).reshape(D, D) / (S * D)
    bf = np.stack(_bfly8(list(np.eye(8))))
    binv = np.kron(np.linalg.inv(bf), np.eye(128))
    gd = _diag_blocks(binv.T @ fwd, 256, 1e-6)
    gdi = _diag_blocks(inv @ binv, 256, 1e-12)
    eye, lo = np.eye(256), np.arange(128) < 64
    roll = lambda v: np.roll(v, 64, axis=1)
    pre = np.concatenate(_half_pre(eye[:, :128], eye[:, 128:], lo, roll, np.where), axis=1)
    gi = []
    for g in range(4):
        post = np.concatenate(_half_post(g, eye[:, :128], eye[:, 128:], lo, roll, np.where), axis=1)
        gi.append(_diag_blocks(np.linalg.inv(pre) @ gdi[g] @ np.linalg.inv(post), 128, 1e-12))
    gi = np.concatenate(gi)

    b = np.arange(N2)
    k1 = np.arange(N1)[:, None] + N1 * np.arange(N2)[None, :]
    th = 2 * np.pi * ((k1[:, :, None] * b[None, None, :]) % S) / S
    gr, gim = np.cos(th), -np.sin(th)
    full = np.block([[gr, -gim], [gim, gr]])
    kap = np.arange(2 * N2)
    src = ((kap >> 3) & 1) * N2 + (kap >> 4) * 8 + (kap & 7)
    gs = full[:, :, src]
    hr, hi = np.swapaxes(gr, 1, 2), -np.swapaxes(gim, 1, 2)
    gsi = np.block([[hr, -hi], [hi, hr]])

    lane = np.arange(128)
    kb = 8 * (lane % 16) + lane // 16
    t128 = 2 * np.pi * ((lane[:, None] * kb[None, :]) % 128) / 128
    nyf = _cplx(np.cos(t128), -np.sin(t128))
    nyi = _cplx(np.cos(t128).T, np.sin(t128).T)
    i16 = np.arange(16)
    t16 = 2 * np.pi * ((i16[:, None] * i16[None, :]) % 16) / 16
    tw = 2 * np.pi * (i16[:, None] * lane[None, :]) / S
    sm = np.zeros((80, 128), np.float32)
    sm[0:16], sm[16:32] = np.cos(tw), np.sin(tw)
    sm[32:48, :16], sm[48:64, :16] = np.cos(t16), -np.sin(t16)
    sm[64:80, :16], sm[64:80, 16:32] = np.cos(t16), -np.sin(t16)

    gfp = _pack_rows(np.concatenate([gd, nyf[None], nyi[None]]))
    return gfp, _pack_rows(gi), sm, _pack_rows(np.stack([gs, gsi]))


def _mask80():
    r = lax.broadcasted_iota(jnp.int32, (80, 80), 0)
    c = lax.broadcasted_iota(jnp.int32, (80, 80), 1)

    def head(i):
        return jnp.where(i < 64, i >> 5, (i - 64) >> 3)

    def pos(i):
        j = i & 31
        return jnp.where(i < 64, jnp.where(j < M, j, j + 8), M + (i & 7))

    same = head(r) == head(c)
    ok = (pos(r) < M) | (pos(c) <= pos(r))
    return jnp.where(same, jnp.where(ok, 1.0, -1e9), -jnp.inf).astype(F32)


def _as_bf(u):
    return pltpu.bitcast(u, BF)


def _as_u32(b):
    return pltpu.bitcast(b, U32)


def _lo_f32(u):
    return pltpu.bitcast(u << 16, F32)


def _hi_f32(u):
    return pltpu.bitcast(u & jnp.uint32(0xFFFF0000), F32)


def _dot(a, b):
    return jnp.dot(a, b, preferred_element_type=F32)


def _dot_nt(a, b):
    return lax.dot_general(a, b, (((1,), (1,)), ((), ())), preferred_element_type=F32)


def _transpose_u32(u):
    return pltpu.bitcast(pltpu.bitcast(u, F32).T, U32)


def _lanes(rows):
    return lax.broadcasted_iota(jnp.int32, (rows, 128), 1)


def _kernel(x_hbm, mem_hbm, wq_hbm, wk_hbm, wv_hbm, wo_hbm, fr_hbm, fi_hbm, gw_hbm,
            gf_hbm, gi_hbm, sm_hbm, gs_hbm,
            out_hbm,
            x_v, raw, wqkv, wo, st, sto, obuf, xb, fraw, fp, gf, gi, sm, gs, y, out_v, mem_ref, gw_ref,
            nyq, xa, ct, a_s, qkv_s, bb_s, g_s, stg, pst, mf, sem):
    KQ = D // NQ
    raw4 = raw.reshape(6, D, 8, DH)
    w_hbm = (wq_hbm, wk_hbm, wv_hbm)
    f_hbm = (fr_hbm, fi_hbm)

    def w_src(c):
        return w_hbm[c // 2].bitcast(U32).at[:, pl.ds(8 * (c % 2), 8), :]

    def wait(dst, k):
        pltpu.make_async_copy(dst, dst, sem.at[k]).wait()

    def x_dst(q):
        return x_v.at[:, pl.ds(pl.multiple_of(q * KQ, KQ), KQ)]

    def w0_dst(q):
        return raw4.at[0, pl.ds(pl.multiple_of(q * KQ, KQ), KQ)]

    def f_copies(h):
        return [(f_hbm[a].at[pl.ds(0, D // 2), pl.ds(128 * (8 * h + c), 128)].bitcast(U32),
                 fraw.at[h, a, c], SEM_F + h) for a in range(2) for c in range(8)]

    copies = []
    for q in range(NQ):
        copies.append((x_hbm.at[:, pl.ds(q * KQ, KQ)], x_dst(q), SEM_X + q))
        copies.append((w_src(0).at[pl.ds(q * KQ, KQ)], w0_dst(q), SEM_W0 + q))
    copies += [(gf_hbm, gf, SEM_GF), (sm_hbm, sm, SEM_SM)]
    copies += [(f_hbm[a].at[pl.ds(D // 2, 1), :], nyq.at[a], SEM_NYQ) for a in range(2)]
    copies += f_copies(0) + [(w_src(1), raw4.at[1], SEM_W + 1)] + f_copies(1) + [(gs_hbm, gs, SEM_GS)]
    copies += [(w_src(c), raw4.at[c], SEM_W + c) for c in (2, 3, 4, 5)]
    copies += [(wo_hbm.bitcast(U32).at[:, pl.ds(128 * j, 128)], wo.at[j], SEM_WO) for j in range(8)]
    copies += [(gi_hbm, gi, SEM_GI), (mem_hbm, mem_ref, SEM_MEM), (gw_hbm, gw_ref, SEM_GW)]
    for src, dst, k in copies:
        pltpu.make_async_copy(src, dst, sem.at[k]).start()

    def relayout(c, jj, d_lo, nd):
        ws = [[], []]
        for d0 in range(0, nd, 64):
            a = raw[c, pl.ds((d_lo + d0) * 8 + jj, 64, stride=8), :]
            ws[0].append(_lo_f32(a).astype(BF))
            ws[1].append(_hi_f32(a).astype(BF))
        return [jnp.concatenate(w, axis=0) for w in ws]

    def store_st(item, res):
        res = [r.reshape(NSEG, 8, 128) for r in res]
        st[item] = _as_u32(jnp.concatenate(res, axis=1).reshape(16 * NSEG, 128).astype(BF))

    def acc(h):
        return y.at[h // 8, (h // 4) % 2, pl.ds(512 * (h % 4), 512), :]

    for h in range(16):
        acc(h)[...] = jnp.zeros((512, 128), F32)

    def k_slice(q, last):
        wait(x_dst(q), SEM_X + q)
        d_lo = pl.multiple_of(q * KQ, KQ)
        cols = pl.ds(d_lo, KQ)
        for s2 in range(NSEG // 2):
            rows = jnp.concatenate([x_v[64 * s2:64 * s2 + 16, cols].astype(F32)[0:8],
                                    x_v[64 * s2 + 32:64 * s2 + 48, cols].astype(F32)[0:8]], axis=0)
            xb[8 * s2:8 * s2 + 8, cols] = _as_u32(rows.astype(BF))
        wait(w0_dst(q), SEM_W0 + q)
        for jj in range(8):
            ws = relayout(0, jj, d_lo, KQ)
            res = []
            for p in range(2):
                wqkv[2 * jj + p, pl.ds(pl.multiple_of(q * (KQ // 2), KQ // 2), KQ // 2), :] = _as_u32(ws[p])
                r = _dot(_as_bf(xb[:, cols]), ws[p]) + acc(2 * jj + p)[...]
                if last:
                    res.append(r)
                else:
                    acc(2 * jj + p)[...] = r
            if last:
                store_st(jj, res)

    def k_body(q, c):
        k_slice(q, False)
        return c

    with jax.named_scope("p0"):
        if ONLY in ("", "p0"):
            lax.fori_loop(0, NQ - 1, k_body, 0)
            k_slice(NQ - 1, True)
        else:
            for q in range(NQ):
                wait(x_dst(q), SEM_X + q)
                wait(w0_dst(q), SEM_W0 + q)

    wait(gf, SEM_GF)
    RB, HB = 128, 64

    def f1(i, c):
        base = pl.multiple_of(i * RB, RB)
        alt = (1 - 2 * (_lanes(16) & 1)).astype(F32).astype(BF)
        u0 = [[] for _ in range(4)]
        for h0 in range(0, RB, HB):
            pieces = []
            for a1 in range(4):
                for r in range(h0, h0 + HB, 16):
                    xs = x_v[pl.ds(base + (QS * a1 + r), 16), :].astype(F32)
                    us = _bfly8([xs[:, 128 * a:128 * a + 128] for a in range(8)])
                    pieces.append(jnp.concatenate(us, axis=1).astype(BF))
                    u0[a1].append(pieces[-1][:, :128])
            ub = jnp.concatenate(pieces, axis=0)
            if h0 + HB == RB:
                for a1 in range(4):
                    xa[pl.ds(4 * a1 + i, 1), :] = _dot_nt(alt, jnp.concatenate(u0[a1], axis=0))[0:1]
            for g in range(4):
                yy = _dot(ub[:, 256 * g:256 * g + 256], _as_bf(gf[g]))
                v = _fft([(yy[HB * a1:HB * a1 + HB, :128], yy[HB * a1:HB * a1 + HB, 128:])
                          for a1 in range(4)], -1)
                for k1 in range(4):
                    rows = pl.ds(base + (QS * k1 + h0), HB)
                    y[g, 0, rows, :] = v[k1][0]
                    y[g, 1, rows, :] = v[k1][1]
        return c

    with jax.named_scope("f1"):
        if ONLY in ("", "f1"):
            lax.fori_loop(0, QS // RB, f1, 0)

    def fprep(h, c):
        ev, od = [], []
        for r in range(8):
            wr = fraw[h, 0, c, pl.ds(r, 32, stride=8), :]
            wi = fraw[h, 1, c, pl.ds(r, 32, stride=8), :]
            ev.append((wr & jnp.uint32(0xFFFF)) | (wi << 16))
            od.append((wr >> 16) | (wi & jnp.uint32(0xFFFF0000)))
        for g, cls in enumerate(CLASSES):
            t = _transpose_u32(jnp.concatenate([(od if k % 2 else ev)[k // 2] for k in cls], axis=0))
            for q in range(128 // N1):
                row = pl.multiple_of(((8 * h + c) * (128 // N1) + q) * PITCH, 8)
                fp[g, pl.ds(row, N1), :] = t[q * N1:(q + 1) * N1]

    def nyquist():
        twc, tws = sm[0:16], sm[16:32]
        u = _dot(sm[32:64, 0:16].astype(BF), xa[...].astype(BF))
        ur, ui = u[0:16], u[16:32]
        u = jnp.concatenate([ur * twc + ui * tws, ui * twc - ur * tws], axis=1).astype(BF)
        yield
        xx = _dot(u, _as_bf(gf[4]))
        xr, xi = xx[:, :128], xx[:, 128:]
        w = (pltpu.bitcast(nyq[0].astype(F32), U32) >> 16) | pltpu.bitcast(nyq[1].astype(F32), U32)
        w = jnp.concatenate([w[:, 128 * a:128 * a + 128] for a in range(16)], axis=0)
        wt = _transpose_u32(jnp.concatenate([w] * 8, axis=0))
        blk = _lanes(16) >> 4
        wm = wt[0:16]
        for j in range(1, 8):
            wm = jnp.where(blk == j, wt[16 * j:16 * j + 16], wm)
        wr, wi = _lo_f32(wm), _hi_f32(wm)
        z = jnp.concatenate([xr * wr - xi * wi, xr * wi + xi * wr], axis=1).astype(BF)
        yield
        pp = _dot(z, _as_bf(gf[5]))
        pr, pi = pp[:, :128], pp[:, 128:]
        pp = jnp.concatenate([pr * twc - pi * tws, pi * twc + pr * tws], axis=0).astype(BF)
        yield
        cc = _dot(sm[64:80, 0:32].astype(BF), pp) * (1.0 / (S * D))
        ct[...] = jnp.concatenate([cc, jnp.zeros((112, 128), F32)], axis=0).T
        yield

    def s_mid(g, k1):
        def rows(a0, r):
            return slice(QS * k1 + N2 * a0 + r, QS * k1 + N2 * a0 + r + 8)

        us = [[] for _ in range(8)]
        for r in range(0, N2, 8):
            v = [_cmul_const((y[g, 0, rows(a0, r), :], y[g, 1, rows(a0, r), :]), a0 * k1, N1, -1)
                 for a0 in range(8)]
            v = _fft(v, -1)
            for k0 in range(8):
                us[k0].append(jnp.concatenate(v[k0], axis=0).astype(BF))
        zs = []
        for k0 in range(8):
            ka = k1 + 4 * k0
            xx = _dot(_as_bf(gs[0, ka]), jnp.concatenate(us[k0], axis=0))
            w32 = fp[g, pl.ds(ka, N2, stride=PITCH), :]
            wr, wi = _lo_f32(w32), _hi_f32(w32)
            xr, xi = xx[:N2], xx[N2:]
            zs.append(jnp.concatenate([xr * wr - xi * wi, xr * wi + xi * wr], axis=0).astype(BF))
        yield
        ps = [_dot(_as_bf(gs[1, k1 + 4 * k0]), zs[k0]) for k0 in range(8)]
        for r in range(0, N2, 8):
            v = _fft([(pp[r:r + 8], pp[N2 + r:N2 + r + 8]) for pp in ps], 1)
            for a0 in range(8):
                vr, vi = _cmul_const(v[a0], a0 * k1, N1, 1)
                y[g, 0, rows(a0, r), :] = vr
                y[g, 1, rows(a0, r), :] = vi
        yield

    def bulk(ch, jj0, n, after_dot):
        for i in range(n):
            jj = jj0 + i
            item = 8 * ch + jj
            ws = relayout(ch, jj, 0, D)
            res = []
            for p in range(2):
                wqkv[2 * item + p] = _as_u32(ws[p])
                res.append(_dot(_as_bf(xb[...]), ws[p]))
                after_dot(2 * i + p)
            store_st(item, res)

    def loop_a(h, c):
        wait(fraw.at[h], SEM_F + h)
        ny = nyquist()

        def after_dot(q):
            if q < 4:
                next(ny)
            fprep(h, q)

        bulk(1, 4 * h, 4, after_dot)
        return c

    def loop_b(g, c):
        wait(raw4.at[g + 2], SEM_W + 2 + g)
        units = [s_mid(g, k1) for k1 in range(4)]

        def after_dot(q):
            if q % 2 == 0:
                next(units[q // 4])

        bulk(g + 2, 0, 8, after_dot)
        return c

    wait(sm, SEM_SM)
    wait(nyq, SEM_NYQ)
    wait(raw4.at[1], SEM_W + 1)
    with jax.named_scope("loop_a"):
        if ONLY in ("", "a"):
            lax.fori_loop(0, 2, loop_a, 0)
        else:
            wait(fraw.at[0], SEM_F)
            wait(fraw.at[1], SEM_F + 1)
    wait(gs, SEM_GS)
    with jax.named_scope("loop_b"):
        if ONLY in ("", "b"):
            lax.fori_loop(0, 4, loop_b, 0)
        else:
            for g in range(4):
                wait(raw4.at[g + 2], SEM_W + 2 + g)
    wait(wo, SEM_WO)
    wait(gi, SEM_GI)
    wait(mem_ref, SEM_MEM)
    wait(gw_ref, SEM_GW)

    scale = DH ** -0.5

    mf[...] = _mask80()

    def softmax(s):
        fill = mf[...]
        s = jnp.where(fill > 0.0, s * scale, fill)
        m = jnp.max(s, axis=-1, keepdims=True)
        e = jnp.exp(s - m)
        l = jnp.sum(e, axis=-1, keepdims=True)
        return (e * (1.0 / l)).astype(BF)

    def lhs_rows(mem, seg):
        xs = x_v[pl.ds(pl.multiple_of(seg * SEG, SEG), SEG), :].astype(F32)
        return jnp.concatenate([mem, xs[8:SEG]], axis=0).astype(BF)

    def proj2(a, m, j):
        return jnp.concatenate([_dot(a, _as_bf(wqkv[H * m + 2 * j + p])).astype(BF) for p in range(2)], axis=0)

    def proj_first(a):
        if not KSPLIT:
            return [proj2(a, m, 0) for m in range(3)]
        part = [_dot(a[:, :D // 2], _as_bf(wqkv[H * (i // 2) + i % 2, 0:D // 4, :])) for i in range(6)]
        full = [(_dot(a[:, D // 2:], _as_bf(wqkv[H * (i // 2) + i % 2, D // 4:D // 2, :])) + part[i]).astype(BF)
                for i in range(6)]
        return [jnp.concatenate(full[2 * m:2 * m + 2], axis=0) for m in range(3)]

    def step(a, seg, first, hook=None):
        R = 32 if first else 48
        qkv, ps = {}, {}
        srow = pl.multiple_of(seg * 8, 8)

        def put(m, j, r):
            if "qkv"[m] in STAGE:
                stg[m, j % 8] = _as_u32(r)
            else:
                qkv[m, j] = r

        def get(m, j):
            r = _as_bf(stg[m, j % 8]) if "qkv"[m] in STAGE else qkv[m, j]
            return jnp.concatenate([r, _as_bf(st[NP * m + j, pl.ds(srow, 8), :])], axis=0)

        def proj(j, m):
            if j == 0:
                if m == 0:
                    r = [_as_bf(qkv_s[m]) for m in range(3)] if first else proj_first(a)
                    for mm in range(3):
                        put(mm, 0, r[mm])
            else:
                put(m, j, proj2(a, m, j))

        def scores(j):
            pp = softmax(_dot_nt(get(0, j), get(1, j)))
            if "p" in STAGE:
                pst[j % 8] = _as_u32(pp)
            else:
                ps[j] = pp

        def pv(j):
            o = _dot(_as_bf(pst[j % 8]) if "p" in STAGE else ps[j], get(2, j))
            for i in range(2):
                h = 2 * j + i
                if first:
                    ob = o[32 * i:32 * i + 32].astype(BF)
                    sto[h] = o[64 + 8 * i:72 + 8 * i]
                else:
                    ob = jnp.concatenate([o[32 * i:32 * i + 32], o[64 + 8 * i:72 + 8 * i], sto[h]],
                                         axis=0).astype(BF)
                obuf[h, 0:R // 2, :] = _as_u32(ob)

        def wo_part(j, h0, h1):
            og = jnp.concatenate([_as_bf(obuf[h, 0:R // 2, :]) for h in range(h0, h1)], axis=1)
            return _dot(og, _as_bf(wo[j, h0 * 64:h1 * 64, :]))

        parts = []
        for i in range(NP + 4):
            for ch in ORDER:
                if ch in "qkv":
                    m = "qkv".index(ch)
                    if i < NP:
                        proj(i, m)
                    elif m < 2:
                        parts.append(wo_part(2 * (i - NP) + len(parts) % 2, 0, SPLIT))
                elif ch == "s" and 0 <= i - LAG1 < NP:
                    scores(i - LAG1)
                elif ch == "p" and 0 <= i - LAG2 < NP:
                    pv(i - LAG2)
            if hook is not None and i == HOOK_AT:
                hook()
        return jnp.concatenate([wo_part(j, SPLIT, H) + parts[j] for j in range(8)], axis=1)

    def start_pair(mem, t):
        a = lhs_rows(mem, 2 * t)
        a_s[...] = _as_u32(a)
        for m, r in enumerate(proj_first(a)):
            qkv_s[m] = _as_u32(r)

    def pair(t, c):
        base = pl.multiple_of(t * 64, 64)
        lane = _lanes(64)
        lo = lane < 64
        roll = (lambda v: v + 1.0) if _E('NOROLL', 0) else (lambda v: pltpu.roll(v, 64, 1))
        a1 = t // 8
        off = pl.multiple_of((t % 8) * 64, 64)
        s2 = (1 - 2 * (a1 & 1)).astype(F32)
        sg = (1 - (a1 & 2)).astype(F32)
        cc, ss = sg * (1 - (a1 & 1)).astype(F32), sg * (a1 & 1).astype(F32)

        def irfft_group(g):
            q = [[y[g, e, pl.ds(off + QS * k1, 64), :] for e in range(2)] for k1 in range(4)]
            br, bi = q[1][0] + s2 * q[3][0], q[1][1] + s2 * q[3][1]
            vr = q[0][0] + s2 * q[2][0] + (cc * br - ss * bi)
            vi = q[0][1] + s2 * q[2][1] + (cc * bi + ss * br)
            tin = _half_pre(vr, vi, lo, roll, jnp.where)
            tp, tm = [_dot(tin[e].astype(BF), _as_bf(gi[2 * g + e])) for e in range(2)]
            if g == 0:
                nyc = jnp.sum(jnp.where(lane == t // 2,
                                        ct[pl.ds(pl.multiple_of((t % 2) * 64, 64), 64), :], 0.0),
                              axis=-1, keepdims=True)
                tp = tp + nyc * (1 - 2 * (lane & 1)).astype(F32)
            return list(_half_post(g, tp, tm, lo, roll, jnp.where))

        def spectral_part():
            ts = sum([irfft_group(g) for g in range(4)], [])
            b = jnp.concatenate(_bfly8_t(ts), axis=1).astype(BF).astype(F32)
            xs = x_v[pl.ds(base, 64), :].astype(F32)
            gate = jax.nn.sigmoid(jnp.sum(xs * gw_ref[...].astype(F32), axis=-1, keepdims=True))
            bb = (1.0 - gate) * b
            bb_s[...] = jnp.concatenate([bb[0:8], bb[8:32] + gate[8:32] * bb_s[8:32], bb[32:64]], axis=0)
            g_s[...] = jnp.broadcast_to(gate, (64, 128))

        res_a = step(_as_bf(a_s[...]), 2 * t, True)
        bb_s[8:32] = res_a[8:32]
        a = lhs_rows(res_a[0:8].astype(BF).astype(F32), 2 * t + 1)
        res_b = step(a, 2 * t + 1, False, None if NOSPEC else spectral_part)

        def gated(r0, r1, res):
            return bb_s[r0:r1] + jnp.concatenate([g_s[r0:r1]] * 8, axis=1) * res

        out_v[pl.ds(base, 64), :] = jnp.concatenate(
            [gated(0, 8, res_b[40:48]), bb_s[8:32], gated(32, 40, res_b[32:40]), gated(40, 64, res_b[8:32])],
            axis=0).astype(BF)
        cp = pltpu.make_async_copy(out_v.at[pl.ds(base, 64), :], out_hbm.at[pl.ds(base, 64), :],
                                   sem.at[SEM_OUT])
        if DMAPOS == 0:
            cp.start()
        start_pair(res_b[0:8].astype(BF).astype(F32), jnp.minimum(t + 1, S // 64 - 1))
        if DMAPOS == 1:
            cp.start()
        return c

    with jax.named_scope("chain"):
        if ONLY in ("", "chain"):
            start_pair(mem_ref[...].astype(F32), 0)
            lax.fori_loop(0, S // 64, pair, 0)
            if DMAPOS == 2:
                pltpu.make_async_copy(out_v, out_hbm, sem.at[SEM_OUT]).start()
    with jax.named_scope("fin"):
        if ONLY in ("", "chain"):
            pltpu.make_async_copy(out_v, out_hbm, sem.at[SEM_OUT]).wait()


@functools.partial(jax.jit, static_argnames=("A_seg_len",))
def pallas_gated_mix__memory_aug_recurrent_mem_tr__spectral_gfnet__prompt_kernel(
    A_x, A_mem0, A_Wq, A_Wk, A_Wv, A_Wo, A_seg_len, B_x, B_w_r, B_w_i, gate_w,
):
    assert A_x.shape == (1, S, D) and A_mem0.shape == (1, M, D) and A_Wq.shape == (D, H, DH)
    assert int(A_seg_len) == SEG
    consts = [jnp.asarray(c) for c in _constants()]
    any_spec = pl.BlockSpec(memory_space=pl.ANY)
    out = pl.pallas_call(
        _kernel,
        out_shape=jax.ShapeDtypeStruct((S, D), BF),
        in_specs=[any_spec] * 13,
        out_specs=any_spec,
        scratch_shapes=[
            pltpu.VMEM((S, D), BF),
            pltpu.VMEM((6, D * 8, DH), U32),
            pltpu.VMEM((3 * H, D // 2, DH), U32),
            pltpu.VMEM((8, H * DH // 2, 128), U32),
            pltpu.VMEM((3 * NP, 8 * NSEG, 128), U32),
            pltpu.VMEM((H, 8, 128), F32),
            pltpu.VMEM((H, 24, 128), U32),
            pltpu.VMEM((4 * NSEG, D), U32),
            pltpu.VMEM((2, 2, 8, 256, 128), U32),
            pltpu.VMEM((4, N2 * PITCH, 128), U32),
            pltpu.VMEM((6, 128, 256), U32),
            pltpu.VMEM((8, 64, 128), U32),
            pltpu.VMEM((80, 128), F32),
            pltpu.VMEM((2, N1, N2, 2 * N2), U32),
            pltpu.VMEM((4, 2, S, 128), F32),
            pltpu.VMEM((S, D), BF),
            pltpu.VMEM((M, D), BF),
            pltpu.VMEM((1, D), BF),
            pltpu.VMEM((2, 1, S), BF),
            pltpu.VMEM((16, 128), F32),
            pltpu.VMEM((128, 128), F32),
            pltpu.VMEM((16, D), U32),
            pltpu.VMEM((3, 32, 128), U32),
            pltpu.VMEM((64, D), F32),
            pltpu.VMEM((64, 128), F32),
            pltpu.VMEM((3, 8, 32, 128), U32),
            pltpu.VMEM((8, 40, 80), U32),
            pltpu.VMEM((80, 80), F32),
            pltpu.SemaphoreType.DMA((NSEM,)),
        ],
        compiler_params=pltpu.CompilerParams(vmem_limit_bytes=120 * 1024 * 1024),
    )(
        A_x.reshape(S, D), A_mem0.reshape(M, D), A_Wq, A_Wk, A_Wv,
        A_Wo.reshape(H * DH, D), B_w_r.T, B_w_i.T, gate_w.reshape(1, D), *consts,
    )
    return out.reshape(1, S, D)
```

```python
import functools
import math
import os

import numpy as np
import jax
import jax.numpy as jnp
from jax import lax
import jax.experimental.pallas as pl
import jax.experimental.pallas.tpu as pltpu

BF, F32, U32 = jnp.bfloat16, jnp.float32, jnp.uint32

S, D, H, DH, M, SEG = 2048, 1024, 32, 128, 8, 32
NSEG = S // SEG
NP = H // 2
N1, N2 = 32, 64
QS = S // 4
PITCH = N1 + 8
CLASSES = ((0, 8, 4, 12), (1, 15, 9, 7), (2, 14, 10, 6), (3, 13, 11, 5))
_E = lambda k, d: int(os.environ.get(k, d))
LAG1, LAG2, SPLIT = _E("LAG1", 1), _E("LAG2", 2), _E("SPLIT", 28)
HOOK_AT = _E("HOOK_AT", 17)
ONLY = os.environ.get("ONLY", "")
KSPLIT = _E("KSPLIT", 1)
NOSPEC = _E("NOSPEC", 0)
STAGE = os.environ.get("STAGE", "qkvp")
ORDER = os.environ.get("ORDER", "vqskp")
DMAPOS = _E("DMAPOS", 0)
B0, BD, BW, BV, BL = _E("B0", 0), _E("BD", 10), _E("BW", 8), _E("BV", 8), _E("BL", 8)
PINCB = _E("PINCB", 1)
NQ = 4
(SEM_W, SEM_GF, SEM_GI, SEM_SM, SEM_GS, SEM_F, SEM_NYQ, SEM_WO, SEM_MEM, SEM_GW, SEM_OUT,
 SEM_X) = 0, 6, 7, 8, 9, 10, 12, 13, 14, 15, 16, 17
SEM_W0 = SEM_X + NQ
NSEM = SEM_W0 + NQ
RSQ2 = float(np.float32(math.sqrt(0.5)))


def _bfly8(x):
    s = [x[i] + x[i + 4] for i in range(4)]
    d = [x[i] - x[i + 4] for i in range(4)]
    e, f = s[0] + s[2], s[1] + s[3]
    t1, t2 = (d[1] - d[3]) * RSQ2, (d[1] + d[3]) * RSQ2
    return [e + f, e - f, d[0] + t1, t2 + d[2], s[0] - s[2], s[1] - s[3], d[0] - t1, t2 - d[2]]


def _bfly8_t(t):
    e, f = t[0] + t[1], t[0] - t[1]
    s = [e + t[4], f + t[5], e - t[4], f - t[5]]
    t1, t2 = t[2] - t[6], t[3] + t[7]
    d = [t[2] + t[6], (t1 + t2) * RSQ2, t[3] - t[7], (t2 - t1) * RSQ2]
    return [s[i] + d[i] for i in range(4)] + [s[i] - d[i] for i in range(4)]


def _half_pre(vr, vi, lo, roll, where):
    ri = roll(vi)
    return where(lo, vr, ri), where(lo, ri, vr)


def _half_post(g, tp, tm, lo, roll, where):
    if g == 0:
        return tp, tm
    c = float(np.float32(math.cos(math.pi * g / 8)))
    s = float(np.float32(math.sin(math.pi * g / 8)))
    p, r = tp + tm, tp - tm
    rm = roll(where(lo, r, p))
    return where(lo, p, c * rm + s * r), where(lo, rm, c * r - s * rm)


def _cmul_const(v, k, n, sign):
    re, im = v
    k %= n
    if k == 0:
        return re, im
    if 4 * k == n:
        return (-im, re) if sign > 0 else (im, -re)
    if 8 * k == n:
        return (((re - im) * RSQ2, (re + im) * RSQ2) if sign > 0
                else ((re + im) * RSQ2, (im - re) * RSQ2))
    if 8 * k == 3 * n:
        return (((re + im) * -RSQ2, (re - im) * RSQ2) if sign > 0
                else ((im - re) * RSQ2, (re + im) * -RSQ2))
    c, s = math.cos(2 * math.pi * k / n), sign * math.sin(2 * math.pi * k / n)
    return re * c - im * s, re * s + im * c


def _fft(v, sign):
    n = len(v)
    if n == 1:
        return v
    ev, od = _fft(v[0::2], sign), _fft(v[1::2], sign)
    lo, hi = [], []
    for k in range(n // 2):
        er, ei = ev[k]
        if 4 * k == n:
            xr, xi = od[k]
            if sign > 0:
                lo.append((er - xi, ei + xr)); hi.append((er + xi, ei - xr))
            else:
                lo.append((er + xi, ei - xr)); hi.append((er - xi, ei + xr))
            continue
        tr, ti = _cmul_const(od[k], k, n, sign)
        lo.append((er + tr, ei + ti))
        hi.append((er - tr, ei - ti))
    return lo + hi


def _pack_rows(a):
    u = np.ascontiguousarray(a, dtype=np.float32).view(np.uint32)
    b = ((u + 0x7FFF + ((u >> 16) & 1)) >> 16).astype(np.uint32)
    return (b[..., 0::2, :] | (b[..., 1::2, :] << 16)).astype(np.uint32)


def _diag_blocks(full, n, tol):
    k = full.shape[0] // n
    blk = np.kron(np.eye(k), np.ones((n, n)))
    assert np.abs(full * (1 - blk)).max() < tol
    return np.stack([full[n * g:n * g + n, n * g:n * g + n] for g in range(k)])


def _cplx(re, im):
    return np.block([[re, im], [-im, re]])


@functools.lru_cache(maxsize=None)
def _constants():
    k2 = np.stack([np.concatenate([c + 16 * np.arange(32) for c in cls]) for cls in CLASSES])
    n2 = np.arange(D)
    ang = 2 * np.pi * ((k2[:, :, None] * n2[None, None, :]) % D) / D
    rows = np.stack([np.cos(ang), -np.sin(ang)], axis=1)
    wgt = np.where(k2 == 0, 1.0, 2.0)[:, None, :, None]
    fwd = rows.reshape(D, D).T
    inv = (rows * wgt).reshape(D, D) / (S * D)
    bf = np.stack(_bfly8(list(np.eye(8))))
    binv = np.kron(np.linalg.inv(bf), np.eye(128))
    gd = _diag_blocks(binv.T @ fwd, 256, 1e-6)
    gdi = _diag_blocks(inv @ binv, 256, 1e-12)
    eye, lo = np.eye(256), np.arange(128) < 64
    roll = lambda v: np.roll(v, 64, axis=1)
    pre = np.concatenate(_half_pre(eye[:, :128], eye[:, 128:], lo, roll, np.where), axis=1)
    gi = []
    for g in range(4):
        post = np.concatenate(_half_post(g, eye[:, :128], eye[:, 128:], lo, roll, np.where), axis=1)
        gi.append(_diag_blocks(np.linalg.inv(pre) @ gdi[g] @ np.linalg.inv(post), 128, 1e-12))
    gi = np.concatenate(gi)

    b = np.arange(N2)
    k1 = np.arange(N1)[:, None] + N1 * np.arange(N2)[None, :]
    th = 2 * np.pi * ((k1[:, :, None] * b[None, None, :]) % S) / S
    gr, gim = np.cos(th), -np.sin(th)
    full = np.block([[gr, -gim], [gim, gr]])
    kap = np.arange(2 * N2)
    src = ((kap >> 3) & 1) * N2 + (kap >> 4) * 8 + (kap & 7)
    gs = full[:, :, src]
    hr, hi = np.swapaxes(gr, 1, 2), -np.swapaxes(gim, 1, 2)
    gsi = np.block([[hr, -hi], [hi, hr]])

    lane = np.arange(128)
    kb = 8 * (lane % 16) + lane // 16
    t128 = 2 * np.pi * ((lane[:, None] * kb[None, :]) % 128) / 128
    nyf = _cplx(np.cos(t128), -np.sin(t128))
    nyi = _cplx(np.cos(t128).T, np.sin(t128).T)
    i16 = np.arange(16)
    t16 = 2 * np.pi * ((i16[:, None] * i16[None, :]) % 16) / 16
    tw = 2 * np.pi * (i16[:, None] * lane[None, :]) / S
    sm = np.zeros((80, 128), np.float32)
    sm[0:16], sm[16:32] = np.cos(tw), np.sin(tw)
    sm[32:48, :16], sm[48:64, :16] = np.cos(t16), -np.sin(t16)
    sm[64:80, :16], sm[64:80, 16:32] = np.cos(t16), -np.sin(t16)

    gfp = _pack_rows(np.concatenate([gd, nyf[None], nyi[None]]))
    return gfp, _pack_rows(gi), sm, _pack_rows(np.stack([gs, gsi]))


def _mask80():
    r = lax.broadcasted_iota(jnp.int32, (80, 80), 0)
    c = lax.broadcasted_iota(jnp.int32, (80, 80), 1)

    def head(i):
        return jnp.where(i < 64, i >> 5, (i - 64) >> 3)

    def pos(i):
        j = i & 31
        return jnp.where(i < 64, jnp.where(j < M, j, j + 8), M + (i & 7))

    same = head(r) == head(c)
    ok = (pos(r) < M) | (pos(c) <= pos(r))
    return jnp.where(same, jnp.where(ok, 1.0, -1e9), -jnp.inf).astype(F32)


def _as_bf(u):
    return pltpu.bitcast(u, BF)


def _as_u32(b):
    return pltpu.bitcast(b, U32)


def _lo_f32(u):
    return pltpu.bitcast(u << 16, F32)


def _hi_f32(u):
    return pltpu.bitcast(u & jnp.uint32(0xFFFF0000), F32)


def _dot(a, b):
    return jnp.dot(a, b, preferred_element_type=F32)


def _dot_nt(a, b):
    return lax.dot_general(a, b, (((1,), (1,)), ((), ())), preferred_element_type=F32)


def _transpose_u32(u):
    return pltpu.bitcast(pltpu.bitcast(u, F32).T, U32)


def _lanes(rows):
    return lax.broadcasted_iota(jnp.int32, (rows, 128), 1)


def _kernel(x_hbm, mem_hbm, wq_hbm, wk_hbm, wv_hbm, wo_hbm, fr_hbm, fi_hbm, gw_hbm,
            gf_hbm, gi_hbm, sm_hbm, gs_hbm,
            out_hbm,
            x_v, raw, wqkv, wo, st, sto, obuf, sl, fraw, fp, gf, gi, sm, gs, y, out_v, mem_ref, gw_ref,
            nyq, xa, ct, a_s, qkv_s, bb_s, g_s, stg, pst, mf, u_s, v_s, cb, z_s, p_s, zero_s, sem):
    KH = D // 2
    KQ = KH // NQ
    raw4 = raw.reshape(6, D, 8, DH)
    w_hbm = (wq_hbm, wk_hbm, wv_hbm)
    f_hbm = (fr_hbm, fi_hbm)

    def w_src(c):
        return w_hbm[c // 2].bitcast(U32).at[:, pl.ds(8 * (c % 2), 8), :]

    def wait(dst, k):
        pltpu.make_async_copy(dst, dst, sem.at[k]).wait()

    def kslice(q, e):
        return pl.ds(pl.multiple_of(e * KH + q * KQ, KQ), KQ)

    def f_copies(h):
        return [(f_hbm[a].at[pl.ds(0, D // 2), pl.ds(128 * (8 * h + c), 128)].bitcast(U32),
                 fraw.at[h, a, c], SEM_F + h) for a in range(2) for c in range(8)]

    copies = []
    for q in range(NQ):
        copies += [(x_hbm.at[:, kslice(q, e)], x_v.at[:, kslice(q, e)], SEM_X + q) for e in range(2)]
        copies += [(w_src(0).at[kslice(q, e)], raw4.at[0, kslice(q, e)], SEM_W0 + q) for e in range(2)]
    copies += [(gf_hbm, gf, SEM_GF), (sm_hbm, sm, SEM_SM)]
    copies += [(f_hbm[a].at[pl.ds(D // 2, 1), :], nyq.at[a], SEM_NYQ) for a in range(2)]
    copies += f_copies(0) + [(w_src(1), raw4.at[1], SEM_W + 1)] + f_copies(1) + [(gs_hbm, gs, SEM_GS)]
    copies += [(w_src(c), raw4.at[c], SEM_W + c) for c in (2, 3, 4, 5)]
    copies += [(wo_hbm.bitcast(U32).at[:, pl.ds(128 * j, 128)], wo.at[j], SEM_WO) for j in range(8)]
    copies += [(gi_hbm, gi, SEM_GI), (mem_hbm, mem_ref, SEM_MEM), (gw_hbm, gw_ref, SEM_GW)]
    for src, dst, k in copies:
        pltpu.make_async_copy(src, dst, sem.at[k]).start()

    def prep_rhs(ch, jj, k0, nk):
        item = 8 * ch + jj
        a1 = raw[ch, pl.ds(k0 * 8 + jj, nk, stride=8), :]
        a2 = raw[ch, pl.ds((KH + k0) * 8 + jj, nk, stride=8), :]
        b11, b12, b21, b22 = _lo_f32(a1), _hi_f32(a1), _lo_f32(a2), _hi_f32(a2)
        for p, e, b in ((0, 0, b11), (1, 0, b12), (0, 1, b21), (1, 1, b22)):
            row = pl.multiple_of((e * KH + k0) // 2, nk // 2)
            wqkv[2 * item + p, pl.ds(row, nk // 2), :] = _as_u32(b.astype(BF))
        return [v.astype(BF) for v in (b11 + b22, b11, b12 - b22, b21 - b11, b22, b11 + b12, b21 + b22)]

    def strassen(rhs, k0, nk, init, finish, after_dot):
        def prod(i):
            return _dot(_as_bf(sl[i, :, pl.ds(k0, nk)]), rhs[i])

        def plus(i, r):
            return r if init is None else init(i) + r

        m = prod(1)
        cb[0] = m
        after_dot(0, m)
        m = prod(4)
        cb[1] = m
        after_dot(1, m)
        m = prod(0)
        cb[2] = plus(0, m - cb[1])
        cb[3] = plus(3, m - cb[0])
        after_dot(2, m)
        m = prod(3)
        cb[4] = plus(2, cb[0] + m)
        cb[2] = cb[2] + m
        after_dot(3, m)
        m = prod(2)
        cb[5] = plus(1, cb[1] + m)
        cb[3] = cb[3] + m
        after_dot(4, m)
        m = prod(6) + cb[2]
        finish(0, m, cb[5])
        after_dot(5, m)
        m = prod(5) + cb[3]
        finish(1, cb[4], m)
        after_dot(6, m)

    def store_st(item, e, c1, c2):
        r = jnp.concatenate([c.reshape(NSEG // 2, 8, 128) for c in (c1, c2)], axis=1)
        st[item, 256 * e:256 * e + 256, :] = _as_u32(r.reshape(8 * NSEG, 128).astype(BF))

    def pin(i, c):
        if PINCB:
            cb[i, 0:8, :] = jnp.zeros((8, 128), F32)
        zero_s[i] = 0
        z_s[i, 0:8, :] = jnp.zeros((8, 128), U32)
        p_s[i, 0:8, :] = jnp.zeros((8, 128), F32)
        u_s[i, 0:8, :] = jnp.zeros((8, 128), U32)
        stg[i, 0, 0:8, :] = jnp.zeros((8, 128), U32)
        obuf[i, 0:8, :] = jnp.zeros((8, 128), U32)
        return c

    lax.fori_loop(0, 2, pin, 0)

    def acc(jj, i):
        return y.at[jj // 4, (jj // 2) % 2, pl.ds(1024 * (jj % 2) + 256 * i, 256), :]

    for jj in range(8):
        for i in range(4):
            acc(jj, i)[...] = jnp.zeros((256, 128), F32)

    def k_slice(q, last):
        for e in range(2):
            wait(x_v.at[:, kslice(q, e)], SEM_X + q)
        k0 = pl.multiple_of(q * KQ, KQ)

        def rows16(s2, e):
            return jnp.concatenate([x_v[64 * s2:64 * s2 + 16, kslice(q, e)].astype(F32)[0:8],
                                    x_v[64 * s2 + 32:64 * s2 + 48, kslice(q, e)].astype(F32)[0:8]], axis=0)

        for s2 in range(NSEG // 4):
            a11, a12, a21, a22 = rows16(s2, 0), rows16(s2, 1), rows16(s2 + 16, 0), rows16(s2 + 16, 1)
            for i, v in enumerate((a11 + a22, a21 + a22, a11, a22, a11 + a12, a21 - a11, a12 - a22)):
                sl[i, 8 * s2:8 * s2 + 8, pl.ds(k0, KQ)] = _as_u32(v.astype(BF))
        for e in range(2):
            wait(raw4.at[0, kslice(q, e)], SEM_W0 + q)
        for jj in range(8):
            def finish(e, c1, c2):
                if last:
                    store_st(jj, e, c1, c2)
                else:
                    acc(jj, 2 * e)[...] = c1
                    acc(jj, 2 * e + 1)[...] = c2

            strassen(prep_rhs(0, jj, k0, KQ), k0, KQ, lambda i: acc(jj, i)[...], finish, lambda n, m: None)

    def k_body(q, c):
        k_slice(q, False)
        return c

    with jax.named_scope("p0"):
        if ONLY in ("", "p0"):
            lax.fori_loop(0, NQ - 1, k_body, 0)
            k_slice(NQ - 1, True)
        else:
            for q in range(NQ):
                for e in range(2):
                    wait(x_v.at[:, kslice(q, e)], SEM_X + q)
                    wait(raw4.at[0, kslice(q, e)], SEM_W0 + q)

    wait(gf, SEM_GF)
    RB, HB = 128, 64

    def f1(i, c):
        base = pl.multiple_of(i * RB, RB)
        alt = (1 - 2 * (_lanes(16) & 1)).astype(F32).astype(BF)
        u0 = [[] for _ in range(4)]
        for h0 in range(0, RB, HB):
            pieces = []
            for a1 in range(4):
                for r in range(h0, h0 + HB, 16):
                    xs = x_v[pl.ds(base + (QS * a1 + r), 16), :].astype(F32)
                    us = _bfly8([xs[:, 128 * a:128 * a + 128] for a in range(8)])
                    pieces.append(jnp.concatenate(us, axis=1).astype(BF))
                    u0[a1].append(pieces[-1][:, :128])
            ub = jnp.concatenate(pieces, axis=0)
            if h0 + HB == RB:
                for a1 in range(4):
                    xa[pl.ds(4 * a1 + i, 1), :] = _dot_nt(alt, jnp.concatenate(u0[a1], axis=0))[0:1]
            for g in range(4):
                yy = _dot(ub[:, 256 * g:256 * g + 256], _as_bf(gf[g]))
                v = _fft([(yy[HB * a1:HB * a1 + HB, :128], yy[HB * a1:HB * a1 + HB, 128:])
                          for a1 in range(4)], -1)
                for k1 in range(4):
                    rows = pl.ds(base + (QS * k1 + h0), HB)
                    y[g, 0, rows, :] = v[k1][0]
                    y[g, 1, rows, :] = v[k1][1]
        return c

    with jax.named_scope("f1"):
        if ONLY in ("", "f1"):
            lax.fori_loop(0, QS // RB, f1, 0)

    def fprep(h, c):
        ev, od = [], []
        for r in range(8):
            wr = fraw[h, 0, c, pl.ds(r, 32, stride=8), :]
            wi = fraw[h, 1, c, pl.ds(r, 32, stride=8), :]
            ev.append((wr & jnp.uint32(0xFFFF)) | (wi << 16))
            od.append((wr >> 16) | (wi & jnp.uint32(0xFFFF0000)))
        for g, cls in enumerate(CLASSES):
            t = _transpose_u32(jnp.concatenate([(od if k % 2 else ev)[k // 2] for k in cls], axis=0))
            for q in range(128 // N1):
                row = pl.multiple_of(((8 * h + c) * (128 // N1) + q) * PITCH, 8)
                fp[g, pl.ds(row, N1), :] = t[q * N1:(q + 1) * N1]

    def nyquist():
        twc, tws = sm[0:16], sm[16:32]
        u = _dot(sm[32:64, 0:16].astype(BF), xa[...].astype(BF))
        ur, ui = u[0:16], u[16:32]
        u = jnp.concatenate([ur * twc + ui * tws, ui * twc - ur * tws], axis=1).astype(BF)
        yield
        xx = _dot(u, _as_bf(gf[4]))
        xr, xi = xx[:, :128], xx[:, 128:]
        w = (pltpu.bitcast(nyq[0].astype(F32), U32) >> 16) | pltpu.bitcast(nyq[1].astype(F32), U32)
        w = jnp.concatenate([w[:, 128 * a:128 * a + 128] for a in range(16)], axis=0)
        wt = _transpose_u32(jnp.concatenate([w] * 8, axis=0))
        blk = _lanes(16) >> 4
        wm = wt[0:16]
        for j in range(1, 8):
            wm = jnp.where(blk == j, wt[16 * j:16 * j + 16], wm)
        wr, wi = _lo_f32(wm), _hi_f32(wm)
        z = jnp.concatenate([xr * wr - xi * wi, xr * wi + xi * wr], axis=1).astype(BF)
        yield
        pp = _dot(z, _as_bf(gf[5]))
        pr, pi = pp[:, :128], pp[:, 128:]
        pp = jnp.concatenate([pr * twc - pi * tws, pi * twc + pr * tws], axis=0).astype(BF)
        yield
        cc = _dot(sm[64:80, 0:32].astype(BF), pp) * (1.0 / (S * D))
        ct[...] = jnp.concatenate([cc, jnp.zeros((112, 128), F32)], axis=0).T
        yield

    def s_rows(k1, a0, r):
        return pl.ds(r + (QS * k1 + N2 * a0), 8)

    def anchored(v, tok):
        return jnp.where(zero_s[0] != 0, tok, v)

    def s_prep(g, k1, r, tok):
        v = [(y[g, 0, s_rows(k1, a0, r), :], y[g, 1, s_rows(k1, a0, r), :]) for a0 in range(8)]
        v[0] = (anchored(v[0][0], tok), v[0][1])
        v = _fft([_cmul_const(v[a0], a0 * k1, N1, -1) for a0 in range(8)], -1)
        for k0 in range(8):
            u_s[k1 + 4 * k0, pl.ds(r, 8), :] = _as_u32(jnp.concatenate(v[k0], axis=0).astype(BF))

    def s_fwd(g, ka, tok):
        xx = _dot(_as_bf(gs[0, ka]), _as_bf(u_s[ka]))
        w32 = fp[g, pl.ds(ka, N2, stride=PITCH), :]
        wr, wi = _lo_f32(w32), _hi_f32(w32)
        xr, xi = xx[:N2], xx[N2:]
        z_s[ka] = _as_u32(jnp.concatenate([xr * wr - xi * wi, xr * wi + xi * wr], axis=0).astype(BF))

    def s_inv(ka, tok):
        p_s[ka] = _dot(_as_bf(gs[1, ka]), _as_bf(z_s[ka]))

    def s_post(g, k1, r, tok):
        v = [(p_s[k1 + 4 * k0, r:r + 8, :], p_s[k1 + 4 * k0, N2 + r:N2 + r + 8, :]) for k0 in range(8)]
        v[0] = (anchored(v[0][0], tok), anchored(v[0][1], tok))
        v = _fft(v, 1)
        for a0 in range(8):
            vr, vi = _cmul_const(v[a0], a0 * k1, N1, 1)
            v_s[g, 0, s_rows(k1, a0, r), :] = vr
            v_s[g, 1, s_rows(k1, a0, r), :] = vi

    def bulk(ch, jj0, n, events):
        for i in range(n):
            def hook(k, m):
                for piece in events.get(7 * i + k, ()):
                    piece(m[0:8])

            strassen(prep_rhs(ch, jj0 + i, 0, KH), 0, KH, None,
                     functools.partial(store_st, 8 * ch + jj0 + i), hook)

    def spread(events, pieces, q0, q1):
        for i, piece in enumerate(pieces):
            events.setdefault(q0 + ((q1 - q0) * i) // len(pieces), []).append(piece)

    P = functools.partial

    def loop_a(h, c):
        wait(fraw.at[h], SEM_F + h)
        ny = nyquist()
        events = {}
        spread(events, [lambda tok: next(ny)] * 4, 2, 14)
        spread(events, [lambda tok, c=c: fprep(h, c) for c in range(8)], 0, 24)
        r0 = pl.multiple_of(h * (N2 // 2), N2 // 2)
        spread(events, [P(s_prep, 0, k1, r0 + r) for k1 in range(4) for r in range(0, N2 // 2, 8)], 0, 26)
        bulk(1, 4 * h, 4, events)
        return c

    def loop_b(g, c):
        wait(raw4.at[g + 2], SEM_W + 2 + g)
        gn = jnp.minimum(g + 1, 3)
        events = {}
        for k1 in range(4):
            q = B0 + BD * k1
            spread(events, [P(s_fwd, g, k1 + 4 * k0) for k0 in range(8)], q, q + BW)
            spread(events, [P(s_prep, gn, k1, r) for r in range(0, N2, 8)], q + BW, q + BW + BV)
            q += BL
            spread(events, [P(s_inv, k1 + 4 * k0) for k0 in range(8)], q, q + BW)
            spread(events, [P(s_post, g, k1, r) for r in range(0, N2, 8)], q + BW, q + BW + BV)
        assert max(events) < 55
        bulk(g + 2, 0, 8, events)
        return c

    wait(sm, SEM_SM)
    wait(nyq, SEM_NYQ)
    wait(raw4.at[1], SEM_W + 1)
    with jax.named_scope("loop_a"):
        if ONLY in ("", "a"):
            lax.fori_loop(0, 2, loop_a, 0)
        else:
            wait(fraw.at[0], SEM_F)
            wait(fraw.at[1], SEM_F + 1)
    wait(gs, SEM_GS)
    with jax.named_scope("loop_b"):
        if ONLY in ("", "b"):
            lax.fori_loop(0, 4, loop_b, 0)
        else:
            for g in range(4):
                wait(raw4.at[g + 2], SEM_W + 2 + g)
    wait(wo, SEM_WO)
    wait(gi, SEM_GI)
    wait(mem_ref, SEM_MEM)
    wait(gw_ref, SEM_GW)

    scale = DH ** -0.5

    mf[...] = _mask80()

    def softmax(s):
        fill = mf[...]
        s = jnp.where(fill > 0.0, s * scale, fill)
        m = jnp.max(s, axis=-1, keepdims=True)
        e = jnp.exp(s - m)
        l = jnp.sum(e, axis=-1, keepdims=True)
        return (e * (1.0 / l)).astype(BF)

    def lhs_rows(mem, seg):
        xs = x_v[pl.ds(pl.multiple_of(seg * SEG, SEG), SEG), :].astype(F32)
        return jnp.concatenate([mem, xs[8:SEG]], axis=0).astype(BF)

    def proj2(a, m, j):
        return jnp.concatenate([_dot(a, _as_bf(wqkv[H * m + 2 * j + p])).astype(BF) for p in range(2)], axis=0)

    def proj_first(a):
        if not KSPLIT:
            return [proj2(a, m, 0) for m in range(3)]
        part = [_dot(a[:, :D // 2], _as_bf(wqkv[H * (i // 2) + i % 2, 0:D // 4, :])) for i in range(6)]
        full = [(_dot(a[:, D // 2:], _as_bf(wqkv[H * (i // 2) + i % 2, D // 4:D // 2, :])) + part[i]).astype(BF)
                for i in range(6)]
        return [jnp.concatenate(full[2 * m:2 * m + 2], axis=0) for m in range(3)]

    def step(a, seg, first, hook=None):
        R = 32 if first else 48
        qkv, ps = {}, {}
        srow = pl.multiple_of(seg * 8, 8)

        def put(m, j, r):
            if "qkv"[m] in STAGE:
                stg[m, j % 8] = _as_u32(r)
            else:
                qkv[m, j] = r

        def get(m, j):
            r = _as_bf(stg[m, j % 8]) if "qkv"[m] in STAGE else qkv[m, j]
            return jnp.concatenate([r, _as_bf(st[NP * m + j, pl.ds(srow, 8), :])], axis=0)

        def proj(j, m):
            if j == 0:
                if m == 0:
                    r = [_as_bf(qkv_s[m]) for m in range(3)] if first else proj_first(a)
                    for mm in range(3):
                        put(mm, 0, r[mm])
            else:
                put(m, j, proj2(a, m, j))

        def scores(j):
            pp = softmax(_dot_nt(get(0, j), get(1, j)))
            if "p" in STAGE:
                pst[j % 8] = _as_u32(pp)
            else:
                ps[j] = pp

        def pv(j):
            o = _dot(_as_bf(pst[j % 8]) if "p" in STAGE else ps[j], get(2, j))
            for i in range(2):
                h = 2 * j + i
                if first:
                    ob = o[32 * i:32 * i + 32].astype(BF)
                    sto[h] = o[64 + 8 * i:72 + 8 * i]
                else:
                    ob = jnp.concatenate([o[32 * i:32 * i + 32], o[64 + 8 * i:72 + 8 * i], sto[h]],
                                         axis=0).astype(BF)
                obuf[h, 0:R // 2, :] = _as_u32(ob)

        def wo_part(j, h0, h1):
            og = jnp.concatenate([_as_bf(obuf[h, 0:R // 2, :]) for h in range(h0, h1)], axis=1)
            return _dot(og, _as_bf(wo[j, h0 * 64:h1 * 64, :]))

        parts = []
        for i in range(NP + 4):
            for ch in ORDER:
                if ch in "qkv":
                    m = "qkv".index(ch)
                    if i < NP:
                        proj(i, m)
                    elif m < 2:
                        parts.append(wo_part(2 * (i - NP) + len(parts) % 2, 0, SPLIT))
                elif ch == "s" and 0 <= i - LAG1 < NP:
                    scores(i - LAG1)
                elif ch == "p" and 0 <= i - LAG2 < NP:
                    pv(i - LAG2)
            if hook is not None and i == HOOK_AT:
                hook()
        return jnp.concatenate([wo_part(j, SPLIT, H) + parts[j] for j in range(8)], axis=1)

    def start_pair(mem, t):
        a = lhs_rows(mem, 2 * t)
        a_s[...] = _as_u32(a)
        for m, r in enumerate(proj_first(a)):
            qkv_s[m] = _as_u32(r)

    def pair(t, c):
        base = pl.multiple_of(t * 64, 64)
        lane = _lanes(64)
        lo = lane < 64
        roll = (lambda v: v + 1.0) if _E('NOROLL', 0) else (lambda v: pltpu.roll(v, 64, 1))
        a1 = t // 8
        off = pl.multiple_of((t % 8) * 64, 64)
        s2 = (1 - 2 * (a1 & 1)).astype(F32)
        sg = (1 - (a1 & 2)).astype(F32)
        cc, ss = sg * (1 - (a1 & 1)).astype(F32), sg * (a1 & 1).astype(F32)

        def irfft_group(g):
            q = [[v_s[g, e, pl.ds(off + QS * k1, 64), :] for e in range(2)] for k1 in range(4)]
            br, bi = q[1][0] + s2 * q[3][0], q[1][1] + s2 * q[3][1]
            vr = q[0][0] + s2 * q[2][0] + (cc * br - ss * bi)
            vi = q[0][1] + s2 * q[2][1] + (cc * bi + ss * br)
            tin = _half_pre(vr, vi, lo, roll, jnp.where)
            tp, tm = [_dot(tin[e].astype(BF), _as_bf(gi[2 * g + e])) for e in range(2)]
            if g == 0:
                nyc = jnp.sum(jnp.where(lane == t // 2,
                                        ct[pl.ds(pl.multiple_of((t % 2) * 64, 64), 64), :], 0.0),
                              axis=-1, keepdims=True)
                tp = tp + nyc * (1 - 2 * (lane & 1)).astype(F32)
            return list(_half_post(g, tp, tm, lo, roll, jnp.where))

        def spectral_part():
            ts = sum([irfft_group(g) for g in range(4)], [])
            b = jnp.concatenate(_bfly8_t(ts), axis=1).astype(BF).astype(F32)
            xs = x_v[pl.ds(base, 64), :].astype(F32)
            gate = jax.nn.sigmoid(jnp.sum(xs * gw_ref[...].astype(F32), axis=-1, keepdims=True))
            bb = (1.0 - gate) * b
            bb_s[...] = jnp.concatenate([bb[0:8], bb[8:32] + gate[8:32] * bb_s[8:32], bb[32:64]], axis=0)
            g_s[...] = jnp.broadcast_to(gate, (64, 128))

        res_a = step(_as_bf(a_s[...]), 2 * t, True)
        bb_s[8:32] = res_a[8:32]
        a = lhs_rows(res_a[0:8].astype(BF).astype(F32), 2 * t + 1)
        res_b = step(a, 2 * t + 1, False, None if NOSPEC else spectral_part)

        def gated(r0, r1, res):
            return bb_s[r0:r1] + jnp.concatenate([g_s[r0:r1]] * 8, axis=1) * res

        out_v[pl.ds(base, 64), :] = jnp.concatenate(
            [gated(0, 8, res_b[40:48]), bb_s[8:32], gated(32, 40, res_b[32:40]), gated(40, 64, res_b[8:32])],
            axis=0).astype(BF)
        cp = pltpu.make_async_copy(out_v.at[pl.ds(base, 64), :], out_hbm.at[pl.ds(base, 64), :],
                                   sem.at[SEM_OUT])
        if DMAPOS == 0:
            cp.start()
        start_pair(res_b[0:8].astype(BF).astype(F32), jnp.minimum(t + 1, S // 64 - 1))
        if DMAPOS == 1:
            cp.start()
        return c

    with jax.named_scope("chain"):
        if ONLY in ("", "chain"):
            start_pair(mem_ref[...].astype(F32), 0)
            lax.fori_loop(0, S // 64, pair, 0)
            if DMAPOS == 2:
                pltpu.make_async_copy(out_v, out_hbm, sem.at[SEM_OUT]).start()
    if ONLY not in ("", "chain"):
        def keep(i, c):
            v = st[i, 0:8, :] + wqkv[i, 0:8, :] + fp[i % 4, 0:8, :] + u_s[i % 32, 0:8, :] + pltpu.bitcast(y[i % 4, 0, pl.ds(8 * i, 8), :] + v_s[i % 4, 0, pl.ds(8 * i, 8), :] + ct[pl.ds(i, 8), :] + xa[0:8], U32) + sl[i % 7, 0:8, 0:128]
            out_v[pl.ds(16 * i, 16), 0:128] = _as_bf(v)
            return c
        lax.fori_loop(0, 48, keep, 0)
        pltpu.make_async_copy(out_v, out_hbm, sem.at[SEM_OUT]).start()
        pltpu.make_async_copy(out_v, out_hbm, sem.at[SEM_OUT]).wait()
    with jax.named_scope("fin"):
        if ONLY in ("", "chain"):
            pltpu.make_async_copy(out_v, out_hbm, sem.at[SEM_OUT]).wait()


@functools.partial(jax.jit, static_argnames=("A_seg_len",))
def pallas_gated_mix__memory_aug_recurrent_mem_tr__spectral_gfnet__prompt_kernel(
    A_x, A_mem0, A_Wq, A_Wk, A_Wv, A_Wo, A_seg_len, B_x, B_w_r, B_w_i, gate_w,
):
    assert A_x.shape == (1, S, D) and A_mem0.shape == (1, M, D) and A_Wq.shape == (D, H, DH)
    assert int(A_seg_len) == SEG
    consts = [jnp.asarray(c) for c in _constants()]
    any_spec = pl.BlockSpec(memory_space=pl.ANY)
    out = pl.pallas_call(
        _kernel,
        out_shape=jax.ShapeDtypeStruct((S, D), BF),
        in_specs=[any_spec] * 13,
        out_specs=any_spec,
        scratch_shapes=[
            pltpu.VMEM((S, D), BF),
            pltpu.VMEM((6, D * 8, DH), U32),
            pltpu.VMEM((3 * H, D // 2, DH), U32),
            pltpu.VMEM((8, H * DH // 2, 128), U32),
            pltpu.VMEM((3 * NP, 8 * NSEG, 128), U32),
            pltpu.VMEM((H, 8, 128), F32),
            pltpu.VMEM((H, 24, 128), U32),
            pltpu.VMEM((7, 2 * NSEG, D // 2), U32),
            pltpu.VMEM((2, 2, 8, 256, 128), U32),
            pltpu.VMEM((4, N2 * PITCH, 128), U32),
            pltpu.VMEM((6, 128, 256), U32),
            pltpu.VMEM((8, 64, 128), U32),
            pltpu.VMEM((80, 128), F32),
            pltpu.VMEM((2, N1, N2, 2 * N2), U32),
            pltpu.VMEM((4, 2, S, 128), F32),
            pltpu.VMEM((S, D), BF),
            pltpu.VMEM((M, D), BF),
            pltpu.VMEM((1, D), BF),
            pltpu.VMEM((2, 1, S), BF),
            pltpu.VMEM((16, 128), F32),
            pltpu.VMEM((128, 128), F32),
            pltpu.VMEM((16, D), U32),
            pltpu.VMEM((3, 32, 128), U32),
            pltpu.VMEM((64, D), F32),
            pltpu.VMEM((64, 128), F32),
            pltpu.VMEM((3, 8, 32, 128), U32),
            pltpu.VMEM((8, 40, 80), U32),
            pltpu.VMEM((80, 80), F32),
            pltpu.VMEM((N1, N2, 128), U32),
            pltpu.VMEM((4, 2, S, 128), F32),
            pltpu.VMEM((6, 256, 128), F32),
            pltpu.VMEM((N1, N2, 128), U32),
            pltpu.VMEM((N1, 2 * N2, 128), F32),
            pltpu.SMEM((2,), jnp.int32),
            pltpu.SemaphoreType.DMA((NSEM,)),
        ],
        compiler_params=pltpu.CompilerParams(vmem_limit_bytes=120 * 1024 * 1024),
    )(
        A_x.reshape(S, D), A_mem0.reshape(M, D), A_Wq, A_Wk, A_Wv,
        A_Wo.reshape(H * DH, D), B_w_r.T, B_w_i.T, gate_w.reshape(1, D), *consts,
    )
    return out.reshape(1, S, D)
```

```python
import functools
import math
import os

import numpy as np
import jax
import jax.numpy as jnp
from jax import lax
import jax.experimental.pallas as pl
import jax.experimental.pallas.tpu as pltpu

BF, F32, U32 = jnp.bfloat16, jnp.float32, jnp.uint32

S, D, H, DH, M, SEG = 2048, 1024, 32, 128, 8, 32
NSEG = S // SEG
NP = H // 2
N1, N2 = 32, 64
QS = S // 4
PITCH = N1 + 8
CLASSES = ((0, 8, 4, 12), (1, 15, 9, 7), (2, 14, 10, 6), (3, 13, 11, 5))
_E = lambda k, d: int(os.environ.get(k, d))
LAG1, LAG2, SPLIT = _E("LAG1", 1), _E("LAG2", 2), _E("SPLIT", 28)
HOOK_AT = _E("HOOK_AT", 17)
ONLY = os.environ.get("ONLY", "")
KSPLIT = _E("KSPLIT", 1)
NOSPEC = _E("NOSPEC", 0)
STAGE = os.environ.get("STAGE", "qkvp")
ORDER = os.environ.get("ORDER", "vqskp")
DMAPOS = _E("DMAPOS", 0)
B0, BD, BW, BV, BL = _E("B0", 0), _E("BD", 7), _E("BW", 8), _E("BV", 8), _E("BL", 3)
PINCB = _E("PINCB", 1)
NQ = 2
(SEM_W, SEM_GF, SEM_GI, SEM_SM, SEM_GS, SEM_NYQ, SEM_WO, SEM_MEM, SEM_GW, SEM_OUT, SEM_F, SEM_X,
 SEM_W0) = 0, 6, 7, 8, 9, 10, 11, 12, 13, 14, 15, 19, 23
NSEM = SEM_W0 + NQ
RSQ2 = float(np.float32(math.sqrt(0.5)))


def _bfly8(x):
    s = [x[i] + x[i + 4] for i in range(4)]
    d = [x[i] - x[i + 4] for i in range(4)]
    e, f = s[0] + s[2], s[1] + s[3]
    t1, t2 = (d[1] - d[3]) * RSQ2, (d[1] + d[3]) * RSQ2
    return [e + f, e - f, d[0] + t1, t2 + d[2], s[0] - s[2], s[1] - s[3], d[0] - t1, t2 - d[2]]


def _bfly8_t(t):
    e, f = t[0] + t[1], t[0] - t[1]
    s = [e + t[4], f + t[5], e - t[4], f - t[5]]
    t1, t2 = t[2] - t[6], t[3] + t[7]
    d = [t[2] + t[6], (t1 + t2) * RSQ2, t[3] - t[7], (t2 - t1) * RSQ2]
    return [s[i] + d[i] for i in range(4)] + [s[i] - d[i] for i in range(4)]


def _half_pre(vr, vi, lo, roll, where):
    ri = roll(vi)
    return where(lo, vr, ri), where(lo, ri, vr)


def _half_post(g, tp, tm, lo, roll, where):
    if g == 0:
        return tp, tm
    c = float(np.float32(math.cos(math.pi * g / 8)))
    s = float(np.float32(math.sin(math.pi * g / 8)))
    p, r = tp + tm, tp - tm
    rm = roll(where(lo, r, p))
    return where(lo, p, c * rm + s * r), where(lo, rm, c * r - s * rm)


def _cmul_const(v, k, n, sign):
    re, im = v
    k %= n
    if k == 0:
        return re, im
    if 4 * k == n:
        return (-im, re) if sign > 0 else (im, -re)
    if 8 * k == n:
        return (((re - im) * RSQ2, (re + im) * RSQ2) if sign > 0
                else ((re + im) * RSQ2, (im - re) * RSQ2))
    if 8 * k == 3 * n:
        return (((re + im) * -RSQ2, (re - im) * RSQ2) if sign > 0
                else ((im - re) * RSQ2, (re + im) * -RSQ2))
    c, s = math.cos(2 * math.pi * k / n), sign * math.sin(2 * math.pi * k / n)
    return re * c - im * s, re * s + im * c


def _fft(v, sign):
    n = len(v)
    if n == 1:
        return v
    ev, od = _fft(v[0::2], sign), _fft(v[1::2], sign)
    lo, hi = [], []
    for k in range(n // 2):
        er, ei = ev[k]
        if 4 * k == n:
            xr, xi = od[k]
            if sign > 0:
                lo.append((er - xi, ei + xr)); hi.append((er + xi, ei - xr))
            else:
                lo.append((er + xi, ei - xr)); hi.append((er - xi, ei + xr))
            continue
        tr, ti = _cmul_const(od[k], k, n, sign)
        lo.append((er + tr, ei + ti))
        hi.append((er - tr, ei - ti))
    return lo + hi


def _pack_rows(a):
    u = np.ascontiguousarray(a, dtype=np.float32).view(np.uint32)
    b = ((u + 0x7FFF + ((u >> 16) & 1)) >> 16).astype(np.uint32)
    return (b[..., 0::2, :] | (b[..., 1::2, :] << 16)).astype(np.uint32)


def _diag_blocks(full, n, tol):
    k = full.shape[0] // n
    blk = np.kron(np.eye(k), np.ones((n, n)))
    assert np.abs(full * (1 - blk)).max() < tol
    return np.stack([full[n * g:n * g + n, n * g:n * g + n] for g in range(k)])


def _cplx(re, im):
    return np.block([[re, im], [-im, re]])


@functools.lru_cache(maxsize=None)
def _constants():
    k2 = np.stack([np.concatenate([c + 16 * np.arange(32) for c in cls]) for cls in CLASSES])
    n2 = np.arange(D)
    ang = 2 * np.pi * ((k2[:, :, None] * n2[None, None, :]) % D) / D
    rows = np.stack([np.cos(ang), -np.sin(ang)], axis=1)
    wgt = np.where(k2 == 0, 1.0, 2.0)[:, None, :, None]
    fwd = rows.reshape(D, D).T
    inv = (rows * wgt).reshape(D, D) / (S * D)
    bf = np.stack(_bfly8(list(np.eye(8))))
    binv = np.kron(np.linalg.inv(bf), np.eye(128))
    gd = _diag_blocks(binv.T @ fwd, 256, 1e-6)
    gdi = _diag_blocks(inv @ binv, 256, 1e-12)
    eye, lo = np.eye(256), np.arange(128) < 64
    roll = lambda v: np.roll(v, 64, axis=1)
    pre = np.concatenate(_half_pre(eye[:, :128], eye[:, 128:], lo, roll, np.where), axis=1)
    gi = []
    for g in range(4):
        post = np.concatenate(_half_post(g, eye[:, :128], eye[:, 128:], lo, roll, np.where), axis=1)
        gi.append(_diag_blocks(np.linalg.inv(pre) @ gdi[g] @ np.linalg.inv(post), 128, 1e-12))
    gi = np.concatenate(gi)

    b = np.arange(N2)
    k1 = np.arange(N1)[:, None] + N1 * np.arange(N2)[None, :]
    th = 2 * np.pi * ((k1[:, :, None] * b[None, None, :]) % S) / S
    gr, gim = np.cos(th), -np.sin(th)
    full = np.block([[gr, -gim], [gim, gr]])
    kap = np.arange(2 * N2)
    src = ((kap >> 3) & 1) * N2 + (kap >> 4) * 8 + (kap & 7)
    gs = full[:, :, src]
    hr, hi = np.swapaxes(gr, 1, 2), -np.swapaxes(gim, 1, 2)
    gsi = np.block([[hr, -hi], [hi, hr]])

    lane = np.arange(128)
    kb = 8 * (lane % 16) + lane // 16
    t128 = 2 * np.pi * ((lane[:, None] * kb[None, :]) % 128) / 128
    nyf = _cplx(np.cos(t128), -np.sin(t128))
    nyi = _cplx(np.cos(t128).T, np.sin(t128).T)
    i16 = np.arange(16)
    t16 = 2 * np.pi * ((i16[:, None] * i16[None, :]) % 16) / 16
    tw = 2 * np.pi * (i16[:, None] * lane[None, :]) / S
    sm = np.zeros((80, 128), np.float32)
    sm[0:16], sm[16:32] = np.cos(tw), np.sin(tw)
    sm[32:48, :16], sm[48:64, :16] = np.cos(t16), -np.sin(t16)
    sm[64:80, :16], sm[64:80, 16:32] = np.cos(t16), -np.sin(t16)

    gfp = _pack_rows(np.concatenate([gd, nyf[None], nyi[None]]))
    return gfp, _pack_rows(gi), sm, _pack_rows(np.stack([gs, gsi]))


def _mask80():
    r = lax.broadcasted_iota(jnp.int32, (80, 80), 0)
    c = lax.broadcasted_iota(jnp.int32, (80, 80), 1)

    def head(i):
        return jnp.where(i < 64, i >> 5, (i - 64) >> 3)

    def pos(i):
        j = i & 31
        return jnp.where(i < 64, jnp.where(j < M, j, j + 8), M + (i & 7))

    same = head(r) == head(c)
    ok = (pos(r) < M) | (pos(c) <= pos(r))
    return jnp.where(same, jnp.where(ok, 1.0, -1e9), -jnp.inf).astype(F32)


def _as_bf(u):
    return pltpu.bitcast(u, BF)


def _as_u32(b):
    return pltpu.bitcast(b, U32)


def _lo_f32(u):
    return pltpu.bitcast(u << 16, F32)


def _hi_f32(u):
    return pltpu.bitcast(u & jnp.uint32(0xFFFF0000), F32)


def _dot(a, b):
    return jnp.dot(a, b, preferred_element_type=F32)


def _dot_nt(a, b):
    return lax.dot_general(a, b, (((1,), (1,)), ((), ())), preferred_element_type=F32)


def _transpose_u32(u):
    return pltpu.bitcast(pltpu.bitcast(u, F32).T, U32)


def _lanes(rows):
    return lax.broadcasted_iota(jnp.int32, (rows, 128), 1)


def _kernel(x_hbm, mem_hbm, wq_hbm, wk_hbm, wv_hbm, wo_hbm, fr_hbm, fi_hbm, gw_hbm,
            gf_hbm, gi_hbm, sm_hbm, gs_hbm,
            out_hbm,
            x_v, raw, wqkv, wo, st, sto, obuf, sl, fraw, fp, gf, gi, sm, gs, y, out_v, mem_ref, gw_ref,
            nyq, xa, ct, a_s, qkv_s, bb_s, g_s, stg, pst, mf, u_s, v_s, cb, z_s, p_s, zero_s, sem):
    KH = D // 2
    KQ = KH // NQ
    RB, HB = 128, 64
    raw4 = raw.reshape(6, D, 8, DH)
    w_hbm = (wq_hbm, wk_hbm, wv_hbm)
    f_hbm = (fr_hbm, fi_hbm)

    def w_src(c):
        return w_hbm[c // 2].bitcast(U32).at[:, pl.ds(8 * (c % 2), 8), :]

    def wait(dst, k):
        pltpu.make_async_copy(dst, dst, sem.at[k]).wait()

    def kslice(q, e):
        return pl.ds(e * KH + q * KQ, KQ)

    def x_rows(i, a1):
        return pl.ds(pl.multiple_of(i * RB, RB) + QS * a1, RB)

    def f_copies(h):
        return [(f_hbm[a].at[pl.ds(0, D // 2), pl.ds(128 * (4 * h + c), 128)].bitcast(U32),
                 fraw.at[h, a, c], SEM_F + h) for a in range(2) for c in range(4)]

    def w_copy(c):
        return [(w_src(c), raw4.at[c], SEM_W + c)]

    copies = [(gf_hbm, gf, SEM_GF)]
    copies += [(x_hbm.at[x_rows(i, a1), :], x_v.at[x_rows(i, a1), :], SEM_X + i)
               for i in range(QS // RB) for a1 in range(4)]
    copies += [(sm_hbm, sm, SEM_SM)]
    copies += [(f_hbm[a].at[pl.ds(D // 2, 1), :], nyq.at[a], SEM_NYQ) for a in range(2)]
    copies += [(w_src(0).at[kslice(q, e)], raw4.at[0, kslice(q, e)], SEM_W0 + q)
               for q in range(NQ) for e in range(2)]
    copies += f_copies(0) + w_copy(1) + f_copies(1) + w_copy(2) + f_copies(2) + f_copies(3)
    copies += [(gs_hbm, gs, SEM_GS)] + w_copy(3) + w_copy(4) + w_copy(5)
    copies += [(wo_hbm.bitcast(U32).at[:, pl.ds(128 * j, 128)], wo.at[j], SEM_WO) for j in range(8)]
    copies += [(gi_hbm, gi, SEM_GI), (mem_hbm, mem_ref, SEM_MEM), (gw_hbm, gw_ref, SEM_GW)]
    for src, dst, k in copies:
        pltpu.make_async_copy(src, dst, sem.at[k]).start()

    def prep_rhs(ch, jj, k0, nk):
        item = 8 * ch + jj
        a1 = raw[ch, pl.ds(k0 * 8 + jj, nk, stride=8), :]
        a2 = raw[ch, pl.ds((KH + k0) * 8 + jj, nk, stride=8), :]
        b11, b12, b21, b22 = _lo_f32(a1), _hi_f32(a1), _lo_f32(a2), _hi_f32(a2)
        for p, e, b in ((0, 0, b11), (1, 0, b12), (0, 1, b21), (1, 1, b22)):
            wqkv[2 * item + p, pl.ds((e * KH + k0) // 2, nk // 2), :] = _as_u32(b.astype(BF))
        return [v.astype(BF) for v in (b11 + b22, b11, b12 - b22, b21 - b11, b22, b11 + b12, b21 + b22)]

    def strassen(rhs, k0, nk, init, finish, after_dot):
        def prod(i):
            return _dot(_as_bf(sl[i, :, pl.ds(k0, nk)]), rhs[i])

        def plus(i, r):
            return r if init is None else init(i) + r

        m = prod(1)
        cb[0] = m
        after_dot(0, m)
        m = prod(4)
        cb[1] = m
        after_dot(1, m)
        m = prod(0)
        cb[2] = plus(0, m - cb[1])
        cb[3] = plus(3, m - cb[0])
        after_dot(2, m)
        m = prod(3)
        cb[4] = plus(2, cb[0] + m)
        cb[2] = cb[2] + m
        after_dot(3, m)
        m = prod(2)
        cb[5] = plus(1, cb[1] + m)
        cb[3] = cb[3] + m
        after_dot(4, m)
        m = prod(6) + cb[2]
        finish(0, m, cb[5])
        after_dot(5, m)
        m = prod(5) + cb[3]
        finish(1, cb[4], m)
        after_dot(6, m)

    def store_st(item, e, c1, c2):
        r = jnp.concatenate([c.reshape(NSEG // 2, 8, 128) for c in (c1, c2)], axis=1)
        st[item, 256 * e:256 * e + 256, :] = _as_u32(r.reshape(8 * NSEG, 128).astype(BF))

    def pin(i, c):
        if PINCB:
            cb[i, 0:8, :] = jnp.zeros((8, 128), F32)
        zero_s[i] = 0
        z_s[i, 0:8, :] = jnp.zeros((8, 128), U32)
        p_s[i, 0:8, :] = jnp.zeros((8, 128), F32)
        u_s[i, 0:8, :] = jnp.zeros((8, 128), U32)
        stg[i, 0, 0:8, :] = jnp.zeros((8, 128), U32)
        obuf[i, 0:8, :] = jnp.zeros((8, 128), U32)
        return c

    lax.fori_loop(0, 2, pin, 0)

    wait(gf, SEM_GF)

    def f1(i, c):
        for a1 in range(4):
            wait(x_v.at[x_rows(i, a1), :], SEM_X + i)
        base = pl.multiple_of(i * RB, RB)
        alt = (1 - 2 * (_lanes(16) & 1)).astype(F32).astype(BF)
        u0 = [[] for _ in range(4)]
        for h0 in range(0, RB, HB):
            pieces, first8 = [], []
            for a1 in range(4):
                for r in range(h0, h0 + HB, 16):
                    xs = x_v[pl.ds(base + (QS * a1 + r), 16), :].astype(F32)
                    if r % SEG == 0:
                        first8.append(xs[0:8])
                    us = _bfly8([xs[:, 128 * a:128 * a + 128] for a in range(8)])
                    pieces.append(jnp.concatenate(us, axis=1).astype(BF))
                    u0[a1].append(pieces[-1][:, :128])
            ub = jnp.concatenate(pieces, axis=0)
            for a1 in range(2):
                top = jnp.concatenate(first8[2 * a1:2 * a1 + 2], axis=0)
                bot = jnp.concatenate(first8[2 * a1 + 4:2 * a1 + 6], axis=0)
                a11, a12, a21, a22 = top[:, :KH], top[:, KH:], bot[:, :KH], bot[:, KH:]
                row = pl.multiple_of((base + (QS * a1 + h0)) // 8, 8)
                for k, v in enumerate((a11 + a22, a21 + a22, a11, a22, a11 + a12, a21 - a11, a12 - a22)):
                    sl[k, pl.ds(row, 8), :] = _as_u32(v.astype(BF))
            if h0 + HB == RB:
                for a1 in range(4):
                    xa[pl.ds(4 * a1 + i, 1), :] = _dot_nt(alt, jnp.concatenate(u0[a1], axis=0))[0:1]
            for g in range(4):
                yy = _dot(ub[:, 256 * g:256 * g + 256], _as_bf(gf[g]))
                v = _fft([(yy[HB * a1:HB * a1 + HB, :128], yy[HB * a1:HB * a1 + HB, 128:])
                          for a1 in range(4)], -1)
                for k1 in range(4):
                    rows = pl.ds(base + (QS * k1 + h0), HB)
                    y[g, 0, rows, :] = v[k1][0]
                    y[g, 1, rows, :] = v[k1][1]
        return c

    with jax.named_scope("f1"):
        if ONLY in ("", "f1"):
            lax.fori_loop(0, QS // RB, f1, 0)
        else:
            for i in range(4):
                for a1 in range(4):
                    wait(x_v.at[x_rows(i, a1), :], SEM_X + i)

    def fprep(h, c):
        ev, od = [], []
        for r in range(8):
            wr = fraw[h, 0, c, pl.ds(r, 32, stride=8), :]
            wi = fraw[h, 1, c, pl.ds(r, 32, stride=8), :]
            ev.append((wr & jnp.uint32(0xFFFF)) | (wi << 16))
            od.append((wr >> 16) | (wi & jnp.uint32(0xFFFF0000)))
        for g, cls in enumerate(CLASSES):
            t = _transpose_u32(jnp.concatenate([(od if k % 2 else ev)[k // 2] for k in cls], axis=0))
            for q in range(128 // N1):
                row = pl.multiple_of(((4 * h + c) * (128 // N1) + q) * PITCH, 8)
                fp[g, pl.ds(row, N1), :] = t[q * N1:(q + 1) * N1]

    def nyquist():
        twc, tws = sm[0:16], sm[16:32]
        u = _dot(sm[32:64, 0:16].astype(BF), xa[...].astype(BF))
        ur, ui = u[0:16], u[16:32]
        u = jnp.concatenate([ur * twc + ui * tws, ui * twc - ur * tws], axis=1).astype(BF)
        yield
        xx = _dot(u, _as_bf(gf[4]))
        xr, xi = xx[:, :128], xx[:, 128:]
        w = (pltpu.bitcast(nyq[0].astype(F32), U32) >> 16) | pltpu.bitcast(nyq[1].astype(F32), U32)
        w = jnp.concatenate([w[:, 128 * a:128 * a + 128] for a in range(16)], axis=0)
        wt = _transpose_u32(jnp.concatenate([w] * 8, axis=0))
        blk = _lanes(16) >> 4
        wm = wt[0:16]
        for j in range(1, 8):
            wm = jnp.where(blk == j, wt[16 * j:16 * j + 16], wm)
        wr, wi = _lo_f32(wm), _hi_f32(wm)
        z = jnp.concatenate([xr * wr - xi * wi, xr * wi + xi * wr], axis=1).astype(BF)
        yield
        pp = _dot(z, _as_bf(gf[5]))
        pr, pi = pp[:, :128], pp[:, 128:]
        pp = jnp.concatenate([pr * twc - pi * tws, pi * twc + pr * tws], axis=0).astype(BF)
        yield
        cc = _dot(sm[64:80, 0:32].astype(BF), pp) * (1.0 / (S * D))
        ct[...] = jnp.concatenate([cc, jnp.zeros((112, 128), F32)], axis=0).T
        yield

    def s_rows(k1, a0, r):
        return pl.ds(r + (QS * k1 + N2 * a0), 8)

    def anchored(v, tok):
        return jnp.where(zero_s[0] != 0, tok, v)

    def s_prep(g, k1, r, tok):
        v = [(y[g, 0, s_rows(k1, a0, r), :], y[g, 1, s_rows(k1, a0, r), :]) for a0 in range(8)]
        v[0] = (anchored(v[0][0], tok), v[0][1])
        v = _fft([_cmul_const(v[a0], a0 * k1, N1, -1) for a0 in range(8)], -1)
        for k0 in range(8):
            u_s[k1 + 4 * k0, pl.ds(r, 8), :] = _as_u32(jnp.concatenate(v[k0], axis=0).astype(BF))

    def s_fwd(g, ka, tok):
        xx = _dot(_as_bf(gs[0, ka]), _as_bf(u_s[ka]))
        w32 = fp[g, pl.ds(ka, N2, stride=PITCH), :]
        wr, wi = _lo_f32(w32), _hi_f32(w32)
        xr, xi = xx[:N2], xx[N2:]
        z_s[ka] = _as_u32(jnp.concatenate([xr * wr - xi * wi, xr * wi + xi * wr], axis=0).astype(BF))

    def s_inv(ka, tok):
        p_s[ka] = _dot(_as_bf(gs[1, ka]), _as_bf(z_s[ka]))

    def s_post(g, k1, r, tok):
        v = [(p_s[k1 + 4 * k0, r:r + 8, :], p_s[k1 + 4 * k0, N2 + r:N2 + r + 8, :]) for k0 in range(8)]
        v[0] = (anchored(v[0][0], tok), anchored(v[0][1], tok))
        v = _fft(v, 1)
        for a0 in range(8):
            vr, vi = _cmul_const(v[a0], a0 * k1, N1, 1)
            v_s[g, 0, s_rows(k1, a0, r), :] = vr
            v_s[g, 1, s_rows(k1, a0, r), :] = vi

    def acc(jj, i):
        return v_s.at[jj // 4, (jj // 2) % 2, pl.ds(1024 * (jj % 2) + 256 * i, 256), :]

    def bulk(item0, n, events, q=None):
        k0, nk = (0, KH) if q is None else (q * KQ, KQ)
        for i in range(n):
            item = item0 + i

            def hook(k, m):
                pieces = events.get(7 * i + k, ())
                vec = [pc for pc in pieces if getattr(pc, "func", None) in (s_prep, s_post)]
                for piece in pieces:
                    r = 8 * ((32 * vec.index(piece)) // len(vec)) if piece in vec else 0
                    piece(m[r:r + 8])

            def finish(e, c1, c2):
                if q in (None, NQ - 1):
                    store_st(item, e, c1, c2)
                else:
                    acc(item, 2 * e)[...] = c1
                    acc(item, 2 * e + 1)[...] = c2

            init = None if q in (None, 0) else (lambda k: acc(item, k)[...])
            strassen(prep_rhs(item // 8, item % 8, k0, nk), k0, nk, init, finish, hook)

    def spread(events, pieces, q0, q1):
        for i, piece in enumerate(pieces):
            events.setdefault(q0 + ((q1 - q0) * i) // len(pieces), []).append(piece)

    P = functools.partial

    def loop_a(h, c):
        @pl.when(h % 2 == 0)
        def _():
            wait(raw4.at[1 + h // 2], SEM_W + 1 + h // 2)

        wait(fraw.at[h], SEM_F + h)
        events = {}
        spread(events, [lambda tok, c=c: fprep(h, c) for c in range(4)], 0, 24)
        bulk(8 + 4 * h, 4, events)
        return c

    def loop_b(g, c):
        @pl.when(g < 3)
        def _():
            wait(raw4.at[3 + g], SEM_W + 3 + g)

        gn = jnp.minimum(g + 1, 3)
        events = {}
        for k1 in range(4):
            q = B0 + BD * k1
            spread(events, [P(s_fwd, g, k1 + 4 * k0) for k0 in range(8)], q, q + BW)
            spread(events, [P(s_prep, gn, k1, r) for r in range(0, N2, 8)], q + BW, q + BW + BV)
            q = max(q + BL, 0)
            spread(events, [P(s_inv, k1 + 4 * k0) for k0 in range(8)], q, q + BW)
            spread(events, [P(s_post, g, k1, r) for r in range(0, N2, 8)], q + BW, q + BW + BV)
        assert max(events) < 41
        for q in sorted(q for q in events if q < 0):
            for piece in events[q]:
                piece(None)
        bulk(24 + 6 * g, 6, events)
        return c

    wait(sm, SEM_SM)
    wait(nyq, SEM_NYQ)
    with jax.named_scope("p0"):
        ny = nyquist()
        for q in range(NQ):
            for e in range(2):
                wait(raw4.at[0, kslice(q, e)], SEM_W0 + q)
            events = {}
            if q == 0:
                spread(events, [lambda tok: next(ny)] * 4, 4, 28)
            spread(events, [P(s_prep, 0, k1, r) for k1 in range(4 * q // NQ, 4 * (q + 1) // NQ)
                            for r in range(0, N2, 8)], 0, 52)
            if ONLY in ("", "p0"):
                bulk(0, 8, events, q)
    with jax.named_scope("loop_a"):
        if ONLY in ("", "a"):
            lax.fori_loop(0, 4, loop_a, 0)
        else:
            for h in range(4):
                wait(fraw.at[h], SEM_F + h)
            for h in range(2):
                wait(raw4.at[1 + h], SEM_W + 1 + h)
    wait(gs, SEM_GS)
    with jax.named_scope("loop_b"):
        if ONLY in ("", "b"):
            lax.fori_loop(0, 4, loop_b, 0)
        else:
            for g in range(3):
                wait(raw4.at[g + 3], SEM_W + 3 + g)
    wait(wo, SEM_WO)
    wait(gi, SEM_GI)
    wait(mem_ref, SEM_MEM)
    wait(gw_ref, SEM_GW)

    scale = DH ** -0.5

    mf[...] = _mask80()

    def softmax(s):
        fill = mf[...]
        s = jnp.where(fill > 0.0, s * scale, fill)
        m = jnp.max(s, axis=-1, keepdims=True)
        e = jnp.exp(s - m)
        l = jnp.sum(e, axis=-1, keepdims=True)
        return (e * (1.0 / l)).astype(BF)

    def lhs_rows(mem, seg):
        xs = x_v[pl.ds(pl.multiple_of(seg * SEG, SEG), SEG), :].astype(F32)
        return jnp.concatenate([mem, xs[8:SEG]], axis=0).astype(BF)

    def proj2(a, m, j):
        return jnp.concatenate([_dot(a, _as_bf(wqkv[H * m + 2 * j + p])).astype(BF) for p in range(2)], axis=0)

    def proj_first(a):
        if not KSPLIT:
            return [proj2(a, m, 0) for m in range(3)]
        part = [_dot(a[:, :D // 2], _as_bf(wqkv[H * (i // 2) + i % 2, 0:D // 4, :])) for i in range(6)]
        full = [(_dot(a[:, D // 2:], _as_bf(wqkv[H * (i // 2) + i % 2, D // 4:D // 2, :])) + part[i]).astype(BF)
                for i in range(6)]
        return [jnp.concatenate(full[2 * m:2 * m + 2], axis=0) for m in range(3)]

    def step(a, seg, first, hook=None):
        R = 32 if first else 48
        qkv, ps = {}, {}
        srow = pl.multiple_of(seg * 8, 8)

        def put(m, j, r):
            if "qkv"[m] in STAGE:
                stg[m, j % 8] = _as_u32(r)
            else:
                qkv[m, j] = r

        def get(m, j):
            r = _as_bf(stg[m, j % 8]) if "qkv"[m] in STAGE else qkv[m, j]
            return jnp.concatenate([r, _as_bf(st[NP * m + j, pl.ds(srow, 8), :])], axis=0)

        def proj(j, m):
            if j == 0:
                if m == 0:
                    r = [_as_bf(qkv_s[m]) for m in range(3)] if first else proj_first(a)
                    for mm in range(3):
                        put(mm, 0, r[mm])
            else:
                put(m, j, proj2(a, m, j))

        def scores(j):
            pp = softmax(_dot_nt(get(0, j), get(1, j)))
            if "p" in STAGE:
                pst[j % 8] = _as_u32(pp)
            else:
                ps[j] = pp

        def pv(j):
            o = _dot(_as_bf(pst[j % 8]) if "p" in STAGE else ps[j], get(2, j))
            for i in range(2):
                h = 2 * j + i
                if first:
                    ob = o[32 * i:32 * i + 32].astype(BF)
                    sto[h] = o[64 + 8 * i:72 + 8 * i]
                else:
                    ob = jnp.concatenate([o[32 * i:32 * i + 32], o[64 + 8 * i:72 + 8 * i], sto[h]],
                                         axis=0).astype(BF)
                obuf[h, 0:R // 2, :] = _as_u32(ob)

        def wo_part(j, h0, h1):
            og = jnp.concatenate([_as_bf(obuf[h, 0:R // 2, :]) for h in range(h0, h1)], axis=1)
            return _dot(og, _as_bf(wo[j, h0 * 64:h1 * 64, :]))

        parts = []
        for i in range(NP + 4):
            for ch in ORDER:
                if ch in "qkv":
                    m = "qkv".index(ch)
                    if i < NP:
                        proj(i, m)
                    elif m < 2:
                        parts.append(wo_part(2 * (i - NP) + len(parts) % 2, 0, SPLIT))
                elif ch == "s" and 0 <= i - LAG1 < NP:
                    scores(i - LAG1)
                elif ch == "p" and 0 <= i - LAG2 < NP:
                    pv(i - LAG2)
            if hook is not None and i == HOOK_AT:
                hook()
        return jnp.concatenate([wo_part(j, SPLIT, H) + parts[j] for j in range(8)], axis=1)

    def start_pair(mem, t):
        a = lhs_rows(mem, 2 * t)
        a_s[...] = _as_u32(a)
        for m, r in enumerate(proj_first(a)):
            qkv_s[m] = _as_u32(r)

    def pair(t, c):
        base = pl.multiple_of(t * 64, 64)
        lane = _lanes(64)
        lo = lane < 64
        roll = (lambda v: v + 1.0) if _E('NOROLL', 0) else (lambda v: pltpu.roll(v, 64, 1))
        a1 = t // 8
        off = pl.multiple_of((t % 8) * 64, 64)
        s2 = (1 - 2 * (a1 & 1)).astype(F32)
        sg = (1 - (a1 & 2)).astype(F32)
        cc, ss = sg * (1 - (a1 & 1)).astype(F32), sg * (a1 & 1).astype(F32)

        def irfft_group(g):
            q = [[v_s[g, e, pl.ds(off + QS * k1, 64), :] for e in range(2)] for k1 in range(4)]
            br, bi = q[1][0] + s2 * q[3][0], q[1][1] + s2 * q[3][1]
            vr = q[0][0] + s2 * q[2][0] + (cc * br - ss * bi)
            vi = q[0][1] + s2 * q[2][1] + (cc * bi + ss * br)
            tin = _half_pre(vr, vi, lo, roll, jnp.where)
            tp, tm = [_dot(tin[e].astype(BF), _as_bf(gi[2 * g + e])) for e in range(2)]
            if g == 0:
                nyc = jnp.sum(jnp.where(lane == t // 2,
                                        ct[pl.ds(pl.multiple_of((t % 2) * 64, 64), 64), :], 0.0),
                              axis=-1, keepdims=True)
                tp = tp + nyc * (1 - 2 * (lane & 1)).astype(F32)
            return list(_half_post(g, tp, tm, lo, roll, jnp.where))

        def spectral_part():
            ts = sum([irfft_group(g) for g in range(4)], [])
            b = jnp.concatenate(_bfly8_t(ts), axis=1).astype(BF).astype(F32)
            xs = x_v[pl.ds(base, 64), :].astype(F32)
            gate = jax.nn.sigmoid(jnp.sum(xs * gw_ref[...].astype(F32), axis=-1, keepdims=True))
            bb = (1.0 - gate) * b
            bb_s[...] = jnp.concatenate([bb[0:8], bb[8:32] + gate[8:32] * bb_s[8:32], bb[32:64]], axis=0)
            g_s[...] = jnp.broadcast_to(gate, (64, 128))

        res_a = step(_as_bf(a_s[...]), 2 * t, True)
        bb_s[8:32] = res_a[8:32]
        a = lhs_rows(res_a[0:8].astype(BF).astype(F32), 2 * t + 1)
        res_b = step(a, 2 * t + 1, False, None if NOSPEC else spectral_part)

        def gated(r0, r1, res):
            return bb_s[r0:r1] + jnp.concatenate([g_s[r0:r1]] * 8, axis=1) * res

        out_v[pl.ds(base, 64), :] = jnp.concatenate(
            [gated(0, 8, res_b[40:48]), bb_s[8:32], gated(32, 40, res_b[32:40]), gated(40, 64, res_b[8:32])],
            axis=0).astype(BF)
        cp = pltpu.make_async_copy(out_v.at[pl.ds(base, 64), :], out_hbm.at[pl.ds(base, 64), :],
                                   sem.at[SEM_OUT])
        if DMAPOS == 0:
            cp.start()
        start_pair(res_b[0:8].astype(BF).astype(F32), jnp.minimum(t + 1, S // 64 - 1))
        if DMAPOS == 1:
            cp.start()
        return c

    with jax.named_scope("chain"):
        if ONLY in ("", "chain"):
            start_pair(mem_ref[...].astype(F32), 0)
            lax.fori_loop(0, S // 64, pair, 0)
            if DMAPOS == 2:
                pltpu.make_async_copy(out_v, out_hbm, sem.at[SEM_OUT]).start()
    if ONLY not in ("", "chain"):
        def keep(i, c):
            v = st[i, 0:8, :] + wqkv[i, 0:8, :] + fp[i % 4, 0:8, :] + u_s[i % 32, 0:8, :] + pltpu.bitcast(y[i % 4, 0, pl.ds(8 * i, 8), :] + v_s[i % 4, 0, pl.ds(8 * i, 8), :] + ct[pl.ds(i, 8), :] + xa[0:8], U32) + sl[i % 7, 0:8, 0:128]
            out_v[pl.ds(16 * i, 16), 0:128] = _as_bf(v)
            return c
        lax.fori_loop(0, 48, keep, 0)
        pltpu.make_async_copy(out_v, out_hbm, sem.at[SEM_OUT]).start()
        pltpu.make_async_copy(out_v, out_hbm, sem.at[SEM_OUT]).wait()
    with jax.named_scope("fin"):
        if ONLY in ("", "chain"):
            pltpu.make_async_copy(out_v, out_hbm, sem.at[SEM_OUT]).wait()


@functools.partial(jax.jit, static_argnames=("A_seg_len",))
def pallas_gated_mix__memory_aug_recurrent_mem_tr__spectral_gfnet__prompt_kernel(
    A_x, A_mem0, A_Wq, A_Wk, A_Wv, A_Wo, A_seg_len, B_x, B_w_r, B_w_i, gate_w,
):
    assert A_x.shape == (1, S, D) and A_mem0.shape == (1, M, D) and A_Wq.shape == (D, H, DH)
    assert int(A_seg_len) == SEG
    consts = [jnp.asarray(c) for c in _constants()]
    any_spec = pl.BlockSpec(memory_space=pl.ANY)
    out = pl.pallas_call(
        _kernel,
        out_shape=jax.ShapeDtypeStruct((S, D), BF),
        in_specs=[any_spec] * 13,
        out_specs=any_spec,
        scratch_shapes=[
            pltpu.VMEM((S, D), BF),
            pltpu.VMEM((6, D * 8, DH), U32),
            pltpu.VMEM((3 * H, D // 2, DH), U32),
            pltpu.VMEM((8, H * DH // 2, 128), U32),
            pltpu.VMEM((3 * NP, 8 * NSEG, 128), U32),
            pltpu.VMEM((H, 8, 128), F32),
            pltpu.VMEM((H, 24, 128), U32),
            pltpu.VMEM((7, 2 * NSEG, D // 2), U32),
            pltpu.VMEM((4, 2, 4, 256, 128), U32),
            pltpu.VMEM((4, N2 * PITCH, 128), U32),
            pltpu.VMEM((6, 128, 256), U32),
            pltpu.VMEM((8, 64, 128), U32),
            pltpu.VMEM((80, 128), F32),
            pltpu.VMEM((2, N1, N2, 2 * N2), U32),
            pltpu.VMEM((4, 2, S, 128), F32),
            pltpu.VMEM((S, D), BF),
            pltpu.VMEM((M, D), BF),
            pltpu.VMEM((1, D), BF),
            pltpu.VMEM((2, 1, S), BF),
            pltpu.VMEM((16, 128), F32),
            pltpu.VMEM((128, 128), F32),
            pltpu.VMEM((16, D), U32),
            pltpu.VMEM((3, 32, 128), U32),
            pltpu.VMEM((64, D), F32),
            pltpu.VMEM((64, 128), F32),
            pltpu.VMEM((3, 8, 32, 128), U32),
            pltpu.VMEM((8, 40, 80), U32),
            pltpu.VMEM((80, 80), F32),
            pltpu.VMEM((N1, N2, 128), U32),
            pltpu.VMEM((4, 2, S, 128), F32),
            pltpu.VMEM((6, 256, 128), F32),
            pltpu.VMEM((N1, N2, 128), U32),
            pltpu.VMEM((N1, 2 * N2, 128), F32),
            pltpu.SMEM((2,), jnp.int32),
            pltpu.SemaphoreType.DMA((NSEM,)),
        ],
        compiler_params=pltpu.CompilerParams(vmem_limit_bytes=120 * 1024 * 1024),
    )(
        A_x.reshape(S, D), A_mem0.reshape(M, D), A_Wq, A_Wk, A_Wv,
        A_Wo.reshape(H * DH, D), B_w_r.T, B_w_i.T, gate_w.reshape(1, D), *consts,
    )
    return out.reshape(1, S, D)
```

```python
import functools
import math
import os

import numpy as np
import jax
import jax.numpy as jnp
from jax import lax
import jax.experimental.pallas as pl
import jax.experimental.pallas.tpu as pltpu

BF, F32, U32 = jnp.bfloat16, jnp.float32, jnp.uint32

S, D, H, DH, M, SEG = 2048, 1024, 32, 128, 8, 32
NSEG = S // SEG
NP = H // 2
N1, N2 = 32, 64
QS = S // 4
PITCH = N1 + 8
CLASSES = ((0, 8, 4, 12), (1, 15, 9, 7), (2, 14, 10, 6), (3, 13, 11, 5))
_E = lambda k, d: int(os.environ.get(k, d))
LAG1, LAG2, SPLIT = _E("LAG1", 1), _E("LAG2", 2), _E("SPLIT", 28)
HOOK_AT = _E("HOOK_AT", 17)
ONLY = os.environ.get("ONLY", "")
KSPLIT = _E("KSPLIT", 1)
NOSPEC = _E("NOSPEC", 0)
STAGE = os.environ.get("STAGE", "qkvp")
ORDER = os.environ.get("ORDER", "vqskp")
DMAPOS = _E("DMAPOS", 0)
B0, BD, BW, BV, BL = _E("B0", 0), _E("BD", 7), _E("BW", 8), _E("BV", 8), _E("BL", 3)
PINCB = _E("PINCB", 1)
VATT = _E("VATT", 0)
NTG = _E("NTG", 3)
DL = _E("DL", 0)
NQ = 2
(SEM_W, SEM_GF, SEM_GI, SEM_SM, SEM_GS, SEM_NYQ, SEM_WO, SEM_MEM, SEM_GW, SEM_OUT, SEM_F, SEM_X,
 SEM_W0) = 0, 6, 7, 8, 9, 10, 11, 12, 13, 14, 15, 19, 23
NSEM = SEM_W0 + NQ
RSQ2 = float(np.float32(math.sqrt(0.5)))


def _bfly8(x):
    s = [x[i] + x[i + 4] for i in range(4)]
    d = [x[i] - x[i + 4] for i in range(4)]
    e, f = s[0] + s[2], s[1] + s[3]
    t1, t2 = (d[1] - d[3]) * RSQ2, (d[1] + d[3]) * RSQ2
    return [e + f, e - f, d[0] + t1, t2 + d[2], s[0] - s[2], s[1] - s[3], d[0] - t1, t2 - d[2]]


def _bfly8_t(t):
    e, f = t[0] + t[1], t[0] - t[1]
    s = [e + t[4], f + t[5], e - t[4], f - t[5]]
    t1, t2 = t[2] - t[6], t[3] + t[7]
    d = [t[2] + t[6], (t1 + t2) * RSQ2, t[3] - t[7], (t2 - t1) * RSQ2]
    return [s[i] + d[i] for i in range(4)] + [s[i] - d[i] for i in range(4)]


def _half_pre(vr, vi, lo, roll, where):
    ri = roll(vi)
    return where(lo, vr, ri), where(lo, ri, vr)


def _half_post(g, tp, tm, lo, roll, where):
    if g == 0:
        return tp, tm
    c = float(np.float32(math.cos(math.pi * g / 8)))
    s = float(np.float32(math.sin(math.pi * g / 8)))
    p, r = tp + tm, tp - tm
    rm = roll(where(lo, r, p))
    return where(lo, p, c * rm + s * r), where(lo, rm, c * r - s * rm)


def _cmul_const(v, k, n, sign):
    re, im = v
    k %= n
    if k == 0:
        return re, im
    if 4 * k == n:
        return (-im, re) if sign > 0 else (im, -re)
    if 8 * k == n:
        return (((re - im) * RSQ2, (re + im) * RSQ2) if sign > 0
                else ((re + im) * RSQ2, (im - re) * RSQ2))
    if 8 * k == 3 * n:
        return (((re + im) * -RSQ2, (re - im) * RSQ2) if sign > 0
                else ((im - re) * RSQ2, (re + im) * -RSQ2))
    c, s = math.cos(2 * math.pi * k / n), sign * math.sin(2 * math.pi * k / n)
    return re * c - im * s, re * s + im * c


def _fft(v, sign):
    n = len(v)
    if n == 1:
        return v
    ev, od = _fft(v[0::2], sign), _fft(v[1::2], sign)
    lo, hi = [], []
    for k in range(n // 2):
        er, ei = ev[k]
        if 4 * k == n:
            xr, xi = od[k]
            if sign > 0:
                lo.append((er - xi, ei + xr)); hi.append((er + xi, ei - xr))
            else:
                lo.append((er + xi, ei - xr)); hi.append((er - xi, ei + xr))
            continue
        tr, ti = _cmul_const(od[k], k, n, sign)
        lo.append((er + tr, ei + ti))
        hi.append((er - tr, ei - ti))
    return lo + hi


def _pack_rows(a):
    u = np.ascontiguousarray(a, dtype=np.float32).view(np.uint32)
    b = ((u + 0x7FFF + ((u >> 16) & 1)) >> 16).astype(np.uint32)
    return (b[..., 0::2, :] | (b[..., 1::2, :] << 16)).astype(np.uint32)


def _diag_blocks(full, n, tol):
    k = full.shape[0] // n
    blk = np.kron(np.eye(k), np.ones((n, n)))
    assert np.abs(full * (1 - blk)).max() < tol
    return np.stack([full[n * g:n * g + n, n * g:n * g + n] for g in range(k)])


def _cplx(re, im):
    return np.block([[re, im], [-im, re]])


@functools.lru_cache(maxsize=None)
def _constants():
    k2 = np.stack([np.concatenate([c + 16 * np.arange(32) for c in cls]) for cls in CLASSES])
    n2 = np.arange(D)
    ang = 2 * np.pi * ((k2[:, :, None] * n2[None, None, :]) % D) / D
    rows = np.stack([np.cos(ang), -np.sin(ang)], axis=1)
    wgt = np.where(k2 == 0, 1.0, 2.0)[:, None, :, None]
    fwd = rows.reshape(D, D).T
    inv = (rows * wgt).reshape(D, D) / (S * D)
    bf = np.stack(_bfly8(list(np.eye(8))))
    binv = np.kron(np.linalg.inv(bf), np.eye(128))
    gd = _diag_blocks(binv.T @ fwd, 256, 1e-6)
    gdi = _diag_blocks(inv @ binv, 256, 1e-12)
    eye, lo = np.eye(256), np.arange(128) < 64
    roll = lambda v: np.roll(v, 64, axis=1)
    pre = np.concatenate(_half_pre(eye[:, :128], eye[:, 128:], lo, roll, np.where), axis=1)
    gi = []
    for g in range(4):
        post = np.concatenate(_half_post(g, eye[:, :128], eye[:, 128:], lo, roll, np.where), axis=1)
        gi.append(_diag_blocks(np.linalg.inv(pre) @ gdi[g] @ np.linalg.inv(post), 128, 1e-12))
    gi = np.concatenate(gi)

    b = np.arange(N2)
    k1 = np.arange(N1)[:, None] + N1 * np.arange(N2)[None, :]
    th = 2 * np.pi * ((k1[:, :, None] * b[None, None, :]) % S) / S
    gr, gim = np.cos(th), -np.sin(th)
    full = np.block([[gr, -gim], [gim, gr]])
    kap = np.arange(2 * N2)
    src = ((kap >> 3) & 1) * N2 + (kap >> 4) * 8 + (kap & 7)
    gs = full[:, :, src]
    hr, hi = np.swapaxes(gr, 1, 2), -np.swapaxes(gim, 1, 2)
    gsi = np.block([[hr, -hi], [hi, hr]])

    lane = np.arange(128)
    kb = 8 * (lane % 16) + lane // 16
    t128 = 2 * np.pi * ((lane[:, None] * kb[None, :]) % 128) / 128
    nyf = _cplx(np.cos(t128), -np.sin(t128))
    nyi = _cplx(np.cos(t128).T, np.sin(t128).T)
    i16 = np.arange(16)
    t16 = 2 * np.pi * ((i16[:, None] * i16[None, :]) % 16) / 16
    tw = 2 * np.pi * (i16[:, None] * lane[None, :]) / S
    sm = np.zeros((80, 128), np.float32)
    sm[0:16], sm[16:32] = np.cos(tw), np.sin(tw)
    sm[32:48, :16], sm[48:64, :16] = np.cos(t16), -np.sin(t16)
    sm[64:80, :16], sm[64:80, 16:32] = np.cos(t16), -np.sin(t16)

    gfp = _pack_rows(np.concatenate([gd, nyf[None], nyi[None]]))
    return gfp, _pack_rows(gi), sm, _pack_rows(np.stack([gs, gsi]))


def _mask80():
    r = lax.broadcasted_iota(jnp.int32, (80, 80), 0)
    c = lax.broadcasted_iota(jnp.int32, (80, 80), 1)

    def head(i):
        return jnp.where(i < 64, i >> 5, (i - 64) >> 3)

    def pos(i):
        j = i & 31
        return jnp.where(i < 64, jnp.where(j < M, j, j + 8), M + (i & 7))

    same = head(r) == head(c)
    ok = (pos(r) < M) | (pos(c) <= pos(r))
    return jnp.where(same, jnp.where(ok, 1.0, -1e9), -jnp.inf).astype(F32)


def _as_bf(u):
    return pltpu.bitcast(u, BF)


def _as_u32(b):
    return pltpu.bitcast(b, U32)


def _lo_f32(u):
    return pltpu.bitcast(u << 16, F32)


def _hi_f32(u):
    return pltpu.bitcast(u & jnp.uint32(0xFFFF0000), F32)


def _dot(a, b):
    return jnp.dot(a, b, preferred_element_type=F32)


def _dot_nt(a, b):
    return lax.dot_general(a, b, (((1,), (1,)), ((), ())), preferred_element_type=F32)


def _transpose_u32(u):
    return pltpu.bitcast(pltpu.bitcast(u, F32).T, U32)


def _lanes(rows):
    return lax.broadcasted_iota(jnp.int32, (rows, 128), 1)


def _kernel(x_hbm, mem_hbm, wq_hbm, wk_hbm, wv_hbm, wo_hbm, fr_hbm, fi_hbm, gw_hbm,
            gf_hbm, gi_hbm, sm_hbm, gs_hbm,
            out_hbm,
            x_v, raw, wqkv, wo, st, sl, fraw, fp, gf, gi, gs, y, v_s, out_v, u_s, cb, z_s, p_s,
            sto, obuf, ct, a_s, qkv_s, bb_s, g_s, stg, pst, gw_s, mem_ref, mf, sm, xa, nyq, gw_ref, zero_s, sem):
    KH = D // 2
    KQ = KH // NQ
    RB, HB = 128, _E('HB', 16)
    raw4 = raw.reshape(6, D, 8, DH)
    w_hbm = (wq_hbm, wk_hbm, wv_hbm)
    f_hbm = (fr_hbm, fi_hbm)

    def w_src(c):
        return w_hbm[c // 2].bitcast(U32).at[:, pl.ds(8 * (c % 2), 8), :]

    def wait(dst, k):
        pltpu.make_async_copy(dst, dst, sem.at[k]).wait()

    def kslice(q, e):
        return pl.ds(e * KH + q * KQ, KQ)

    def x_rows(i, a1):
        return pl.ds(pl.multiple_of(i * RB, RB) + QS * a1, RB)

    def f_copies(h):
        return [(f_hbm[a].at[pl.ds(0, D // 2), pl.ds(128 * (4 * h + c), 128)].bitcast(U32),
                 fraw.at[h, a, c], SEM_F + h) for a in range(2) for c in range(4)]

    def w_copy(c):
        return [(w_src(c), raw4.at[c], SEM_W + c)]

    copies = [(gf_hbm.at[0:4], gf.at[0:4], SEM_GF)]
    copies += [(x_hbm.at[x_rows(i, a1), :], x_v.at[x_rows(i, a1), :], SEM_X + i)
               for i in range(QS // RB) for a1 in range(4)]
    copies += [(w_src(0).at[kslice(q, e)], raw4.at[0, kslice(q, e)], SEM_W0 + q)
               for q in range(NQ) for e in range(2)]
    copies += [(sm_hbm, sm, SEM_SM), (gf_hbm.at[4:6], gf.at[4:6], SEM_W)]
    copies += [(f_hbm[a].at[pl.ds(D // 2, 1), :], nyq.at[a], SEM_NYQ) for a in range(2)]
    copies += f_copies(0) + w_copy(1) + f_copies(1) + w_copy(2) + f_copies(2) + f_copies(3)
    copies += [(gs_hbm, gs, SEM_GS)] + w_copy(3) + w_copy(4) + w_copy(5)
    copies += [(wo_hbm.bitcast(U32).at[:, pl.ds(128 * j, 128)], wo.at[j], SEM_WO) for j in range(8)]
    copies += [(gi_hbm, gi, SEM_GI), (mem_hbm, mem_ref, SEM_MEM), (gw_hbm, gw_ref, SEM_GW)]
    for src, dst, k in copies:
        pltpu.make_async_copy(src, dst, sem.at[k]).start()

    def prep_rhs(ch, jj, k0, nk):
        item = 8 * ch + jj
        a1 = raw[ch, pl.ds(k0 * 8 + jj, nk, stride=8), :]
        a2 = raw[ch, pl.ds((KH + k0) * 8 + jj, nk, stride=8), :]
        b11, b12, b21, b22 = _lo_f32(a1), _hi_f32(a1), _lo_f32(a2), _hi_f32(a2)
        for p, e, b in ((0, 0, b11), (1, 0, b12), (0, 1, b21), (1, 1, b22)):
            wqkv[2 * item + p, pl.ds((e * KH + k0) // 2, nk // 2), :] = _as_u32(b.astype(BF))
        return [v.astype(BF) for v in (b11 + b22, b11, b12 - b22, b21 - b11, b22, b11 + b12, b21 + b22)]

    def strassen(rhs, k0, nk, init, finish, after_dot):
        def prod(i):
            return _dot(_as_bf(sl[i, :, pl.ds(k0, nk)]), rhs[i])

        def plus(i, r):
            return r if init is None else init(i) + r

        m = prod(1)
        cb[0] = m
        after_dot(0, m)
        m = prod(4)
        cb[1] = m
        after_dot(1, m)
        m = prod(0)
        cb[2] = plus(0, m - cb[1])
        cb[3] = plus(3, m - cb[0])
        after_dot(2, m)
        m = prod(3)
        cb[4] = plus(2, cb[0] + m)
        cb[2] = cb[2] + m
        after_dot(3, m)
        m = prod(2)
        cb[5] = plus(1, cb[1] + m)
        cb[3] = cb[3] + m
        after_dot(4, m)
        m = prod(6) + cb[2]
        finish(0, m, cb[5])
        after_dot(5, m)
        m = prod(5) + cb[3]
        finish(1, cb[4], m)
        after_dot(6, m)

    def store_st(item, e, c1, c2):
        r = jnp.concatenate([c.reshape(NSEG // 2, 8, 128) for c in (c1, c2)], axis=1)
        st[item, 256 * e:256 * e + 256, :] = _as_u32(r.reshape(8 * NSEG, 128).astype(BF))

    def pin(i, c):
        if PINCB:
            cb[i, 0:8, :] = jnp.zeros((8, 128), F32)
        zero_s[i] = 0
        z_s[i, 0:8, :] = jnp.zeros((8, 128), U32)
        p_s[i, 0:8, :] = jnp.zeros((8, 128), F32)
        u_s[i, 0:8, :] = jnp.zeros((8, 128), U32)
        stg[i, 0, 0:8, :] = jnp.zeros((8, 128), U32)
        obuf[i, 0:8, :] = jnp.zeros((8, 128), U32)
        sto[i] = jnp.zeros((8, 128), F32)
        return c

    lax.fori_loop(0, 2, pin, 0)

    wait(gf.at[0:4], SEM_GF)

    def f1(i, c):
        for a1 in range(4):
            wait(x_v.at[x_rows(i, a1), :], SEM_X + i)
        base = pl.multiple_of(i * RB, RB)
        alt = (1 - 2 * (_lanes(16) & 1)).astype(F32).astype(BF)

        def rows16(r):
            return jnp.concatenate([x_v[pl.ds(r + d, 16), :].astype(F32)[0:8] for d in (0, SEG)], axis=0)

        for r in (0, 64, QS, QS + 64):
            top, bot = rows16(base + r), rows16(base + (r + 2 * QS))
            a11, a12, a21, a22 = top[:, :KH], top[:, KH:], bot[:, :KH], bot[:, KH:]
            row = pl.multiple_of((base + r) // 8, 8)
            for k, v in enumerate((a11 + a22, a21 + a22, a11, a22, a11 + a12, a21 - a11, a12 - a22)):
                sl[k, pl.ds(row, 8), :] = _as_u32(v.astype(BF))
        for h0 in range(0, RB, HB):
            pieces = []
            for a1 in range(4):
                for r in range(h0, h0 + HB, 16):
                    xs = x_v[pl.ds(base + (QS * a1 + r), 16), :].astype(F32)
                    pieces.append(jnp.concatenate(_bfly8([xs[:, 128 * a:128 * a + 128] for a in range(8)]),
                                                  axis=1))
                    z_s[a1, r // 2:r // 2 + 8, :] = _as_u32(pieces[-1][:, :128].astype(BF))
            ub = jnp.concatenate(pieces, axis=0)
            for g in range(4):
                yy = _dot(ub[:, 256 * g:256 * g + 256].astype(BF), _as_bf(gf[g]))
                v = _fft([(yy[HB * a1:HB * a1 + HB, :128], yy[HB * a1:HB * a1 + HB, 128:])
                          for a1 in range(4)], -1)
                for k1 in range(4):
                    rows = pl.ds(base + (QS * k1 + h0), HB)
                    y[g, 0, rows, :] = v[k1][0]
                    y[g, 1, rows, :] = v[k1][1]
                if h0 + HB == RB and g == NTG:
                    for a1 in range(4):
                        xa[pl.ds(4 * a1 + i, 1), :] = _dot_nt(alt, _as_bf(z_s[a1]))[0:1]
        return c

    with jax.named_scope("f1"):
        if ONLY in ("", "f1"):
            lax.fori_loop(0, QS // RB, f1, 0)
        else:
            for i in range(4):
                for a1 in range(4):
                    wait(x_v.at[x_rows(i, a1), :], SEM_X + i)

    def fprep(h, c):
        ev, od = [], []
        for r in range(8):
            wr = fraw[h, 0, c, pl.ds(r, 32, stride=8), :]
            wi = fraw[h, 1, c, pl.ds(r, 32, stride=8), :]
            ev.append((wr & jnp.uint32(0xFFFF)) | (wi << 16))
            od.append((wr >> 16) | (wi & jnp.uint32(0xFFFF0000)))
        for g, cls in enumerate(CLASSES):
            t = _transpose_u32(jnp.concatenate([(od if k % 2 else ev)[k // 2] for k in cls], axis=0))
            for q in range(128 // N1):
                row = pl.multiple_of(((4 * h + c) * (128 // N1) + q) * PITCH, 8)
                fp[g, pl.ds(row, N1), :] = t[q * N1:(q + 1) * N1]

    def nyquist():
        twc, tws = sm[0:16], sm[16:32]
        u = _dot(sm[32:64, 0:16].astype(BF), xa[...].astype(BF))
        ur, ui = u[0:16], u[16:32]
        u = jnp.concatenate([ur * twc + ui * tws, ui * twc - ur * tws], axis=1).astype(BF)
        yield
        xx = _dot(u, _as_bf(gf[4]))
        xr, xi = xx[:, :128], xx[:, 128:]
        w = (pltpu.bitcast(nyq[0].astype(F32), U32) >> 16) | pltpu.bitcast(nyq[1].astype(F32), U32)
        w = jnp.concatenate([w[:, 128 * a:128 * a + 128] for a in range(16)], axis=0)
        wt = _transpose_u32(jnp.concatenate([w] * 8, axis=0))
        blk = _lanes(16) >> 4
        wm = wt[0:16]
        for j in range(1, 8):
            wm = jnp.where(blk == j, wt[16 * j:16 * j + 16], wm)
        wr, wi = _lo_f32(wm), _hi_f32(wm)
        z = jnp.concatenate([xr * wr - xi * wi, xr * wi + xi * wr], axis=1).astype(BF)
        yield
        pp = _dot(z, _as_bf(gf[5]))
        pr, pi = pp[:, :128], pp[:, 128:]
        pp = jnp.concatenate([pr * twc - pi * tws, pi * twc + pr * tws], axis=0).astype(BF)
        yield
        cc = _dot(sm[64:80, 0:32].astype(BF), pp) * (1.0 / (S * D))
        ct[...] = jnp.concatenate([cc, jnp.zeros((112, 128), F32)], axis=0).T
        yield

    def s_rows(k1, a0, r):
        return pl.ds(r + (QS * k1 + N2 * a0), 8)

    def anchored(v, tok):
        return jnp.where(zero_s[0] != 0, tok, v)

    def s_prep(g, k1, r, tok):
        v = [(y[g, 0, s_rows(k1, a0, r), :], y[g, 1, s_rows(k1, a0, r), :]) for a0 in range(8)]
        v[0] = (anchored(v[0][0], tok), v[0][1])
        v = _fft([_cmul_const(v[a0], a0 * k1, N1, -1) for a0 in range(8)], -1)
        for k0 in range(8):
            u_s[k1 + 4 * k0, pl.ds(r, 8), :] = _as_u32(jnp.concatenate(v[k0], axis=0).astype(BF))

    def s_fwd(g, ka, tok):
        xx = _dot(_as_bf(gs[0, ka]), _as_bf(u_s[ka]))
        w32 = fp[g, pl.ds(ka, N2, stride=PITCH), :]
        wr, wi = _lo_f32(w32), _hi_f32(w32)
        xr, xi = xx[:N2], xx[N2:]
        z_s[ka] = _as_u32(jnp.concatenate([xr * wr - xi * wi, xr * wi + xi * wr], axis=0).astype(BF))

    def s_inv(ka, tok):
        p_s[ka] = _dot(_as_bf(gs[1, ka]), _as_bf(z_s[ka]))

    def s_post(g, k1, r, tok):
        v = [(p_s[k1 + 4 * k0, r:r + 8, :], p_s[k1 + 4 * k0, N2 + r:N2 + r + 8, :]) for k0 in range(8)]
        v[0] = (anchored(v[0][0], tok), anchored(v[0][1], tok))
        v = _fft(v, 1)
        for a0 in range(8):
            vr, vi = _cmul_const(v[a0], a0 * k1, N1, 1)
            v_s[g, 0, s_rows(k1, a0, r), :] = vr
            v_s[g, 1, s_rows(k1, a0, r), :] = vi

    def acc(jj, i):
        return v_s.at[jj // 4, (jj // 2) % 2, pl.ds(1024 * (jj % 2) + 256 * i, 256), :]

    def bulk(item0, n, events, q=None):
        k0, nk = (0, KH) if q is None else (q * KQ, KQ)
        for i in range(n):
            item = item0 + i

            def hook(k, m):
                pieces = events.get(7 * i + k, ())
                vec = [pc for pc in pieces if getattr(pc, "func", None) in (s_prep, s_post)]
                for piece in pieces:
                    r = 8 * ((32 * vec.index(piece)) // len(vec)) if piece in vec else 0
                    piece(m[r:r + 8])

            def finish(e, c1, c2):
                if q in (None, NQ - 1):
                    store_st(item, e, c1, c2)
                else:
                    acc(item, 2 * e)[...] = c1
                    acc(item, 2 * e + 1)[...] = c2

            init = None if q in (None, 0) else (lambda k: acc(item, k)[...])
            strassen(prep_rhs(item // 8, item % 8, k0, nk), k0, nk, init, finish, hook)

    def spread(events, pieces, q0, q1):
        for i, piece in enumerate(pieces):
            events.setdefault(q0 + ((q1 - q0) * i) // len(pieces), []).append(piece)

    P = functools.partial

    def loop_a(h, c):
        @pl.when(h % 2 == 0)
        def _():
            wait(raw4.at[1 + h // 2], SEM_W + 1 + h // 2)

        wait(fraw.at[h], SEM_F + h)
        events = {}
        spread(events, [lambda tok, c=c: fprep(h, c) for c in range(4)], 0, 24)
        bulk(8 + 4 * h, 4, events)
        return c

    def loop_b(g, c):
        @pl.when(g < 3)
        def _():
            wait(raw4.at[3 + g], SEM_W + 3 + g)

        gn = jnp.minimum(g + 1, 3)
        events = {}
        for k1 in range(4):
            q = B0 + BD * k1
            spread(events, [P(s_fwd, g, k1 + 4 * k0) for k0 in range(8)], q, q + BW)
            spread(events, [P(s_prep, gn, k1, r) for r in range(0, N2, 8)], q + BW, q + BW + BV)
            q = max(q + BL, 0)
            spread(events, [P(s_inv, k1 + 4 * k0) for k0 in range(8)], q, q + BW)
            spread(events, [P(s_post, g, k1, r) for r in range(0, N2, 8)], q + BW, q + BW + BV)
        assert max(events) < 41
        for q in sorted(q for q in events if q < 0):
            for piece in events[q]:
                piece(None)
        bulk(24 + 6 * g, 6, events)
        return c

    with jax.named_scope("p0"):
        ny = nyquist()
        for q in range(NQ):
            for e in range(2):
                wait(raw4.at[0, kslice(q, e)], SEM_W0 + q)
            events = {}
            if q == NQ - 1:
                wait(sm, SEM_SM)
                wait(gf.at[4:6], SEM_W)
                wait(nyq, SEM_NYQ)
                spread(events, [lambda tok: next(ny)] * 4, 4, 28)
            spread(events, [P(s_prep, 0, k1, r) for k1 in range(4 * q // NQ, 4 * (q + 1) // NQ)
                            for r in range(0, N2, 8)], 0, 52)
            if ONLY in ("", "p0"):
                bulk(0, 8, events, q)
    with jax.named_scope("loop_a"):
        if ONLY in ("", "a"):
            lax.fori_loop(0, 4, loop_a, 0)
        else:
            for h in range(4):
                wait(fraw.at[h], SEM_F + h)
            for h in range(2):
                wait(raw4.at[1 + h], SEM_W + 1 + h)
    wait(gs, SEM_GS)
    with jax.named_scope("loop_b"):
        if ONLY in ("", "b"):
            lax.fori_loop(0, 4, loop_b, 0)
        else:
            for g in range(3):
                wait(raw4.at[g + 3], SEM_W + 3 + g)
    wait(wo, SEM_WO)
    wait(gi, SEM_GI)
    wait(mem_ref, SEM_MEM)
    wait(gw_ref, SEM_GW)

    scale = DH ** -0.5

    mf[...] = _mask80()
    gw_s[...] = jnp.broadcast_to(gw_ref[...].astype(F32).reshape(1, D), (8, D))

    def softmax(s):
        fill = mf[0:s.shape[0], :]
        s = jnp.where(fill > 0.0, s * scale, fill)
        m = jnp.max(s, axis=-1, keepdims=True)
        e = jnp.exp(s - m)
        l = jnp.sum(e, axis=-1, keepdims=True)
        return (e * (1.0 / l)).astype(BF)

    def lhs_rows(mem, seg):
        xs = x_v[pl.ds(pl.multiple_of(seg * SEG, SEG), SEG), :].astype(F32)
        return jnp.concatenate([mem, xs[8:SEG]], axis=0).astype(BF)

    def proj2(a, m, j):
        return jnp.concatenate([_dot(a, _as_bf(wqkv[H * m + 2 * j + p])).astype(BF) for p in range(2)], axis=0)

    def proj_first(a):
        if not KSPLIT:
            return [proj2(a, m, 0) for m in range(3)]
        part = [_dot(a[:, :D // 2], _as_bf(wqkv[H * (i // 2) + i % 2, 0:D // 4, :])) for i in range(6)]
        full = [(_dot(a[:, D // 2:], _as_bf(wqkv[H * (i // 2) + i % 2, D // 4:D // 2, :])) + part[i]).astype(BF)
                for i in range(6)]
        return [jnp.concatenate(full[2 * m:2 * m + 2], axis=0) for m in range(3)]

    def step(a, seg, first, hook=None):
        R = 32 if first else 48
        qkv, ps = {}, {}
        srow = pl.multiple_of(seg * 8, 8)

        def put(m, j, r):
            if "qkv"[m] in STAGE:
                stg[m, j % 8] = _as_u32(r)
            else:
                qkv[m, j] = r

        due = {}

        def after(u, keys):
            for k in keys:
                for o in due.pop(k, ()):
                    u = anchored(u, pltpu.bitcast(o, U32))
            return u

        def get(m, j):
            r = _as_bf(stg[m, j % 8]) if "qkv"[m] in STAGE else qkv[m, j]
            u = st[NP * m + j, pl.ds(srow, 8), :]
            if m == 2:
                u = after(u, [j - DL])
            return jnp.concatenate([r, _as_bf(u)], axis=0)

        def proj(j, m):
            if j == 0:
                if m == 0:
                    r = [_as_bf(qkv_s[m]) for m in range(3)] if first else proj_first(a)
                    for mm in range(3):
                        put(mm, 0, r[mm])
            else:
                put(m, j, proj2(a, m, j))

        def scores(j):
            if VATT:
                pst[j % 8, 0:32, :] = _as_u32(softmax(_dot_nt(_as_bf(stg[0, j % 8]), get(1, j))))
                small(j)
            else:
                pst[j % 8] = _as_u32(softmax(_dot_nt(get(0, j), get(1, j))))

        def small(j):
            qs, ks, vs = [_as_bf(st[NP * m + j, pl.ds(srow, 8), :]).astype(F32) for m in range(3)]
            row = lax.broadcasted_iota(jnp.int32, (8, 1), 0)
            for i in range(2):
                h = 2 * j + i
                km, vm = [_as_bf(stg[m, j % 8, 16 * i:16 * i + 8, :]).astype(F32)[0:8] for m in (1, 2)]
                q = qs[8 * i:8 * i + 8] * scale
                rot = lambda v, r: pltpu.roll(v, r, 0) if r else v
                sc = [jnp.sum(q * rot(km, r), axis=-1, keepdims=True) for r in range(8)]
                for r in range(8):
                    t = jnp.sum(q * rot(ks[8 * i:8 * i + 8], r), axis=-1, keepdims=True)
                    sc.append(jnp.where(row >= r, t, -1e9) if r else t)
                m = functools.reduce(jnp.maximum, sc)
                e = [jnp.exp(t - m) for t in sc]
                l = functools.reduce(jnp.add, e)
                vv = [rot(vm, r) for r in range(8)] + [rot(vs[8 * i:8 * i + 8], r) for r in range(8)]
                o = functools.reduce(jnp.add, [a * b for a, b in zip(e, vv)]) * (1.0 / l)
                due.setdefault(j, []).append(o)
                if first:
                    sto[h] = o
                else:
                    obuf[h, 16:24, :] = _as_u32(jnp.concatenate([o, sto[h]], axis=0).astype(BF))

        def pv(j):
            if VATT:
                o = _dot(_as_bf(pst[j % 8, 0:32, :]), get(2, j))
                for i in range(2):
                    obuf[2 * j + i, 0:16, :] = _as_u32(o[32 * i:32 * i + 32].astype(BF))
                return
            o = _dot(_as_bf(pst[j % 8]), get(2, j))
            for i in range(2):
                h = 2 * j + i
                if first:
                    ob = o[32 * i:32 * i + 32].astype(BF)
                    sto[h] = o[64 + 8 * i:72 + 8 * i]
                else:
                    ob = jnp.concatenate([o[32 * i:32 * i + 32], o[64 + 8 * i:72 + 8 * i], sto[h]],
                                         axis=0).astype(BF)
                obuf[h, 0:R // 2, :] = _as_u32(ob)

        def wo_part(j, h0, h1):
            og = [obuf[h, 0:R // 2, :] for h in range(h0, h1)]
            if h0 > 0:
                og[0] = jnp.concatenate([after(og[0][0:8], list(due)), og[0][8:]], axis=0)
            og = jnp.concatenate([_as_bf(u) for u in og], axis=1)
            return _dot(og, _as_bf(wo[j, h0 * 64:h1 * 64, :]))

        parts = []
        for i in range(NP + 4):
            for ch in ORDER:
                if ch in "qkv":
                    m = "qkv".index(ch)
                    if i < NP:
                        proj(i, m)
                    elif m < 2:
                        parts.append(wo_part(2 * (i - NP) + len(parts) % 2, 0, SPLIT))
                elif ch == "s" and 0 <= i - LAG1 < NP:
                    scores(i - LAG1)
                elif ch == "p" and 0 <= i - LAG2 < NP:
                    pv(i - LAG2)
            if hook is not None and i == HOOK_AT:
                hook()
        return jnp.concatenate([wo_part(j, SPLIT, H) + parts[j] for j in range(8)], axis=1)

    def start_pair(mem, t):
        a = lhs_rows(mem, 2 * t)
        a_s[...] = _as_u32(a)
        for m, r in enumerate(proj_first(a)):
            qkv_s[m] = _as_u32(r)

    def pair(t, c):
        base = pl.multiple_of(t * 64, 64)
        lane = _lanes(64)
        lo = lane < 64
        roll = (lambda v: v + 1.0) if _E('NOROLL', 0) else (lambda v: pltpu.roll(v, 64, 1))
        a1 = t // 8
        off = pl.multiple_of((t % 8) * 64, 64)
        s2 = (1 - 2 * (a1 & 1)).astype(F32)
        sg = (1 - (a1 & 2)).astype(F32)
        cc, ss = sg * (1 - (a1 & 1)).astype(F32), sg * (a1 & 1).astype(F32)

        def irfft_group(g):
            q = [[v_s[g, e, pl.ds(off + QS * k1, 64), :] for e in range(2)] for k1 in range(4)]
            br, bi = q[1][0] + s2 * q[3][0], q[1][1] + s2 * q[3][1]
            vr = q[0][0] + s2 * q[2][0] + (cc * br - ss * bi)
            vi = q[0][1] + s2 * q[2][1] + (cc * bi + ss * br)
            tin = _half_pre(vr, vi, lo, roll, jnp.where)
            tp, tm = [_dot(tin[e].astype(BF), _as_bf(gi[2 * g + e])) for e in range(2)]
            if g == 0:
                nyc = jnp.sum(jnp.where(lane == t // 2,
                                        ct[pl.ds(pl.multiple_of((t % 2) * 64, 64), 64), :], 0.0),
                              axis=-1, keepdims=True)
                tp = tp + nyc * (1 - 2 * (lane & 1)).astype(F32)
            return list(_half_post(g, tp, tm, lo, roll, jnp.where))

        def spectral_part():
            ts = sum([irfft_group(g) for g in range(4)], [])
            b = jnp.concatenate(_bfly8_t(ts), axis=1).astype(BF).astype(F32)
            xs = x_v[pl.ds(base, 64), :].astype(F32)
            gate = jax.nn.sigmoid(jnp.sum(xs * jnp.concatenate([gw_s[...]] * 8, axis=0), axis=-1, keepdims=True))
            bb = (1.0 - gate) * b
            bb_s[...] = jnp.concatenate([bb[0:8], bb[8:32] + gate[8:32] * bb_s[8:32], bb[32:64]], axis=0)
            g_s[...] = jnp.broadcast_to(gate, (64, 128))

        res_a = step(_as_bf(a_s[...]), 2 * t, True)
        bb_s[8:32] = res_a[8:32]
        a = lhs_rows(res_a[0:8].astype(BF).astype(F32), 2 * t + 1)
        res_b = step(a, 2 * t + 1, False, None if NOSPEC else spectral_part)

        def gated(r0, r1, res):
            return bb_s[r0:r1] + jnp.concatenate([g_s[r0:r1]] * 8, axis=1) * res

        out_v[pl.ds(base, 64), :] = jnp.concatenate(
            [gated(0, 8, res_b[40:48]), bb_s[8:32], gated(32, 40, res_b[32:40]), gated(40, 64, res_b[8:32])],
            axis=0).astype(BF)
        cp = pltpu.make_async_copy(out_v.at[pl.ds(base, 64), :], out_hbm.at[pl.ds(base, 64), :],
                                   sem.at[SEM_OUT])
        if DMAPOS == 0:
            cp.start()
        start_pair(res_b[0:8].astype(BF).astype(F32), jnp.minimum(t + 1, S // 64 - 1))
        if DMAPOS == 1:
            cp.start()
        return c

    with jax.named_scope("chain"):
        if ONLY in ("", "chain"):
            start_pair(mem_ref[...].astype(F32), 0)
            lax.fori_loop(0, S // 64, pair, 0, unroll=_E("UNROLL", 1))
            if DMAPOS == 2:
                pltpu.make_async_copy(out_v, out_hbm, sem.at[SEM_OUT]).start()
    if ONLY not in ("", "chain"):
        def keep(i, c):
            v = st[i, 0:8, :] + wqkv[i, 0:8, :] + fp[i % 4, 0:8, :] + u_s[i % 32, 0:8, :] + pltpu.bitcast(y[i % 4, 0, pl.ds(8 * i, 8), :] + v_s[i % 4, 0, pl.ds(8 * i, 8), :] + ct[pl.ds(i, 8), :] + xa[0:8], U32) + sl[i % 7, 0:8, 0:128]
            out_v[pl.ds(16 * i, 16), 0:128] = _as_bf(v)
            return c
        lax.fori_loop(0, 48, keep, 0)
        pltpu.make_async_copy(out_v, out_hbm, sem.at[SEM_OUT]).start()
        pltpu.make_async_copy(out_v, out_hbm, sem.at[SEM_OUT]).wait()
    for i in range(_E("PADK", 0)):
        if i < 6:
            raw[i] = jnp.full((8192, 128), i, U32)
        elif i < 12:
            wqkv[16 * (i - 6):16 * (i - 5)] = jnp.full((16, 512, 128), i, U32)
        elif i < 15:
            st[16 * (i - 12):16 * (i - 11)] = jnp.full((16, 512, 128), i, U32)
        elif i < 17:
            y[2 * (i - 15):2 * (i - 14)] = jnp.full((2, 2, 2048, 128), i, F32)
        elif i < 19:
            v_s[2 * (i - 17):2 * (i - 16)] = jnp.full((2, 2, 2048, 128), i, F32)
        elif i < 21:
            wo[4 * (i - 19):4 * (i - 18)] = jnp.full((4, 2048, 128), i, U32)
    with jax.named_scope("fin"):
        if ONLY in ("", "chain"):
            pltpu.make_async_copy(out_v, out_hbm, sem.at[SEM_OUT]).wait()


@jax.jit
def pallas_gated_mix__memory_aug_recurrent_mem_tr__spectral_gfnet__prompt_kernel(
    A_x, A_mem0, A_Wq, A_Wk, A_Wv, A_Wo, A_seg_len, B_x, B_w_r, B_w_i, gate_w,
):
    assert A_x.shape == (1, S, D) and A_mem0.shape == (1, M, D) and A_Wq.shape == (D, H, DH)
    consts = [jnp.asarray(c) for c in _constants()]
    any_spec = pl.BlockSpec(memory_space=pl.ANY)
    out = pl.pallas_call(
        _kernel,
        out_shape=jax.ShapeDtypeStruct((S, D), BF),
        in_specs=[any_spec] * 13,
        out_specs=any_spec,
        scratch_shapes=[
            pltpu.VMEM((S, D), BF),
            pltpu.VMEM((6, D * 8, DH), U32),
            pltpu.VMEM((3 * H, D // 2, DH), U32),
            pltpu.VMEM((8, H * DH // 2, 128), U32),
            pltpu.VMEM((3 * NP, 8 * NSEG, 128), U32),
            pltpu.VMEM((7, 2 * NSEG, D // 2), U32),
            pltpu.VMEM((4, 2, 4, 256, 128), U32),
            pltpu.VMEM((4, N2 * PITCH, 128), U32),
            pltpu.VMEM((6, 128, 256), U32),
            pltpu.VMEM((8, 64, 128), U32),
            pltpu.VMEM((2, N1, N2, 2 * N2), U32),
            pltpu.VMEM((4, 2, S, 128), F32),
            pltpu.VMEM((4, 2, S, 128), F32),
            pltpu.VMEM((S, D), BF),
            pltpu.VMEM((N1, N2, 128), U32),
            pltpu.VMEM((6, 256, 128), F32),
            pltpu.VMEM((N1, N2, 128), U32),
            pltpu.VMEM((N1, 2 * N2, 128), F32),
            pltpu.VMEM((H, 8, 128), F32),
            pltpu.VMEM((H, 24, 128), U32),
            pltpu.VMEM((128, 128), F32),
            pltpu.VMEM((16, D), U32),
            pltpu.VMEM((3, 32, 128), U32),
            pltpu.VMEM((64, D), F32),
            pltpu.VMEM((64, 128), F32),
            pltpu.VMEM((3, 8, 32, 128), U32),
            pltpu.VMEM((8, 40, 80), U32),
            pltpu.VMEM((8, D), F32),
            pltpu.VMEM((M, D), BF),
            pltpu.VMEM((80, 80), F32),
            pltpu.VMEM((80, 128), F32),
            pltpu.VMEM((16, 128), F32),
            pltpu.VMEM((2, 1, S), BF),
            pltpu.VMEM((D,), BF),
            pltpu.SMEM((2,), jnp.int32),
            pltpu.SemaphoreType.DMA((NSEM,)),
        ],
        compiler_params=pltpu.CompilerParams(vmem_limit_bytes=120 * 1024 * 1024),
    )(
        A_x.reshape(S, D), A_mem0.reshape(M, D), A_Wq, A_Wk, A_Wv,
        A_Wo.reshape(H * DH, D), B_w_r.T, B_w_i.T, gate_w, *consts,
    )
    return out.reshape(1, S, D)
```

```python
import functools
import math

import numpy as np
import jax
import jax.numpy as jnp
from jax import lax
import jax.experimental.pallas as pl
import jax.experimental.pallas.tpu as pltpu

BF, F32, U32 = jnp.bfloat16, jnp.float32, jnp.uint32

S, D, H, DH, M, SEG = 2048, 1024, 32, 128, 8, 32
NSEG = S // SEG
NP = H // 2
N1, N2 = 32, 64
QS = S // 4
PITCH = N1 + 8
CLASSES = ((0, 8, 4, 12), (1, 15, 9, 7), (2, 14, 10, 6), (3, 13, 11, 5))
LAG1, LAG2, SPLIT, HOOK_AT = 1, 2, 28, 17
ORDER = "vqskp"
BD, BW, BV, BL = 7, 8, 8, 3
NQ = 2
(SEM_W, SEM_GF, SEM_GI, SEM_SM, SEM_GS, SEM_NYQ, SEM_WO, SEM_MEM, SEM_GW, SEM_OUT, SEM_F, SEM_X,
 SEM_W0) = 0, 6, 7, 8, 9, 10, 11, 12, 13, 14, 15, 19, 23
NSEM = SEM_W0 + NQ
RSQ2 = float(np.float32(math.sqrt(0.5)))


def _bfly8(x):
    s = [x[i] + x[i + 4] for i in range(4)]
    d = [x[i] - x[i + 4] for i in range(4)]
    e, f = s[0] + s[2], s[1] + s[3]
    t1, t2 = (d[1] - d[3]) * RSQ2, (d[1] + d[3]) * RSQ2
    return [e + f, e - f, d[0] + t1, t2 + d[2], s[0] - s[2], s[1] - s[3], d[0] - t1, t2 - d[2]]


def _bfly8_t(t):
    e, f = t[0] + t[1], t[0] - t[1]
    s = [e + t[4], f + t[5], e - t[4], f - t[5]]
    t1, t2 = t[2] - t[6], t[3] + t[7]
    d = [t[2] + t[6], (t1 + t2) * RSQ2, t[3] - t[7], (t2 - t1) * RSQ2]
    return [s[i] + d[i] for i in range(4)] + [s[i] - d[i] for i in range(4)]


def _half_pre(vr, vi, lo, roll, where):
    ri = roll(vi)
    return where(lo, vr, ri), where(lo, ri, vr)


def _half_post(g, tp, tm, lo, roll, where):
    if g == 0:
        return tp, tm
    c = float(np.float32(math.cos(math.pi * g / 8)))
    s = float(np.float32(math.sin(math.pi * g / 8)))
    p, r = tp + tm, tp - tm
    rm = roll(where(lo, r, p))
    return where(lo, p, c * rm + s * r), where(lo, rm, c * r - s * rm)


def _cmul_const(v, k, n, sign):
    re, im = v
    k %= n
    if k == 0:
        return re, im
    if 4 * k == n:
        return (-im, re) if sign > 0 else (im, -re)
    if 8 * k == n:
        return (((re - im) * RSQ2, (re + im) * RSQ2) if sign > 0
                else ((re + im) * RSQ2, (im - re) * RSQ2))
    if 8 * k == 3 * n:
        return (((re + im) * -RSQ2, (re - im) * RSQ2) if sign > 0
                else ((im - re) * RSQ2, (re + im) * -RSQ2))
    c, s = math.cos(2 * math.pi * k / n), sign * math.sin(2 * math.pi * k / n)
    return re * c - im * s, re * s + im * c


def _fft(v, sign):
    n = len(v)
    if n == 1:
        return v
    ev, od = _fft(v[0::2], sign), _fft(v[1::2], sign)
    lo, hi = [], []
    for k in range(n // 2):
        er, ei = ev[k]
        if 4 * k == n:
            xr, xi = od[k]
            if sign > 0:
                lo.append((er - xi, ei + xr)); hi.append((er + xi, ei - xr))
            else:
                lo.append((er + xi, ei - xr)); hi.append((er - xi, ei + xr))
            continue
        tr, ti = _cmul_const(od[k], k, n, sign)
        lo.append((er + tr, ei + ti))
        hi.append((er - tr, ei - ti))
    return lo + hi


def _pack_rows(a):
    u = np.ascontiguousarray(a, dtype=np.float32).view(np.uint32)
    b = ((u + 0x7FFF + ((u >> 16) & 1)) >> 16).astype(np.uint32)
    return (b[..., 0::2, :] | (b[..., 1::2, :] << 16)).astype(np.uint32)


def _diag_blocks(full, n, tol):
    k = full.shape[0] // n
    blk = np.kron(np.eye(k), np.ones((n, n)))
    assert np.abs(full * (1 - blk)).max() < tol
    return np.stack([full[n * g:n * g + n, n * g:n * g + n] for g in range(k)])


def _cplx(re, im):
    return np.block([[re, im], [-im, re]])


@functools.lru_cache(maxsize=None)
def _constants():
    k2 = np.stack([np.concatenate([c + 16 * np.arange(32) for c in cls]) for cls in CLASSES])
    n2 = np.arange(D)
    ang = 2 * np.pi * ((k2[:, :, None] * n2[None, None, :]) % D) / D
    rows = np.stack([np.cos(ang), -np.sin(ang)], axis=1)
    wgt = np.where(k2 == 0, 1.0, 2.0)[:, None, :, None]
    fwd = rows.reshape(D, D).T
    inv = (rows * wgt).reshape(D, D) / (S * D)
    bf = np.stack(_bfly8(list(np.eye(8))))
    binv = np.kron(np.linalg.inv(bf), np.eye(128))
    gd = _diag_blocks(binv.T @ fwd, 256, 1e-6)
    gdi = _diag_blocks(inv @ binv, 256, 1e-12)
    eye, lo = np.eye(256), np.arange(128) < 64
    roll = lambda v: np.roll(v, 64, axis=1)
    pre = np.concatenate(_half_pre(eye[:, :128], eye[:, 128:], lo, roll, np.where), axis=1)
    gi = []
    for g in range(4):
        post = np.concatenate(_half_post(g, eye[:, :128], eye[:, 128:], lo, roll, np.where), axis=1)
        gi.append(_diag_blocks(np.linalg.inv(pre) @ gdi[g] @ np.linalg.inv(post), 128, 1e-12))
    gi = np.concatenate(gi)

    b = np.arange(N2)
    k1 = np.arange(N1)[:, None] + N1 * np.arange(N2)[None, :]
    th = 2 * np.pi * ((k1[:, :, None] * b[None, None, :]) % S) / S
    gr, gim = np.cos(th), -np.sin(th)
    full = np.block([[gr, -gim], [gim, gr]])
    kap = np.arange(2 * N2)
    src = ((kap >> 3) & 1) * N2 + (kap >> 4) * 8 + (kap & 7)
    gs = full[:, :, src]
    hr, hi = np.swapaxes(gr, 1, 2), -np.swapaxes(gim, 1, 2)
    gsi = np.block([[hr, -hi], [hi, hr]])

    lane = np.arange(128)
    kb = 8 * (lane % 16) + lane // 16
    t128 = 2 * np.pi * ((lane[:, None] * kb[None, :]) % 128) / 128
    nyf = _cplx(np.cos(t128), -np.sin(t128))
    nyi = _cplx(np.cos(t128).T, np.sin(t128).T)
    i16 = np.arange(16)
    t16 = 2 * np.pi * ((i16[:, None] * i16[None, :]) % 16) / 16
    tw = 2 * np.pi * (i16[:, None] * lane[None, :]) / S
    sm = np.zeros((96, 128), np.float32)
    sm[0:16], sm[16:32] = np.cos(tw), np.sin(tw)
    sm[32:48, :16], sm[48:64, :16] = np.cos(t16), -np.sin(t16)
    sm[64:80, :16], sm[64:80, 16:32] = np.cos(t16), -np.sin(t16)

    gfp = _pack_rows(np.concatenate([gd, nyf[None], nyi[None]]))
    return gfp, _pack_rows(gi), sm, _pack_rows(np.stack([gs, gsi]))


def _mask80():
    r = lax.broadcasted_iota(jnp.int32, (80, 80), 0)
    c = lax.broadcasted_iota(jnp.int32, (80, 80), 1)

    def head(i):
        return jnp.where(i < 64, i >> 5, (i - 64) >> 3)

    def pos(i):
        j = i & 31
        return jnp.where(i < 64, jnp.where(j < M, j, j + 8), M + (i & 7))

    same = head(r) == head(c)
    ok = (pos(r) < M) | (pos(c) <= pos(r))
    return jnp.where(same, jnp.where(ok, 1.0, -1e9), -jnp.inf).astype(F32)


def _as_bf(u):
    return pltpu.bitcast(u, BF)


def _as_u32(b):
    return pltpu.bitcast(b, U32)


def _lo_f32(u):
    return pltpu.bitcast(u << 16, F32)


def _hi_f32(u):
    return pltpu.bitcast(u & jnp.uint32(0xFFFF0000), F32)


def _dot(a, b):
    return jnp.dot(a, b, preferred_element_type=F32)


def _dot_nt(a, b):
    return lax.dot_general(a, b, (((1,), (1,)), ((), ())), preferred_element_type=F32)


def _transpose_u32(u):
    return pltpu.bitcast(pltpu.bitcast(u, F32).T, U32)


def _lanes(rows):
    return lax.broadcasted_iota(jnp.int32, (rows, 128), 1)


def _kernel(x_hbm, mem_hbm, wq_hbm, wk_hbm, wv_hbm, wo_hbm, fr_hbm, fi_hbm, gw_hbm,
            gf_hbm, gi_hbm, sm_hbm, gs_hbm,
            out_hbm,
            x_v, raw, wqkv, wo, st, sl, fraw, fp, gf, gi, gs, y, v_s, out_v, u_s, cb, z_s, p_s,
            sto, obuf, ct, a_s, bb_s, g_s, stg, pst, gw_s, mem_ref, mf, sm, xa, nyq, gw_ref, zero_s, sem):
    KH = D // 2
    KQ = KH // NQ
    RB, HB = 128, 16
    raw4 = raw.reshape(6, D, 8, DH)
    w_hbm = (wq_hbm, wk_hbm, wv_hbm)
    f_hbm = (fr_hbm, fi_hbm)

    def w_src(c):
        return w_hbm[c // 2].bitcast(U32).at[:, pl.ds(8 * (c % 2), 8), :]

    def wait(dst, k):
        pltpu.make_async_copy(dst, dst, sem.at[k]).wait()

    def kslice(q, e):
        return pl.ds(e * KH + q * KQ, KQ)

    def x_rows(i, a1):
        return pl.ds(pl.multiple_of(i * RB, RB) + QS * a1, RB)

    def f_copies(h):
        return [(f_hbm[a].at[pl.ds(0, D // 2), pl.ds(128 * (4 * h + c), 128)].bitcast(U32),
                 fraw.at[h, a, c], SEM_F + h) for a in range(2) for c in range(4)]

    def w_copy(c):
        return [(w_src(c), raw4.at[c], SEM_W + c)]

    copies = [(gf_hbm.at[0:4], gf.at[0:4], SEM_GF)]
    copies += [(x_hbm.at[x_rows(i, a1), :], x_v.at[x_rows(i, a1), :], SEM_X + i)
               for i in range(QS // RB) for a1 in range(4)]
    copies += [(w_src(0).at[kslice(q, e)], raw4.at[0, kslice(q, e)], SEM_W0 + q)
               for q in range(NQ) for e in range(2)]
    copies += [(sm_hbm, sm, SEM_SM), (gf_hbm.at[4:6], gf.at[4:6], SEM_W)]
    copies += [(f_hbm[a].at[pl.ds(D // 2, 1), :], nyq.at[a], SEM_NYQ) for a in range(2)]
    copies += f_copies(0) + w_copy(1) + f_copies(1) + w_copy(2) + f_copies(2) + f_copies(3)
    copies += [(gs_hbm, gs, SEM_GS)] + w_copy(3) + w_copy(4) + w_copy(5)
    copies += [(wo_hbm.bitcast(U32).at[:, pl.ds(128 * j, 128)], wo.at[j], SEM_WO) for j in range(8)]
    copies += [(gi_hbm, gi, SEM_GI), (mem_hbm, mem_ref, SEM_MEM), (gw_hbm, gw_ref.at[pl.ds(0, D)], SEM_GW)]
    for src, dst, k in copies:
        pltpu.make_async_copy(src, dst, sem.at[k]).start()

    def prep_rhs(ch, jj, k0, nk):
        item = 8 * ch + jj
        a1 = raw[ch, pl.ds(k0 * 8 + jj, nk, stride=8), :]
        a2 = raw[ch, pl.ds((KH + k0) * 8 + jj, nk, stride=8), :]
        b11, b12, b21, b22 = _lo_f32(a1), _hi_f32(a1), _lo_f32(a2), _hi_f32(a2)
        for p, e, b in ((0, 0, b11), (1, 0, b12), (0, 1, b21), (1, 1, b22)):
            wqkv[2 * item + p, pl.ds((e * KH + k0) // 2, nk // 2), :] = _as_u32(b.astype(BF))
        return [v.astype(BF) for v in (b11 + b22, b11, b12 - b22, b21 - b11, b22, b11 + b12, b21 + b22)]

    def strassen(rhs, k0, nk, init, finish, after_dot):
        def prod(i):
            return _dot(_as_bf(sl[i, :, pl.ds(k0, nk)]), rhs[i])

        def plus(i, r):
            return r if init is None else init(i) + r

        m = prod(1)
        cb[0] = m
        after_dot(0, m)
        m = prod(4)
        cb[1] = m
        after_dot(1, m)
        m = prod(0)
        cb[2] = plus(0, m - cb[1])
        cb[3] = plus(3, m - cb[0])
        after_dot(2, m)
        m = prod(3)
        cb[4] = plus(2, cb[0] + m)
        cb[2] = cb[2] + m
        after_dot(3, m)
        m = prod(2)
        cb[5] = plus(1, cb[1] + m)
        cb[3] = cb[3] + m
        after_dot(4, m)
        m = prod(6) + cb[2]
        finish(0, m, cb[5])
        after_dot(5, m)
        m = prod(5) + cb[3]
        finish(1, cb[4], m)
        after_dot(6, m)

    def store_st(item, e, c1, c2):
        r = jnp.concatenate([c.reshape(NSEG // 2, 8, 128) for c in (c1, c2)], axis=1)
        st[item, 256 * e:256 * e + 256, :] = _as_u32(r.reshape(8 * NSEG, 128).astype(BF))

    def pin(i, c):
        cb[i, 0:8, :] = jnp.zeros((8, 128), F32)
        zero_s[i] = 0
        z_s[i, 0:8, :] = jnp.zeros((8, 128), U32)
        p_s[i, 0:8, :] = jnp.zeros((8, 128), F32)
        u_s[i, 0:8, :] = jnp.zeros((8, 128), U32)
        stg[i, 0, 0:8, :] = jnp.zeros((8, 128), U32)
        obuf[i, 0:8, :] = jnp.zeros((8, 128), U32)
        sto[i] = jnp.zeros((8, 128), F32)
        return c

    lax.fori_loop(0, 2, pin, 0)

    wait(gf.at[0:4], SEM_GF)

    def f1(i, c):
        for a1 in range(4):
            wait(x_v.at[x_rows(i, a1), :], SEM_X + i)
        base = pl.multiple_of(i * RB, RB)
        alt = (1 - 2 * (_lanes(16) & 1)).astype(F32).astype(BF)

        def rows16(r):
            return jnp.concatenate([x_v[pl.ds(r + d, 16), :].astype(F32)[0:8] for d in (0, SEG)], axis=0)

        for r in (0, 64, QS, QS + 64):
            top, bot = rows16(base + r), rows16(base + (r + 2 * QS))
            a11, a12, a21, a22 = top[:, :KH], top[:, KH:], bot[:, :KH], bot[:, KH:]
            row = pl.multiple_of((base + r) // 8, 8)
            for k, v in enumerate((a11 + a22, a21 + a22, a11, a22, a11 + a12, a21 - a11, a12 - a22)):
                sl[k, pl.ds(row, 8), :] = _as_u32(v.astype(BF))
        for h0 in range(0, RB, HB):
            pieces = []
            for a1 in range(4):
                for r in range(h0, h0 + HB, 16):
                    xs = x_v[pl.ds(base + (QS * a1 + r), 16), :].astype(F32)
                    pieces.append(jnp.concatenate(_bfly8([xs[:, 128 * a:128 * a + 128] for a in range(8)]),
                                                  axis=1))
                    z_s[a1, r // 2:r // 2 + 8, :] = _as_u32(pieces[-1][:, :128].astype(BF))
            ub = jnp.concatenate(pieces, axis=0)
            for g in range(4):
                yy = _dot(ub[:, 256 * g:256 * g + 256].astype(BF), _as_bf(gf[g]))
                v = _fft([(yy[HB * a1:HB * a1 + HB, :128], yy[HB * a1:HB * a1 + HB, 128:])
                          for a1 in range(4)], -1)
                for k1 in range(4):
                    rows = pl.ds(base + (QS * k1 + h0), HB)
                    y[g, 0, rows, :] = v[k1][0]
                    y[g, 1, rows, :] = v[k1][1]
                if h0 + HB == RB and g == 3:
                    for a1 in range(4):
                        xa[pl.ds(4 * a1 + i, 1), :] = _dot_nt(alt, _as_bf(z_s[a1]))[0:1]
        return c

    with jax.named_scope("f1"):
        lax.fori_loop(0, QS // RB, f1, 0)

    def fprep(h, c):
        ev, od = [], []
        for r in range(8):
            wr = fraw[h, 0, c, pl.ds(r, 32, stride=8), :]
            wi = fraw[h, 1, c, pl.ds(r, 32, stride=8), :]
            ev.append((wr & jnp.uint32(0xFFFF)) | (wi << 16))
            od.append((wr >> 16) | (wi & jnp.uint32(0xFFFF0000)))
        for g, cls in enumerate(CLASSES):
            t = _transpose_u32(jnp.concatenate([(od if k % 2 else ev)[k // 2] for k in cls], axis=0))
            for q in range(128 // N1):
                row = pl.multiple_of(((4 * h + c) * (128 // N1) + q) * PITCH, 8)
                fp[g, pl.ds(row, N1), :] = t[q * N1:(q + 1) * N1]

    def nyquist():
        twc, tws = sm[0:16], sm[16:32]
        u = _dot(sm[32:64, 0:16].astype(BF), xa[0:16, :].astype(BF))
        ur, ui = u[0:16], u[16:32]
        u = jnp.concatenate([ur * twc + ui * tws, ui * twc - ur * tws], axis=1).astype(BF)
        yield
        xx = _dot(u, _as_bf(gf[4]))
        xr, xi = xx[:, :128], xx[:, 128:]
        w = (pltpu.bitcast(nyq[0].astype(F32), U32) >> 16) | pltpu.bitcast(nyq[1].astype(F32), U32)
        w = jnp.concatenate([w[:, 128 * a:128 * a + 128] for a in range(16)], axis=0)
        wt = _transpose_u32(jnp.concatenate([w] * 8, axis=0))
        blk = _lanes(16) >> 4
        wm = wt[0:16]
        for j in range(1, 8):
            wm = jnp.where(blk == j, wt[16 * j:16 * j + 16], wm)
        wr, wi = _lo_f32(wm), _hi_f32(wm)
        z = jnp.concatenate([xr * wr - xi * wi, xr * wi + xi * wr], axis=1).astype(BF)
        yield
        pp = _dot(z, _as_bf(gf[5]))
        pr, pi = pp[:, :128], pp[:, 128:]
        pp = jnp.concatenate([pr * twc - pi * tws, pi * twc + pr * tws], axis=0).astype(BF)
        yield
        cc = _dot(sm[64:80, 0:32].astype(BF), pp) * (1.0 / (S * D))
        ct[...] = jnp.concatenate([cc, jnp.zeros((112, 128), F32)], axis=0).T
        yield

    def s_rows(k1, a0, r):
        return pl.ds(r + (QS * k1 + N2 * a0), 8)

    def anchored(v, tok):
        return jnp.where(zero_s[0] != 0, tok, v)

    def s_prep(g, k1, r, tok):
        v = [(y[g, 0, s_rows(k1, a0, r), :], y[g, 1, s_rows(k1, a0, r), :]) for a0 in range(8)]
        v[0] = (anchored(v[0][0], tok), v[0][1])
        v = _fft([_cmul_const(v[a0], a0 * k1, N1, -1) for a0 in range(8)], -1)
        for k0 in range(8):
            u_s[k1 + 4 * k0, pl.ds(r, 8), :] = _as_u32(jnp.concatenate(v[k0], axis=0).astype(BF))

    def s_fwd(g, ka, tok):
        xx = _dot(_as_bf(gs[0, ka]), _as_bf(u_s[ka]))
        w32 = fp[g, pl.ds(ka, N2, stride=PITCH), :]
        wr, wi = _lo_f32(w32), _hi_f32(w32)
        xr, xi = xx[:N2], xx[N2:]
        z_s[ka] = _as_u32(jnp.concatenate([xr * wr - xi * wi, xr * wi + xi * wr], axis=0).astype(BF))

    def s_inv(ka, tok):
        p_s[ka] = _dot(_as_bf(gs[1, ka]), _as_bf(z_s[ka]))

    def s_post(g, k1, r, tok):
        v = [(p_s[k1 + 4 * k0, r:r + 8, :], p_s[k1 + 4 * k0, N2 + r:N2 + r + 8, :]) for k0 in range(8)]
        v[0] = (anchored(v[0][0], tok), anchored(v[0][1], tok))
        v = _fft(v, 1)
        for a0 in range(8):
            vr, vi = _cmul_const(v[a0], a0 * k1, N1, 1)
            v_s[g, 0, s_rows(k1, a0, r), :] = vr
            v_s[g, 1, s_rows(k1, a0, r), :] = vi

    def acc(jj, i):
        return v_s.at[jj // 4, (jj // 2) % 2, pl.ds(1024 * (jj % 2) + 256 * i, 256), :]

    def bulk(item0, n, events, q=None):
        k0, nk = (0, KH) if q is None else (q * KQ, KQ)
        for i in range(n):
            item = item0 + i

            def hook(k, m):
                pieces = events.get(7 * i + k, ())
                vec = [pc for pc in pieces if isinstance(pc, P) and pc.func in (s_prep, s_post)]
                for piece in pieces:
                    r = 8 * ((32 * vec.index(piece)) // len(vec)) if piece in vec else 0
                    piece(m[r:r + 8])

            def finish(e, c1, c2):
                if q in (None, NQ - 1):
                    store_st(item, e, c1, c2)
                else:
                    acc(item, 2 * e)[...] = c1
                    acc(item, 2 * e + 1)[...] = c2

            init = None if q in (None, 0) else (lambda k: acc(item, k)[...])
            strassen(prep_rhs(item // 8, item % 8, k0, nk), k0, nk, init, finish, hook)

    def spread(events, pieces, q0, q1):
        for i, piece in enumerate(pieces):
            events.setdefault(q0 + ((q1 - q0) * i) // len(pieces), []).append(piece)

    P = functools.partial

    def loop_a(h, c):
        @pl.when(h % 2 == 0)
        def _():
            wait(raw4.at[1 + h // 2], SEM_W + 1 + h // 2)

        wait(fraw.at[h], SEM_F + h)
        events = {}
        spread(events, [lambda tok, c=c: fprep(h, c) for c in range(4)], 0, 24)
        bulk(8 + 4 * h, 4, events)
        return c

    def loop_b(g, c):
        @pl.when(g < 3)
        def _():
            wait(raw4.at[3 + g], SEM_W + 3 + g)

        gn = jnp.minimum(g + 1, 3)
        events = {}
        for k1 in range(4):
            q = BD * k1
            spread(events, [P(s_fwd, g, k1 + 4 * k0) for k0 in range(8)], q, q + BW)
            spread(events, [P(s_prep, gn, k1, r) for r in range(0, N2, 8)], q + BW, q + BW + BV)
            q += BL
            spread(events, [P(s_inv, k1 + 4 * k0) for k0 in range(8)], q, q + BW)
            spread(events, [P(s_post, g, k1, r) for r in range(0, N2, 8)], q + BW, q + BW + BV)
        assert max(events) < 41
        bulk(24 + 6 * g, 6, events)
        return c

    with jax.named_scope("p0"):
        ny = nyquist()
        for q in range(NQ):
            for e in range(2):
                wait(raw4.at[0, kslice(q, e)], SEM_W0 + q)
            events = {}
            if q == NQ - 1:
                wait(sm, SEM_SM)
                wait(gf.at[4:6], SEM_W)
                wait(nyq, SEM_NYQ)
                spread(events, [lambda tok: next(ny)] * 4, 4, 28)
            spread(events, [P(s_prep, 0, k1, r) for k1 in range(4 * q // NQ, 4 * (q + 1) // NQ)
                            for r in range(0, N2, 8)], 0, 52)
            bulk(0, 8, events, q)
    with jax.named_scope("loop_a"):
        lax.fori_loop(0, 4, loop_a, 0)
    wait(gs, SEM_GS)
    with jax.named_scope("loop_b"):
        lax.fori_loop(0, 4, loop_b, 0)
    wait(wo, SEM_WO)
    wait(gi, SEM_GI)
    wait(mem_ref, SEM_MEM)
    wait(gw_ref.at[pl.ds(0, D)], SEM_GW)

    scale = DH ** -0.5

    mf[0:80, :] = _mask80()
    gw_s[...] = jnp.broadcast_to(gw_ref[pl.ds(0, D)].astype(F32).reshape(1, D), (8, D))

    def softmax(s):
        fill = mf[0:80, :]
        s = jnp.where(fill > 0.0, s * scale, fill)
        m = jnp.max(s, axis=-1, keepdims=True)
        e = jnp.exp(s - m)
        l = jnp.sum(e, axis=-1, keepdims=True)
        return (e * (1.0 / l)).astype(BF)

    def lhs_rows(mem, seg):
        xs = x_v[pl.ds(pl.multiple_of(seg * SEG, SEG), SEG), :].astype(F32)
        return jnp.concatenate([mem, xs[8:SEG]], axis=0).astype(BF)

    def proj2(a, m, j):
        return jnp.concatenate([_dot(a, _as_bf(wqkv[H * m + 2 * j + p])).astype(BF) for p in range(2)], axis=0)

    def proj_first(a):
        part = [_dot(a[:, :D // 2], _as_bf(wqkv[H * (i // 2) + i % 2, 0:D // 4, :])) for i in range(6)]
        full = [(_dot(a[:, D // 2:], _as_bf(wqkv[H * (i // 2) + i % 2, D // 4:D // 2, :])) + part[i]).astype(BF)
                for i in range(6)]
        for m in range(3):
            stg[m, 0] = _as_u32(jnp.concatenate(full[2 * m:2 * m + 2], axis=0))

    def step(a, seg, first, hook=None):
        R = 32 if first else 48
        srow = pl.multiple_of(seg * 8, 8)

        def get(m, j):
            return _as_bf(jnp.concatenate([stg[m, j % 8], st[NP * m + j, pl.ds(srow, 8), :]], axis=0))

        def proj(j, m):
            if j > 0:
                stg[m, j % 8] = _as_u32(proj2(a, m, j))
            elif m == 0 and not first:
                proj_first(a)

        def scores(j):
            pst[j % 8] = _as_u32(softmax(_dot_nt(get(0, j), get(1, j))))

        def pv(j):
            o = _dot(_as_bf(pst[j % 8]), get(2, j))
            for i in range(2):
                h = 2 * j + i
                if first:
                    ob = o[32 * i:32 * i + 32]
                    sto[h] = o[64 + 8 * i:72 + 8 * i]
                else:
                    ob = jnp.concatenate([o[32 * i:32 * i + 32], o[64 + 8 * i:72 + 8 * i], sto[h]], axis=0)
                obuf[h, 0:R // 2, :] = _as_u32(ob.astype(BF))

        def wo_part(j, h0, h1):
            og = jnp.concatenate([_as_bf(obuf[h, 0:R // 2, :]) for h in range(h0, h1)], axis=1)
            return _dot(og, _as_bf(wo[j, h0 * 64:h1 * 64, :]))

        parts = []
        for i in range(NP + 4):
            for ch in ORDER:
                if ch in "qkv":
                    m = "qkv".index(ch)
                    if i < NP:
                        proj(i, m)
                    elif m < 2:
                        parts.append(wo_part(2 * (i - NP) + len(parts) % 2, 0, SPLIT))
                elif ch == "s" and 0 <= i - LAG1 < NP:
                    scores(i - LAG1)
                elif ch == "p" and 0 <= i - LAG2 < NP:
                    pv(i - LAG2)
            if hook is not None and i == HOOK_AT:
                hook()
        return jnp.concatenate([wo_part(j, SPLIT, H) + parts[j] for j in range(8)], axis=1)

    def start_pair(mem, t):
        a = lhs_rows(mem, 2 * t)
        a_s[...] = _as_u32(a)
        proj_first(a)

    def pair(t, c):
        base = pl.multiple_of(t * 64, 64)
        lane = _lanes(64)
        lo = lane < 64
        roll = lambda v: pltpu.roll(v, 64, 1)
        a1 = t // 8
        off = pl.multiple_of((t % 8) * 64, 64)
        s2 = (1 - 2 * (a1 & 1)).astype(F32)
        sg = (1 - (a1 & 2)).astype(F32)
        cc, ss = sg * (1 - (a1 & 1)).astype(F32), sg * (a1 & 1).astype(F32)

        def irfft_group(g):
            q = [[v_s[g, e, pl.ds(off + QS * k1, 64), :] for e in range(2)] for k1 in range(4)]
            br, bi = q[1][0] + s2 * q[3][0], q[1][1] + s2 * q[3][1]
            vr = q[0][0] + s2 * q[2][0] + (cc * br - ss * bi)
            vi = q[0][1] + s2 * q[2][1] + (cc * bi + ss * br)
            tin = _half_pre(vr, vi, lo, roll, jnp.where)
            tp, tm = [_dot(tin[e].astype(BF), _as_bf(gi[2 * g + e])) for e in range(2)]
            if g == 0:
                nyc = jnp.sum(jnp.where(lane == t // 2,
                                        ct[pl.ds(pl.multiple_of((t % 2) * 64, 64), 64), :], 0.0),
                              axis=-1, keepdims=True)
                tp = tp + nyc * (1 - 2 * (lane & 1)).astype(F32)
            return list(_half_post(g, tp, tm, lo, roll, jnp.where))

        def spectral_part():
            ts = sum([irfft_group(g) for g in range(4)], [])
            b = jnp.concatenate(_bfly8_t(ts), axis=1).astype(BF).astype(F32)
            xs = x_v[pl.ds(base, 64), :].astype(F32)
            gate = jax.nn.sigmoid(jnp.sum(xs * jnp.concatenate([gw_s[...]] * 8, axis=0), axis=-1, keepdims=True))
            bb = (1.0 - gate) * b
            bb_s[...] = jnp.concatenate([bb[0:8], bb[8:32] + gate[8:32] * bb_s[8:32], bb[32:64]], axis=0)
            g_s[...] = jnp.broadcast_to(gate, (64, 128))

        res_a = step(_as_bf(a_s[...]), 2 * t, True)
        bb_s[8:32] = res_a[8:32]
        a = lhs_rows(res_a[0:8], 2 * t + 1)
        res_b = step(a, 2 * t + 1, False, spectral_part)

        def gated(r0, r1, res):
            return bb_s[r0:r1] + jnp.concatenate([g_s[r0:r1]] * 8, axis=1) * res

        out_v[pl.ds(base, 64), :] = jnp.concatenate(
            [gated(0, 8, res_b[40:48]), bb_s[8:32], gated(32, 40, res_b[32:40]), gated(40, 64, res_b[8:32])],
            axis=0).astype(BF)
        pltpu.make_async_copy(out_v.at[pl.ds(base, 64), :], out_hbm.at[pl.ds(base, 64), :],
                              sem.at[SEM_OUT]).start()
        start_pair(res_b[0:8], jnp.minimum(t + 1, S // 64 - 1))
        return c

    with jax.named_scope("chain"):
        start_pair(mem_ref[...].astype(F32), 0)
        lax.fori_loop(0, S // 64, pair, 0)
    pltpu.make_async_copy(out_v, out_hbm, sem.at[SEM_OUT]).wait()


@jax.jit
def pallas_gated_mix__memory_aug_recurrent_mem_tr__spectral_gfnet__prompt_kernel(
    A_x, A_mem0, A_Wq, A_Wk, A_Wv, A_Wo, A_seg_len, B_x, B_w_r, B_w_i, gate_w,
):
    assert A_x.shape == (1, S, D) and A_mem0.shape == (1, M, D) and A_Wq.shape == (D, H, DH)
    consts = [jnp.asarray(c) for c in _constants()]
    any_spec = pl.BlockSpec(memory_space=pl.ANY)
    out = pl.pallas_call(
        _kernel,
        out_shape=jax.ShapeDtypeStruct((S, D), BF),
        in_specs=[any_spec] * 13,
        out_specs=any_spec,
        scratch_shapes=[
            pltpu.VMEM((S, D), BF),
            pltpu.VMEM((6, D * 8, DH), U32),
            pltpu.VMEM((3 * H, D // 2, DH), U32),
            pltpu.VMEM((8, H * DH // 2, 128), U32),
            pltpu.VMEM((3 * NP, 8 * NSEG, 128), U32),
            pltpu.VMEM((7, 2 * NSEG, D // 2), U32),
            pltpu.VMEM((4, 2, 4, 256, 128), U32),
            pltpu.VMEM((4, N2 * PITCH, 128), U32),
            pltpu.VMEM((6, 128, 256), U32),
            pltpu.VMEM((8, 64, 128), U32),
            pltpu.VMEM((2, N1, N2, 2 * N2), U32),
            pltpu.VMEM((4, 2, S, 128), F32),
            pltpu.VMEM((4, 2, S, 128), F32),
            pltpu.VMEM((S, D), BF),
            pltpu.VMEM((N1, N2, 128), U32),
            pltpu.VMEM((6, 256, 128), F32),
            pltpu.VMEM((N1, N2, 128), U32),
            pltpu.VMEM((N1, 2 * N2, 128), F32),
            pltpu.VMEM((H, 8, 128), F32),
            pltpu.VMEM((H, 24, 128), U32),
            pltpu.VMEM((128, 128), F32),
            pltpu.VMEM((16, D), U32),
            pltpu.VMEM((64, D), F32),
            pltpu.VMEM((64, 128), F32),
            pltpu.VMEM((3, 8, 32, 128), U32),
            pltpu.VMEM((8, 40, 80), U32),
            pltpu.VMEM((8, D), F32),
            pltpu.VMEM((M, D), BF),
            pltpu.VMEM((96, 80), F32),
            pltpu.VMEM((96, 128), F32),
            pltpu.VMEM((32, 128), F32),
            pltpu.VMEM((2, 1, S), BF),
            pltpu.VMEM((8 * D,), BF),
            pltpu.SMEM((2,), jnp.int32),
            pltpu.SemaphoreType.DMA((NSEM,)),
        ],
        compiler_params=pltpu.CompilerParams(vmem_limit_bytes=120 * 1024 * 1024),
    )(
        A_x.reshape(S, D), A_mem0.reshape(M, D), A_Wq, A_Wk, A_Wv,
        A_Wo.reshape(H * DH, D), B_w_r.T, B_w_i.T, gate_w, *consts,
    )
    return out.reshape(1, S, D)
```

```python
import functools
import itertools
import math

import numpy as np
import jax
import jax.numpy as jnp
from jax import lax
import jax.experimental.pallas as pl
import jax.experimental.pallas.tpu as pltpu

BF, F32, U32 = jnp.bfloat16, jnp.float32, jnp.uint32

S, D, H, DH, M, SEG = 2048, 1024, 32, 128, 8, 32
NSEG = S // SEG
NP = H // 2
N1, N2 = 32, 64
QS = S // 4
PITCH = N1 + 8
CLASSES = ((0, 8, 4, 12), (1, 15, 9, 7), (2, 14, 10, 6), (3, 13, 11, 5))
LAG1, LAG2, SPLIT, HOOK_AT = 1, 2, 27, 18
ORDER = "qksvp"
UNROLL = 2
DEADL = 0
ROT = 0
NMF = 1
AVAL = 1
OPQ = 0
DEFER = 0
NEWTON = 1
SPLIT11 = 1
NY0, NY1 = 32, 40
BD, BW, BV, BL = 7, 8, 8, 3
NQ = 2
(SEM_W, SEM_GF, SEM_GI, SEM_SM, SEM_GS, SEM_NYQ, SEM_WO, SEM_MEM, SEM_GW, SEM_OUT, SEM_F, SEM_X,
 SEM_W0) = 0, 6, 7, 8, 9, 10, 11, 12, 13, 14, 15, 19, 23
NSEM = SEM_W0 + 6
RSQ2 = float(np.float32(math.sqrt(0.5)))


def _bfly8(x):
    s = [x[i] + x[i + 4] for i in range(4)]
    d = [x[i] - x[i + 4] for i in range(4)]
    e, f = s[0] + s[2], s[1] + s[3]
    t1, t2 = (d[1] - d[3]) * RSQ2, (d[1] + d[3]) * RSQ2
    return [e + f, e - f, d[0] + t1, t2 + d[2], s[0] - s[2], s[1] - s[3], d[0] - t1, t2 - d[2]]


def _bfly8_t(t):
    e, f = t[0] + t[1], t[0] - t[1]
    s = [e + t[4], f + t[5], e - t[4], f - t[5]]
    t1, t2 = t[2] - t[6], t[3] + t[7]
    d = [t[2] + t[6], (t1 + t2) * RSQ2, t[3] - t[7], (t2 - t1) * RSQ2]
    return [s[i] + d[i] for i in range(4)] + [s[i] - d[i] for i in range(4)]


def _half_pre(vr, vi, lo, roll, where):
    ri = roll(vi)
    return where(lo, vr, ri), where(lo, ri, vr)


def _half_post(g, tp, tm, lo, roll, where):
    if g == 0:
        return tp, tm
    c = float(np.float32(math.cos(math.pi * g / 8)))
    s = float(np.float32(math.sin(math.pi * g / 8)))
    p, r = tp + tm, tp - tm
    rm = roll(where(lo, r, p))
    return where(lo, p, c * rm + s * r), where(lo, rm, c * r - s * rm)


def _cmul_const(v, k, n, sign):
    re, im = v
    k %= n
    if k == 0:
        return re, im
    if 4 * k == n:
        return (-im, re) if sign > 0 else (im, -re)
    if 8 * k == n:
        return (((re - im) * RSQ2, (re + im) * RSQ2) if sign > 0
                else ((re + im) * RSQ2, (im - re) * RSQ2))
    if 8 * k == 3 * n:
        return (((re + im) * -RSQ2, (re - im) * RSQ2) if sign > 0
                else ((im - re) * RSQ2, (re + im) * -RSQ2))
    c, s = math.cos(2 * math.pi * k / n), sign * math.sin(2 * math.pi * k / n)
    return re * c - im * s, re * s + im * c


def _fft(v, sign):
    n = len(v)
    if n == 1:
        return v
    ev, od = _fft(v[0::2], sign), _fft(v[1::2], sign)
    lo, hi = [], []
    for k in range(n // 2):
        er, ei = ev[k]
        if 4 * k == n:
            xr, xi = od[k]
            if sign > 0:
                lo.append((er - xi, ei + xr)); hi.append((er + xi, ei - xr))
            else:
                lo.append((er + xi, ei - xr)); hi.append((er - xi, ei + xr))
            continue
        tr, ti = _cmul_const(od[k], k, n, sign)
        lo.append((er + tr, ei + ti))
        hi.append((er - tr, ei - ti))
    return lo + hi


def _pack_rows(a):
    u = np.ascontiguousarray(a, dtype=np.float32).view(np.uint32)
    b = ((u + 0x7FFF + ((u >> 16) & 1)) >> 16).astype(np.uint32)
    return (b[..., 0::2, :] | (b[..., 1::2, :] << 16)).astype(np.uint32)


def _diag_blocks(full, n, tol):
    k = full.shape[0] // n
    blk = np.kron(np.eye(k), np.ones((n, n)))
    assert np.abs(full * (1 - blk)).max() < tol
    return np.stack([full[n * g:n * g + n, n * g:n * g + n] for g in range(k)])


def _cplx(re, im):
    return np.block([[re, im], [-im, re]])


@functools.lru_cache(maxsize=None)
def _constants():
    k2 = np.stack([np.concatenate([c + 16 * np.arange(32) for c in cls]) for cls in CLASSES])
    n2 = np.arange(D)
    ang = 2 * np.pi * ((k2[:, :, None] * n2[None, None, :]) % D) / D
    rows = np.stack([np.cos(ang), -np.sin(ang)], axis=1)
    wgt = np.where(k2 == 0, 1.0, 2.0)[:, None, :, None]
    fwd = rows.reshape(D, D).T
    inv = (rows * wgt).reshape(D, D) / (S * D)
    bf = np.stack(_bfly8(list(np.eye(8))))
    binv = np.kron(np.linalg.inv(bf), np.eye(128))
    gd = _diag_blocks(binv.T @ fwd, 256, 1e-6)
    gdi = _diag_blocks(inv @ binv, 256, 1e-12)
    eye, lo = np.eye(256), np.arange(128) < 64
    roll = lambda v: np.roll(v, 64, axis=1)
    pre = np.concatenate(_half_pre(eye[:, :128], eye[:, 128:], lo, roll, np.where), axis=1)
    gi = []
    for g in range(4):
        post = np.concatenate(_half_post(g, eye[:, :128], eye[:, 128:], lo, roll, np.where), axis=1)
        gi.append(_diag_blocks(np.linalg.inv(pre) @ gdi[g] @ np.linalg.inv(post), 128, 1e-12))
    gi = np.concatenate(gi)

    b = np.arange(N2)
    k1 = np.arange(N1)[:, None] + N1 * np.arange(N2)[None, :]
    th = 2 * np.pi * ((k1[:, :, None] * b[None, None, :]) % S) / S
    gr, gim = np.cos(th), -np.sin(th)
    full = np.block([[gr, -gim], [gim, gr]])
    kap = np.arange(2 * N2)
    src = ((kap >> 3) & 1) * N2 + (kap >> 4) * 8 + (kap & 7)
    gs = full[:, :, src]
    hr, hi = np.swapaxes(gr, 1, 2), -np.swapaxes(gim, 1, 2)
    gsi = np.block([[hr, -hi], [hi, hr]])

    lane = np.arange(128)
    kb = 8 * (lane % 16) + lane // 16
    t128 = 2 * np.pi * ((lane[:, None] * kb[None, :]) % 128) / 128
    nyf = _cplx(np.cos(t128), -np.sin(t128))
    nyi = _cplx(np.cos(t128).T, np.sin(t128).T)
    i16 = np.arange(16)
    t16 = 2 * np.pi * ((i16[:, None] * i16[None, :]) % 16) / 16
    tw = 2 * np.pi * (i16[:, None] * lane[None, :]) / S
    sm = np.zeros((96, 128), np.float32)
    sm[0:16], sm[16:32] = np.cos(tw), np.sin(tw)
    sm[32:48, :16], sm[48:64, :16] = np.cos(t16), -np.sin(t16)
    sm[64:80, :16], sm[64:80, 16:32] = np.cos(t16), -np.sin(t16)

    gfp = _pack_rows(np.concatenate([gd, nyf[None], nyi[None]]))
    return gfp, _pack_rows(gi), sm, _pack_rows(np.stack([gs, gsi]))


def _mask80():
    r = lax.broadcasted_iota(jnp.int32, (80, 80), 0)
    c = lax.broadcasted_iota(jnp.int32, (80, 80), 1)

    def head(i):
        return jnp.where(i < 64, i >> 5, (i - 64) >> 3)

    def pos(i):
        j = i & 31
        return jnp.where(i < 64, jnp.where(j < M, j, j + 8), M + (i & 7))

    same = head(r) == head(c)
    ok = (pos(r) < M) | (pos(c) <= pos(r))
    return jnp.where(same, jnp.where(ok, 1.0, -1e9), -jnp.inf).astype(F32)


def _as_bf(u):
    return pltpu.bitcast(u, BF)


def _as_u32(b):
    return pltpu.bitcast(b, U32)


def _lo_f32(u):
    return pltpu.bitcast(u << 16, F32)


def _hi_f32(u):
    return pltpu.bitcast(u & jnp.uint32(0xFFFF0000), F32)


def _dot(a, b):
    return jnp.dot(a, b, preferred_element_type=F32)


def _dot_nt(a, b):
    return lax.dot_general(a, b, (((1,), (1,)), ((), ())), preferred_element_type=F32)


def _transpose_u32(u):
    return pltpu.bitcast(pltpu.bitcast(u, F32).T, U32)


def _lanes(rows):
    return lax.broadcasted_iota(jnp.int32, (rows, 128), 1)


def _kernel(x_hbm, mem_hbm, wq_hbm, wk_hbm, wv_hbm, wo_hbm, fr_hbm, fi_hbm, gw_hbm,
            gf_hbm, gi_hbm, sm_hbm, gs_hbm,
            out_hbm,
            x_v, raw, wqkv, wo, st, sl, fraw, fp, gf, gi, gs, y, v_s, out_v, u_s, cb, z_s, p_s,
            sto, obuf, ct, a_s, pa_s, bb_s, g_s, stg, pst, rst, gw_s, mem_ref, mf, sm, xa, nyq, gw_ref, zero_s, sem):
    KH = D // 2
    KQ = KH // NQ
    RB, HB = 128, 16
    raw4 = raw.reshape(6, D, 8, DH)
    w_hbm = (wq_hbm, wk_hbm, wv_hbm)
    f_hbm = (fr_hbm, fi_hbm)

    def w_src(c):
        return w_hbm[c // 2].bitcast(U32).at[:, pl.ds(8 * (c % 2), 8), :]

    def wait(dst, k):
        pltpu.make_async_copy(dst, dst, sem.at[k]).wait()

    def w_half(ref, q, e):
        return ref.at[pl.ds(pl.multiple_of(q * KQ, KQ) + e * KH, KQ)]

    def x_rows(i, a1):
        return pl.ds(pl.multiple_of(i * RB, RB) + QS * a1, RB)

    def f_copies(h):
        return [(f_hbm[a].at[pl.ds(0, D // 2), pl.ds(128 * (4 * h + c), 128)].bitcast(U32),
                 fraw.at[h, a, c], SEM_F + h) for a in range(2) for c in range(4)]

    def w_copy(c):
        return [(w_src(c), raw4.at[c], SEM_W + c)]

    copies = [(gf_hbm.at[0:4], gf.at[0:4], SEM_GF)]
    copies += [(x_hbm.at[x_rows(i, a1), :], x_v.at[x_rows(i, a1), :], SEM_X + i)
               for i in range(QS // RB) for a1 in range(4)]
    for n in range(6):
        copies += [(w_half(w_src(n // 2), n % 2, e), w_half(raw4.at[n // 2], n % 2, e), SEM_W0 + n)
                   for e in range(2)]
        if n >= 2:
            copies += f_copies(n - 2)
    copies += [(sm_hbm, sm, SEM_SM), (gf_hbm.at[4:6], gf.at[4:6], SEM_W)]
    copies += [(f_hbm[a].at[pl.ds(D // 2, 1), :], nyq.at[a], SEM_NYQ) for a in range(2)]
    copies += [(gs_hbm, gs, SEM_GS)] + w_copy(3) + w_copy(4) + w_copy(5)
    copies += [(wo_hbm.bitcast(U32).at[:, pl.ds(128 * j, 128)], wo.at[j], SEM_WO) for j in range(8)]
    copies += [(gi_hbm, gi, SEM_GI), (mem_hbm, mem_ref, SEM_MEM), (gw_hbm, gw_ref.at[pl.ds(0, D)], SEM_GW)]
    for src, dst, k in copies:
        pltpu.make_async_copy(src, dst, sem.at[k]).start()

    def prep_rhs(ch, jj, k0, nk):
        item = 8 * ch + jj
        a1 = raw[ch, pl.ds(k0 * 8 + jj, nk, stride=8), :]
        a2 = raw[ch, pl.ds((KH + k0) * 8 + jj, nk, stride=8), :]
        b11, b12, b21, b22 = _lo_f32(a1), _hi_f32(a1), _lo_f32(a2), _hi_f32(a2)
        for p, e, b in ((0, 0, b11), (1, 0, b12), (0, 1, b21), (1, 1, b22)):
            row = pl.multiple_of(k0 // 2, nk // 2) + e * KH // 2
            wqkv[2 * item + p, pl.ds(row, nk // 2), :] = _as_u32(b.astype(BF))
        return [v.astype(BF) for v in (b11 + b22, b11, b12 - b22, b21 - b11, b22, b11 + b12, b21 + b22)]

    def strassen(rhs, k0, nk, item, init, keep, after_dot):
        def prod(i):
            return _dot(_as_bf(sl[i, :, pl.ds(k0, nk)]), rhs[i])

        def plus(i, r):
            return r if init is None else init(i) + r

        c12, c21 = (cb.at[5], cb.at[4]) if keep is None else (keep(1), keep(2))
        m = prod(1)
        cb[0] = m
        after_dot(0, m)
        m = prod(4)
        cb[1] = m
        after_dot(1, m)
        m1 = prod(0)
        cb[3] = plus(3, m1 - cb[0])
        if keep is None or SPLIT11:
            cb[2] = plus(0, m1 - cb[1])
        after_dot(2, m1)
        m = prod(3)
        c21[...] = plus(2, cb[0] + m)
        cb[2] = cb[2] + m if keep is None or SPLIT11 else plus(0, m1 - cb[1]) + m
        after_dot(3, m)
        m = prod(2)
        c12[...] = plus(1, cb[1] + m)
        cb[3] = cb[3] + m
        after_dot(4, m)
        for k, (i, acc) in enumerate(((6, 2), (5, 3))):
            m = prod(i) + cb[acc]
            if keep is not None:
                keep(3 * k)[...] = m
            store_st(item, k, *((m, c12[...]) if k == 0 else (c21[...], m)))
            after_dot(5 + k, m)

    def store_st(item, e, c1, c2):
        r = jnp.concatenate([c.reshape(NSEG // 2, 8, 128) for c in (c1, c2)], axis=1)
        st[item, 256 * e:256 * e + 256, :] = _as_u32(r.reshape(8 * NSEG, 128).astype(BF))

    def pin(i, c):
        if 1:
            cb[i, 0:8, :] = jnp.zeros((8, 128), F32)
        zero_s[i] = 0
        z_s[i, 0:8, :] = jnp.zeros((8, 128), U32)
        p_s[i, 0:8, :] = jnp.zeros((8, 128), F32)
        u_s[i, 0:8, :] = jnp.zeros((8, 128), U32)
        stg[i, 0, 0:8, :] = jnp.zeros((8, 128), U32)
        obuf[i, 0:8, :] = jnp.zeros((8, 128), U32)
        sto[i] = jnp.zeros((8, 128), F32)
        rst[i, 0:8, :] = jnp.zeros((8, 128), F32)
        if 1:
            a_s[i, 0:8, 0:128] = jnp.zeros((8, 128), U32)
        pa_s[i, 0:8, :] = jnp.zeros((8, 128), F32)
        if 0:
            bb_s[pl.ds(pl.multiple_of(8 * i, 8), 8), 0:128] = jnp.zeros((8, 128), F32)
            g_s[pl.ds(pl.multiple_of(8 * i, 8), 8), :] = jnp.zeros((8, 128), F32)
        return c

    lax.fori_loop(0, 2, pin, 0)

    def fill_mask(i, c):
        mf[i, 0:80, :] = _mask80()
        return c

    lax.fori_loop(0, NMF, fill_mask, 0)
    fraw[4] = jnp.zeros(fraw.shape[1:], U32)

    wait(gf.at[0:4], SEM_GF)

    def f1(i, c):
        for a1 in range(4):
            wait(x_v.at[x_rows(i, a1), :], SEM_X + i)
        base = pl.multiple_of(i * RB, RB)
        alt = (1 - 2 * (_lanes(16) & 1)).astype(F32).astype(BF)

        def rows16(r):
            return jnp.concatenate([x_v[pl.ds(r + d, 16), :].astype(F32)[0:8] for d in (0, SEG)], axis=0)

        for r in (0, 64, QS, QS + 64):
            top, bot = rows16(base + r), rows16(base + (r + 2 * QS))
            a11, a12, a21, a22 = top[:, :KH], top[:, KH:], bot[:, :KH], bot[:, KH:]
            row = pl.multiple_of((base + r) // 8, 8)
            for k, v in enumerate((a11 + a22, a21 + a22, a11, a22, a11 + a12, a21 - a11, a12 - a22)):
                sl[k, pl.ds(row, 8), :] = _as_u32(v.astype(BF))
        for h0 in range(0, RB, HB):
            pieces = []
            for a1 in range(4):
                for r in range(h0, h0 + HB, 16):
                    xs = x_v[pl.ds(base + (QS * a1 + r), 16), :].astype(F32)
                    pieces.append(jnp.concatenate(_bfly8([xs[:, 128 * a:128 * a + 128] for a in range(8)]),
                                                  axis=1))
                    z_s[a1, r // 2:r // 2 + 8, :] = _as_u32(pieces[-1][:, :128].astype(BF))
            ub = jnp.concatenate(pieces, axis=0)
            for g in range(4):
                yy = _dot(ub[:, 256 * g:256 * g + 256].astype(BF), _as_bf(gf[g]))
                v = _fft([(yy[HB * a1:HB * a1 + HB, :128], yy[HB * a1:HB * a1 + HB, 128:])
                          for a1 in range(4)], -1)
                for k1 in range(4):
                    rows = pl.ds(base + (QS * k1 + h0), HB)
                    y[g, 0, rows, :] = v[k1][0]
                    y[g, 1, rows, :] = v[k1][1]
                if h0 + HB == RB and g == 3:
                    for a1 in range(4):
                        xa[pl.ds(4 * a1 + i, 1), :] = _dot_nt(alt, _as_bf(z_s[a1]))[0:1]
        return c

    with jax.named_scope("f1"):
        lax.fori_loop(0, QS // RB, f1, 0)

    def fprep(src, h, c):
        ev, od = [], []
        for r in range(8):
            wr = fraw[src, 0, c, pl.ds(r, 32, stride=8), :]
            wi = fraw[src, 1, c, pl.ds(r, 32, stride=8), :]
            ev.append((wr & jnp.uint32(0xFFFF)) | (wi << 16))
            od.append((wr >> 16) | (wi & jnp.uint32(0xFFFF0000)))
        for g, cls in enumerate(CLASSES):
            t = _transpose_u32(jnp.concatenate([(od if k % 2 else ev)[k // 2] for k in cls], axis=0))
            for q in range(128 // N1):
                row = pl.multiple_of(((4 * h + c) * (128 // N1) + q) * PITCH, 8)
                fp[g, pl.ds(row, N1), :] = t[q * N1:(q + 1) * N1]

    def nyquist():
        twc, tws = sm[0:16], sm[16:32]
        u = _dot(sm[32:64, 0:16].astype(BF), xa[0:16, :].astype(BF))
        ur, ui = u[0:16], u[16:32]
        u = jnp.concatenate([ur * twc + ui * tws, ui * twc - ur * tws], axis=1).astype(BF)
        yield
        xx = _dot(u, _as_bf(gf[4]))
        xr, xi = xx[:, :128], xx[:, 128:]
        w = (pltpu.bitcast(nyq[0].astype(F32), U32) >> 16) | pltpu.bitcast(nyq[1].astype(F32), U32)
        w = jnp.concatenate([w[:, 128 * a:128 * a + 128] for a in range(16)], axis=0)
        wt = _transpose_u32(jnp.concatenate([w] * 8, axis=0))
        blk = _lanes(16) >> 4
        wm = wt[0:16]
        for j in range(1, 8):
            wm = jnp.where(blk == j, wt[16 * j:16 * j + 16], wm)
        wr, wi = _lo_f32(wm), _hi_f32(wm)
        z = jnp.concatenate([xr * wr - xi * wi, xr * wi + xi * wr], axis=1).astype(BF)
        yield
        pp = _dot(z, _as_bf(gf[5]))
        pr, pi = pp[:, :128], pp[:, 128:]
        pp = jnp.concatenate([pr * twc - pi * tws, pi * twc + pr * tws], axis=0).astype(BF)
        yield
        cc = _dot(sm[64:80, 0:32].astype(BF), pp) * (1.0 / (S * D))
        ct[...] = jnp.concatenate([cc, jnp.zeros((112, 128), F32)], axis=0).T
        yield

    def s_rows(k1, a0, r):
        return pl.ds(r + (QS * k1 + N2 * a0), 8)

    def anchored(v, tok, inst=0):
        return jnp.where(zero_s[inst] != 0, tok, v)

    def s_prep(g, k1, r, tok):
        v = [(y[g, 0, s_rows(k1, a0, r), :], y[g, 1, s_rows(k1, a0, r), :]) for a0 in range(8)]
        if tok is not None:
            v[0] = (anchored(v[0][0], tok), v[0][1])
        v = _fft([_cmul_const(v[a0], a0 * k1, N1, -1) for a0 in range(8)], -1)
        for k0 in range(8):
            u_s[k1 + 4 * k0, pl.ds(r, 8), :] = _as_u32(jnp.concatenate(v[k0], axis=0).astype(BF))

    def s_fwd(g, ka, tok):
        xx = _dot(_as_bf(gs[0, ka]), _as_bf(u_s[ka]))
        w32 = fp[g, pl.ds(ka, N2, stride=PITCH), :]
        wr, wi = _lo_f32(w32), _hi_f32(w32)
        xr, xi = xx[:N2], xx[N2:]
        z_s[ka] = _as_u32(jnp.concatenate([xr * wr - xi * wi, xr * wi + xi * wr], axis=0).astype(BF))

    def s_inv(ka, tok):
        p_s[ka] = _dot(_as_bf(gs[1, ka]), _as_bf(z_s[ka]))

    def s_post(g, k1, r, tok):
        v = [(p_s[k1 + 4 * k0, r:r + 8, :], p_s[k1 + 4 * k0, N2 + r:N2 + r + 8, :]) for k0 in range(8)]
        v[0] = (anchored(v[0][0], tok), anchored(v[0][1], tok))
        v = _fft(v, 1)
        for a0 in range(8):
            vr, vi = _cmul_const(v[a0], a0 * k1, N1, 1)
            v_s[g, 0, s_rows(k1, a0, r), :] = vr
            v_s[g, 1, s_rows(k1, a0, r), :] = vi

    def bulk(where, n, events, q=None):
        k0, nk = (0, KH) if q is None else (pl.multiple_of(q * KQ, KQ), KQ)
        for i in range(n):
            ch, jj = where(i)

            def hook(k, m):
                pieces = events.get(7 * i + k, ())
                vec = [pc for pc in pieces if isinstance(pc, P) and pc.func in (s_prep, s_post)]
                for piece in pieces:
                    r = 8 * ((32 * vec.index(piece)) // len(vec)) if piece in vec else 0
                    piece(m[r:r + 8])

            def keep(k):
                return v_s.at[jj // 4, (jj // 2) % 2, pl.ds(1024 * (jj % 2) + 256 * k, 256), :]

            def init(k):
                return jnp.where(q > 0, keep(k)[...], 0.0)

            strassen(prep_rhs(ch, jj, k0, nk), k0, nk, 8 * ch + jj,
                     None if q is None else init, None if q is None else keep, hook)

    def spread(events, pieces, q0, q1):
        for i, piece in enumerate(pieces):
            events.setdefault(q0 + ((q1 - q0) * i) // len(pieces), []).append(piece)

    P = functools.partial

    def loop_a(n, c):
        for e in range(2):
            wait(w_half(raw4.at[n // 2], n % 2, e), SEM_W0 + n)
        h = jnp.maximum(n - 2, 0)

        @pl.when(n >= 2)
        def _():
            wait(fraw.at[h], SEM_F + h)

        src = jnp.where(n >= 2, h, 4)
        events = {}
        spread(events, [lambda tok, c=c: fprep(src, h, c) for c in range(4)], 0, 48)
        bulk(lambda i: (n // 2, i), 8, events, n % 2)
        return c

    def loop_b(g, c):
        @pl.when(g < 3)
        def _():
            wait(raw4.at[3 + g], SEM_W + 3 + g)

        gn = jnp.minimum(g + 1, 3)
        events = {}
        for k1 in range(4):
            q = BD * k1
            spread(events, [P(s_fwd, g, k1 + 4 * k0) for k0 in range(8)], q, q + BW)
            spread(events, [P(s_prep, gn, k1, r) for r in range(0, N2, 8)], q + BW, q + BW + BV)
            q += BL
            spread(events, [P(s_inv, k1 + 4 * k0) for k0 in range(8)], q, q + BW)
            spread(events, [P(s_post, g, k1, r) for r in range(0, N2, 8)], q + BW, q + BW + BV)
        ny = nyquist()
        spread(events, [lambda tok: next(ny)] * 4, NY0, NY1)
        assert max(events) < 41
        bulk(lambda i: ((24 + 6 * g + i) // 8, (24 + 6 * g + i) % 8), 6, events)
        return c

    def prep0(i, c):
        for k1 in range(4):
            s_prep(0, k1, pl.multiple_of(i * 8, 8), None)
        return c

    lax.fori_loop(0, N2 // 8, prep0, 0)
    with jax.named_scope("loop_a"):
        lax.fori_loop(0, 6, loop_a, 0)
    wait(sm, SEM_SM)
    wait(gf.at[4:6], SEM_W)
    wait(nyq, SEM_NYQ)
    wait(gs, SEM_GS)
    with jax.named_scope("loop_b"):
        lax.fori_loop(0, 4, loop_b, 0)
    wait(wo, SEM_WO)
    wait(gi, SEM_GI)
    wait(mem_ref, SEM_MEM)
    wait(gw_ref.at[pl.ds(0, D)], SEM_GW)

    scale = DH ** -0.5

    for i in range(UNROLL):
        gw_s[i] = jnp.broadcast_to(gw_ref[pl.ds(0, D)].astype(F32).reshape(1, D), (8, D))

    uses = itertools.count()

    def softmax(s):
        fill = mf[next(uses) % NMF, 0:80, :]
        s = jnp.where(fill > 0.0, s * scale, fill)
        m = jnp.max(s, axis=-1, keepdims=True)
        e = jnp.exp(s - m)
        l = jnp.sum(e, axis=-1, keepdims=True)
        if NEWTON:
            r = pl.reciprocal(l, approx=True)
            r = r * (2.0 - l * r)
        else:
            r = 1.0 / l
        return e, r

    def lhs_rows(mem, seg):
        xs = x_v[pl.ds(pl.multiple_of(seg * SEG, SEG), SEG), :].astype(F32)
        return jnp.concatenate([mem, xs[8:SEG]], axis=0).astype(BF)

    def proj2(a, m, j):
        return jnp.concatenate([_dot(_as_bf(a[...]), _as_bf(wqkv[H * m + 2 * j + p])).astype(BF)
                                for p in range(2)], axis=0)

    def proj_lo(a):
        for i in range(6):
            pa_s[i] = _dot(_as_bf(a[:, :KH]), _as_bf(wqkv[H * (i // 2) + i % 2, 0:KH // 2, :]))

    def proj_hi(a):
        full = [(_dot(_as_bf(a[:, KH:]), _as_bf(wqkv[H * (i // 2) + i % 2, KH // 2:KH, :]))
                 + pa_s[i]).astype(BF) for i in range(6)]
        for m in range(3):
            stg[m, 0] = _as_u32(jnp.concatenate(full[2 * m:2 * m + 2], axis=0))

    def step(a, seg, first, hook=None, inst=0):
        R = 32 if first else 48
        srow = pl.multiple_of(seg * 8, 8)
        if AVAL:
            a = a[...]

        def get(m, j):
            return _as_bf(jnp.concatenate([stg[m, j % 8], st[NP * m + j, pl.ds(srow, 8), :]], axis=0))

        def proj(j, m):
            if j > 0:
                stg[m, j % 8] = _as_u32(proj2(a, m, j))
            elif m == 0:
                if not first:
                    proj_lo(a)
                if not (first and ROT):
                    proj_hi(a)

        def scores(j):
            e, r = softmax(_dot_nt(get(0, j), get(1, j)))
            if DEFER:
                pst[j % 8] = _as_u32(e.astype(BF))
                rst[j % 8, 0:80, :] = jnp.broadcast_to(r, (80, 128))
            else:
                pst[j % 8] = _as_u32((e * r).astype(BF))

        def pv(j):
            o = _dot(_as_bf(pst[j % 8]), get(2, j))
            if DEFER:
                o = o * rst[j % 8, 0:80, :]
            for i in range(2):
                h = 2 * j + i
                if first:
                    ob = o[32 * i:32 * i + 32]
                    sto[h] = o[64 + 8 * i:72 + 8 * i]
                else:
                    ob = jnp.concatenate([o[32 * i:32 * i + 32], o[64 + 8 * i:72 + 8 * i], sto[h]], axis=0)
                obuf[h, 0:R // 2, :] = _as_u32(ob.astype(BF))

        def wo_part(j, h0, h1):
            og = jnp.concatenate([_as_bf(obuf[h, 0:R // 2, :]) for h in range(h0, h1)], axis=1)
            return _dot(og, _as_bf(wo[j, h0 * 64:h1 * 64, :]))

        parts = []
        for i in range(NP + 4):
            for ch in ORDER:
                if ch in "qkv":
                    m = "qkv".index(ch)
                    if i < NP:
                        proj(i, m)
                    elif m < 2:
                        parts.append(wo_part(2 * (i - NP) + len(parts) % 2, 0, SPLIT))
                elif ch == "s" and 0 <= i - LAG1 < NP:
                    scores(i - LAG1)
                elif ch == "p" and 0 <= i - LAG2 < NP:
                    pv(i - LAG2)
            if hook is not None and i == HOOK_AT:
                tok = hook()
        if hook is not None and DEADL:
            parts = [jnp.concatenate([anchored(p[0:8], tok[:, 128 * j:128 * j + 128], inst), p[8:]], axis=0)
                     for j, p in enumerate(parts)]
        return jnp.concatenate([wo_part(j, SPLIT, H) + parts[j] for j in range(8)], axis=1)

    def start_pair(mem, t):
        a = a_s.at[0]
        a_s[zero_s[1] if OPQ else 0] = _as_u32(lhs_rows(mem, 2 * t))
        proj_lo(a)
        if ROT:
            proj_hi(a)

    def pair(t, inst):
        base = pl.multiple_of(t * 64, 64)
        lane = _lanes(64) + zero_s[inst]
        lo = lane < 64
        roll = lambda v: pltpu.roll(v, 64, 1)
        a1 = t // 8
        off = pl.multiple_of((t % 8) * 64, 64)
        s2 = (1 - 2 * (a1 & 1)).astype(F32)
        sg = (1 - (a1 & 2)).astype(F32)
        cc, ss = sg * (1 - (a1 & 1)).astype(F32), sg * (a1 & 1).astype(F32)

        def irfft_group(g):
            q = [[v_s[g, e, pl.ds(off + QS * k1, 64), :] for e in range(2)] for k1 in range(4)]
            br, bi = q[1][0] + s2 * q[3][0], q[1][1] + s2 * q[3][1]
            vr = q[0][0] + s2 * q[2][0] + (cc * br - ss * bi)
            vi = q[0][1] + s2 * q[2][1] + (cc * bi + ss * br)
            tin = _half_pre(vr, vi, lo, roll, jnp.where)
            tp, tm = [_dot(tin[e].astype(BF), _as_bf(gi[2 * g + e])) for e in range(2)]
            if g == 0:
                nyc = jnp.sum(jnp.where(lane == t // 2,
                                        ct[pl.ds(pl.multiple_of((t % 2) * 64, 64), 64), :], 0.0),
                              axis=-1, keepdims=True)
                tp = tp + nyc * (1 - 2 * (lane & 1)).astype(F32)
            return list(_half_post(g, tp, tm, lo, roll, jnp.where))

        def spectral_part():
            ts = sum([irfft_group(g) for g in range(4)], [])
            b = jnp.concatenate(_bfly8_t(ts), axis=1).astype(BF).astype(F32)
            xs = x_v[pl.ds(base, 64), :].astype(F32)
            gate = jax.nn.sigmoid(jnp.sum(xs * jnp.concatenate([gw_s[inst]] * 8, axis=0), axis=-1, keepdims=True))
            bb = (1.0 - gate) * b
            bb_s[...] = jnp.concatenate([bb[0:8], bb[8:32] + gate[8:32] * bb_s[8:32], bb[32:64]], axis=0)
            g_s[...] = jnp.broadcast_to(gate, (64, 128))
            return functools.reduce(jnp.maximum, [bb[r:r + 8] for r in range(0, 64, 8)])

        res_a = step(a_s.at[0], 2 * t, True)
        bb_s[8:32] = res_a[8:32]
        a_s[zero_s[1] + 1 if OPQ else 1] = _as_u32(lhs_rows(res_a[0:8], 2 * t + 1))
        res_b = step(a_s.at[1], 2 * t + 1, False, spectral_part, inst)

        def gated(r0, r1, res):
            return bb_s[r0:r1] + jnp.concatenate([g_s[r0:r1]] * 8, axis=1) * res

        out_v[pl.ds(base, 64), :] = jnp.concatenate(
            [gated(0, 8, res_b[40:48]), bb_s[8:32], gated(32, 40, res_b[32:40]), gated(40, 64, res_b[8:32])],
            axis=0).astype(BF)
        start_pair(res_b[0:8], jnp.minimum(t + 1, S // 64 - 1))

    def pairs(u, c):
        for i in range(UNROLL):
            pair(UNROLL * u + i, i)
        rows = pl.ds(pl.multiple_of(u * (64 * UNROLL), 64), 64 * UNROLL)
        pltpu.make_async_copy(out_v.at[rows, :], out_hbm.at[rows, :], sem.at[SEM_OUT]).start()
        return c

    with jax.named_scope("chain"):
        start_pair(mem_ref[...].astype(F32), 0)
        lax.fori_loop(0, S // (64 * UNROLL), pairs, 0)
    pltpu.make_async_copy(out_v, out_hbm, sem.at[SEM_OUT]).wait()


@jax.jit
def pallas_gated_mix__memory_aug_recurrent_mem_tr__spectral_gfnet__prompt_kernel(
    A_x, A_mem0, A_Wq, A_Wk, A_Wv, A_Wo, A_seg_len, B_x, B_w_r, B_w_i, gate_w,
):
    assert A_x.shape == (1, S, D) and A_mem0.shape == (1, M, D) and A_Wq.shape == (D, H, DH)
    consts = [jnp.asarray(c) for c in _constants()]
    any_spec = pl.BlockSpec(memory_space=pl.ANY)
    out = pl.pallas_call(
        _kernel,
        out_shape=jax.ShapeDtypeStruct((S, D), BF),
        in_specs=[any_spec] * 13,
        out_specs=any_spec,
        scratch_shapes=[
            pltpu.VMEM((S, D), BF),
            pltpu.VMEM((6, D * 8, DH), U32),
            pltpu.VMEM((3 * H, D // 2, DH), U32),
            pltpu.VMEM((8, H * DH // 2, 128), U32),
            pltpu.VMEM((3 * NP, 8 * NSEG, 128), U32),
            pltpu.VMEM((7, 2 * NSEG, D // 2), U32),
            pltpu.VMEM((5, 2, 4, 256, 128), U32),
            pltpu.VMEM((4, N2 * PITCH, 128), U32),
            pltpu.VMEM((6, 128, 256), U32),
            pltpu.VMEM((8, 64, 128), U32),
            pltpu.VMEM((2, N1, N2, 2 * N2), U32),
            pltpu.VMEM((4, 2, S, 128), F32),
            pltpu.VMEM((4, 2, S, 128), F32),
            pltpu.VMEM((S, D), BF),
            pltpu.VMEM((N1, N2, 128), U32),
            pltpu.VMEM((6, 256, 128), F32),
            pltpu.VMEM((N1, N2, 128), U32),
            pltpu.VMEM((N1, 2 * N2, 128), F32),
            pltpu.VMEM((H, 8, 128), F32),
            pltpu.VMEM((H, 24, 128), U32),
            pltpu.VMEM((128, 128), F32),
            pltpu.VMEM((2, 16, D), U32),
            pltpu.VMEM((6, 32, 128), F32),
            pltpu.VMEM((64, D), F32),
            pltpu.VMEM((64, 128), F32),
            pltpu.VMEM((3, 8, 32, 128), U32),
            pltpu.VMEM((8, 40, 80), U32),
            pltpu.VMEM((8, 96, 128), F32),
            pltpu.VMEM((UNROLL, 8, D), F32),
            pltpu.VMEM((M, D), BF),
            pltpu.VMEM((NMF, 96, 80), F32),
            pltpu.VMEM((96, 128), F32),
            pltpu.VMEM((32, 128), F32),
            pltpu.VMEM((2, 1, S), BF),
            pltpu.VMEM((8 * D,), BF),
            pltpu.SMEM((2,), jnp.int32),
            pltpu.SemaphoreType.DMA((NSEM,)),
        ],
        compiler_params=pltpu.CompilerParams(vmem_limit_bytes=120 * 1024 * 1024),
    )(
        A_x.reshape(S, D), A_mem0.reshape(M, D), A_Wq, A_Wk, A_Wv,
        A_Wo.reshape(H * DH, D), B_w_r.T, B_w_i.T, gate_w, *consts,
    )
    return out.reshape(1, S, D)
```

```python
import functools
import itertools
import math

import numpy as np
import jax
import jax.numpy as jnp
from jax import lax
import jax.experimental.pallas as pl
import jax.experimental.pallas.tpu as pltpu

BF, F32, U32 = jnp.bfloat16, jnp.float32, jnp.uint32

S, D, H, DH, M, SEG = 2048, 1024, 32, 128, 8, 32
NSEG = S // SEG
NP = H // 2
N1, N2 = 32, 64
QS = S // 4
PITCH = N1 + 8
CLASSES = ((0, 8, 4, 12), (1, 15, 9, 7), (2, 14, 10, 6), (3, 13, 11, 5))
LAG1, LAG2, SPLIT, HOOK_AT = 1, 2, 27, 18
ORDER = "qksvp"
UNROLL = 2
DEADL = 0
ROT = 0
NMF = 1
AVAL = 1
OPQ = 0
DEFER = 0
NEWTON = 1
SPLIT11 = 1
NY0, NY1 = 32, 40
BD, BW, BV, BL = 7, 8, 8, 3
NQ = 2
(SEM_W, SEM_GF, SEM_GI, SEM_SM, SEM_GS, SEM_NYQ, SEM_WO, SEM_MEM, SEM_GW, SEM_OUT, SEM_F, SEM_X,
 SEM_W0) = 0, 6, 7, 8, 9, 10, 11, 12, 13, 14, 15, 19, 23
NSEM = SEM_W0 + 6
RSQ2 = float(np.float32(math.sqrt(0.5)))


def _bfly8(x):
    s = [x[i] + x[i + 4] for i in range(4)]
    d = [x[i] - x[i + 4] for i in range(4)]
    e, f = s[0] + s[2], s[1] + s[3]
    t1, t2 = (d[1] - d[3]) * RSQ2, (d[1] + d[3]) * RSQ2
    return [e + f, e - f, d[0] + t1, t2 + d[2], s[0] - s[2], s[1] - s[3], d[0] - t1, t2 - d[2]]


def _bfly8_t(t):
    e, f = t[0] + t[1], t[0] - t[1]
    s = [e + t[4], f + t[5], e - t[4], f - t[5]]
    t1, t2 = t[2] - t[6], t[3] + t[7]
    d = [t[2] + t[6], (t1 + t2) * RSQ2, t[3] - t[7], (t2 - t1) * RSQ2]
    return [s[i] + d[i] for i in range(4)] + [s[i] - d[i] for i in range(4)]


def _half_pre(vr, vi, lo, roll, where):
    ri = roll(vi)
    return where(lo, vr, ri), where(lo, ri, vr)


def _half_post(g, tp, tm, lo, roll, where):
    if g == 0:
        return tp, tm
    c = float(np.float32(math.cos(math.pi * g / 8)))
    s = float(np.float32(math.sin(math.pi * g / 8)))
    p, r = tp + tm, tp - tm
    rm = roll(where(lo, r, p))
    return where(lo, p, c * rm + s * r), where(lo, rm, c * r - s * rm)


def _cmul_const(v, k, n, sign):
    re, im = v
    k %= n
    if k == 0:
        return re, im
    if 4 * k == n:
        return (-im, re) if sign > 0 else (im, -re)
    if 8 * k == n:
        return (((re - im) * RSQ2, (re + im) * RSQ2) if sign > 0
                else ((re + im) * RSQ2, (im - re) * RSQ2))
    if 8 * k == 3 * n:
        return (((re + im) * -RSQ2, (re - im) * RSQ2) if sign > 0
                else ((im - re) * RSQ2, (re + im) * -RSQ2))
    c, s = math.cos(2 * math.pi * k / n), sign * math.sin(2 * math.pi * k / n)
    return re * c - im * s, re * s + im * c


def _fft(v, sign):
    n = len(v)
    if n == 1:
        return v
    ev, od = _fft(v[0::2], sign), _fft(v[1::2], sign)
    lo, hi = [], []
    for k in range(n // 2):
        er, ei = ev[k]
        if 4 * k == n:
            xr, xi = od[k]
            if sign > 0:
                lo.append((er - xi, ei + xr)); hi.append((er + xi, ei - xr))
            else:
                lo.append((er + xi, ei - xr)); hi.append((er - xi, ei + xr))
            continue
        tr, ti = _cmul_const(od[k], k, n, sign)
        lo.append((er + tr, ei + ti))
        hi.append((er - tr, ei - ti))
    return lo + hi


def _pack_rows(a):
    u = np.ascontiguousarray(a, dtype=np.float32).view(np.uint32)
    b = ((u + 0x7FFF + ((u >> 16) & 1)) >> 16).astype(np.uint32)
    return (b[..., 0::2, :] | (b[..., 1::2, :] << 16)).astype(np.uint32)


def _diag_blocks(full, n, tol):
    k = full.shape[0] // n
    blk = np.kron(np.eye(k), np.ones((n, n)))
    assert np.abs(full * (1 - blk)).max() < tol
    return np.stack([full[n * g:n * g + n, n * g:n * g + n] for g in range(k)])


def _cplx(re, im):
    return np.block([[re, im], [-im, re]])


@functools.lru_cache(maxsize=None)
def _constants():
    k2 = np.stack([np.concatenate([c + 16 * np.arange(32) for c in cls]) for cls in CLASSES])
    n2 = np.arange(D)
    ang = 2 * np.pi * ((k2[:, :, None] * n2[None, None, :]) % D) / D
    rows = np.stack([np.cos(ang), -np.sin(ang)], axis=1)
    wgt = np.where(k2 == 0, 1.0, 2.0)[:, None, :, None]
    fwd = rows.reshape(D, D).T
    inv = (rows * wgt).reshape(D, D) / (S * D)
    bf = np.stack(_bfly8(list(np.eye(8))))
    binv = np.kron(np.linalg.inv(bf), np.eye(128))
    gd = _diag_blocks(binv.T @ fwd, 256, 1e-6)
    gdi = _diag_blocks(inv @ binv, 256, 1e-12)
    eye, lo = np.eye(256), np.arange(128) < 64
    roll = lambda v: np.roll(v, 64, axis=1)
    pre = np.concatenate(_half_pre(eye[:, :128], eye[:, 128:], lo, roll, np.where), axis=1)
    gi = []
    for g in range(4):
        post = np.concatenate(_half_post(g, eye[:, :128], eye[:, 128:], lo, roll, np.where), axis=1)
        gi.append(_diag_blocks(np.linalg.inv(pre) @ gdi[g] @ np.linalg.inv(post), 128, 1e-12))
    gi = np.concatenate(gi)

    b = np.arange(N2)
    k1 = np.arange(N1)[:, None] + N1 * np.arange(N2)[None, :]
    th = 2 * np.pi * ((k1[:, :, None] * b[None, None, :]) % S) / S
    gr, gim = np.cos(th), -np.sin(th)
    full = np.block([[gr, -gim], [gim, gr]])
    kap = np.arange(2 * N2)
    src = ((kap >> 3) & 1) * N2 + (kap >> 4) * 8 + (kap & 7)
    gs = full[:, :, src]
    hr, hi = np.swapaxes(gr, 1, 2), -np.swapaxes(gim, 1, 2)
    gsi = np.block([[hr, -hi], [hi, hr]])

    lane = np.arange(128)
    kb = 8 * (lane % 16) + lane // 16
    t128 = 2 * np.pi * ((lane[:, None] * kb[None, :]) % 128) / 128
    nyf = _cplx(np.cos(t128), -np.sin(t128))
    nyi = _cplx(np.cos(t128).T, np.sin(t128).T)
    i16 = np.arange(16)
    t16 = 2 * np.pi * ((i16[:, None] * i16[None, :]) % 16) / 16
    tw = 2 * np.pi * (i16[:, None] * lane[None, :]) / S
    sm = np.zeros((96, 128), np.float32)
    sm[0:16], sm[16:32] = np.cos(tw), np.sin(tw)
    sm[32:48, :16], sm[48:64, :16] = np.cos(t16), -np.sin(t16)
    sm[64:80, :16], sm[64:80, 16:32] = np.cos(t16), -np.sin(t16)

    gfp = _pack_rows(np.concatenate([gd, nyf[None], nyi[None]]))
    return gfp, _pack_rows(gi), sm, _pack_rows(np.stack([gs, gsi]))


def _mask80():
    r = lax.broadcasted_iota(jnp.int32, (80, 80), 0)
    c = lax.broadcasted_iota(jnp.int32, (80, 80), 1)

    def head(i):
        return jnp.where(i < 64, i >> 5, (i - 64) >> 3)

    def pos(i):
        j = i & 31
        return jnp.where(i < 64, jnp.where(j < M, j, j + 8), M + (i & 7))

    same = head(r) == head(c)
    ok = (pos(r) < M) | (pos(c) <= pos(r))
    return jnp.where(same, jnp.where(ok, 1.0, -1e9), -jnp.inf).astype(F32)


def _as_bf(u):
    return pltpu.bitcast(u, BF)


def _as_u32(b):
    return pltpu.bitcast(b, U32)


def _lo_f32(u):
    return pltpu.bitcast(u << 16, F32)


def _hi_f32(u):
    return pltpu.bitcast(u & jnp.uint32(0xFFFF0000), F32)


def _dot(a, b):
    return jnp.dot(a, b, preferred_element_type=F32)


def _dot_nt(a, b):
    return lax.dot_general(a, b, (((1,), (1,)), ((), ())), preferred_element_type=F32)


def _transpose_u32(u):
    return pltpu.bitcast(pltpu.bitcast(u, F32).T, U32)


def _lanes(rows):
    return lax.broadcasted_iota(jnp.int32, (rows, 128), 1)


def _kernel(x_hbm, mem_hbm, wq_hbm, wk_hbm, wv_hbm, wo_hbm, fr_hbm, fi_hbm, gw_hbm,
            gf_hbm, gi_hbm, sm_hbm, gs_hbm,
            out_hbm,
            x_v, raw, wqkv, wo, st, sl, fraw, fp, gf, gi, gs, y, v_s, out_v, u_s, cb, z_s, p_s,
            sto, obuf, ct, a_s, pa_s, bb_s, g_s, stg, pst, rst, gw_s, mem_ref, mf, sm, xa, nyq, gw_ref, zero_s, sem):
    KH = D // 2
    KQ = KH // NQ
    RB, HB = 128, 16
    raw4 = raw.reshape(6, D, 8, DH)
    w_hbm = (wq_hbm, wk_hbm, wv_hbm)
    f_hbm = (fr_hbm, fi_hbm)

    def w_src(c):
        return w_hbm[c // 2].bitcast(U32).at[:, pl.ds(8 * (c % 2), 8), :]

    def wait(dst, k):
        pltpu.make_async_copy(dst, dst, sem.at[k]).wait()

    def w_half(ref, q, e):
        return ref.at[pl.ds(pl.multiple_of(q * KQ, KQ) + e * KH, KQ)]

    def x_rows(i, a1):
        return pl.ds(pl.multiple_of(i * RB, RB) + QS * a1, RB)

    def f_copies(h):
        return [(f_hbm[a].at[pl.ds(0, D // 2), pl.ds(128 * (4 * h + c), 128)].bitcast(U32),
                 fraw.at[h, a, c], SEM_F + h) for a in range(2) for c in range(4)]

    def w_copy(c):
        return [(w_src(c), raw4.at[c], SEM_W + c)]

    copies = [(gf_hbm.at[0:4], gf.at[0:4], SEM_GF)]
    copies += [(x_hbm.at[x_rows(i, a1), :], x_v.at[x_rows(i, a1), :], SEM_X + i)
               for i in range(QS // RB) for a1 in range(4)]
    for n in range(6):
        copies += [(w_half(w_src(n // 2), n % 2, e), w_half(raw4.at[n // 2], n % 2, e), SEM_W0 + n)
                   for e in range(2)]
        if n >= 2:
            copies += f_copies(n - 2)
    copies += [(sm_hbm, sm, SEM_SM), (gf_hbm.at[4:6], gf.at[4:6], SEM_W)]
    copies += [(f_hbm[a].at[pl.ds(D // 2, 1), :], nyq.at[a], SEM_NYQ) for a in range(2)]
    copies += [(gs_hbm, gs, SEM_GS)] + w_copy(3) + w_copy(4) + w_copy(5)
    copies += [(wo_hbm.bitcast(U32).at[:, pl.ds(128 * j, 128)], wo.at[j], SEM_WO) for j in range(8)]
    copies += [(gi_hbm, gi, SEM_GI), (mem_hbm, mem_ref, SEM_MEM), (gw_hbm, gw_ref.at[pl.ds(0, D)], SEM_GW)]
    for src, dst, k in copies:
        pltpu.make_async_copy(src, dst, sem.at[k]).start()

    def prep_rhs(ch, jj, k0, nk):
        item = 8 * ch + jj
        a1 = raw[ch, pl.ds(k0 * 8 + jj, nk, stride=8), :]
        a2 = raw[ch, pl.ds((KH + k0) * 8 + jj, nk, stride=8), :]
        b11, b12, b21, b22 = _lo_f32(a1), _hi_f32(a1), _lo_f32(a2), _hi_f32(a2)
        for p, e, b in ((0, 0, b11), (1, 0, b12), (0, 1, b21), (1, 1, b22)):
            row = pl.multiple_of(k0 // 2, nk // 2) + e * KH // 2
            wqkv[2 * item + p, pl.ds(row, nk // 2), :] = _as_u32(b.astype(BF))
        return [v.astype(BF) for v in (b11 + b22, b11, b12 - b22, b21 - b11, b22, b11 + b12, b21 + b22)]

    def strassen(rhs, q, item, init, keep, after_dot):
        def prod(i):
            lhs = sl[q, i] if q is not None else jnp.concatenate([sl[k, i] for k in range(NQ)], axis=1)
            return _dot(_as_bf(lhs), rhs[i])

        def plus(i, r):
            return r if init is None else init(i) + r

        c12, c21 = (cb.at[5], cb.at[4]) if keep is None else (keep(1), keep(2))
        m = prod(1)
        cb[0] = m
        after_dot(0, m)
        m = prod(4)
        cb[1] = m
        after_dot(1, m)
        m1 = prod(0)
        cb[3] = plus(3, m1 - cb[0])
        if keep is None or SPLIT11:
            cb[2] = plus(0, m1 - cb[1])
        after_dot(2, m1)
        m = prod(3)
        c21[...] = plus(2, cb[0] + m)
        cb[2] = cb[2] + m if keep is None or SPLIT11 else plus(0, m1 - cb[1]) + m
        after_dot(3, m)
        m = prod(2)
        c12[...] = plus(1, cb[1] + m)
        cb[3] = cb[3] + m
        after_dot(4, m)
        for k, (i, acc) in enumerate(((6, 2), (5, 3))):
            m = prod(i) + cb[acc]
            if keep is not None:
                keep(3 * k)[...] = m
            store_st(item, k, *((m, c12[...]) if k == 0 else (c21[...], m)))
            after_dot(5 + k, m)

    def store_st(item, e, c1, c2):
        r = jnp.concatenate([c.reshape(NSEG // 2, 8, 128) for c in (c1, c2)], axis=1)
        st[item, 256 * e:256 * e + 256, :] = _as_u32(r.reshape(8 * NSEG, 128).astype(BF))

    def pin(i, c):
        if 1:
            cb[i, 0:8, :] = jnp.zeros((8, 128), F32)
        zero_s[i] = 0
        z_s[i, 0:8, :] = jnp.zeros((8, 128), U32)
        p_s[i, 0:8, :] = jnp.zeros((8, 128), F32)
        u_s[i, 0:8, :] = jnp.zeros((8, 128), U32)
        stg[i, 0, 0:8, :] = jnp.zeros((8, 128), U32)
        obuf[i, 0:8, :] = jnp.zeros((8, 128), U32)
        sto[i] = jnp.zeros((8, 128), F32)
        rst[i, 0:8, :] = jnp.zeros((8, 128), F32)
        if 1:
            a_s[i, 0:8, 0:128] = jnp.zeros((8, 128), U32)
        pa_s[i, 0:8, :] = jnp.zeros((8, 128), F32)
        if 0:
            bb_s[pl.ds(pl.multiple_of(8 * i, 8), 8), 0:128] = jnp.zeros((8, 128), F32)
            g_s[pl.ds(pl.multiple_of(8 * i, 8), 8), :] = jnp.zeros((8, 128), F32)
        return c

    lax.fori_loop(0, 2, pin, 0)

    def fill_mask(i, c):
        mf[i, 0:80, :] = _mask80()
        return c

    lax.fori_loop(0, NMF, fill_mask, 0)
    fraw[4] = jnp.zeros(fraw.shape[1:], U32)

    wait(gf.at[0:4], SEM_GF)

    def f1(i, c):
        for a1 in range(4):
            wait(x_v.at[x_rows(i, a1), :], SEM_X + i)
        base = pl.multiple_of(i * RB, RB)
        alt = (1 - 2 * (_lanes(16) & 1)).astype(F32).astype(BF)

        def rows16(r):
            return jnp.concatenate([x_v[pl.ds(r + d, 16), :].astype(F32)[0:8] for d in (0, SEG)], axis=0)

        for r in (0, 64, QS, QS + 64):
            top, bot = rows16(base + r), rows16(base + (r + 2 * QS))
            a11, a12, a21, a22 = top[:, :KH], top[:, KH:], bot[:, :KH], bot[:, KH:]
            row = pl.multiple_of((base + r) // 8, 8)
            for k, v in enumerate((a11 + a22, a21 + a22, a11, a22, a11 + a12, a21 - a11, a12 - a22)):
                for q in range(NQ):
                    sl[q, k, pl.ds(row, 8), :] = _as_u32(v[:, q * KQ:(q + 1) * KQ].astype(BF))
        for h0 in range(0, RB, HB):
            pieces = []
            for a1 in range(4):
                for r in range(h0, h0 + HB, 16):
                    xs = x_v[pl.ds(base + (QS * a1 + r), 16), :].astype(F32)
                    pieces.append(jnp.concatenate(_bfly8([xs[:, 128 * a:128 * a + 128] for a in range(8)]),
                                                  axis=1))
                    z_s[a1, r // 2:r // 2 + 8, :] = _as_u32(pieces[-1][:, :128].astype(BF))
            ub = jnp.concatenate(pieces, axis=0)
            for g in range(4):
                yy = _dot(ub[:, 256 * g:256 * g + 256].astype(BF), _as_bf(gf[g]))
                v = _fft([(yy[HB * a1:HB * a1 + HB, :128], yy[HB * a1:HB * a1 + HB, 128:])
                          for a1 in range(4)], -1)
                for k1 in range(4):
                    rows = pl.ds(base + (QS * k1 + h0), HB)
                    y[g, 0, rows, :] = v[k1][0]
                    y[g, 1, rows, :] = v[k1][1]
                if h0 + HB == RB and g == 3:
                    for a1 in range(4):
                        xa[pl.ds(4 * a1 + i, 1), :] = _dot_nt(alt, _as_bf(z_s[a1]))[0:1]
        return c

    with jax.named_scope("f1"):
        lax.fori_loop(0, QS // RB, f1, 0)

    def fprep(src, h, c):
        ev, od = [], []
        for r in range(8):
            wr = fraw[src, 0, c, pl.ds(r, 32, stride=8), :]
            wi = fraw[src, 1, c, pl.ds(r, 32, stride=8), :]
            ev.append((wr & jnp.uint32(0xFFFF)) | (wi << 16))
            od.append((wr >> 16) | (wi & jnp.uint32(0xFFFF0000)))
        for g, cls in enumerate(CLASSES):
            t = _transpose_u32(jnp.concatenate([(od if k % 2 else ev)[k // 2] for k in cls], axis=0))
            for q in range(128 // N1):
                row = pl.multiple_of(((4 * h + c) * (128 // N1) + q) * PITCH, 8)
                fp[g, pl.ds(row, N1), :] = t[q * N1:(q + 1) * N1]

    def nyquist():
        twc, tws = sm[0:16], sm[16:32]
        u = _dot(sm[32:64, 0:16].astype(BF), xa[0:16, :].astype(BF))
        ur, ui = u[0:16], u[16:32]
        u = jnp.concatenate([ur * twc + ui * tws, ui * twc - ur * tws], axis=1).astype(BF)
        yield
        xx = _dot(u, _as_bf(gf[4]))
        xr, xi = xx[:, :128], xx[:, 128:]
        w = (pltpu.bitcast(nyq[0].astype(F32), U32) >> 16) | pltpu.bitcast(nyq[1].astype(F32), U32)
        w = jnp.concatenate([w[:, 128 * a:128 * a + 128] for a in range(16)], axis=0)
        wt = _transpose_u32(jnp.concatenate([w] * 8, axis=0))
        blk = _lanes(16) >> 4
        wm = wt[0:16]
        for j in range(1, 8):
            wm = jnp.where(blk == j, wt[16 * j:16 * j + 16], wm)
        wr, wi = _lo_f32(wm), _hi_f32(wm)
        z = jnp.concatenate([xr * wr - xi * wi, xr * wi + xi * wr], axis=1).astype(BF)
        yield
        pp = _dot(z, _as_bf(gf[5]))
        pr, pi = pp[:, :128], pp[:, 128:]
        pp = jnp.concatenate([pr * twc - pi * tws, pi * twc + pr * tws], axis=0).astype(BF)
        yield
        cc = _dot(sm[64:80, 0:32].astype(BF), pp) * (1.0 / (S * D))
        ct[...] = jnp.concatenate([cc, jnp.zeros((112, 128), F32)], axis=0).T
        yield

    def s_rows(k1, a0, r):
        return pl.ds(r + (QS * k1 + N2 * a0), 8)

    def anchored(v, tok, inst=0):
        return jnp.where(zero_s[inst] != 0, tok, v)

    def s_prep(g, k1, r, tok):
        v = [(y[g, 0, s_rows(k1, a0, r), :], y[g, 1, s_rows(k1, a0, r), :]) for a0 in range(8)]
        if tok is not None:
            v[0] = (anchored(v[0][0], tok), v[0][1])
        v = _fft([_cmul_const(v[a0], a0 * k1, N1, -1) for a0 in range(8)], -1)
        for k0 in range(8):
            u_s[k1 + 4 * k0, pl.ds(r, 8), :] = _as_u32(jnp.concatenate(v[k0], axis=0).astype(BF))

    def s_fwd(g, ka, tok):
        xx = _dot(_as_bf(gs[0, ka]), _as_bf(u_s[ka]))
        w32 = fp[g, pl.ds(ka, N2, stride=PITCH), :]
        wr, wi = _lo_f32(w32), _hi_f32(w32)
        xr, xi = xx[:N2], xx[N2:]
        z_s[ka] = _as_u32(jnp.concatenate([xr * wr - xi * wi, xr * wi + xi * wr], axis=0).astype(BF))

    def s_inv(ka, tok):
        p_s[ka] = _dot(_as_bf(gs[1, ka]), _as_bf(z_s[ka]))

    def s_post(g, k1, r, tok):
        v = [(p_s[k1 + 4 * k0, r:r + 8, :], p_s[k1 + 4 * k0, N2 + r:N2 + r + 8, :]) for k0 in range(8)]
        v[0] = (anchored(v[0][0], tok), anchored(v[0][1], tok))
        v = _fft(v, 1)
        for a0 in range(8):
            vr, vi = _cmul_const(v[a0], a0 * k1, N1, 1)
            v_s[g, 0, s_rows(k1, a0, r), :] = vr
            v_s[g, 1, s_rows(k1, a0, r), :] = vi

    def bulk(where, n, events, q=None):
        k0, nk = (0, KH) if q is None else (pl.multiple_of(q * KQ, KQ), KQ)
        for i in range(n):
            ch, jj = where(i)

            def hook(k, m):
                pieces = events.get(7 * i + k, ())
                vec = [pc for pc in pieces if isinstance(pc, P) and pc.func in (s_prep, s_post)]
                for piece in pieces:
                    r = 8 * ((32 * vec.index(piece)) // len(vec)) if piece in vec else 0
                    piece(m[r:r + 8])

            def keep(k):
                return v_s.at[jj // 4, (jj // 2) % 2, pl.ds(1024 * (jj % 2) + 256 * k, 256), :]

            def init(k):
                return jnp.where(q > 0, keep(k)[...], 0.0)

            strassen(prep_rhs(ch, jj, k0, nk), q, 8 * ch + jj,
                     None if q is None else init, None if q is None else keep, hook)

    def spread(events, pieces, q0, q1):
        for i, piece in enumerate(pieces):
            events.setdefault(q0 + ((q1 - q0) * i) // len(pieces), []).append(piece)

    P = functools.partial

    def loop_a(n, c):
        for e in range(2):
            wait(w_half(raw4.at[n // 2], n % 2, e), SEM_W0 + n)
        h = jnp.maximum(n - 2, 0)

        @pl.when(n >= 2)
        def _():
            wait(fraw.at[h], SEM_F + h)

        src = jnp.where(n >= 2, h, 4)
        events = {}
        spread(events, [lambda tok, c=c: fprep(src, h, c) for c in range(4)], 0, 48)
        bulk(lambda i: (n // 2, i), 8, events, n % 2)
        return c

    def loop_b(g, c):
        @pl.when(g < 3)
        def _():
            wait(raw4.at[3 + g], SEM_W + 3 + g)

        gn = jnp.minimum(g + 1, 3)
        events = {}
        for k1 in range(4):
            q = BD * k1
            spread(events, [P(s_fwd, g, k1 + 4 * k0) for k0 in range(8)], q, q + BW)
            spread(events, [P(s_prep, gn, k1, r) for r in range(0, N2, 8)], q + BW, q + BW + BV)
            q += BL
            spread(events, [P(s_inv, k1 + 4 * k0) for k0 in range(8)], q, q + BW)
            spread(events, [P(s_post, g, k1, r) for r in range(0, N2, 8)], q + BW, q + BW + BV)
        ny = nyquist()
        spread(events, [lambda tok: next(ny)] * 4, NY0, NY1)
        assert max(events) < 41
        bulk(lambda i: ((24 + 6 * g + i) // 8, (24 + 6 * g + i) % 8), 6, events)
        return c

    def prep0(i, c):
        for k1 in range(4):
            s_prep(0, k1, pl.multiple_of(i * 8, 8), None)
        return c

    lax.fori_loop(0, N2 // 8, prep0, 0)
    with jax.named_scope("loop_a"):
        lax.fori_loop(0, 6, loop_a, 0)
    wait(sm, SEM_SM)
    wait(gf.at[4:6], SEM_W)
    wait(nyq, SEM_NYQ)
    wait(gs, SEM_GS)
    with jax.named_scope("loop_b"):
        lax.fori_loop(0, 4, loop_b, 0)
    wait(wo, SEM_WO)
    wait(gi, SEM_GI)
    wait(mem_ref, SEM_MEM)
    wait(gw_ref.at[pl.ds(0, D)], SEM_GW)

    scale = DH ** -0.5

    for i in range(UNROLL):
        gw_s[i] = jnp.broadcast_to(gw_ref[pl.ds(0, D)].astype(F32).reshape(1, D), (8, D))

    uses = itertools.count()

    def softmax(s):
        fill = mf[next(uses) % NMF, 0:80, :]
        s = jnp.where(fill > 0.0, s * scale, fill)
        m = jnp.max(s, axis=-1, keepdims=True)
        e = jnp.exp(s - m)
        l = jnp.sum(e, axis=-1, keepdims=True)
        if NEWTON:
            r = pl.reciprocal(l, approx=True)
            r = r * (2.0 - l * r)
        else:
            r = 1.0 / l
        return e, r

    def lhs_rows(mem, seg):
        xs = x_v[pl.ds(pl.multiple_of(seg * SEG, SEG), SEG), :].astype(F32)
        return jnp.concatenate([mem, xs[8:SEG]], axis=0).astype(BF)

    def proj2(a, m, j):
        return jnp.concatenate([_dot(_as_bf(a[...]), _as_bf(wqkv[H * m + 2 * j + p])).astype(BF)
                                for p in range(2)], axis=0)

    def proj_lo(a):
        for i in range(6):
            pa_s[i] = _dot(_as_bf(a[:, :KH]), _as_bf(wqkv[H * (i // 2) + i % 2, 0:KH // 2, :]))

    def proj_hi(a):
        full = [(_dot(_as_bf(a[:, KH:]), _as_bf(wqkv[H * (i // 2) + i % 2, KH // 2:KH, :]))
                 + pa_s[i]).astype(BF) for i in range(6)]
        for m in range(3):
            stg[m, 0] = _as_u32(jnp.concatenate(full[2 * m:2 * m + 2], axis=0))

    def step(a, seg, first, hook=None, inst=0):
        R = 32 if first else 48
        srow = pl.multiple_of(seg * 8, 8)
        if AVAL:
            a = a[...]

        def get(m, j):
            return _as_bf(jnp.concatenate([stg[m, j % 8], st[NP * m + j, pl.ds(srow, 8), :]], axis=0))

        def proj(j, m):
            if j > 0:
                stg[m, j % 8] = _as_u32(proj2(a, m, j))
            elif m == 0:
                if not first:
                    proj_lo(a)
                if not (first and ROT):
                    proj_hi(a)

        def scores(j):
            e, r = softmax(_dot_nt(get(0, j), get(1, j)))
            if DEFER:
                pst[j % 8] = _as_u32(e.astype(BF))
                rst[j % 8, 0:80, :] = jnp.broadcast_to(r, (80, 128))
            else:
                pst[j % 8] = _as_u32((e * r).astype(BF))

        def pv(j):
            o = _dot(_as_bf(pst[j % 8]), get(2, j))
            if DEFER:
                o = o * rst[j % 8, 0:80, :]
            for i in range(2):
                h = 2 * j + i
                if first:
                    ob = o[32 * i:32 * i + 32]
                    sto[h] = o[64 + 8 * i:72 + 8 * i]
                else:
                    ob = jnp.concatenate([o[32 * i:32 * i + 32], o[64 + 8 * i:72 + 8 * i], sto[h]], axis=0)
                obuf[h, 0:R // 2, :] = _as_u32(ob.astype(BF))

        def wo_part(j, h0, h1):
            og = jnp.concatenate([_as_bf(obuf[h, 0:R // 2, :]) for h in range(h0, h1)], axis=1)
            return _dot(og, _as_bf(wo[j, h0 * 64:h1 * 64, :]))

        parts = []
        for i in range(NP + 4):
            for ch in ORDER:
                if ch in "qkv":
                    m = "qkv".index(ch)
                    if i < NP:
                        proj(i, m)
                    elif m < 2:
                        parts.append(wo_part(2 * (i - NP) + len(parts) % 2, 0, SPLIT))
                elif ch == "s" and 0 <= i - LAG1 < NP:
                    scores(i - LAG1)
                elif ch == "p" and 0 <= i - LAG2 < NP:
                    pv(i - LAG2)
            if hook is not None and i == HOOK_AT:
                tok = hook()
        if hook is not None and DEADL:
            parts = [jnp.concatenate([anchored(p[0:8], tok[:, 128 * j:128 * j + 128], inst), p[8:]], axis=0)
                     for j, p in enumerate(parts)]
        return jnp.concatenate([wo_part(j, SPLIT, H) + parts[j] for j in range(8)], axis=1)

    def start_pair(mem, t):
        a = a_s.at[0]
        a_s[zero_s[1] if OPQ else 0] = _as_u32(lhs_rows(mem, 2 * t))
        proj_lo(a)
        if ROT:
            proj_hi(a)

    def pair(t, inst):
        base = pl.multiple_of(t * 64, 64)
        lane = _lanes(64) + zero_s[inst]
        lo = lane < 64
        roll = lambda v: pltpu.roll(v, 64, 1)
        a1 = t // 8
        off = pl.multiple_of((t % 8) * 64, 64)
        s2 = (1 - 2 * (a1 & 1)).astype(F32)
        sg = (1 - (a1 & 2)).astype(F32)
        cc, ss = sg * (1 - (a1 & 1)).astype(F32), sg * (a1 & 1).astype(F32)

        def irfft_group(g):
            q = [[v_s[g, e, pl.ds(off + QS * k1, 64), :] for e in range(2)] for k1 in range(4)]
            br, bi = q[1][0] + s2 * q[3][0], q[1][1] + s2 * q[3][1]
            vr = q[0][0] + s2 * q[2][0] + (cc * br - ss * bi)
            vi = q[0][1] + s2 * q[2][1] + (cc * bi + ss * br)
            tin = _half_pre(vr, vi, lo, roll, jnp.where)
            tp, tm = [_dot(tin[e].astype(BF), _as_bf(gi[2 * g + e])) for e in range(2)]
            if g == 0:
                nyc = jnp.sum(jnp.where(lane == t // 2,
                                        ct[pl.ds(pl.multiple_of((t % 2) * 64, 64), 64), :], 0.0),
                              axis=-1, keepdims=True)
                tp = tp + nyc * (1 - 2 * (lane & 1)).astype(F32)
            return list(_half_post(g, tp, tm, lo, roll, jnp.where))

        def spectral_part():
            ts = sum([irfft_group(g) for g in range(4)], [])
            b = jnp.concatenate(_bfly8_t(ts), axis=1).astype(BF).astype(F32)
            xs = x_v[pl.ds(base, 64), :].astype(F32)
            gate = jax.nn.sigmoid(jnp.sum(xs * jnp.concatenate([gw_s[inst]] * 8, axis=0), axis=-1, keepdims=True))
            bb = (1.0 - gate) * b
            bb_s[...] = jnp.concatenate([bb[0:8], bb[8:32] + gate[8:32] * bb_s[8:32], bb[32:64]], axis=0)
            g_s[...] = jnp.broadcast_to(gate, (64, 128))
            return functools.reduce(jnp.maximum, [bb[r:r + 8] for r in range(0, 64, 8)])

        res_a = step(a_s.at[0], 2 * t, True)
        bb_s[8:32] = res_a[8:32]
        a_s[zero_s[1] + 1 if OPQ else 1] = _as_u32(lhs_rows(res_a[0:8], 2 * t + 1))
        res_b = step(a_s.at[1], 2 * t + 1, False, spectral_part, inst)

        def gated(r0, r1, res):
            return bb_s[r0:r1] + jnp.concatenate([g_s[r0:r1]] * 8, axis=1) * res

        out_v[pl.ds(base, 64), :] = jnp.concatenate(
            [gated(0, 8, res_b[40:48]), bb_s[8:32], gated(32, 40, res_b[32:40]), gated(40, 64, res_b[8:32])],
            axis=0).astype(BF)
        start_pair(res_b[0:8], jnp.minimum(t + 1, S // 64 - 1))

    def pairs(u, c):
        for i in range(UNROLL):
            pair(UNROLL * u + i, i)
        rows = pl.ds(pl.multiple_of(u * (64 * UNROLL), 64), 64 * UNROLL)
        pltpu.make_async_copy(out_v.at[rows, :], out_hbm.at[rows, :], sem.at[SEM_OUT]).start()
        return c

    with jax.named_scope("chain"):
        start_pair(mem_ref[...].astype(F32), 0)
        lax.fori_loop(0, S // (64 * UNROLL), pairs, 0)
    pltpu.make_async_copy(out_v, out_hbm, sem.at[SEM_OUT]).wait()


@jax.jit
def pallas_gated_mix__memory_aug_recurrent_mem_tr__spectral_gfnet__prompt_kernel(
    A_x, A_mem0, A_Wq, A_Wk, A_Wv, A_Wo, A_seg_len, B_x, B_w_r, B_w_i, gate_w,
):
    assert A_x.shape == (1, S, D) and A_mem0.shape == (1, M, D) and A_Wq.shape == (D, H, DH)
    consts = [jnp.asarray(c) for c in _constants()]
    any_spec = pl.BlockSpec(memory_space=pl.ANY)
    out = pl.pallas_call(
        _kernel,
        out_shape=jax.ShapeDtypeStruct((S, D), BF),
        in_specs=[any_spec] * 13,
        out_specs=any_spec,
        scratch_shapes=[
            pltpu.VMEM((S, D), BF),
            pltpu.VMEM((6, D * 8, DH), U32),
            pltpu.VMEM((3 * H, D // 2, DH), U32),
            pltpu.VMEM((8, H * DH // 2, 128), U32),
            pltpu.VMEM((3 * NP, 8 * NSEG, 128), U32),
            pltpu.VMEM((NQ, 7, 2 * NSEG, D // 2 // NQ), U32),
            pltpu.VMEM((5, 2, 4, 256, 128), U32),
            pltpu.VMEM((4, N2 * PITCH, 128), U32),
            pltpu.VMEM((6, 128, 256), U32),
            pltpu.VMEM((8, 64, 128), U32),
            pltpu.VMEM((2, N1, N2, 2 * N2), U32),
            pltpu.VMEM((4, 2, S, 128), F32),
            pltpu.VMEM((4, 2, S, 128), F32),
            pltpu.VMEM((S, D), BF),
            pltpu.VMEM((N1, N2, 128), U32),
            pltpu.VMEM((6, 256, 128), F32),
            pltpu.VMEM((N1, N2, 128), U32),
            pltpu.VMEM((N1, 2 * N2, 128), F32),
            pltpu.VMEM((H, 8, 128), F32),
            pltpu.VMEM((H, 24, 128), U32),
            pltpu.VMEM((128, 128), F32),
            pltpu.VMEM((2, 16, D), U32),
            pltpu.VMEM((6, 32, 128), F32),
            pltpu.VMEM((64, D), F32),
            pltpu.VMEM((64, 128), F32),
            pltpu.VMEM((3, 8, 32, 128), U32),
            pltpu.VMEM((8, 40, 80), U32),
            pltpu.VMEM((8, 96, 128), F32),
            pltpu.VMEM((UNROLL, 8, D), F32),
            pltpu.VMEM((M, D), BF),
            pltpu.VMEM((NMF, 96, 80), F32),
            pltpu.VMEM((96, 128), F32),
            pltpu.VMEM((32, 128), F32),
            pltpu.VMEM((2, 1, S), BF),
            pltpu.VMEM((8 * D,), BF),
            pltpu.SMEM((2,), jnp.int32),
            pltpu.SemaphoreType.DMA((NSEM,)),
        ],
        compiler_params=pltpu.CompilerParams(vmem_limit_bytes=120 * 1024 * 1024),
    )(
        A_x.reshape(S, D), A_mem0.reshape(M, D), A_Wq, A_Wk, A_Wv,
        A_Wo.reshape(H * DH, D), B_w_r.T, B_w_i.T, gate_w, *consts,
    )
    return out.reshape(1, S, D)
```

```python
import functools
import itertools
import math

import numpy as np
import jax
import jax.numpy as jnp
from jax import lax
import jax.experimental.pallas as pl
import jax.experimental.pallas.tpu as pltpu

BF, F32, U32 = jnp.bfloat16, jnp.float32, jnp.uint32

S, D, H, DH, M, SEG = 2048, 1024, 32, 128, 8, 32
NSEG = S // SEG
NP = H // 2
N1, N2 = 32, 64
QS = S // 4
PITCH = N1 + 8
CLASSES = ((0, 8, 4, 12), (1, 15, 9, 7), (2, 14, 10, 6), (3, 13, 11, 5))
LAG1, LAG2, SPLIT, HOOK_AT = 1, 2, 27, 18
ORDER = "qksvp"
NMF = 1
WSP, W0, W1 = 2, 0, 40
SP3, NSP = 13, 4
HOOKS = ((1, 18), (3, 18), (2, 18), (0, 18))
NEWTON = 1
SPLIT11 = 1
NY0, NY1 = 32, 40
BD, BW, BV, BL = 7, 8, 8, 3
NQ = 2
(SEM_W, SEM_GF, SEM_GI, SEM_SM, SEM_GS, SEM_NYQ, SEM_NYM, SEM_MEM, SEM_GW, SEM_OUT, SEM_F, SEM_X,
 SEM_W0) = 0, 6, 7, 8, 9, 10, 11, 12, 13, 14, 15, 19, 23
SEM_WO = SEM_W0 + 6
NSEM = SEM_WO + 4
RSQ2 = float(np.float32(math.sqrt(0.5)))


def _bfly8(x):
    s = [x[i] + x[i + 4] for i in range(4)]
    d = [x[i] - x[i + 4] for i in range(4)]
    e, f = s[0] + s[2], s[1] + s[3]
    t1, t2 = (d[1] - d[3]) * RSQ2, (d[1] + d[3]) * RSQ2
    return [e + f, e - f, d[0] + t1, t2 + d[2], s[0] - s[2], s[1] - s[3], d[0] - t1, t2 - d[2]]


def _bfly8_t(t):
    e, f = t[0] + t[1], t[0] - t[1]
    s = [e + t[4], f + t[5], e - t[4], f - t[5]]
    t1, t2 = t[2] - t[6], t[3] + t[7]
    d = [t[2] + t[6], (t1 + t2) * RSQ2, t[3] - t[7], (t2 - t1) * RSQ2]
    return [s[i] + d[i] for i in range(4)] + [s[i] - d[i] for i in range(4)]


def _half_pre(vr, vi, lo, roll, where):
    ri = roll(vi)
    return where(lo, vr, ri), where(lo, ri, vr)


def _half_post(g, tp, tm, lo, roll, where):
    if g == 0:
        return tp, tm
    c = float(np.float32(math.cos(math.pi * g / 8)))
    s = float(np.float32(math.sin(math.pi * g / 8)))
    p, r = tp + tm, tp - tm
    rm = roll(where(lo, r, p))
    return where(lo, p, c * rm + s * r), where(lo, rm, c * r - s * rm)


def _cmul_const(v, k, n, sign):
    re, im = v
    k %= n
    if k == 0:
        return re, im
    if 4 * k == n:
        return (-im, re) if sign > 0 else (im, -re)
    if 8 * k == n:
        return (((re - im) * RSQ2, (re + im) * RSQ2) if sign > 0
                else ((re + im) * RSQ2, (im - re) * RSQ2))
    if 8 * k == 3 * n:
        return (((re + im) * -RSQ2, (re - im) * RSQ2) if sign > 0
                else ((im - re) * RSQ2, (re + im) * -RSQ2))
    c, s = math.cos(2 * math.pi * k / n), sign * math.sin(2 * math.pi * k / n)
    return re * c - im * s, re * s + im * c


def _fft(v, sign):
    n = len(v)
    if n == 1:
        return v
    ev, od = _fft(v[0::2], sign), _fft(v[1::2], sign)
    lo, hi = [], []
    for k in range(n // 2):
        er, ei = ev[k]
        if 4 * k == n:
            xr, xi = od[k]
            if sign > 0:
                lo.append((er - xi, ei + xr)); hi.append((er + xi, ei - xr))
            else:
                lo.append((er + xi, ei - xr)); hi.append((er - xi, ei + xr))
            continue
        tr, ti = _cmul_const(od[k], k, n, sign)
        lo.append((er + tr, ei + ti))
        hi.append((er - tr, ei - ti))
    return lo + hi


def _pack_rows(a):
    u = np.ascontiguousarray(a, dtype=np.float32).view(np.uint32)
    b = ((u + 0x7FFF + ((u >> 16) & 1)) >> 16).astype(np.uint32)
    return (b[..., 0::2, :] | (b[..., 1::2, :] << 16)).astype(np.uint32)


def _diag_blocks(full, n, tol):
    k = full.shape[0] // n
    blk = np.kron(np.eye(k), np.ones((n, n)))
    assert np.abs(full * (1 - blk)).max() < tol
    return np.stack([full[n * g:n * g + n, n * g:n * g + n] for g in range(k)])


def _cplx(re, im):
    return np.block([[re, im], [-im, re]])


@functools.lru_cache(maxsize=None)
def _constants():
    k2 = np.stack([np.concatenate([c + 16 * np.arange(32) for c in cls]) for cls in CLASSES])
    n2 = np.arange(D)
    ang = 2 * np.pi * ((k2[:, :, None] * n2[None, None, :]) % D) / D
    rows = np.stack([np.cos(ang), -np.sin(ang)], axis=1)
    wgt = np.where(k2 == 0, 1.0, 2.0)[:, None, :, None]
    fwd = rows.reshape(D, D).T
    inv = (rows * wgt).reshape(D, D) / (S * D)
    bf = np.stack(_bfly8(list(np.eye(8))))
    binv = np.kron(np.linalg.inv(bf), np.eye(128))
    gd = _diag_blocks(binv.T @ fwd, 256, 1e-6)
    gdi = _diag_blocks(inv @ binv, 256, 1e-12)
    eye, lo = np.eye(256), np.arange(128) < 64
    roll = lambda v: np.roll(v, 64, axis=1)
    pre = np.concatenate(_half_pre(eye[:, :128], eye[:, 128:], lo, roll, np.where), axis=1)
    gi = []
    for g in range(4):
        post = np.concatenate(_half_post(g, eye[:, :128], eye[:, 128:], lo, roll, np.where), axis=1)
        gi.append(_diag_blocks(np.linalg.inv(pre) @ gdi[g] @ np.linalg.inv(post), 128, 1e-12))
    gi = np.concatenate(gi)

    b = np.arange(N2)
    k1 = np.arange(N1)[:, None] + N1 * np.arange(N2)[None, :]
    th = 2 * np.pi * ((k1[:, :, None] * b[None, None, :]) % S) / S
    gr, gim = np.cos(th), -np.sin(th)
    full = np.block([[gr, -gim], [gim, gr]])
    kap = np.arange(2 * N2)
    src = ((kap >> 3) & 1) * N2 + (kap >> 4) * 8 + (kap & 7)
    gs = full[:, :, src]
    hr, hi = np.swapaxes(gr, 1, 2), -np.swapaxes(gim, 1, 2)
    gsi = np.block([[hr, -hi], [hi, hr]])

    lane = np.arange(128)
    kb = 8 * (lane % 16) + lane // 16
    t128 = 2 * np.pi * ((lane[:, None] * kb[None, :]) % 128) / 128
    nyf = _cplx(np.cos(t128), -np.sin(t128))
    nyi = _cplx(np.cos(t128).T, np.sin(t128).T)
    i16 = np.arange(16)
    t16 = 2 * np.pi * ((i16[:, None] * i16[None, :]) % 16) / 16
    tw = 2 * np.pi * (i16[:, None] * lane[None, :]) / S
    sm = np.zeros((96, 128), np.float32)
    sm[0:16], sm[16:32] = np.cos(tw), np.sin(tw)
    sm[32:48, :16], sm[48:64, :16] = np.cos(t16), -np.sin(t16)
    sm[64:80, :16], sm[64:80, 16:32] = np.cos(t16), -np.sin(t16)

    gfp = _pack_rows(np.concatenate([gd, nyf[None], nyi[None]]))
    return gfp, _pack_rows(gi), sm, _pack_rows(np.stack([gs, gsi]))


def _mask80():
    r = lax.broadcasted_iota(jnp.int32, (80, 80), 0)
    c = lax.broadcasted_iota(jnp.int32, (80, 80), 1)

    def head(i):
        return jnp.where(i < 64, i >> 5, (i - 64) >> 3)

    def pos(i):
        j = i & 31
        return jnp.where(i < 64, jnp.where(j < M, j, j + 8), M + (i & 7))

    same = head(r) == head(c)
    ok = (pos(r) < M) | (pos(c) <= pos(r))
    return jnp.where(same, jnp.where(ok, 1.0, -1e9), -jnp.inf).astype(F32)


def _as_bf(u):
    return pltpu.bitcast(u, BF)


def _as_u32(b):
    return pltpu.bitcast(b, U32)


def _lo_f32(u):
    return pltpu.bitcast(u << 16, F32)


def _hi_f32(u):
    return pltpu.bitcast(u & jnp.uint32(0xFFFF0000), F32)


def _dot(a, b):
    return jnp.dot(a, b, preferred_element_type=F32)


def _dot_nt(a, b):
    return lax.dot_general(a, b, (((1,), (1,)), ((), ())), preferred_element_type=F32)


def _transpose_u32(u):
    return pltpu.bitcast(pltpu.bitcast(u, F32).T, U32)


def _lanes(rows):
    return lax.broadcasted_iota(jnp.int32, (rows, 128), 1)


def _kernel(x_hbm, mem_hbm, wq_hbm, wk_hbm, wv_hbm, wo_hbm, fr_hbm, fi_hbm, gw_hbm,
            gf_hbm, gi_hbm, sm_hbm, gs_hbm,
            out_hbm,
            x_v, raw_a, raw_b, wqkv, wo, st, sl, fraw, fp, gf, gi, gs, y, v_s, out_v, u_s, cb, z_s, p_s,
            sto, obuf, ct, a_s, pa_s, bb_s, g_s, stg, pst, ra_s, lc, gw_s, mem_ref, mf, sm, xa, nyq, gw_ref, zero_s, sem):
    KH = D // 2
    KQ = KH // NQ
    RB, HB = 128, 16
    raw4 = [r.reshape(3, D, 8, DH) for r in (raw_a, raw_b)]
    w_hbm = (wq_hbm, wk_hbm, wv_hbm)
    f_hbm = (fr_hbm, fi_hbm)

    def w_src(c):
        return w_hbm[c // 2].bitcast(U32).at[:, pl.ds(8 * (c % 2), 8), :]

    def wait(dst, k):
        pltpu.make_async_copy(dst, dst, sem.at[k]).wait()

    def w_half(ref, q, e):
        return ref.at[pl.ds(pl.multiple_of(q * KQ, KQ) + e * KH, KQ)]

    def x_rows(i, a1):
        return pl.ds(pl.multiple_of(i * RB, RB) + QS * a1, RB)

    def f_copies(h):
        return [(f_hbm[a].at[pl.ds(0, D // 2), pl.ds(128 * (4 * h + c), 128)].bitcast(U32),
                 fraw.at[h, a, c], SEM_F + h) for a in range(2) for c in range(4)]

    def w_copy(c):
        return [(w_src(c), raw4[1].at[c - 3], SEM_W + c)]

    copies = [(gf_hbm.at[0:4], gf.at[0:4], SEM_GF)]
    copies += [(x_hbm.at[x_rows(i, a1), :], x_v.at[x_rows(i, a1), :], SEM_X + i)
               for i in range(QS // RB) for a1 in range(4)]
    for n in range(6):
        copies += [(w_half(w_src(n // 2), n % 2, e), w_half(raw4[0].at[n // 2], n % 2, e), SEM_W0 + n)
                   for e in range(2)]
        if n >= 2:
            copies += f_copies(n - 2)
    copies += [(sm_hbm, sm, SEM_SM), (gf_hbm.at[4:6], gf.at[4:6], SEM_NYM)]
    copies += [(f_hbm[a].at[pl.ds(D // 2, 1), :], nyq.at[a], SEM_NYQ) for a in range(2)]
    copies += [(gs_hbm, gs, SEM_GS)]
    for g in range(4):
        copies += w_copy(3 + g) if g < 3 else []
        copies += [(wo_hbm.bitcast(U32).at[:, pl.ds(128 * j, 128)], wo.at[j], SEM_WO + g) for j in (g, g + 4)]
    copies += [(gi_hbm, gi, SEM_GI), (mem_hbm, mem_ref, SEM_MEM), (gw_hbm, gw_ref.at[pl.ds(0, D)], SEM_GW)]
    for src, dst, k in copies:
        pltpu.make_async_copy(src, dst, sem.at[k]).start()

    def prep_rhs(raw, ch, jj, k0, nk):
        item = 8 * ch + jj
        a1 = raw[pl.ds(k0 * 8 + jj, nk, stride=8), :]
        a2 = raw[pl.ds((KH + k0) * 8 + jj, nk, stride=8), :]
        b11, b12, b21, b22 = _lo_f32(a1), _hi_f32(a1), _lo_f32(a2), _hi_f32(a2)
        for p, e, b in ((0, 0, b11), (1, 0, b12), (0, 1, b21), (1, 1, b22)):
            row = pl.multiple_of(k0 // 2, nk // 2) + e * KH // 2
            wqkv[2 * item + p, pl.ds(row, nk // 2), :] = _as_u32(b.astype(BF))
        return [v.astype(BF) for v in (b11 + b22, b11, b12 - b22, b21 - b11, b22, b11 + b12, b21 + b22)]

    def strassen(rhs, q, item, init, keep, after_dot):
        def prod(i):
            lhs = sl[q, i] if q is not None else jnp.concatenate([sl[k, i] for k in range(NQ)], axis=1)
            return _dot(_as_bf(lhs), rhs[i])

        def plus(i, r):
            return r if init is None else init(i) + r

        c12, c21 = (cb.at[5], cb.at[4]) if keep is None else (keep(1), keep(2))
        m = prod(1)
        cb[0] = m
        after_dot(0, m)
        m = prod(4)
        cb[1] = m
        after_dot(1, m)
        m1 = prod(0)
        cb[3] = plus(3, m1 - cb[0])
        if keep is None or SPLIT11:
            cb[2] = plus(0, m1 - cb[1])
        after_dot(2, m1)
        m = prod(3)
        c21[...] = plus(2, cb[0] + m)
        cb[2] = cb[2] + m if keep is None or SPLIT11 else plus(0, m1 - cb[1]) + m
        after_dot(3, m)
        m = prod(2)
        c12[...] = plus(1, cb[1] + m)
        cb[3] = cb[3] + m
        after_dot(4, m)
        for k, (i, acc) in enumerate(((6, 2), (5, 3))):
            m = prod(i) + cb[acc]
            if keep is not None:
                keep(3 * k)[...] = m
            store_st(item, k, *((m, c12[...]) if k == 0 else (c21[...], m)))
            after_dot(5 + k, m)

    def store_st(item, e, c1, c2):
        r = jnp.concatenate([c.reshape(NSEG // 2, 8, 128) for c in (c1, c2)], axis=1)
        st[item, 256 * e:256 * e + 256, :] = _as_u32(r.reshape(8 * NSEG, 128).astype(BF))

    def pin(i, c):
        if 1:
            cb[i, 0:8, :] = jnp.zeros((8, 128), F32)
        zero_s[i] = 0
        z_s[i, 0:8, :] = jnp.zeros((8, 128), U32)
        p_s[i, 0:8, :] = jnp.zeros((8, 128), F32)
        u_s[i, 0:8, :] = jnp.zeros((8, 128), U32)
        stg[i, 0, 0:8, :] = jnp.zeros((8, 128), U32)
        obuf[i, 0:8, :] = jnp.zeros((8, 128), U32)
        sto[i, 0:8, :] = jnp.zeros((8, 128), F32)
        lc[i, 0, 0:8, :] = jnp.zeros((8, 128), U32)
        if 1:
            ra_s[pl.ds(pl.multiple_of(8 * i, 8), 8), 0:128] = jnp.zeros((8, 128), F32)
        if 1:
            a_s[i, 0:8, 0:128] = jnp.zeros((8, 128), U32)
        pa_s[i, 0:8, :] = jnp.zeros((8, 128), F32)
        if 0:
            bb_s[pl.ds(pl.multiple_of(8 * i, 8), 8), 0:128] = jnp.zeros((8, 128), F32)
            g_s[pl.ds(pl.multiple_of(8 * i, 8), 8), :] = jnp.zeros((8, 128), F32)
        return c

    lax.fori_loop(0, 2, pin, 0)

    def fill_mask(i, c):
        mf[i, 0:80, :] = _mask80()
        return c

    lax.fori_loop(0, NMF, fill_mask, 0)
    fraw[4] = jnp.zeros(fraw.shape[1:], U32)

    wait(gf.at[0:4], SEM_GF)

    def f1(i, c):
        for a1 in range(4):
            wait(x_v.at[x_rows(i, a1), :], SEM_X + i)
        base = pl.multiple_of(i * RB, RB)
        alt = (1 - 2 * (_lanes(16) & 1)).astype(F32).astype(BF)

        def rows16(r):
            return jnp.concatenate([x_v[pl.ds(r + d, 16), :].astype(F32)[0:8] for d in (0, SEG)], axis=0)

        for r in (0, 64, QS, QS + 64):
            top, bot = rows16(base + r), rows16(base + (r + 2 * QS))
            a11, a12, a21, a22 = top[:, :KH], top[:, KH:], bot[:, :KH], bot[:, KH:]
            row = pl.multiple_of((base + r) // 8, 8)
            for k, v in enumerate((a11 + a22, a21 + a22, a11, a22, a11 + a12, a21 - a11, a12 - a22)):
                for q in range(NQ):
                    sl[q, k, pl.ds(row, 8), :] = _as_u32(v[:, q * KQ:(q + 1) * KQ].astype(BF))
        for h0 in range(0, RB, HB):
            pieces = []
            for a1 in range(4):
                for r in range(h0, h0 + HB, 16):
                    xs = x_v[pl.ds(base + (QS * a1 + r), 16), :].astype(F32)
                    pieces.append(jnp.concatenate(_bfly8([xs[:, 128 * a:128 * a + 128] for a in range(8)]),
                                                  axis=1))
                    z_s[a1, r // 2:r // 2 + 8, :] = _as_u32(pieces[-1][:, :128].astype(BF))
            ub = jnp.concatenate(pieces, axis=0)
            for g in range(4):
                yy = _dot(ub[:, 256 * g:256 * g + 256].astype(BF), _as_bf(gf[g]))
                v = _fft([(yy[HB * a1:HB * a1 + HB, :128], yy[HB * a1:HB * a1 + HB, 128:])
                          for a1 in range(4)], -1)
                for k1 in range(4):
                    rows = pl.ds(base + (QS * k1 + h0), HB)
                    y[g, 0, rows, :] = v[k1][0]
                    y[g, 1, rows, :] = v[k1][1]
                if h0 + HB == RB and g == 3:
                    for a1 in range(4):
                        xa[pl.ds(4 * a1 + i, 1), :] = _dot_nt(alt, _as_bf(z_s[a1]))[0:1]
        return c

    with jax.named_scope("f1"):
        lax.fori_loop(0, QS // RB, f1, 0)

    def fprep(src, h, c):
        ev, od = [], []
        for r in range(8):
            wr = fraw[src, 0, c, pl.ds(r, 32, stride=8), :]
            wi = fraw[src, 1, c, pl.ds(r, 32, stride=8), :]
            ev.append((wr & jnp.uint32(0xFFFF)) | (wi << 16))
            od.append((wr >> 16) | (wi & jnp.uint32(0xFFFF0000)))
        for g, cls in enumerate(CLASSES):
            t = _transpose_u32(jnp.concatenate([(od if k % 2 else ev)[k // 2] for k in cls], axis=0))
            for q in range(128 // N1):
                row = pl.multiple_of(((4 * h + c) * (128 // N1) + q) * PITCH, 8)
                fp[g, pl.ds(row, N1), :] = t[q * N1:(q + 1) * N1]

    def nyquist():
        twc, tws = sm[0:16], sm[16:32]
        u = _dot(sm[32:64, 0:16].astype(BF), xa[0:16, :].astype(BF))
        ur, ui = u[0:16], u[16:32]
        u = jnp.concatenate([ur * twc + ui * tws, ui * twc - ur * tws], axis=1).astype(BF)
        yield
        xx = _dot(u, _as_bf(gf[4]))
        xr, xi = xx[:, :128], xx[:, 128:]
        w = (pltpu.bitcast(nyq[0].astype(F32), U32) >> 16) | pltpu.bitcast(nyq[1].astype(F32), U32)
        w = jnp.concatenate([w[:, 128 * a:128 * a + 128] for a in range(16)], axis=0)
        wt = _transpose_u32(jnp.concatenate([w] * 8, axis=0))
        blk = _lanes(16) >> 4
        wm = wt[0:16]
        for j in range(1, 8):
            wm = jnp.where(blk == j, wt[16 * j:16 * j + 16], wm)
        wr, wi = _lo_f32(wm), _hi_f32(wm)
        z = jnp.concatenate([xr * wr - xi * wi, xr * wi + xi * wr], axis=1).astype(BF)
        yield
        pp = _dot(z, _as_bf(gf[5]))
        pr, pi = pp[:, :128], pp[:, 128:]
        pp = jnp.concatenate([pr * twc - pi * tws, pi * twc + pr * tws], axis=0).astype(BF)
        yield
        cc = _dot(sm[64:80, 0:32].astype(BF), pp) * (1.0 / (S * D))
        ct[...] = jnp.concatenate([cc, jnp.zeros((112, 128), F32)], axis=0).T
        yield

    def s_rows(k1, a0, r):
        return pl.ds(r + (QS * k1 + N2 * a0), 8)

    def anchored(v, tok, inst=0):
        return jnp.where(zero_s[inst] != 0, tok, v)

    def s_prep(g, k1, r, tok):
        v = [(y[g, 0, s_rows(k1, a0, r), :], y[g, 1, s_rows(k1, a0, r), :]) for a0 in range(8)]
        if tok is not None:
            v[0] = (anchored(v[0][0], tok), v[0][1])
        v = _fft([_cmul_const(v[a0], a0 * k1, N1, -1) for a0 in range(8)], -1)
        for k0 in range(8):
            u_s[k1 + 4 * k0, pl.ds(r, 8), :] = _as_u32(jnp.concatenate(v[k0], axis=0).astype(BF))

    def s_fwd(g, ka, tok):
        xx = _dot(_as_bf(gs[0, ka]), _as_bf(u_s[ka]))
        w32 = fp[g, pl.ds(ka, N2, stride=PITCH), :]
        wr, wi = _lo_f32(w32), _hi_f32(w32)
        xr, xi = xx[:N2], xx[N2:]
        z_s[ka] = _as_u32(jnp.concatenate([xr * wr - xi * wi, xr * wi + xi * wr], axis=0).astype(BF))

    def s_inv(ka, tok):
        p_s[ka] = _dot(_as_bf(gs[1, ka]), _as_bf(z_s[ka]))

    def s_post(g, k1, r, tok):
        v = [(p_s[k1 + 4 * k0, r:r + 8, :], p_s[k1 + 4 * k0, N2 + r:N2 + r + 8, :]) for k0 in range(8)]
        v[0] = (anchored(v[0][0], tok), anchored(v[0][1], tok))
        v = _fft(v, 1)
        for a0 in range(8):
            vr, vi = _cmul_const(v[a0], a0 * k1, N1, 1)
            v_s[g, 0, s_rows(k1, a0, r), :] = vr
            v_s[g, 1, s_rows(k1, a0, r), :] = vi

    def wc_block(c, jc):
        return raw_a.at[c // 2, pl.ds(pl.multiple_of(4096 * (c % 2) + 1024 * jc, 1024), 1024), :]

    def wo_comb(jc, p, r, tok):
        nr = 64 // WSP
        u = [wo[jc + 4 * f, 128 * p + 64 * e + r:128 * p + 64 * e + r + nr, :] for e in range(2) for f in range(2)]
        tok = jnp.concatenate([pltpu.bitcast(tok, U32)] * (nr // 8), axis=0)
        u[0], u[3] = anchored(u[0], tok), anchored(u[3], tok)
        b11, b12, b21, b22 = [_as_bf(v).astype(F32) for v in u]
        for c, v in enumerate((b11 + b22, b12 - b22, b21 - b11, b11 + b12, b21 + b22)):
            wc_block(c, jc)[64 * p + r:64 * p + r + nr, :] = _as_u32(v.astype(BF))

    def bulk(where, n, events, q=None):
        k0, nk = (0, KH) if q is None else (pl.multiple_of(q * KQ, KQ), KQ)
        for i in range(n):
            ch, jj = where(i)

            def hook(k, m):
                pieces = events.get(7 * i + k, ())
                vec = [pc for pc in pieces if isinstance(pc, P) and pc.func in (s_prep, s_post, wo_comb)]
                for piece in pieces:
                    r = 8 * ((32 * vec.index(piece)) // len(vec)) if piece in vec else 0
                    piece(m[r:r + 8])

            def keep(k):
                return v_s.at[jj // 4, (jj // 2) % 2, pl.ds(1024 * (jj % 2) + 256 * k, 256), :]

            def init(k):
                return jnp.where(q > 0, keep(k)[...], 0.0)

            raw = raw_b.at[ch - 3] if q is None else raw_a.at[ch]
            strassen(prep_rhs(raw, ch, jj, k0, nk), q, 8 * ch + jj,
                     None if q is None else init, None if q is None else keep, hook)

    def spread(events, pieces, q0, q1):
        for i, piece in enumerate(pieces):
            events.setdefault(q0 + ((q1 - q0) * i) // len(pieces), []).append(piece)

    P = functools.partial

    def loop_a(n, c):
        for e in range(2):
            wait(w_half(raw4[0].at[n // 2], n % 2, e), SEM_W0 + n)
        h = jnp.maximum(n - 2, 0)

        @pl.when(n >= 2)
        def _():
            wait(fraw.at[h], SEM_F + h)

        src = jnp.where(n >= 2, h, 4)
        events = {}
        spread(events, [lambda tok, c=c: fprep(src, h, c) for c in range(4)], 0, 48)
        bulk(lambda i: (n // 2, i), 8, events, n % 2)
        return c

    def loop_b(g, c):
        @pl.when(g < 3)
        def _():
            wait(raw4[1].at[g], SEM_W + 3 + g)

        for e in range(2):
            wait(wo.at[g + 4 * e], SEM_WO + g)
        gn = jnp.minimum(g + 1, 3)
        events = {}
        for k1 in range(4):
            q = BD * k1
            spread(events, [P(s_fwd, g, k1 + 4 * k0) for k0 in range(8)], q, q + BW)
            spread(events, [P(s_prep, gn, k1, r) for r in range(0, N2, 8)], q + BW, q + BW + BV)
            q += BL
            spread(events, [P(s_inv, k1 + 4 * k0) for k0 in range(8)], q, q + BW)
            spread(events, [P(s_post, g, k1, r) for r in range(0, N2, 8)], q + BW, q + BW + BV)
        spread(events, [P(wo_comb, g, p, r) for p in range(NP) for r in range(0, 64, 64 // WSP)], W0, W1)
        ny = nyquist()
        spread(events, [lambda tok: next(ny)] * 4, NY0, NY1)
        assert max(events) < 41
        bulk(lambda i: ((24 + 6 * g + i) // 8, (24 + 6 * g + i) % 8), 6, events)
        return c

    def prep0(i, c):
        for k1 in range(4):
            s_prep(0, k1, pl.multiple_of(i * 8, 8), None)
        return c

    lax.fori_loop(0, N2 // 8, prep0, 0)
    with jax.named_scope("loop_a"):
        lax.fori_loop(0, 6, loop_a, 0)
    wait(sm, SEM_SM)
    wait(gf.at[4:6], SEM_NYM)
    wait(nyq, SEM_NYQ)
    wait(gs, SEM_GS)
    with jax.named_scope("loop_b"):
        lax.fori_loop(0, 4, loop_b, 0)
    wait(gi, SEM_GI)
    wait(mem_ref, SEM_MEM)
    wait(gw_ref.at[pl.ds(0, D)], SEM_GW)

    scale = DH ** -0.5

    gw_s[...] = jnp.broadcast_to(gw_ref[pl.ds(0, D)].astype(F32).reshape(1, D), (8, D))

    uses = itertools.count()

    def softmax(s):
        fill = mf[next(uses) % NMF, 0:80, :]
        s = jnp.where(fill > 0.0, s * scale, fill)
        m = jnp.max(s, axis=-1, keepdims=True)
        e = jnp.exp(s - m)
        l = jnp.sum(e, axis=-1, keepdims=True)
        if NEWTON:
            r = pl.reciprocal(l, approx=True)
            r = r * (2.0 - l * r)
        else:
            r = 1.0 / l
        return e, r

    def lhs_rows(mem, seg):
        xs = x_v[pl.ds(pl.multiple_of(seg * SEG, SEG), SEG), :].astype(F32)
        return jnp.concatenate([mem, xs[8:SEG]], axis=0).astype(BF)

    def proj2(a, m, j):
        return jnp.concatenate([_dot(_as_bf(a[...]), _as_bf(wqkv[H * m + 2 * j + p])).astype(BF)
                                for p in range(2)], axis=0)

    def proj_lo(a):
        for i in range(6):
            pa_s[i] = _dot(_as_bf(a[:, :KH]), _as_bf(wqkv[H * (i // 2) + i % 2, 0:KH // 2, :]))

    def proj_hi(a):
        full = [(_dot(_as_bf(a[:, KH:]), _as_bf(wqkv[H * (i // 2) + i % 2, KH // 2:KH, :]))
                 + pa_s[i]).astype(BF) for i in range(6)]
        for m in range(3):
            stg[m, 0] = _as_u32(jnp.concatenate(full[2 * m:2 * m + 2], axis=0))

    def step(a, seg, k, hooks):
        srow = pl.multiple_of(seg * 8, 8)
        a = a[...]

        def get(m, j):
            return _as_bf(jnp.concatenate([stg[m, j % 8], st[NP * m + j, pl.ds(srow, 8), :]], axis=0))

        def proj(j, m):
            if j > 0:
                stg[m, j % 8] = _as_u32(proj2(a, m, j))
            elif m == 0:
                if k > 0:
                    proj_lo(a)
                proj_hi(a)

        def scores(j):
            e, r = softmax(_dot_nt(get(0, j), get(1, j)))
            pst[j % 8] = _as_u32((e * r).astype(BF))

        def pv(j):
            o = _dot(_as_bf(pst[j % 8]), get(2, j))
            if k < 3:
                for i in range(2):
                    sto[2 * j + i, 8 * k:8 * k + 8, :] = o[64 + 8 * i:72 + 8 * i]
                    obuf[2 * j + i] = _as_u32(o[32 * i:32 * i + 32].astype(BF))
            else:
                a11, a12 = o[0:32], o[32:64]
                a21, a22 = [jnp.concatenate([sto[2 * j + i, 0:24, :], o[64 + 8 * i:72 + 8 * i]], axis=0)
                            for i in range(2)]
                for i, v in enumerate((a11 + a22, a21 + a22, a11, a22, a11 + a12, a21 - a11, a12 - a22)):
                    lc[i, j] = _as_u32(v.astype(BF))

        def wo_part(j, h0, h1):
            og = jnp.concatenate([_as_bf(obuf[h]) for h in range(h0, h1)], axis=1)
            return _dot(og, _as_bf(wo[j, h0 * 64:h1 * 64, :]))

        def prod(i, jc, p0, p1):
            lhs = jnp.concatenate([_as_bf(lc[i, p]) for p in range(p0, p1)], axis=1)
            if i in (1, 4):
                e = i // 4
                rhs = jnp.concatenate([wo[jc + 4 * e, 128 * p + 64 * e:128 * p + 64 * e + 64, :]
                                       for p in range(p0, p1)], axis=0)
            else:
                rhs = wc_block((0, None, 1, 2, None, 3, 4)[i], jc)[64 * p0:64 * p1, :]
            return _dot(lhs, _as_bf(rhs))

        early = [(i, jc) for i in (0, 3, 4, 6) for jc in range(4)]
        parts = []
        for i in range(NP + 4):
            for ch in ORDER:
                if ch in "qkv":
                    m = "qkv".index(ch)
                    if i < NP:
                        proj(i, m)
                    elif m < 2 and k < 3:
                        parts.append(wo_part(len(parts), 0, SPLIT))
                    elif m < 2:
                        parts += [prod(*early[len(parts) + n], 0, SP3) for n in range(2)]
                elif ch == "s" and 0 <= i - LAG1 < NP:
                    scores(i - LAG1)
                elif ch == "p" and 0 <= i - LAG2 < NP:
                    pv(i - LAG2)
            if (k, i) in hooks:
                hooks[k, i]()
        if k < 3:
            return jnp.concatenate([wo_part(j, SPLIT, H) + parts[j] for j in range(8)], axis=1)
        mm = {key: prod(*key, SP3, NP) + parts[n] for n, key in enumerate(early)}
        c11 = [mm[0, jc] + mm[3, jc] - mm[4, jc] + mm[6, jc] for jc in range(4)]
        mm.update({(2, jc): prod(2, jc, 0, NP) for jc in range(4)})
        c12 = [mm[2, jc] + mm[4, jc] for jc in range(4)]
        mm.update({(1, jc): prod(1, jc, 0, NP) for jc in range(4)})
        c21 = [mm[1, jc] + mm[3, jc] for jc in range(4)]
        c22 = [prod(5, jc, 0, NP) + (mm[0, jc] - mm[1, jc] + mm[2, jc]) for jc in range(4)]
        return jnp.concatenate(c11 + c12, axis=1), jnp.concatenate(c21 + c22, axis=1)

    def start_quad(mem, u):
        a_s[0] = _as_u32(lhs_rows(mem, 4 * u))
        proj_lo(a_s.at[0])

    def quad(u, c):
        NR = 128 // NSP
        a1 = u // 4
        s2 = (1 - 2 * (a1 & 1)).astype(F32)
        sg = (1 - (a1 & 2)).astype(F32)
        cc, ss = sg * (1 - (a1 & 1)).astype(F32), sg * (a1 & 1).astype(F32)
        base = pl.multiple_of(u * 128, 128)
        lane = _lanes(NR)
        lo = lane < 64
        roll = lambda v: pltpu.roll(v, 64, 1)

        def spectral_part(r0):
            off = pl.multiple_of((u % 4) * 128, 128) + r0

            def irfft_group(g):
                q = [[v_s[g, e, pl.ds(off + QS * k1, NR), :] for e in range(2)] for k1 in range(4)]
                br, bi = q[1][0] + s2 * q[3][0], q[1][1] + s2 * q[3][1]
                vr = q[0][0] + s2 * q[2][0] + (cc * br - ss * bi)
                vi = q[0][1] + s2 * q[2][1] + (cc * bi + ss * br)
                tin = _half_pre(vr, vi, lo, roll, jnp.where)
                tp, tm = [_dot(tin[e].astype(BF), _as_bf(gi[2 * g + e])) for e in range(2)]
                if g == 0:
                    nyc = jnp.sum(jnp.where(lane == u, ct[r0:r0 + NR, :], 0.0), axis=-1, keepdims=True)
                    tp = tp + nyc * (1 - 2 * (lane & 1)).astype(F32)
                return list(_half_post(g, tp, tm, lo, roll, jnp.where))

            ts = sum([irfft_group(g) for g in range(4)], [])
            b = jnp.concatenate(_bfly8_t(ts), axis=1).astype(BF).astype(F32)
            xs = x_v[pl.ds(base + r0, NR), :].astype(F32)
            gate = jax.nn.sigmoid(jnp.sum(xs * jnp.concatenate([gw_s[...]] * (NR // 8), axis=0),
                                          axis=-1, keepdims=True))
            bb_s[r0:r0 + NR, :] = (1.0 - gate) * b
            g_s[r0:r0 + NR, :] = jnp.broadcast_to(gate, (NR, 128))

        hooks = {HOOKS[n]: functools.partial(spectral_part, n * NR) for n in range(NSP)}
        for k in range(3):
            res = step(a_s.at[k % 2], 4 * u + k, k, hooks)
            ra_s[32 * k + 8:32 * k + 32, :] = res[8:32]
            a_s[(k + 1) % 2] = _as_u32(lhs_rows(res[0:8], 4 * u + k + 1))
        res, first8 = step(a_s.at[1], 4 * u + 3, 3, hooks)
        att = []
        for k in range(4):
            att += [first8[8 * k:8 * k + 8], ra_s[32 * k + 8:32 * k + 32, :] if k < 3 else res[8:32]]
        out_v[pl.ds(base, 128), :] = (bb_s[...] + jnp.concatenate([g_s[...]] * 8, axis=1)
                                      * jnp.concatenate(att, axis=0)).astype(BF)
        pltpu.make_async_copy(out_v.at[pl.ds(base, 128), :], out_hbm.at[pl.ds(base, 128), :],
                              sem.at[SEM_OUT]).start()
        start_quad(res[0:8], jnp.minimum(u + 1, S // 128 - 1))
        return c

    with jax.named_scope("chain"):
        start_quad(mem_ref[...].astype(F32), 0)
        lax.fori_loop(0, S // 128, quad, 0)
    pltpu.make_async_copy(out_v, out_hbm, sem.at[SEM_OUT]).wait()


@jax.jit
def pallas_gated_mix__memory_aug_recurrent_mem_tr__spectral_gfnet__prompt_kernel(
    A_x, A_mem0, A_Wq, A_Wk, A_Wv, A_Wo, A_seg_len, B_x, B_w_r, B_w_i, gate_w,
):
    assert A_x.shape == (1, S, D) and A_mem0.shape == (1, M, D) and A_Wq.shape == (D, H, DH)
    consts = [jnp.asarray(c) for c in _constants()]
    any_spec = pl.BlockSpec(memory_space=pl.ANY)
    out = pl.pallas_call(
        _kernel,
        out_shape=jax.ShapeDtypeStruct((S, D), BF),
        in_specs=[any_spec] * 13,
        out_specs=any_spec,
        scratch_shapes=[
            pltpu.VMEM((S, D), BF),
            pltpu.VMEM((3, D * 8, DH), U32),
            pltpu.VMEM((3, D * 8, DH), U32),
            pltpu.VMEM((3 * H, D // 2, DH), U32),
            pltpu.VMEM((8, H * DH // 2, 128), U32),
            pltpu.VMEM((3 * NP, 8 * NSEG, 128), U32),
            pltpu.VMEM((NQ, 7, 2 * NSEG, D // 2 // NQ), U32),
            pltpu.VMEM((5, 2, 4, 256, 128), U32),
            pltpu.VMEM((4, N2 * PITCH, 128), U32),
            pltpu.VMEM((6, 128, 256), U32),
            pltpu.VMEM((8, 64, 128), U32),
            pltpu.VMEM((2, N1, N2, 2 * N2), U32),
            pltpu.VMEM((4, 2, S, 128), F32),
            pltpu.VMEM((4, 2, S, 128), F32),
            pltpu.VMEM((S, D), BF),
            pltpu.VMEM((N1, N2, 128), U32),
            pltpu.VMEM((6, 256, 128), F32),
            pltpu.VMEM((N1, N2, 128), U32),
            pltpu.VMEM((N1, 2 * N2, 128), F32),
            pltpu.VMEM((H, 32, 128), F32),
            pltpu.VMEM((H, 16, 128), U32),
            pltpu.VMEM((128, 128), F32),
            pltpu.VMEM((2, 16, D), U32),
            pltpu.VMEM((6, 32, 128), F32),
            pltpu.VMEM((128, D), F32),
            pltpu.VMEM((128, 128), F32),
            pltpu.VMEM((3, 8, 32, 128), U32),
            pltpu.VMEM((8, 40, 80), U32),
            pltpu.VMEM((128, D), F32),
            pltpu.VMEM((7, NP, 16, 128), U32),
            pltpu.VMEM((8, D), F32),
            pltpu.VMEM((M, D), BF),
            pltpu.VMEM((NMF, 96, 80), F32),
            pltpu.VMEM((96, 128), F32),
            pltpu.VMEM((32, 128), F32),
            pltpu.VMEM((2, 1, S), BF),
            pltpu.VMEM((8 * D,), BF),
            pltpu.SMEM((2,), jnp.int32),
            pltpu.SemaphoreType.DMA((NSEM,)),
        ],
        compiler_params=pltpu.CompilerParams(vmem_limit_bytes=120 * 1024 * 1024),
    )(
        A_x.reshape(S, D), A_mem0.reshape(M, D), A_Wq, A_Wk, A_Wv,
        A_Wo.reshape(H * DH, D), B_w_r.T, B_w_i.T, gate_w, *consts,
    )
    return out.reshape(1, S, D)
```

```python
import functools
import itertools
import math

import numpy as np
import jax
import jax.numpy as jnp
from jax import lax
import jax.experimental.pallas as pl
import jax.experimental.pallas.tpu as pltpu

BF, F32, U32 = jnp.bfloat16, jnp.float32, jnp.uint32

S, D, H, DH, M, SEG = 2048, 1024, 32, 128, 8, 32
NSEG = S // SEG
NP = H // 2
N1, N2 = 32, 64
QS = S // 4
PITCH = N1 + 8
CLASSES = ((0, 8, 4, 12), (1, 15, 9, 7), (2, 14, 10, 6), (3, 13, 11, 5))
LAG1, LAG2, SPLIT, HOOK_AT = 1, 2, 27, 18
ORDER = "qksvp"
NMF = 1
STG, PB, SE = 1, 16, 6
WSP, W0, W1 = 8, 0, 40
SP3, NSP = 13, 4
HOOKS = ((1, 18), (3, 18), (2, 18), (0, 18))
NEWTON = 1
SPLIT11 = 1
NY0, NY1 = 32, 40
BD, BW, BV, BL = 7, 8, 8, 3
NQ = 2
(SEM_W, SEM_GF, SEM_GI, SEM_SM, SEM_GS, SEM_NYQ, SEM_NYM, SEM_MEM, SEM_GW, SEM_OUT, SEM_F, SEM_X,
 SEM_W0) = 0, 6, 7, 8, 9, 10, 11, 12, 13, 14, 15, 19, 23
SEM_WO = SEM_W0 + 6
NSEM = SEM_WO + 4
RSQ2 = float(np.float32(math.sqrt(0.5)))


def _bfly8(x):
    s = [x[i] + x[i + 4] for i in range(4)]
    d = [x[i] - x[i + 4] for i in range(4)]
    e, f = s[0] + s[2], s[1] + s[3]
    t1, t2 = (d[1] - d[3]) * RSQ2, (d[1] + d[3]) * RSQ2
    return [e + f, e - f, d[0] + t1, t2 + d[2], s[0] - s[2], s[1] - s[3], d[0] - t1, t2 - d[2]]


def _bfly8_t(t):
    e, f = t[0] + t[1], t[0] - t[1]
    s = [e + t[4], f + t[5], e - t[4], f - t[5]]
    t1, t2 = t[2] - t[6], t[3] + t[7]
    d = [t[2] + t[6], (t1 + t2) * RSQ2, t[3] - t[7], (t2 - t1) * RSQ2]
    return [s[i] + d[i] for i in range(4)] + [s[i] - d[i] for i in range(4)]


def _half_pre(vr, vi, lo, roll, where):
    ri = roll(vi)
    return where(lo, vr, ri), where(lo, ri, vr)


def _half_post(g, tp, tm, lo, roll, where):
    if g == 0:
        return tp, tm
    c = float(np.float32(math.cos(math.pi * g / 8)))
    s = float(np.float32(math.sin(math.pi * g / 8)))
    p, r = tp + tm, tp - tm
    rm = roll(where(lo, r, p))
    return where(lo, p, c * rm + s * r), where(lo, rm, c * r - s * rm)


def _cmul_const(v, k, n, sign):
    re, im = v
    k %= n
    if k == 0:
        return re, im
    if 4 * k == n:
        return (-im, re) if sign > 0 else (im, -re)
    if 8 * k == n:
        return (((re - im) * RSQ2, (re + im) * RSQ2) if sign > 0
                else ((re + im) * RSQ2, (im - re) * RSQ2))
    if 8 * k == 3 * n:
        return (((re + im) * -RSQ2, (re - im) * RSQ2) if sign > 0
                else ((im - re) * RSQ2, (re + im) * -RSQ2))
    c, s = math.cos(2 * math.pi * k / n), sign * math.sin(2 * math.pi * k / n)
    return re * c - im * s, re * s + im * c


def _fft(v, sign):
    n = len(v)
    if n == 1:
        return v
    ev, od = _fft(v[0::2], sign), _fft(v[1::2], sign)
    lo, hi = [], []
    for k in range(n // 2):
        er, ei = ev[k]
        if 4 * k == n:
            xr, xi = od[k]
            if sign > 0:
                lo.append((er - xi, ei + xr)); hi.append((er + xi, ei - xr))
            else:
                lo.append((er + xi, ei - xr)); hi.append((er - xi, ei + xr))
            continue
        tr, ti = _cmul_const(od[k], k, n, sign)
        lo.append((er + tr, ei + ti))
        hi.append((er - tr, ei - ti))
    return lo + hi


def _pack_rows(a):
    u = np.ascontiguousarray(a, dtype=np.float32).view(np.uint32)
    b = ((u + 0x7FFF + ((u >> 16) & 1)) >> 16).astype(np.uint32)
    return (b[..., 0::2, :] | (b[..., 1::2, :] << 16)).astype(np.uint32)


def _diag_blocks(full, n, tol):
    k = full.shape[0] // n
    blk = np.kron(np.eye(k), np.ones((n, n)))
    assert np.abs(full * (1 - blk)).max() < tol
    return np.stack([full[n * g:n * g + n, n * g:n * g + n] for g in range(k)])


def _cplx(re, im):
    return np.block([[re, im], [-im, re]])


@functools.lru_cache(maxsize=None)
def _constants():
    k2 = np.stack([np.concatenate([c + 16 * np.arange(32) for c in cls]) for cls in CLASSES])
    n2 = np.arange(D)
    ang = 2 * np.pi * ((k2[:, :, None] * n2[None, None, :]) % D) / D
    rows = np.stack([np.cos(ang), -np.sin(ang)], axis=1)
    wgt = np.where(k2 == 0, 1.0, 2.0)[:, None, :, None]
    fwd = rows.reshape(D, D).T
    inv = (rows * wgt).reshape(D, D) / (S * D)
    bf = np.stack(_bfly8(list(np.eye(8))))
    binv = np.kron(np.linalg.inv(bf), np.eye(128))
    gd = _diag_blocks(binv.T @ fwd, 256, 1e-6)
    gdi = _diag_blocks(inv @ binv, 256, 1e-12)
    eye, lo = np.eye(256), np.arange(128) < 64
    roll = lambda v: np.roll(v, 64, axis=1)
    pre = np.concatenate(_half_pre(eye[:, :128], eye[:, 128:], lo, roll, np.where), axis=1)
    gi = []
    for g in range(4):
        post = np.concatenate(_half_post(g, eye[:, :128], eye[:, 128:], lo, roll, np.where), axis=1)
        gi.append(_diag_blocks(np.linalg.inv(pre) @ gdi[g] @ np.linalg.inv(post), 128, 1e-12))
    gi = np.concatenate(gi)

    b = np.arange(N2)
    k1 = np.arange(N1)[:, None] + N1 * np.arange(N2)[None, :]
    th = 2 * np.pi * ((k1[:, :, None] * b[None, None, :]) % S) / S
    gr, gim = np.cos(th), -np.sin(th)
    full = np.block([[gr, -gim], [gim, gr]])
    kap = np.arange(2 * N2)
    src = ((kap >> 3) & 1) * N2 + (kap >> 4) * 8 + (kap & 7)
    gs = full[:, :, src]
    hr, hi = np.swapaxes(gr, 1, 2), -np.swapaxes(gim, 1, 2)
    gsi = np.block([[hr, -hi], [hi, hr]])

    lane = np.arange(128)
    kb = 8 * (lane % 16) + lane // 16
    t128 = 2 * np.pi * ((lane[:, None] * kb[None, :]) % 128) / 128
    nyf = _cplx(np.cos(t128), -np.sin(t128))
    nyi = _cplx(np.cos(t128).T, np.sin(t128).T)
    i16 = np.arange(16)
    t16 = 2 * np.pi * ((i16[:, None] * i16[None, :]) % 16) / 16
    tw = 2 * np.pi * (i16[:, None] * lane[None, :]) / S
    sm = np.zeros((96, 128), np.float32)
    sm[0:16], sm[16:32] = np.cos(tw), np.sin(tw)
    sm[32:48, :16], sm[48:64, :16] = np.cos(t16), -np.sin(t16)
    sm[64:80, :16], sm[64:80, 16:32] = np.cos(t16), -np.sin(t16)

    gfp = _pack_rows(np.concatenate([gd, nyf[None], nyi[None]]))
    return gfp, _pack_rows(gi), sm, _pack_rows(np.stack([gs, gsi]))


def _mask80():
    r = lax.broadcasted_iota(jnp.int32, (80, 80), 0)
    c = lax.broadcasted_iota(jnp.int32, (80, 80), 1)

    def head(i):
        return jnp.where(i < 64, i >> 5, (i - 64) >> 3)

    def pos(i):
        j = i & 31
        return jnp.where(i < 64, jnp.where(j < M, j, j + 8), M + (i & 7))

    same = head(r) == head(c)
    ok = (pos(r) < M) | (pos(c) <= pos(r))
    return jnp.where(same, jnp.where(ok, 1.0, -1e9), -jnp.inf).astype(F32)


def _as_bf(u):
    return pltpu.bitcast(u, BF)


def _as_u32(b):
    return pltpu.bitcast(b, U32)


def _lo_f32(u):
    return pltpu.bitcast(u << 16, F32)


def _hi_f32(u):
    return pltpu.bitcast(u & jnp.uint32(0xFFFF0000), F32)


def _dot(a, b):
    return jnp.dot(a, b, preferred_element_type=F32)


def _dot_nt(a, b):
    return lax.dot_general(a, b, (((1,), (1,)), ((), ())), preferred_element_type=F32)


def _transpose_u32(u):
    return pltpu.bitcast(pltpu.bitcast(u, F32).T, U32)


def _lanes(rows):
    return lax.broadcasted_iota(jnp.int32, (rows, 128), 1)


def _kernel(x_hbm, mem_hbm, wq_hbm, wk_hbm, wv_hbm, wo_hbm, fr_hbm, fi_hbm, gw_hbm,
            gf_hbm, gi_hbm, sm_hbm, gs_hbm,
            out_hbm,
            x_v, raw_a, raw_b, wqkv, wo, st, sl, fraw, fp, gf, gi, gs, y, v_s, out_v, u_s, cb, z_s, p_s, rs_u, rs_c,
            sto, obuf, ct, a_s, pa_s, bb_s, g_s, stg, pst, ra_s, lc, gw_s, mem_ref, mf, sm, xa, nyq, gw_ref, zero_s, sem):
    KH = D // 2
    KQ = KH // NQ
    RB, HB = 128, 16
    raw4 = [r.reshape(3, D, 8, DH) for r in (raw_a, raw_b)]
    w_hbm = (wq_hbm, wk_hbm, wv_hbm)
    f_hbm = (fr_hbm, fi_hbm)

    def w_src(c):
        return w_hbm[c // 2].bitcast(U32).at[:, pl.ds(8 * (c % 2), 8), :]

    def wait(dst, k):
        pltpu.make_async_copy(dst, dst, sem.at[k]).wait()

    def w_half(ref, q, e):
        return ref.at[pl.ds(pl.multiple_of(q * KQ, KQ) + e * KH, KQ)]

    def x_rows(i, a1):
        return pl.ds(pl.multiple_of(i * RB, RB) + QS * a1, RB)

    def f_copies(h):
        return [(f_hbm[a].at[pl.ds(0, D // 2), pl.ds(128 * (4 * h + c), 128)].bitcast(U32),
                 fraw.at[h, a, c], SEM_F + h) for a in range(2) for c in range(4)]

    def w_copy(c):
        return [(w_src(c), raw4[1].at[c - 3], SEM_W + c)]

    copies = [(gf_hbm.at[0:4], gf.at[0:4], SEM_GF)]
    copies += [(x_hbm.at[x_rows(i, a1), :], x_v.at[x_rows(i, a1), :], SEM_X + i)
               for i in range(QS // RB) for a1 in range(4)]
    for n in range(6):
        copies += [(w_half(w_src(n // 2), n % 2, e), w_half(raw4[0].at[n // 2], n % 2, e), SEM_W0 + n)
                   for e in range(2)]
        if n >= 2:
            copies += f_copies(n - 2)
    copies += [(sm_hbm, sm, SEM_SM), (gf_hbm.at[4:6], gf.at[4:6], SEM_NYM)]
    copies += [(f_hbm[a].at[pl.ds(D // 2, 1), :], nyq.at[a], SEM_NYQ) for a in range(2)]
    copies += [(gs_hbm, gs, SEM_GS)]
    for g in range(4):
        copies += w_copy(3 + g) if g < 3 else []
        copies += [(wo_hbm.bitcast(U32).at[:, pl.ds(128 * j, 128)], wo.at[j], SEM_WO + g) for j in (g, g + 4)]
    copies += [(gi_hbm, gi, SEM_GI), (mem_hbm, mem_ref, SEM_MEM), (gw_hbm, gw_ref.at[pl.ds(0, D)], SEM_GW)]
    for src, dst, k in copies:
        pltpu.make_async_copy(src, dst, sem.at[k]).start()

    def prep_rhs(raw, ch, jj, k0, nk):
        item = 8 * ch + jj
        a1 = raw[pl.ds(k0 * 8 + jj, nk, stride=8), :]
        a2 = raw[pl.ds((KH + k0) * 8 + jj, nk, stride=8), :]
        b11, b12, b21, b22 = _lo_f32(a1), _hi_f32(a1), _lo_f32(a2), _hi_f32(a2)
        for p, e, b in ((0, 0, b11), (1, 0, b12), (0, 1, b21), (1, 1, b22)):
            row = pl.multiple_of(k0 // 2, nk // 2) + e * KH // 2
            wqkv[2 * item + p, pl.ds(row, nk // 2), :] = _as_u32(b.astype(BF))
        return [v.astype(BF) for v in (b11 + b22, b11, b12 - b22, b21 - b11, b22, b11 + b12, b21 + b22)]

    def stage_rhs(item, par, d0, tok):
        raw, jj = raw_b.at[item // 8 - 3], item % 8
        a = [raw[pl.ds((e * KH + d0) * 8 + jj, PB, stride=8), :] for e in range(2)]
        if tok is not None:
            tok = jnp.concatenate([pltpu.bitcast(tok, U32)] * (PB // 8), axis=0)
            a = [anchored(v, tok) for v in a]
        b11, b12, b21, b22 = _lo_f32(a[0]), _hi_f32(a[0]), _lo_f32(a[1]), _hi_f32(a[1])
        for p, e, b in ((0, 0, b11), (1, 0, b12), (0, 1, b21), (1, 1, b22)):
            u = _as_u32(b.astype(BF))
            wqkv[2 * item + p, pl.ds((e * KH + d0) // 2, PB // 2), :] = u
            if p == e:
                rs_u[par, p, d0 // 2:(d0 + PB) // 2, :] = u
        rs_c[par, d0:d0 + PB, :] = jnp.concatenate(
            [b11 + b22, b12 - b22, b21 - b11, b11 + b12, b21 + b22], axis=1).astype(BF)

    def staged_rhs(par):
        c = lambda i: (lambda: rs_c[par, :, 128 * i:128 * i + 128])
        return [c(0), lambda: _as_bf(rs_u[par, 0]), c(1), c(2), lambda: _as_bf(rs_u[par, 1]), c(3), c(4)]

    def strassen(rhs, q, item, init, keep, after_dot):
        def prod(i):
            lhs = sl[q, i] if q is not None else jnp.concatenate([sl[k, i] for k in range(NQ)], axis=1)
            return _dot(_as_bf(lhs), rhs[i]() if callable(rhs[i]) else rhs[i])

        def plus(i, r):
            return r if init is None else init(i) + r

        c12, c21 = (cb.at[5], cb.at[4]) if keep is None else (keep(1), keep(2))
        m = prod(1)
        cb[0] = m
        after_dot(0, m)
        m = prod(4)
        cb[1] = m
        after_dot(1, m)
        m1 = prod(0)
        cb[3] = plus(3, m1 - cb[0])
        if keep is None or SPLIT11:
            cb[2] = plus(0, m1 - cb[1])
        after_dot(2, m1)
        m = prod(3)
        c21[...] = plus(2, cb[0] + m)
        cb[2] = cb[2] + m if keep is None or SPLIT11 else plus(0, m1 - cb[1]) + m
        after_dot(3, m)
        m = prod(2)
        c12[...] = plus(1, cb[1] + m)
        cb[3] = cb[3] + m
        after_dot(4, m)
        for k, (i, acc) in enumerate(((6, 2), (5, 3))):
            m = prod(i) + cb[acc]
            if keep is not None:
                keep(3 * k)[...] = m
            store_st(item, k, *((m, c12[...]) if k == 0 else (c21[...], m)))
            after_dot(5 + k, m)

    def store_st(item, e, c1, c2):
        r = jnp.concatenate([c.reshape(NSEG // 2, 8, 128) for c in (c1, c2)], axis=1)
        st[item, 256 * e:256 * e + 256, :] = _as_u32(r.reshape(8 * NSEG, 128).astype(BF))

    def pin(i, c):
        if 1:
            cb[i, 0:8, :] = jnp.zeros((8, 128), F32)
        zero_s[i] = 0
        rs_u[i, 0, 0:8, :] = jnp.zeros((8, 128), U32)
        rs_c[i, 0:16, 0:128] = jnp.zeros((16, 128), BF)
        z_s[i, 0:8, :] = jnp.zeros((8, 128), U32)
        p_s[i, 0:8, :] = jnp.zeros((8, 128), F32)
        u_s[i, 0:8, :] = jnp.zeros((8, 128), U32)
        stg[i, 0, 0:8, :] = jnp.zeros((8, 128), U32)
        obuf[i, 0:8, :] = jnp.zeros((8, 128), U32)
        sto[i, 0:8, :] = jnp.zeros((8, 128), F32)
        lc[i, 0, 0:8, :] = jnp.zeros((8, 128), U32)
        if 1:
            ra_s[pl.ds(pl.multiple_of(8 * i, 8), 8), 0:128] = jnp.zeros((8, 128), F32)
        if 1:
            a_s[i, 0:8, 0:128] = jnp.zeros((8, 128), U32)
        pa_s[i, 0:8, :] = jnp.zeros((8, 128), F32)
        if 0:
            bb_s[pl.ds(pl.multiple_of(8 * i, 8), 8), 0:128] = jnp.zeros((8, 128), F32)
            g_s[pl.ds(pl.multiple_of(8 * i, 8), 8), :] = jnp.zeros((8, 128), F32)
        return c

    lax.fori_loop(0, 2, pin, 0)

    def fill_mask(i, c):
        mf[i, 0:80, :] = _mask80()
        return c

    lax.fori_loop(0, NMF, fill_mask, 0)
    fraw[4] = jnp.zeros(fraw.shape[1:], U32)

    wait(gf.at[0:4], SEM_GF)

    def f1(i, c):
        for a1 in range(4):
            wait(x_v.at[x_rows(i, a1), :], SEM_X + i)
        base = pl.multiple_of(i * RB, RB)
        alt = (1 - 2 * (_lanes(16) & 1)).astype(F32).astype(BF)

        def rows16(r):
            return jnp.concatenate([x_v[pl.ds(r + d, 16), :].astype(F32)[0:8] for d in (0, SEG)], axis=0)

        for r in (0, 64, QS, QS + 64):
            top, bot = rows16(base + r), rows16(base + (r + 2 * QS))
            a11, a12, a21, a22 = top[:, :KH], top[:, KH:], bot[:, :KH], bot[:, KH:]
            row = pl.multiple_of((base + r) // 8, 8)
            for k, v in enumerate((a11 + a22, a21 + a22, a11, a22, a11 + a12, a21 - a11, a12 - a22)):
                for q in range(NQ):
                    sl[q, k, pl.ds(row, 8), :] = _as_u32(v[:, q * KQ:(q + 1) * KQ].astype(BF))
        for h0 in range(0, RB, HB):
            pieces = []
            for a1 in range(4):
                for r in range(h0, h0 + HB, 16):
                    xs = x_v[pl.ds(base + (QS * a1 + r), 16), :].astype(F32)
                    pieces.append(jnp.concatenate(_bfly8([xs[:, 128 * a:128 * a + 128] for a in range(8)]),
                                                  axis=1))
                    z_s[a1, r // 2:r // 2 + 8, :] = _as_u32(pieces[-1][:, :128].astype(BF))
            ub = jnp.concatenate(pieces, axis=0)
            for g in range(4):
                yy = _dot(ub[:, 256 * g:256 * g + 256].astype(BF), _as_bf(gf[g]))
                v = _fft([(yy[HB * a1:HB * a1 + HB, :128], yy[HB * a1:HB * a1 + HB, 128:])
                          for a1 in range(4)], -1)
                for k1 in range(4):
                    rows = pl.ds(base + (QS * k1 + h0), HB)
                    y[g, 0, rows, :] = v[k1][0]
                    y[g, 1, rows, :] = v[k1][1]
                if h0 + HB == RB and g == 3:
                    for a1 in range(4):
                        xa[pl.ds(4 * a1 + i, 1), :] = _dot_nt(alt, _as_bf(z_s[a1]))[0:1]
        return c

    with jax.named_scope("f1"):
        lax.fori_loop(0, QS // RB, f1, 0)

    def fprep(src, h, c):
        ev, od = [], []
        for r in range(8):
            wr = fraw[src, 0, c, pl.ds(r, 32, stride=8), :]
            wi = fraw[src, 1, c, pl.ds(r, 32, stride=8), :]
            ev.append((wr & jnp.uint32(0xFFFF)) | (wi << 16))
            od.append((wr >> 16) | (wi & jnp.uint32(0xFFFF0000)))
        for g, cls in enumerate(CLASSES):
            t = _transpose_u32(jnp.concatenate([(od if k % 2 else ev)[k // 2] for k in cls], axis=0))
            for q in range(128 // N1):
                row = pl.multiple_of(((4 * h + c) * (128 // N1) + q) * PITCH, 8)
                fp[g, pl.ds(row, N1), :] = t[q * N1:(q + 1) * N1]

    def nyquist():
        twc, tws = sm[0:16], sm[16:32]
        u = _dot(sm[32:64, 0:16].astype(BF), xa[0:16, :].astype(BF))
        ur, ui = u[0:16], u[16:32]
        u = jnp.concatenate([ur * twc + ui * tws, ui * twc - ur * tws], axis=1).astype(BF)
        yield
        xx = _dot(u, _as_bf(gf[4]))
        xr, xi = xx[:, :128], xx[:, 128:]
        w = (pltpu.bitcast(nyq[0].astype(F32), U32) >> 16) | pltpu.bitcast(nyq[1].astype(F32), U32)
        w = jnp.concatenate([w[:, 128 * a:128 * a + 128] for a in range(16)], axis=0)
        wt = _transpose_u32(jnp.concatenate([w] * 8, axis=0))
        blk = _lanes(16) >> 4
        wm = wt[0:16]
        for j in range(1, 8):
            wm = jnp.where(blk == j, wt[16 * j:16 * j + 16], wm)
        wr, wi = _lo_f32(wm), _hi_f32(wm)
        z = jnp.concatenate([xr * wr - xi * wi, xr * wi + xi * wr], axis=1).astype(BF)
        yield
        pp = _dot(z, _as_bf(gf[5]))
        pr, pi = pp[:, :128], pp[:, 128:]
        pp = jnp.concatenate([pr * twc - pi * tws, pi * twc + pr * tws], axis=0).astype(BF)
        yield
        cc = _dot(sm[64:80, 0:32].astype(BF), pp) * (1.0 / (S * D))
        ct[...] = jnp.concatenate([cc, jnp.zeros((112, 128), F32)], axis=0).T
        yield

    def s_rows(k1, a0, r):
        return pl.ds(r + (QS * k1 + N2 * a0), 8)

    def anchored(v, tok, inst=0):
        return jnp.where(zero_s[inst] != 0, tok, v)

    def s_prep(g, k1, r, tok):
        v = [(y[g, 0, s_rows(k1, a0, r), :], y[g, 1, s_rows(k1, a0, r), :]) for a0 in range(8)]
        if tok is not None:
            v[0] = (anchored(v[0][0], tok), v[0][1])
        v = _fft([_cmul_const(v[a0], a0 * k1, N1, -1) for a0 in range(8)], -1)
        for k0 in range(8):
            u_s[k1 + 4 * k0, pl.ds(r, 8), :] = _as_u32(jnp.concatenate(v[k0], axis=0).astype(BF))

    def s_fwd(g, ka, tok):
        xx = _dot(_as_bf(gs[0, ka]), _as_bf(u_s[ka]))
        w32 = fp[g, pl.ds(ka, N2, stride=PITCH), :]
        wr, wi = _lo_f32(w32), _hi_f32(w32)
        xr, xi = xx[:N2], xx[N2:]
        z_s[ka] = _as_u32(jnp.concatenate([xr * wr - xi * wi, xr * wi + xi * wr], axis=0).astype(BF))

    def s_inv(ka, tok):
        p_s[ka] = _dot(_as_bf(gs[1, ka]), _as_bf(z_s[ka]))

    def s_post(g, k1, r, tok):
        v = [(p_s[k1 + 4 * k0, r:r + 8, :], p_s[k1 + 4 * k0, N2 + r:N2 + r + 8, :]) for k0 in range(8)]
        v[0] = (anchored(v[0][0], tok), anchored(v[0][1], tok))
        v = _fft(v, 1)
        for a0 in range(8):
            vr, vi = _cmul_const(v[a0], a0 * k1, N1, 1)
            v_s[g, 0, s_rows(k1, a0, r), :] = vr
            v_s[g, 1, s_rows(k1, a0, r), :] = vi

    def wc_block(c, jc):
        return raw_a.at[c // 2, pl.ds(pl.multiple_of(4096 * (c % 2) + 1024 * jc, 1024), 1024), :]

    def wo_comb(jc, p, r, tok):
        nr = 64 // WSP
        u = [wo[jc + 4 * f, 128 * p + 64 * e + r:128 * p + 64 * e + r + nr, :] for e in range(2) for f in range(2)]
        tok = jnp.concatenate([pltpu.bitcast(tok, U32)] * (nr // 8), axis=0)
        u[0], u[3] = anchored(u[0], tok), anchored(u[3], tok)
        b11, b12, b21, b22 = [_as_bf(v).astype(F32) for v in u]
        for c, v in enumerate((b11 + b22, b12 - b22, b21 - b11, b11 + b12, b21 + b22)):
            wc_block(c, jc)[64 * p + r:64 * p + r + nr, :] = _as_u32(v.astype(BF))

    def bulk(where, n, events, q=None):
        k0, nk = (0, KH) if q is None else (pl.multiple_of(q * KQ, KQ), KQ)
        for i in range(n):
            ch, jj = where(i)

            def hook(k, m):
                pieces = events.get(7 * i + k, ())
                vec = [pc for pc in pieces if isinstance(pc, P) and pc.func in (s_prep, s_post, wo_comb, stage_rhs)]
                for piece in pieces:
                    r = 8 * ((32 * vec.index(piece)) // len(vec)) if piece in vec else 0
                    piece(m[r:r + 8])

            def keep(k):
                return v_s.at[jj // 4, (jj // 2) % 2, pl.ds(1024 * (jj % 2) + 256 * k, 256), :]

            def init(k):
                return jnp.where(q > 0, keep(k)[...], 0.0)

            raw = raw_b.at[ch - 3] if q is None else raw_a.at[ch]
            rhs = staged_rhs(i % 2) if q is None and STG else prep_rhs(raw, ch, jj, k0, nk)
            strassen(rhs, q, 8 * ch + jj,
                     None if q is None else init, None if q is None else keep, hook)

    def spread(events, pieces, q0, q1):
        for i, piece in enumerate(pieces):
            events.setdefault(q0 + ((q1 - q0) * i) // len(pieces), []).append(piece)

    P = functools.partial

    def loop_a(n, c):
        for e in range(2):
            wait(w_half(raw4[0].at[n // 2], n % 2, e), SEM_W0 + n)
        h = jnp.maximum(n - 2, 0)

        @pl.when(n >= 2)
        def _():
            wait(fraw.at[h], SEM_F + h)

        src = jnp.where(n >= 2, h, 4)
        events = {}
        spread(events, [lambda tok, c=c: fprep(src, h, c) for c in range(4)], 0, 48)
        bulk(lambda i: (n // 2, i), 8, events, n % 2)
        return c

    def loop_b(g, c):
        @pl.when((g < 3) & (g >= STG))
        def _():
            wait(raw4[1].at[g], SEM_W + 3 + g)

        for e in range(2):
            wait(wo.at[g + 4 * e], SEM_WO + g)
        gn = jnp.minimum(g + 1, 3)
        events = {}
        for k1 in range(4):
            q = BD * k1
            spread(events, [P(s_fwd, g, k1 + 4 * k0) for k0 in range(8)], q, q + BW)
            spread(events, [P(s_prep, gn, k1, r) for r in range(0, N2, 8)], q + BW, q + BW + BV)
            q += BL
            spread(events, [P(s_inv, k1 + 4 * k0) for k0 in range(8)], q, q + BW)
            spread(events, [P(s_post, g, k1, r) for r in range(0, N2, 8)], q + BW, q + BW + BV)
        spread(events, [P(wo_comb, g, p, r) for p in range(NP) for r in range(0, 64, 64 // WSP)], W0, W1)
        for i in range(6 if STG else 0):
            nxt = jnp.minimum(24 + 6 * g + i + 1, 3 * NP - 1)
            spread(events, [P(stage_rhs, nxt, (i + 1) % 2, d0) for d0 in range(0, KH, PB)], 7 * i, 7 * i + SE)
        ny = nyquist()
        spread(events, [lambda tok: next(ny)] * 4, NY0, NY1)
        assert max(events) < 41
        bulk(lambda i: ((24 + 6 * g + i) // 8, (24 + 6 * g + i) % 8), 6, events)
        return c

    def prep0(i, c):
        for k1 in range(4):
            s_prep(0, k1, pl.multiple_of(i * 8, 8), None)
        return c

    lax.fori_loop(0, N2 // 8, prep0, 0)
    with jax.named_scope("loop_a"):
        lax.fori_loop(0, 6, loop_a, 0)
    wait(sm, SEM_SM)
    wait(gf.at[4:6], SEM_NYM)
    wait(nyq, SEM_NYQ)
    wait(gs, SEM_GS)
    with jax.named_scope("loop_b"):
        if STG:
            wait(raw4[1].at[0], SEM_W + 3)
            for d0 in range(0, KH, PB):
                stage_rhs(24, 0, d0, None)
        lax.fori_loop(0, 4, loop_b, 0)
    wait(gi, SEM_GI)
    wait(mem_ref, SEM_MEM)
    wait(gw_ref.at[pl.ds(0, D)], SEM_GW)

    scale = DH ** -0.5

    gw_s[...] = jnp.broadcast_to(gw_ref[pl.ds(0, D)].astype(F32).reshape(1, D), (8, D))

    uses = itertools.count()

    def softmax(s):
        fill = mf[next(uses) % NMF, 0:80, :]
        s = jnp.where(fill > 0.0, s * scale, fill)
        m = jnp.max(s, axis=-1, keepdims=True)
        e = jnp.exp(s - m)
        l = jnp.sum(e, axis=-1, keepdims=True)
        if NEWTON:
            r = pl.reciprocal(l, approx=True)
            r = r * (2.0 - l * r)
        else:
            r = 1.0 / l
        return e, r

    def lhs_rows(mem, seg):
        xs = x_v[pl.ds(pl.multiple_of(seg * SEG, SEG), SEG), :].astype(F32)
        return jnp.concatenate([mem, xs[8:SEG]], axis=0).astype(BF)

    def proj2(a, m, j):
        return jnp.concatenate([_dot(_as_bf(a[...]), _as_bf(wqkv[H * m + 2 * j + p])).astype(BF)
                                for p in range(2)], axis=0)

    def proj_lo(a):
        for i in range(6):
            pa_s[i] = _dot(_as_bf(a[:, :KH]), _as_bf(wqkv[H * (i // 2) + i % 2, 0:KH // 2, :]))

    def proj_hi(a):
        full = [(_dot(_as_bf(a[:, KH:]), _as_bf(wqkv[H * (i // 2) + i % 2, KH // 2:KH, :]))
                 + pa_s[i]).astype(BF) for i in range(6)]
        for m in range(3):
            stg[m, 0] = _as_u32(jnp.concatenate(full[2 * m:2 * m + 2], axis=0))

    def step(a, seg, k, hooks):
        srow = pl.multiple_of(seg * 8, 8)
        a = a[...]

        def get(m, j):
            return _as_bf(jnp.concatenate([stg[m, j % 8], st[NP * m + j, pl.ds(srow, 8), :]], axis=0))

        def proj(j, m):
            if j > 0:
                stg[m, j % 8] = _as_u32(proj2(a, m, j))
            elif m == 0:
                if k > 0:
                    proj_lo(a)
                proj_hi(a)

        def scores(j):
            e, r = softmax(_dot_nt(get(0, j), get(1, j)))
            pst[j % 8] = _as_u32((e * r).astype(BF))

        def pv(j):
            o = _dot(_as_bf(pst[j % 8]), get(2, j))
            if k < 3:
                for i in range(2):
                    sto[2 * j + i, 8 * k:8 * k + 8, :] = o[64 + 8 * i:72 + 8 * i]
                    obuf[2 * j + i] = _as_u32(o[32 * i:32 * i + 32].astype(BF))
            else:
                a11, a12 = o[0:32], o[32:64]
                a21, a22 = [jnp.concatenate([sto[2 * j + i, 0:24, :], o[64 + 8 * i:72 + 8 * i]], axis=0)
                            for i in range(2)]
                for i, v in enumerate((a11 + a22, a21 + a22, a11, a22, a11 + a12, a21 - a11, a12 - a22)):
                    lc[i, j] = _as_u32(v.astype(BF))

        def wo_part(j, h0, h1):
            og = jnp.concatenate([_as_bf(obuf[h]) for h in range(h0, h1)], axis=1)
            return _dot(og, _as_bf(wo[j, h0 * 64:h1 * 64, :]))

        def prod(i, jc, p0, p1):
            lhs = jnp.concatenate([_as_bf(lc[i, p]) for p in range(p0, p1)], axis=1)
            if i in (1, 4):
                e = i // 4
                rhs = jnp.concatenate([wo[jc + 4 * e, 128 * p + 64 * e:128 * p + 64 * e + 64, :]
                                       for p in range(p0, p1)], axis=0)
            else:
                rhs = wc_block((0, None, 1, 2, None, 3, 4)[i], jc)[64 * p0:64 * p1, :]
            return _dot(lhs, _as_bf(rhs))

        early = [(i, jc) for i in (0, 3, 4, 6) for jc in range(4)]
        parts = []
        for i in range(NP + 4):
            for ch in ORDER:
                if ch in "qkv":
                    m = "qkv".index(ch)
                    if i < NP:
                        proj(i, m)
                    elif m < 2 and k < 3:
                        parts.append(wo_part(len(parts), 0, SPLIT))
                    elif m < 2:
                        parts += [prod(*early[len(parts) + n], 0, SP3) for n in range(2)]
                elif ch == "s" and 0 <= i - LAG1 < NP:
                    scores(i - LAG1)
                elif ch == "p" and 0 <= i - LAG2 < NP:
                    pv(i - LAG2)
            if (k, i) in hooks:
                hooks[k, i]()
        if k < 3:
            return jnp.concatenate([wo_part(j, SPLIT, H) + parts[j] for j in range(8)], axis=1)
        mm = {key: prod(*key, SP3, NP) + parts[n] for n, key in enumerate(early)}
        c11 = [mm[0, jc] + mm[3, jc] - mm[4, jc] + mm[6, jc] for jc in range(4)]
        mm.update({(2, jc): prod(2, jc, 0, NP) for jc in range(4)})
        c12 = [mm[2, jc] + mm[4, jc] for jc in range(4)]
        mm.update({(1, jc): prod(1, jc, 0, NP) for jc in range(4)})
        c21 = [mm[1, jc] + mm[3, jc] for jc in range(4)]
        c22 = [prod(5, jc, 0, NP) + (mm[0, jc] - mm[1, jc] + mm[2, jc]) for jc in range(4)]
        return jnp.concatenate(c11 + c12, axis=1), jnp.concatenate(c21 + c22, axis=1)

    def start_quad(mem, u):
        a_s[0] = _as_u32(lhs_rows(mem, 4 * u))
        proj_lo(a_s.at[0])

    def quad(u, c):
        NR = 128 // NSP
        a1 = u // 4
        s2 = (1 - 2 * (a1 & 1)).astype(F32)
        sg = (1 - (a1 & 2)).astype(F32)
        cc, ss = sg * (1 - (a1 & 1)).astype(F32), sg * (a1 & 1).astype(F32)
        base = pl.multiple_of(u * 128, 128)
        lane = _lanes(NR)
        lo = lane < 64
        roll = lambda v: pltpu.roll(v, 64, 1)

        def spectral_part(r0):
            off = pl.multiple_of((u % 4) * 128, 128) + r0

            def irfft_group(g):
                q = [[v_s[g, e, pl.ds(off + QS * k1, NR), :] for e in range(2)] for k1 in range(4)]
                br, bi = q[1][0] + s2 * q[3][0], q[1][1] + s2 * q[3][1]
                vr = q[0][0] + s2 * q[2][0] + (cc * br - ss * bi)
                vi = q[0][1] + s2 * q[2][1] + (cc * bi + ss * br)
                tin = _half_pre(vr, vi, lo, roll, jnp.where)
                tp, tm = [_dot(tin[e].astype(BF), _as_bf(gi[2 * g + e])) for e in range(2)]
                if g == 0:
                    nyc = jnp.sum(jnp.where(lane == u, ct[r0:r0 + NR, :], 0.0), axis=-1, keepdims=True)
                    tp = tp + nyc * (1 - 2 * (lane & 1)).astype(F32)
                return list(_half_post(g, tp, tm, lo, roll, jnp.where))

            ts = sum([irfft_group(g) for g in range(4)], [])
            b = jnp.concatenate(_bfly8_t(ts), axis=1).astype(BF).astype(F32)
            xs = x_v[pl.ds(base + r0, NR), :].astype(F32)
            gate = jax.nn.sigmoid(jnp.sum(xs * jnp.concatenate([gw_s[...]] * (NR // 8), axis=0),
                                          axis=-1, keepdims=True))
            bb_s[r0:r0 + NR, :] = (1.0 - gate) * b
            g_s[r0:r0 + NR, :] = jnp.broadcast_to(gate, (NR, 128))

        hooks = {HOOKS[n]: functools.partial(spectral_part, n * NR) for n in range(NSP)}
        for k in range(3):
            res = step(a_s.at[k % 2], 4 * u + k, k, hooks)
            ra_s[32 * k + 8:32 * k + 32, :] = res[8:32]
            a_s[(k + 1) % 2] = _as_u32(lhs_rows(res[0:8], 4 * u + k + 1))
        res, first8 = step(a_s.at[1], 4 * u + 3, 3, hooks)
        att = []
        for k in range(4):
            att += [first8[8 * k:8 * k + 8], ra_s[32 * k + 8:32 * k + 32, :] if k < 3 else res[8:32]]
        out_v[pl.ds(base, 128), :] = (bb_s[...] + jnp.concatenate([g_s[...]] * 8, axis=1)
                                      * jnp.concatenate(att, axis=0)).astype(BF)
        pltpu.make_async_copy(out_v.at[pl.ds(base, 128), :], out_hbm.at[pl.ds(base, 128), :],
                              sem.at[SEM_OUT]).start()
        start_quad(res[0:8], jnp.minimum(u + 1, S // 128 - 1))
        return c

    with jax.named_scope("chain"):
        start_quad(mem_ref[...].astype(F32), 0)
        lax.fori_loop(0, S // 128, quad, 0)
    pltpu.make_async_copy(out_v, out_hbm, sem.at[SEM_OUT]).wait()


@jax.jit
def pallas_gated_mix__memory_aug_recurrent_mem_tr__spectral_gfnet__prompt_kernel(
    A_x, A_mem0, A_Wq, A_Wk, A_Wv, A_Wo, A_seg_len, B_x, B_w_r, B_w_i, gate_w,
):
    assert A_x.shape == (1, S, D) and A_mem0.shape == (1, M, D) and A_Wq.shape == (D, H, DH)
    consts = [jnp.asarray(c) for c in _constants()]
    any_spec = pl.BlockSpec(memory_space=pl.ANY)
    out = pl.pallas_call(
        _kernel,
        out_shape=jax.ShapeDtypeStruct((S, D), BF),
        in_specs=[any_spec] * 13,
        out_specs=any_spec,
        scratch_shapes=[
            pltpu.VMEM((S, D), BF),
            pltpu.VMEM((3, D * 8, DH), U32),
            pltpu.VMEM((3, D * 8, DH), U32),
            pltpu.VMEM((3 * H, D // 2, DH), U32),
            pltpu.VMEM((8, H * DH // 2, 128), U32),
            pltpu.VMEM((3 * NP, 8 * NSEG, 128), U32),
            pltpu.VMEM((NQ, 7, 2 * NSEG, D // 2 // NQ), U32),
            pltpu.VMEM((5, 2, 4, 256, 128), U32),
            pltpu.VMEM((4, N2 * PITCH, 128), U32),
            pltpu.VMEM((6, 128, 256), U32),
            pltpu.VMEM((8, 64, 128), U32),
            pltpu.VMEM((2, N1, N2, 2 * N2), U32),
            pltpu.VMEM((4, 2, S, 128), F32),
            pltpu.VMEM((4, 2, S, 128), F32),
            pltpu.VMEM((S, D), BF),
            pltpu.VMEM((N1, N2, 128), U32),
            pltpu.VMEM((6, 256, 128), F32),
            pltpu.VMEM((N1, N2, 128), U32),
            pltpu.VMEM((N1, 2 * N2, 128), F32),
            pltpu.VMEM((2, 2, D // 4, 128), U32),
            pltpu.VMEM((2, D // 2, 5 * 128), BF),
            pltpu.VMEM((H, 32, 128), F32),
            pltpu.VMEM((H, 16, 128), U32),
            pltpu.VMEM((128, 128), F32),
            pltpu.VMEM((2, 16, D), U32),
            pltpu.VMEM((6, 32, 128), F32),
            pltpu.VMEM((128, D), F32),
            pltpu.VMEM((128, 128), F32),
            pltpu.VMEM((3, 8, 32, 128), U32),
            pltpu.VMEM((8, 40, 80), U32),
            pltpu.VMEM((128, D), F32),
            pltpu.VMEM((7, NP, 16, 128), U32),
            pltpu.VMEM((8, D), F32),
            pltpu.VMEM((M, D), BF),
            pltpu.VMEM((NMF, 96, 80), F32),
            pltpu.VMEM((96, 128), F32),
            pltpu.VMEM((32, 128), F32),
            pltpu.VMEM((2, 1, S), BF),
            pltpu.VMEM((8 * D,), BF),
            pltpu.SMEM((2,), jnp.int32),
            pltpu.SemaphoreType.DMA((NSEM,)),
        ],
        compiler_params=pltpu.CompilerParams(vmem_limit_bytes=120 * 1024 * 1024),
    )(
        A_x.reshape(S, D), A_mem0.reshape(M, D), A_Wq, A_Wk, A_Wv,
        A_Wo.reshape(H * DH, D), B_w_r.T, B_w_i.T, gate_w, *consts,
    )
    return out.reshape(1, S, D)
```

```python
import functools
import itertools
import math

import numpy as np
import jax
import jax.numpy as jnp
from jax import lax
import jax.experimental.pallas as pl
import jax.experimental.pallas.tpu as pltpu

BF, F32, U32 = jnp.bfloat16, jnp.float32, jnp.uint32

S, D, H, DH, M, SEG = 2048, 1024, 32, 128, 8, 32
NSEG = S // SEG
NP = H // 2
N1, N2 = 32, 64
QS = S // 4
PITCH = N1 + 8
CLASSES = ((0, 8, 4, 12), (1, 15, 9, 7), (2, 14, 10, 6), (3, 13, 11, 5))
LAG1, LAG2, SPLIT, HOOK_AT = 1, 2, 27, 18
ORDER = "qksvp"
NMF = 1
STG, PB, SE = 1, 16, 6
WSP, W0, W1 = 8, 0, 40
T0 = 6
HMAP = "0122"
SP3 = 13
NEWTON = 1
SPLIT11 = 1
NY0, NY1 = 32, 40
BD, BW, BV, BL = 7, 8, 8, 3
NQ = 2
(SEM_W, SEM_GF, SEM_GI, SEM_SM, SEM_GS, SEM_NYQ, SEM_NYM, SEM_MEM, SEM_GW, SEM_OUT, SEM_F, SEM_X,
 SEM_W0) = 0, 6, 7, 8, 9, 10, 11, 12, 13, 14, 15, 19, 23
SEM_WO = SEM_W0 + 6
NSEM = SEM_WO + 4
RSQ2 = float(np.float32(math.sqrt(0.5)))


def _bfly8(x):
    s = [x[i] + x[i + 4] for i in range(4)]
    d = [x[i] - x[i + 4] for i in range(4)]
    e, f = s[0] + s[2], s[1] + s[3]
    t1, t2 = (d[1] - d[3]) * RSQ2, (d[1] + d[3]) * RSQ2
    return [e + f, e - f, d[0] + t1, t2 + d[2], s[0] - s[2], s[1] - s[3], d[0] - t1, t2 - d[2]]


def _bfly8_t(t):
    e, f = t[0] + t[1], t[0] - t[1]
    s = [e + t[4], f + t[5], e - t[4], f - t[5]]
    t1, t2 = t[2] - t[6], t[3] + t[7]
    d = [t[2] + t[6], (t1 + t2) * RSQ2, t[3] - t[7], (t2 - t1) * RSQ2]
    return [s[i] + d[i] for i in range(4)] + [s[i] - d[i] for i in range(4)]


def _half_pre(vr, vi, lo, roll, where):
    ri = roll(vi)
    return where(lo, vr, ri), where(lo, ri, vr)


def _half_post(g, tp, tm, lo, roll, where):
    if g == 0:
        return tp, tm
    c = float(np.float32(math.cos(math.pi * g / 8)))
    s = float(np.float32(math.sin(math.pi * g / 8)))
    p, r = tp + tm, tp - tm
    rm = roll(where(lo, r, p))
    return where(lo, p, c * rm + s * r), where(lo, rm, c * r - s * rm)


def _cmul_const(v, k, n, sign):
    re, im = v
    k %= n
    if k == 0:
        return re, im
    if 4 * k == n:
        return (-im, re) if sign > 0 else (im, -re)
    if 8 * k == n:
        return (((re - im) * RSQ2, (re + im) * RSQ2) if sign > 0
                else ((re + im) * RSQ2, (im - re) * RSQ2))
    if 8 * k == 3 * n:
        return (((re + im) * -RSQ2, (re - im) * RSQ2) if sign > 0
                else ((im - re) * RSQ2, (re + im) * -RSQ2))
    c, s = math.cos(2 * math.pi * k / n), sign * math.sin(2 * math.pi * k / n)
    return re * c - im * s, re * s + im * c


def _fft(v, sign):
    n = len(v)
    if n == 1:
        return v
    ev, od = _fft(v[0::2], sign), _fft(v[1::2], sign)
    lo, hi = [], []
    for k in range(n // 2):
        er, ei = ev[k]
        if 4 * k == n:
            xr, xi = od[k]
            if sign > 0:
                lo.append((er - xi, ei + xr)); hi.append((er + xi, ei - xr))
            else:
                lo.append((er + xi, ei - xr)); hi.append((er - xi, ei + xr))
            continue
        tr, ti = _cmul_const(od[k], k, n, sign)
        lo.append((er + tr, ei + ti))
        hi.append((er - tr, ei - ti))
    return lo + hi


def _pack_rows(a):
    u = np.ascontiguousarray(a, dtype=np.float32).view(np.uint32)
    b = ((u + 0x7FFF + ((u >> 16) & 1)) >> 16).astype(np.uint32)
    return (b[..., 0::2, :] | (b[..., 1::2, :] << 16)).astype(np.uint32)


def _diag_blocks(full, n, tol):
    k = full.shape[0] // n
    blk = np.kron(np.eye(k), np.ones((n, n)))
    assert np.abs(full * (1 - blk)).max() < tol
    return np.stack([full[n * g:n * g + n, n * g:n * g + n] for g in range(k)])


def _cplx(re, im):
    return np.block([[re, im], [-im, re]])


@functools.lru_cache(maxsize=None)
def _constants():
    k2 = np.stack([np.concatenate([c + 16 * np.arange(32) for c in cls]) for cls in CLASSES])
    n2 = np.arange(D)
    ang = 2 * np.pi * ((k2[:, :, None] * n2[None, None, :]) % D) / D
    rows = np.stack([np.cos(ang), -np.sin(ang)], axis=1)
    wgt = np.where(k2 == 0, 1.0, 2.0)[:, None, :, None]
    fwd = rows.reshape(D, D).T
    inv = (rows * wgt).reshape(D, D) / (S * D)
    bf = np.stack(_bfly8(list(np.eye(8))))
    binv = np.kron(np.linalg.inv(bf), np.eye(128))
    gd = _diag_blocks(binv.T @ fwd, 256, 1e-6)
    gdi = _diag_blocks(inv @ binv, 256, 1e-12)
    eye, lo = np.eye(256), np.arange(128) < 64
    roll = lambda v: np.roll(v, 64, axis=1)
    pre = np.concatenate(_half_pre(eye[:, :128], eye[:, 128:], lo, roll, np.where), axis=1)
    gi = []
    for g in range(4):
        post = np.concatenate(_half_post(g, eye[:, :128], eye[:, 128:], lo, roll, np.where), axis=1)
        gi.append(_diag_blocks(np.linalg.inv(pre) @ gdi[g] @ np.linalg.inv(post), 128, 1e-12))
    gi = np.concatenate(gi)

    b = np.arange(N2)
    k1 = np.arange(N1)[:, None] + N1 * np.arange(N2)[None, :]
    th = 2 * np.pi * ((k1[:, :, None] * b[None, None, :]) % S) / S
    gr, gim = np.cos(th), -np.sin(th)
    full = np.block([[gr, -gim], [gim, gr]])
    kap = np.arange(2 * N2)
    src = ((kap >> 3) & 1) * N2 + (kap >> 4) * 8 + (kap & 7)
    gs = full[:, :, src]
    hr, hi = np.swapaxes(gr, 1, 2), -np.swapaxes(gim, 1, 2)
    gsi = np.block([[hr, -hi], [hi, hr]])

    lane = np.arange(128)
    kb = 8 * (lane % 16) + lane // 16
    t128 = 2 * np.pi * ((lane[:, None] * kb[None, :]) % 128) / 128
    nyf = _cplx(np.cos(t128), -np.sin(t128))
    nyi = _cplx(np.cos(t128).T, np.sin(t128).T)
    i16 = np.arange(16)
    t16 = 2 * np.pi * ((i16[:, None] * i16[None, :]) % 16) / 16
    tw = 2 * np.pi * (i16[:, None] * lane[None, :]) / S
    sm = np.zeros((96, 128), np.float32)
    sm[0:16], sm[16:32] = np.cos(tw), np.sin(tw)
    sm[32:48, :16], sm[48:64, :16] = np.cos(t16), -np.sin(t16)
    sm[64:80, :16], sm[64:80, 16:32] = np.cos(t16), -np.sin(t16)

    gfp = _pack_rows(np.concatenate([gd, nyf[None], nyi[None]]))
    return gfp, _pack_rows(gi), sm, _pack_rows(np.stack([gs, gsi]))


def _mask80():
    r = lax.broadcasted_iota(jnp.int32, (80, 80), 0)
    c = lax.broadcasted_iota(jnp.int32, (80, 80), 1)

    def head(i):
        return jnp.where(i < 64, i >> 5, (i - 64) >> 3)

    def pos(i):
        j = i & 31
        return jnp.where(i < 64, jnp.where(j < M, j, j + 8), M + (i & 7))

    same = head(r) == head(c)
    ok = (pos(r) < M) | (pos(c) <= pos(r))
    return jnp.where(same, jnp.where(ok, 1.0, -1e9), -jnp.inf).astype(F32)


def _as_bf(u):
    return pltpu.bitcast(u, BF)


def _as_u32(b):
    return pltpu.bitcast(b, U32)


def _lo_f32(u):
    return pltpu.bitcast(u << 16, F32)


def _hi_f32(u):
    return pltpu.bitcast(u & jnp.uint32(0xFFFF0000), F32)


def _dot(a, b):
    return jnp.dot(a, b, preferred_element_type=F32)


def _dot_nt(a, b):
    return lax.dot_general(a, b, (((1,), (1,)), ((), ())), preferred_element_type=F32)


def _transpose_u32(u):
    return pltpu.bitcast(pltpu.bitcast(u, F32).T, U32)


def _lanes(rows):
    return lax.broadcasted_iota(jnp.int32, (rows, 128), 1)


def _kernel(x_hbm, mem_hbm, wq_hbm, wk_hbm, wv_hbm, wo_hbm, fr_hbm, fi_hbm, gw_hbm,
            gf_hbm, gi_hbm, sm_hbm, gs_hbm,
            out_hbm,
            x_v, raw_a, raw_b, wqkv, wo, st, sl, fraw, fp, gf, gi, gs, y, v_s, out_v, u_s, cb, z_s, p_s, rs_u, rs_c,
            sto, obuf, ct, a_s, pa_s, bb_s, g_s, stg, pst, ra_s, ts_s, lc, gw_s, mem_ref, mf, sm, xa, nyq, gw_ref, zero_s, sem):
    KH = D // 2
    KQ = KH // NQ
    RB, HB = 128, 16
    raw4 = [r.reshape(3, D, 8, DH) for r in (raw_a, raw_b)]
    w_hbm = (wq_hbm, wk_hbm, wv_hbm)
    f_hbm = (fr_hbm, fi_hbm)

    def w_src(c):
        return w_hbm[c // 2].bitcast(U32).at[:, pl.ds(8 * (c % 2), 8), :]

    def wait(dst, k):
        pltpu.make_async_copy(dst, dst, sem.at[k]).wait()

    def w_half(ref, q, e):
        return ref.at[pl.ds(pl.multiple_of(q * KQ, KQ) + e * KH, KQ)]

    def x_rows(i, a1):
        return pl.ds(pl.multiple_of(i * RB, RB) + QS * a1, RB)

    def f_copies(h):
        return [(f_hbm[a].at[pl.ds(0, D // 2), pl.ds(128 * (4 * h + c), 128)].bitcast(U32),
                 fraw.at[h, a, c], SEM_F + h) for a in range(2) for c in range(4)]

    def w_copy(c):
        return [(w_src(c), raw4[1].at[c - 3], SEM_W + c)]

    copies = [(gf_hbm.at[0:4], gf.at[0:4], SEM_GF)]
    copies += [(x_hbm.at[x_rows(i, a1), :], x_v.at[x_rows(i, a1), :], SEM_X + i)
               for i in range(QS // RB) for a1 in range(4)]
    for n in range(6):
        copies += [(w_half(w_src(n // 2), n % 2, e), w_half(raw4[0].at[n // 2], n % 2, e), SEM_W0 + n)
                   for e in range(2)]
        if n >= 2:
            copies += f_copies(n - 2)
    copies += [(sm_hbm, sm, SEM_SM), (gf_hbm.at[4:6], gf.at[4:6], SEM_NYM)]
    copies += [(f_hbm[a].at[pl.ds(D // 2, 1), :], nyq.at[a], SEM_NYQ) for a in range(2)]
    copies += [(gs_hbm, gs, SEM_GS)]
    for g in range(4):
        copies += w_copy(3 + g) if g < 3 else []
        copies += [(wo_hbm.bitcast(U32).at[:, pl.ds(128 * j, 128)], wo.at[j], SEM_WO + g) for j in (g, g + 4)]
    copies += [(gi_hbm, gi, SEM_GI), (mem_hbm, mem_ref, SEM_MEM), (gw_hbm, gw_ref.at[pl.ds(0, D)], SEM_GW)]
    for src, dst, k in copies:
        pltpu.make_async_copy(src, dst, sem.at[k]).start()

    def prep_rhs(raw, ch, jj, k0, nk):
        item = 8 * ch + jj
        a1 = raw[pl.ds(k0 * 8 + jj, nk, stride=8), :]
        a2 = raw[pl.ds((KH + k0) * 8 + jj, nk, stride=8), :]
        b11, b12, b21, b22 = _lo_f32(a1), _hi_f32(a1), _lo_f32(a2), _hi_f32(a2)
        for p, e, b in ((0, 0, b11), (1, 0, b12), (0, 1, b21), (1, 1, b22)):
            row = pl.multiple_of(k0 // 2, nk // 2) + e * KH // 2
            wqkv[2 * item + p, pl.ds(row, nk // 2), :] = _as_u32(b.astype(BF))
        return [v.astype(BF) for v in (b11 + b22, b11, b12 - b22, b21 - b11, b22, b11 + b12, b21 + b22)]

    def stage_rhs(item, par, d0, tok):
        raw, jj = raw_b.at[item // 8 - 3], item % 8
        a = [raw[pl.ds((e * KH + d0) * 8 + jj, PB, stride=8), :] for e in range(2)]
        if tok is not None:
            tok = jnp.concatenate([pltpu.bitcast(tok, U32)] * (PB // 8), axis=0)
            a = [anchored(v, tok) for v in a]
        b11, b12, b21, b22 = _lo_f32(a[0]), _hi_f32(a[0]), _lo_f32(a[1]), _hi_f32(a[1])
        for p, e, b in ((0, 0, b11), (1, 0, b12), (0, 1, b21), (1, 1, b22)):
            u = _as_u32(b.astype(BF))
            wqkv[2 * item + p, pl.ds((e * KH + d0) // 2, PB // 2), :] = u
            if p == e:
                rs_u[par, p, d0 // 2:(d0 + PB) // 2, :] = u
        rs_c[par, d0:d0 + PB, :] = jnp.concatenate(
            [b11 + b22, b12 - b22, b21 - b11, b11 + b12, b21 + b22], axis=1).astype(BF)

    def staged_rhs(par):
        c = lambda i: (lambda: rs_c[par, :, 128 * i:128 * i + 128])
        return [c(0), lambda: _as_bf(rs_u[par, 0]), c(1), c(2), lambda: _as_bf(rs_u[par, 1]), c(3), c(4)]

    def strassen(rhs, q, item, init, keep, after_dot):
        def prod(i):
            lhs = sl[q, i] if q is not None else jnp.concatenate([sl[k, i] for k in range(NQ)], axis=1)
            return _dot(_as_bf(lhs), rhs[i]() if callable(rhs[i]) else rhs[i])

        def plus(i, r):
            return r if init is None else init(i) + r

        c12, c21 = (cb.at[5], cb.at[4]) if keep is None else (keep(1), keep(2))
        m = prod(1)
        cb[0] = m
        after_dot(0, m)
        m = prod(4)
        cb[1] = m
        after_dot(1, m)
        m1 = prod(0)
        cb[3] = plus(3, m1 - cb[0])
        if keep is None or SPLIT11:
            cb[2] = plus(0, m1 - cb[1])
        after_dot(2, m1)
        m = prod(3)
        c21[...] = plus(2, cb[0] + m)
        cb[2] = cb[2] + m if keep is None or SPLIT11 else plus(0, m1 - cb[1]) + m
        after_dot(3, m)
        m = prod(2)
        c12[...] = plus(1, cb[1] + m)
        cb[3] = cb[3] + m
        after_dot(4, m)
        for k, (i, acc) in enumerate(((6, 2), (5, 3))):
            m = prod(i) + cb[acc]
            if keep is not None:
                keep(3 * k)[...] = m
            store_st(item, k, *((m, c12[...]) if k == 0 else (c21[...], m)))
            after_dot(5 + k, m)

    def store_st(item, e, c1, c2):
        r = jnp.concatenate([c.reshape(NSEG // 2, 8, 128) for c in (c1, c2)], axis=1)
        st[item, 256 * e:256 * e + 256, :] = _as_u32(r.reshape(8 * NSEG, 128).astype(BF))

    def pin(i, c):
        if 1:
            cb[i, 0:8, :] = jnp.zeros((8, 128), F32)
        zero_s[i] = 0
        rs_u[i, 0, 0:8, :] = jnp.zeros((8, 128), U32)
        rs_c[i, 0:16, 0:128] = jnp.zeros((16, 128), BF)
        z_s[i, 0:8, :] = jnp.zeros((8, 128), U32)
        p_s[i, 0:8, :] = jnp.zeros((8, 128), F32)
        u_s[i, 0:8, :] = jnp.zeros((8, 128), U32)
        stg[i, 0, 0:8, :] = jnp.zeros((8, 128), U32)
        obuf[i, 0:8, :] = jnp.zeros((8, 128), U32)
        sto[i, 0:8, :] = jnp.zeros((8, 128), F32)
        lc[i, 0, 0:8, :] = jnp.zeros((8, 128), U32)
        ts_s[pl.ds(pl.multiple_of(8 * i, 8), 8), 0:128] = jnp.zeros((8, 128), F32)
        if 1:
            ra_s[pl.ds(pl.multiple_of(8 * i, 8), 8), 0:128] = jnp.zeros((8, 128), F32)
        if 1:
            a_s[i, 0:8, 0:128] = jnp.zeros((8, 128), U32)
        pa_s[i, 0:8, :] = jnp.zeros((8, 128), F32)
        if 0:
            bb_s[pl.ds(pl.multiple_of(8 * i, 8), 8), 0:128] = jnp.zeros((8, 128), F32)
            g_s[pl.ds(pl.multiple_of(8 * i, 8), 8), :] = jnp.zeros((8, 128), F32)
        return c

    lax.fori_loop(0, 2, pin, 0)

    def fill_mask(i, c):
        mf[i, 0:80, :] = _mask80()
        return c

    lax.fori_loop(0, NMF, fill_mask, 0)
    fraw[4] = jnp.zeros(fraw.shape[1:], U32)

    wait(gf.at[0:4], SEM_GF)

    def f1(i, c):
        for a1 in range(4):
            wait(x_v.at[x_rows(i, a1), :], SEM_X + i)
        base = pl.multiple_of(i * RB, RB)
        alt = (1 - 2 * (_lanes(16) & 1)).astype(F32).astype(BF)

        def rows16(r):
            return jnp.concatenate([x_v[pl.ds(r + d, 16), :].astype(F32)[0:8] for d in (0, SEG)], axis=0)

        for r in (0, 64, QS, QS + 64):
            top, bot = rows16(base + r), rows16(base + (r + 2 * QS))
            a11, a12, a21, a22 = top[:, :KH], top[:, KH:], bot[:, :KH], bot[:, KH:]
            row = pl.multiple_of((base + r) // 8, 8)
            for k, v in enumerate((a11 + a22, a21 + a22, a11, a22, a11 + a12, a21 - a11, a12 - a22)):
                for q in range(NQ):
                    sl[q, k, pl.ds(row, 8), :] = _as_u32(v[:, q * KQ:(q + 1) * KQ].astype(BF))
        for h0 in range(0, RB, HB):
            pieces = []
            for a1 in range(4):
                for r in range(h0, h0 + HB, 16):
                    xs = x_v[pl.ds(base + (QS * a1 + r), 16), :].astype(F32)
                    pieces.append(jnp.concatenate(_bfly8([xs[:, 128 * a:128 * a + 128] for a in range(8)]),
                                                  axis=1))
                    z_s[a1, r // 2:r // 2 + 8, :] = _as_u32(pieces[-1][:, :128].astype(BF))
            ub = jnp.concatenate(pieces, axis=0)
            for g in range(4):
                yy = _dot(ub[:, 256 * g:256 * g + 256].astype(BF), _as_bf(gf[g]))
                v = _fft([(yy[HB * a1:HB * a1 + HB, :128], yy[HB * a1:HB * a1 + HB, 128:])
                          for a1 in range(4)], -1)
                for k1 in range(4):
                    rows = pl.ds(base + (QS * k1 + h0), HB)
                    y[g, 0, rows, :] = v[k1][0]
                    y[g, 1, rows, :] = v[k1][1]
                if h0 + HB == RB and g == 3:
                    for a1 in range(4):
                        xa[pl.ds(4 * a1 + i, 1), :] = _dot_nt(alt, _as_bf(z_s[a1]))[0:1]
        return c

    with jax.named_scope("f1"):
        lax.fori_loop(0, QS // RB, f1, 0)

    def fprep(src, h, c):
        ev, od = [], []
        for r in range(8):
            wr = fraw[src, 0, c, pl.ds(r, 32, stride=8), :]
            wi = fraw[src, 1, c, pl.ds(r, 32, stride=8), :]
            ev.append((wr & jnp.uint32(0xFFFF)) | (wi << 16))
            od.append((wr >> 16) | (wi & jnp.uint32(0xFFFF0000)))
        for g, cls in enumerate(CLASSES):
            t = _transpose_u32(jnp.concatenate([(od if k % 2 else ev)[k // 2] for k in cls], axis=0))
            for q in range(128 // N1):
                row = pl.multiple_of(((4 * h + c) * (128 // N1) + q) * PITCH, 8)
                fp[g, pl.ds(row, N1), :] = t[q * N1:(q + 1) * N1]

    def nyquist():
        twc, tws = sm[0:16], sm[16:32]
        u = _dot(sm[32:64, 0:16].astype(BF), xa[0:16, :].astype(BF))
        ur, ui = u[0:16], u[16:32]
        u = jnp.concatenate([ur * twc + ui * tws, ui * twc - ur * tws], axis=1).astype(BF)
        yield
        xx = _dot(u, _as_bf(gf[4]))
        xr, xi = xx[:, :128], xx[:, 128:]
        w = (pltpu.bitcast(nyq[0].astype(F32), U32) >> 16) | pltpu.bitcast(nyq[1].astype(F32), U32)
        w = jnp.concatenate([w[:, 128 * a:128 * a + 128] for a in range(16)], axis=0)
        wt = _transpose_u32(jnp.concatenate([w] * 8, axis=0))
        blk = _lanes(16) >> 4
        wm = wt[0:16]
        for j in range(1, 8):
            wm = jnp.where(blk == j, wt[16 * j:16 * j + 16], wm)
        wr, wi = _lo_f32(wm), _hi_f32(wm)
        z = jnp.concatenate([xr * wr - xi * wi, xr * wi + xi * wr], axis=1).astype(BF)
        yield
        pp = _dot(z, _as_bf(gf[5]))
        pr, pi = pp[:, :128], pp[:, 128:]
        pp = jnp.concatenate([pr * twc - pi * tws, pi * twc + pr * tws], axis=0).astype(BF)
        yield
        cc = _dot(sm[64:80, 0:32].astype(BF), pp) * (1.0 / (S * D))
        ct[...] = jnp.concatenate([cc, jnp.zeros((112, 128), F32)], axis=0).T
        yield

    def s_rows(k1, a0, r):
        return pl.ds(r + (QS * k1 + N2 * a0), 8)

    def anchored(v, tok, inst=0):
        return jnp.where(zero_s[inst] != 0, tok, v)

    def s_prep(g, k1, r, tok):
        v = [(y[g, 0, s_rows(k1, a0, r), :], y[g, 1, s_rows(k1, a0, r), :]) for a0 in range(8)]
        if tok is not None:
            v[0] = (anchored(v[0][0], tok), v[0][1])
        v = _fft([_cmul_const(v[a0], a0 * k1, N1, -1) for a0 in range(8)], -1)
        for k0 in range(8):
            u_s[k1 + 4 * k0, pl.ds(r, 8), :] = _as_u32(jnp.concatenate(v[k0], axis=0).astype(BF))

    def s_fwd(g, ka, tok):
        xx = _dot(_as_bf(gs[0, ka]), _as_bf(u_s[ka]))
        w32 = fp[g, pl.ds(ka, N2, stride=PITCH), :]
        wr, wi = _lo_f32(w32), _hi_f32(w32)
        xr, xi = xx[:N2], xx[N2:]
        z_s[ka] = _as_u32(jnp.concatenate([xr * wr - xi * wi, xr * wi + xi * wr], axis=0).astype(BF))

    def s_inv(ka, tok):
        p_s[ka] = _dot(_as_bf(gs[1, ka]), _as_bf(z_s[ka]))

    def s_post(g, k1, r, tok):
        v = [(p_s[k1 + 4 * k0, r:r + 8, :], p_s[k1 + 4 * k0, N2 + r:N2 + r + 8, :]) for k0 in range(8)]
        v[0] = (anchored(v[0][0], tok), anchored(v[0][1], tok))
        v = _fft(v, 1)
        for a0 in range(8):
            vr, vi = _cmul_const(v[a0], a0 * k1, N1, 1)
            v_s[g, 0, s_rows(k1, a0, r), :] = vr
            v_s[g, 1, s_rows(k1, a0, r), :] = vi

    def wc_block(c, jc):
        return raw_a.at[c // 2, pl.ds(pl.multiple_of(4096 * (c % 2) + 1024 * jc, 1024), 1024), :]

    def wo_comb(jc, p, r, tok):
        nr = 64 // WSP
        u = [wo[jc + 4 * f, 128 * p + 64 * e + r:128 * p + 64 * e + r + nr, :] for e in range(2) for f in range(2)]
        tok = jnp.concatenate([pltpu.bitcast(tok, U32)] * (nr // 8), axis=0)
        u[0], u[3] = anchored(u[0], tok), anchored(u[3], tok)
        b11, b12, b21, b22 = [_as_bf(v).astype(F32) for v in u]
        for c, v in enumerate((b11 + b22, b12 - b22, b21 - b11, b11 + b12, b21 + b22)):
            wc_block(c, jc)[64 * p + r:64 * p + r + nr, :] = _as_u32(v.astype(BF))

    def bulk(where, n, events, q=None):
        k0, nk = (0, KH) if q is None else (pl.multiple_of(q * KQ, KQ), KQ)
        for i in range(n):
            ch, jj = where(i)

            def hook(k, m):
                pieces = events.get(7 * i + k, ())
                vec = [pc for pc in pieces if isinstance(pc, P) and pc.func in (s_prep, s_post, wo_comb, stage_rhs)]
                for piece in pieces:
                    r = 8 * ((32 * vec.index(piece)) // len(vec)) if piece in vec else 0
                    piece(m[r:r + 8])

            def keep(k):
                return v_s.at[jj // 4, (jj // 2) % 2, pl.ds(1024 * (jj % 2) + 256 * k, 256), :]

            def init(k):
                return jnp.where(q > 0, keep(k)[...], 0.0)

            raw = raw_b.at[ch - 3] if q is None else raw_a.at[ch]
            rhs = staged_rhs(i % 2) if q is None and STG else prep_rhs(raw, ch, jj, k0, nk)
            strassen(rhs, q, 8 * ch + jj,
                     None if q is None else init, None if q is None else keep, hook)

    def spread(events, pieces, q0, q1):
        for i, piece in enumerate(pieces):
            events.setdefault(q0 + ((q1 - q0) * i) // len(pieces), []).append(piece)

    P = functools.partial

    def loop_a(n, c):
        for e in range(2):
            wait(w_half(raw4[0].at[n // 2], n % 2, e), SEM_W0 + n)
        h = jnp.maximum(n - 2, 0)

        @pl.when(n >= 2)
        def _():
            wait(fraw.at[h], SEM_F + h)

        src = jnp.where(n >= 2, h, 4)
        events = {}
        spread(events, [lambda tok, c=c: fprep(src, h, c) for c in range(4)], 0, 48)
        bulk(lambda i: (n // 2, i), 8, events, n % 2)
        return c

    def loop_b(g, c):
        @pl.when((g < 3) & (g >= STG))
        def _():
            wait(raw4[1].at[g], SEM_W + 3 + g)

        for e in range(2):
            wait(wo.at[g + 4 * e], SEM_WO + g)
        gn = jnp.minimum(g + 1, 3)
        events = {}
        for k1 in range(4):
            q = BD * k1
            spread(events, [P(s_fwd, g, k1 + 4 * k0) for k0 in range(8)], q, q + BW)
            spread(events, [P(s_prep, gn, k1, r) for r in range(0, N2, 8)], q + BW, q + BW + BV)
            q += BL
            spread(events, [P(s_inv, k1 + 4 * k0) for k0 in range(8)], q, q + BW)
            spread(events, [P(s_post, g, k1, r) for r in range(0, N2, 8)], q + BW, q + BW + BV)
        spread(events, [P(wo_comb, g, p, r) for p in range(NP) for r in range(0, 64, 64 // WSP)], W0, W1)
        for i in range(6 if STG else 0):
            nxt = jnp.minimum(24 + 6 * g + i + 1, 3 * NP - 1)
            spread(events, [P(stage_rhs, nxt, (i + 1) % 2, d0) for d0 in range(0, KH, PB)], 7 * i, 7 * i + SE)
        ny = nyquist()
        spread(events, [lambda tok: next(ny)] * 4, NY0, NY1)
        assert max(events) < 41
        bulk(lambda i: ((24 + 6 * g + i) // 8, (24 + 6 * g + i) % 8), 6, events)
        return c

    def prep0(i, c):
        for k1 in range(4):
            s_prep(0, k1, pl.multiple_of(i * 8, 8), None)
        return c

    lax.fori_loop(0, N2 // 8, prep0, 0)
    with jax.named_scope("loop_a"):
        lax.fori_loop(0, 6, loop_a, 0)
    wait(sm, SEM_SM)
    wait(gf.at[4:6], SEM_NYM)
    wait(nyq, SEM_NYQ)
    wait(gs, SEM_GS)
    with jax.named_scope("loop_b"):
        if STG:
            wait(raw4[1].at[0], SEM_W + 3)
            for d0 in range(0, KH, PB):
                stage_rhs(24, 0, d0, None)
        lax.fori_loop(0, 4, loop_b, 0)
    wait(gi, SEM_GI)
    wait(mem_ref, SEM_MEM)
    wait(gw_ref.at[pl.ds(0, D)], SEM_GW)

    scale = DH ** -0.5

    gw_s[...] = jnp.broadcast_to(gw_ref[pl.ds(0, D)].astype(F32).reshape(1, D), (8, D))

    uses = itertools.count()

    def softmax(s):
        fill = mf[next(uses) % NMF, 0:80, :]
        s = jnp.where(fill > 0.0, s * scale, fill)
        m = jnp.max(s, axis=-1, keepdims=True)
        e = jnp.exp(s - m)
        l = jnp.sum(e, axis=-1, keepdims=True)
        if NEWTON:
            r = pl.reciprocal(l, approx=True)
            r = r * (2.0 - l * r)
        else:
            r = 1.0 / l
        return e, r

    def lhs_rows(mem, seg):
        xs = x_v[pl.ds(pl.multiple_of(seg * SEG, SEG), SEG), :].astype(F32)
        return jnp.concatenate([mem, xs[8:SEG]], axis=0).astype(BF)

    def proj2(a, m, j):
        return jnp.concatenate([_dot(_as_bf(a[...]), _as_bf(wqkv[H * m + 2 * j + p])).astype(BF)
                                for p in range(2)], axis=0)

    def proj_lo(a):
        for i in range(6):
            pa_s[i] = _dot(_as_bf(a[:, :KH]), _as_bf(wqkv[H * (i // 2) + i % 2, 0:KH // 2, :]))

    def proj_hi(a):
        full = [(_dot(_as_bf(a[:, KH:]), _as_bf(wqkv[H * (i // 2) + i % 2, KH // 2:KH, :]))
                 + pa_s[i]).astype(BF) for i in range(6)]
        for m in range(3):
            stg[m, 0] = _as_u32(jnp.concatenate(full[2 * m:2 * m + 2], axis=0))

    def step(a, seg, k, hooks, late):
        srow = pl.multiple_of(seg * 8, 8)
        a = a[...]

        def get(m, j):
            return _as_bf(jnp.concatenate([stg[m, j % 8], st[NP * m + j, pl.ds(srow, 8), :]], axis=0))

        def proj(j, m):
            if j > 0:
                stg[m, j % 8] = _as_u32(proj2(a, m, j))
            elif m == 0:
                if k > 0:
                    proj_lo(a)
                proj_hi(a)

        def scores(j):
            e, r = softmax(_dot_nt(get(0, j), get(1, j)))
            pst[j % 8] = _as_u32((e * r).astype(BF))

        def pv(j):
            o = _dot(_as_bf(pst[j % 8]), get(2, j))
            if k < 3:
                for i in range(2):
                    sto[2 * j + i, 8 * k:8 * k + 8, :] = o[64 + 8 * i:72 + 8 * i]
                    obuf[2 * j + i] = _as_u32(o[32 * i:32 * i + 32].astype(BF))
            else:
                a11, a12 = o[0:32], o[32:64]
                a21, a22 = [jnp.concatenate([sto[2 * j + i, 0:24, :], o[64 + 8 * i:72 + 8 * i]], axis=0)
                            for i in range(2)]
                for i, v in enumerate((a11 + a22, a21 + a22, a11, a22, a11 + a12, a21 - a11, a12 - a22)):
                    lc[i, j] = _as_u32(v.astype(BF))

        def wo_part(j, h0, h1):
            og = jnp.concatenate([_as_bf(obuf[h]) for h in range(h0, h1)], axis=1)
            return _dot(og, _as_bf(wo[j, h0 * 64:h1 * 64, :]))

        def prod(i, jc, p0, p1):
            lhs = jnp.concatenate([_as_bf(lc[i, p]) for p in range(p0, p1)], axis=1)
            if i in (1, 4):
                e = i // 4
                rhs = jnp.concatenate([wo[jc + 4 * e, 128 * p + 64 * e:128 * p + 64 * e + 64, :]
                                       for p in range(p0, p1)], axis=0)
            else:
                rhs = wc_block((0, None, 1, 2, None, 3, 4)[i], jc)[64 * p0:64 * p1, :]
            return _dot(lhs, _as_bf(rhs))

        early = [(i, jc) for i in (0, 3, 4, 6) for jc in range(4)]
        parts = []
        for i in range(NP + 4):
            for ch in ORDER:
                if ch in "qkv":
                    m = "qkv".index(ch)
                    if i < NP:
                        proj(i, m)
                    elif m < 2 and k < 3:
                        parts.append(wo_part(len(parts), 0, SPLIT))
                    elif m < 2:
                        parts += [prod(*early[len(parts) + n], 0, SP3) for n in range(2)]
                elif ch == "s" and 0 <= i - LAG1 < NP:
                    scores(i - LAG1)
                elif ch == "p" and 0 <= i - LAG2 < NP:
                    pv(i - LAG2)
            if i == HOOK_AT:
                for hook in hooks[k]:
                    hook()
        if k < 3:
            return jnp.concatenate([wo_part(j, SPLIT, H) + parts[j] for j in range(8)], axis=1)
        mm = {key: prod(*key, SP3, NP) + parts[n] for n, key in enumerate(early)}
        c11 = [mm[0, jc] + mm[3, jc] - mm[4, jc] + mm[6, jc] for jc in range(4)]
        mm.update({(2, jc): prod(2, jc, 0, NP) for jc in range(4)})
        c12 = [mm[2, jc] + mm[4, jc] for jc in range(4)]
        toks = parts[T0:] + [mm[3, 3] + c11[0]] * 0 + [mm[0, 3], mm[4, 3]] + [mm[2, jc] for jc in range(4)]
        for n, piece in enumerate(late):
            piece(toks[(n * len(toks)) // len(late)][0:8])
        mm.update({(1, jc): prod(1, jc, 0, NP) for jc in range(4)})
        c21 = [mm[1, jc] + mm[3, jc] for jc in range(4)]
        c22 = [prod(5, jc, 0, NP) + (mm[0, jc] - mm[1, jc] + mm[2, jc]) for jc in range(4)]
        return jnp.concatenate(c11 + c12, axis=1), jnp.concatenate(c21 + c22, axis=1)

    def start_quad(mem, u):
        a_s[0] = _as_u32(lhs_rows(mem, 4 * u))
        proj_lo(a_s.at[0])

    def quad(u, c):
        base = pl.multiple_of(u * 128, 128)
        roll = lambda v: pltpu.roll(v, 64, 1)
        a1 = u // 4
        s2 = (1 - 2 * (a1 & 1)).astype(F32)
        sg = (1 - (a1 & 2)).astype(F32)
        cc, ss = sg * (1 - (a1 & 1)).astype(F32), sg * (a1 & 1).astype(F32)

        def irfft_dots(r0):
            off = pl.multiple_of((u % 4) * 128, 128) + r0
            for g in range(4):
                q = [[v_s[g, e, pl.ds(off + QS * k1, SEG), :] for e in range(2)] for k1 in range(4)]
                br, bi = q[1][0] + s2 * q[3][0], q[1][1] + s2 * q[3][1]
                vr = q[0][0] + s2 * q[2][0] + (cc * br - ss * bi)
                vi = q[0][1] + s2 * q[2][1] + (cc * bi + ss * br)
                tin = _half_pre(vr, vi, _lanes(SEG) < 64, roll, jnp.where)
                for e in range(2):
                    ts_s[r0:r0 + SEG, 128 * (2 * g + e):128 * (2 * g + e + 1)] = _dot(
                        tin[e].astype(BF), _as_bf(gi[2 * g + e]))

        def mix(r0, tok):
            lane = _lanes(8)
            t = [anchored(ts_s[r0:r0 + 8, 128 * i:128 * i + 128], tok) for i in range(8)]
            nyc = jnp.sum(jnp.where(lane == u, anchored(ct[r0:r0 + 8, :], tok), 0.0), axis=-1, keepdims=True)
            t[0] = t[0] + nyc * (1 - 2 * (lane & 1)).astype(F32)
            t = sum([list(_half_post(g, t[2 * g], t[2 * g + 1], lane < 64, roll, jnp.where))
                     for g in range(4)], [])
            b = jnp.concatenate(_bfly8_t(t), axis=1).astype(BF).astype(F32)
            xg = x_v[pl.ds(base + r0, 8), :].astype(F32) * gw_s[...]
            xg = functools.reduce(jnp.add, [xg[:, 128 * i:128 * i + 128] for i in range(8)])
            gate = jax.nn.sigmoid(jnp.sum(anchored(xg, tok), axis=-1, keepdims=True))
            bb = (1.0 - gate) * b
            if r0 % SEG and r0 < 96:
                out_v[pl.ds(base + r0, 8), :] = (bb + gate * ra_s[r0:r0 + 8, :]).astype(BF)
            else:
                bb_s[r0:r0 + 8, :] = bb
                g_s[r0:r0 + 8, :] = jnp.broadcast_to(gate, (8, 128))

        hooks = [[P(irfft_dots, SEG * n) for n in range(4) if HMAP[n] == str(k)] for k in range(4)]
        late = [P(mix, r0) for r0 in range(0, 128, 8)]
        for k in range(3):
            res = step(a_s.at[k % 2], 4 * u + k, k, hooks, late)
            ra_s[32 * k + 8:32 * k + 32, :] = res[8:32]
            a_s[(k + 1) % 2] = _as_u32(lhs_rows(res[0:8], 4 * u + k + 1))
        res, first8 = step(a_s.at[1], 4 * u + 3, 3, hooks, late)

        def emit(r0, n, att):
            out_v[pl.ds(base + r0, n), :] = (
                bb_s[r0:r0 + n, :] + jnp.concatenate([g_s[r0:r0 + n, :]] * 8, axis=1) * att).astype(BF)

        emit(104, 24, res[8:32])
        for k in range(4):
            emit(32 * k, 8, first8[8 * k:8 * k + 8])
        pltpu.make_async_copy(out_v.at[pl.ds(base, 128), :], out_hbm.at[pl.ds(base, 128), :],
                              sem.at[SEM_OUT]).start()
        start_quad(res[0:8], jnp.minimum(u + 1, S // 128 - 1))
        return c

    with jax.named_scope("chain"):
        start_quad(mem_ref[...].astype(F32), 0)
        lax.fori_loop(0, S // 128, quad, 0)
    pltpu.make_async_copy(out_v, out_hbm, sem.at[SEM_OUT]).wait()


@jax.jit
def pallas_gated_mix__memory_aug_recurrent_mem_tr__spectral_gfnet__prompt_kernel(
    A_x, A_mem0, A_Wq, A_Wk, A_Wv, A_Wo, A_seg_len, B_x, B_w_r, B_w_i, gate_w,
):
    assert A_x.shape == (1, S, D) and A_mem0.shape == (1, M, D) and A_Wq.shape == (D, H, DH)
    consts = [jnp.asarray(c) for c in _constants()]
    any_spec = pl.BlockSpec(memory_space=pl.ANY)
    out = pl.pallas_call(
        _kernel,
        out_shape=jax.ShapeDtypeStruct((S, D), BF),
        in_specs=[any_spec] * 13,
        out_specs=any_spec,
        scratch_shapes=[
            pltpu.VMEM((S, D), BF),
            pltpu.VMEM((3, D * 8, DH), U32),
            pltpu.VMEM((3, D * 8, DH), U32),
            pltpu.VMEM((3 * H, D // 2, DH), U32),
            pltpu.VMEM((8, H * DH // 2, 128), U32),
            pltpu.VMEM((3 * NP, 8 * NSEG, 128), U32),
            pltpu.VMEM((NQ, 7, 2 * NSEG, D // 2 // NQ), U32),
            pltpu.VMEM((5, 2, 4, 256, 128), U32),
            pltpu.VMEM((4, N2 * PITCH, 128), U32),
            pltpu.VMEM((6, 128, 256), U32),
            pltpu.VMEM((8, 64, 128), U32),
            pltpu.VMEM((2, N1, N2, 2 * N2), U32),
            pltpu.VMEM((4, 2, S, 128), F32),
            pltpu.VMEM((4, 2, S, 128), F32),
            pltpu.VMEM((S, D), BF),
            pltpu.VMEM((N1, N2, 128), U32),
            pltpu.VMEM((6, 256, 128), F32),
            pltpu.VMEM((N1, N2, 128), U32),
            pltpu.VMEM((N1, 2 * N2, 128), F32),
            pltpu.VMEM((2, 2, D // 4, 128), U32),
            pltpu.VMEM((2, D // 2, 5 * 128), BF),
            pltpu.VMEM((H, 32, 128), F32),
            pltpu.VMEM((H, 16, 128), U32),
            pltpu.VMEM((128, 128), F32),
            pltpu.VMEM((2, 16, D), U32),
            pltpu.VMEM((6, 32, 128), F32),
            pltpu.VMEM((128, D), F32),
            pltpu.VMEM((128, 128), F32),
            pltpu.VMEM((3, 8, 32, 128), U32),
            pltpu.VMEM((8, 40, 80), U32),
            pltpu.VMEM((128, D), F32),
            pltpu.VMEM((128, D), F32),
            pltpu.VMEM((7, NP, 16, 128), U32),
            pltpu.VMEM((8, D), F32),
            pltpu.VMEM((M, D), BF),
            pltpu.VMEM((NMF, 96, 80), F32),
            pltpu.VMEM((96, 128), F32),
            pltpu.VMEM((32, 128), F32),
            pltpu.VMEM((2, 1, S), BF),
            pltpu.VMEM((8 * D,), BF),
            pltpu.SMEM((2,), jnp.int32),
            pltpu.SemaphoreType.DMA((NSEM,)),
        ],
        compiler_params=pltpu.CompilerParams(vmem_limit_bytes=120 * 1024 * 1024),
    )(
        A_x.reshape(S, D), A_mem0.reshape(M, D), A_Wq, A_Wk, A_Wv,
        A_Wo.reshape(H * DH, D), B_w_r.T, B_w_i.T, gate_w, *consts,
    )
    return out.reshape(1, S, D)
```

```python
import functools
import math

import numpy as np
import jax
import jax.numpy as jnp
from jax import lax
import jax.experimental.pallas as pl
import jax.experimental.pallas.tpu as pltpu

BF, F32, U32 = jnp.bfloat16, jnp.float32, jnp.uint32

S, D, H, DH, M, SEG = 2048, 1024, 32, 128, 8, 32
NSEG = S // SEG
NP = H // 2
N1, N2 = 32, 64
QS = S // 4
PITCH = N1 + 8
CLASSES = ((0, 8, 4, 12), (1, 15, 9, 7), (2, 14, 10, 6), (3, 13, 11, 5))
LAG1, LAG2, SPLIT, HOOK_AT = 1, 2, 27, 18
ORDER = "qksvp"
PB, SE = 16, 6
WSP, W0, W1 = 8, 0, 40
T0 = 6
HMAP = "0123"
SP3 = 13
NY0, NY1 = 32, 40
BD, BW, BV, BL = 7, 8, 8, 3
NQ = 2
(SEM_W, SEM_GF, SEM_GI, SEM_SM, SEM_GS, SEM_NYQ, SEM_NYM, SEM_MEM, SEM_GW, SEM_OUT, SEM_F, SEM_X,
 SEM_W0) = 0, 6, 7, 8, 9, 10, 11, 12, 13, 14, 15, 19, 23
SEM_WO = SEM_W0 + 6
NSEM = SEM_WO + 4
RSQ2 = float(np.float32(math.sqrt(0.5)))


def _bfly8(x):
    s = [x[i] + x[i + 4] for i in range(4)]
    d = [x[i] - x[i + 4] for i in range(4)]
    e, f = s[0] + s[2], s[1] + s[3]
    t1, t2 = (d[1] - d[3]) * RSQ2, (d[1] + d[3]) * RSQ2
    return [e + f, e - f, d[0] + t1, t2 + d[2], s[0] - s[2], s[1] - s[3], d[0] - t1, t2 - d[2]]


def _bfly8_t(t):
    e, f = t[0] + t[1], t[0] - t[1]
    s = [e + t[4], f + t[5], e - t[4], f - t[5]]
    t1, t2 = t[2] - t[6], t[3] + t[7]
    d = [t[2] + t[6], (t1 + t2) * RSQ2, t[3] - t[7], (t2 - t1) * RSQ2]
    return [s[i] + d[i] for i in range(4)] + [s[i] - d[i] for i in range(4)]


def _half_pre(vr, vi, lo, roll, where):
    ri = roll(vi)
    return where(lo, vr, ri), where(lo, ri, vr)


def _half_post(g, tp, tm, lo, roll, where):
    if g == 0:
        return tp, tm
    c = float(np.float32(math.cos(math.pi * g / 8)))
    s = float(np.float32(math.sin(math.pi * g / 8)))
    p, r = tp + tm, tp - tm
    rm = roll(where(lo, r, p))
    return where(lo, p, c * rm + s * r), where(lo, rm, c * r - s * rm)


def _cmul_const(v, k, n, sign):
    re, im = v
    k %= n
    if k == 0:
        return re, im
    if 4 * k == n:
        return (-im, re) if sign > 0 else (im, -re)
    if 8 * k == n:
        return (((re - im) * RSQ2, (re + im) * RSQ2) if sign > 0
                else ((re + im) * RSQ2, (im - re) * RSQ2))
    if 8 * k == 3 * n:
        return (((re + im) * -RSQ2, (re - im) * RSQ2) if sign > 0
                else ((im - re) * RSQ2, (re + im) * -RSQ2))
    c, s = math.cos(2 * math.pi * k / n), sign * math.sin(2 * math.pi * k / n)
    return re * c - im * s, re * s + im * c


def _fft(v, sign):
    n = len(v)
    if n == 1:
        return v
    ev, od = _fft(v[0::2], sign), _fft(v[1::2], sign)
    lo, hi = [], []
    for k in range(n // 2):
        er, ei = ev[k]
        if 4 * k == n:
            xr, xi = od[k]
            if sign > 0:
                lo.append((er - xi, ei + xr)); hi.append((er + xi, ei - xr))
            else:
                lo.append((er + xi, ei - xr)); hi.append((er - xi, ei + xr))
            continue
        tr, ti = _cmul_const(od[k], k, n, sign)
        lo.append((er + tr, ei + ti))
        hi.append((er - tr, ei - ti))
    return lo + hi


def _pack_rows(a):
    u = np.ascontiguousarray(a, dtype=np.float32).view(np.uint32)
    b = ((u + 0x7FFF + ((u >> 16) & 1)) >> 16).astype(np.uint32)
    return (b[..., 0::2, :] | (b[..., 1::2, :] << 16)).astype(np.uint32)


def _diag_blocks(full, n, tol):
    k = full.shape[0] // n
    blk = np.kron(np.eye(k), np.ones((n, n)))
    assert np.abs(full * (1 - blk)).max() < tol
    return np.stack([full[n * g:n * g + n, n * g:n * g + n] for g in range(k)])


@functools.lru_cache(maxsize=None)
def _constants():
    k2 = np.stack([np.concatenate([c + 16 * np.arange(32) for c in cls]) for cls in CLASSES])
    n2 = np.arange(D)
    ang = 2 * np.pi * ((k2[:, :, None] * n2[None, None, :]) % D) / D
    rows = np.stack([np.cos(ang), -np.sin(ang)], axis=1)
    wgt = np.where(k2 == 0, 1.0, 2.0)[:, None, :, None]
    fwd = rows.reshape(D, D).T
    inv = (rows * wgt).reshape(D, D) / (S * D)
    bf = np.stack(_bfly8(list(np.eye(8))))
    binv = np.kron(np.linalg.inv(bf), np.eye(128))
    gd = _diag_blocks(binv.T @ fwd, 256, 1e-6)
    gdi = _diag_blocks(inv @ binv, 256, 1e-12)
    eye, lo = np.eye(256), np.arange(128) < 64
    roll = lambda v: np.roll(v, 64, axis=1)
    pre = np.concatenate(_half_pre(eye[:, :128], eye[:, 128:], lo, roll, np.where), axis=1)
    gi = []
    for g in range(4):
        post = np.concatenate(_half_post(g, eye[:, :128], eye[:, 128:], lo, roll, np.where), axis=1)
        gi.append(_diag_blocks(np.linalg.inv(pre) @ gdi[g] @ np.linalg.inv(post), 128, 1e-12))
    gi = np.concatenate(gi)

    b = np.arange(N2)
    k1 = np.arange(N1)[:, None] + N1 * np.arange(N2)[None, :]
    th = 2 * np.pi * ((k1[:, :, None] * b[None, None, :]) % S) / S
    gr, gim = np.cos(th), -np.sin(th)
    full = np.block([[gr, -gim], [gim, gr]])
    kap = np.arange(2 * N2)
    src = ((kap >> 3) & 1) * N2 + (kap >> 4) * 8 + (kap & 7)
    gs = full[:, :, src]
    hr, hi = np.swapaxes(gr, 1, 2), -np.swapaxes(gim, 1, 2)
    gsi = np.block([[hr, -hi], [hi, hr]])

    lane = np.arange(128)
    kb = 8 * (lane % 16) + lane // 16
    t128 = 2 * np.pi * ((lane[:, None] * kb[None, :]) % 128) / 128
    nym = np.concatenate([np.cos(t128), np.sin(t128)], axis=1)
    i16 = np.arange(16)
    t16 = 2 * np.pi * ((i16[:, None] * i16[None, :]) % 16) / 16
    tw = 2 * np.pi * (i16[:, None] * lane[None, :]) / S
    sm = np.zeros((96, 128), np.float32)
    sm[0:16], sm[16:32] = np.cos(tw), np.sin(tw)
    sm[32:48, :16], sm[48:64, :16] = np.cos(t16), -np.sin(t16)
    sm[64:80, :16], sm[64:80, 16:32] = np.cos(t16), -np.sin(t16)

    return _pack_rows(gd), _pack_rows(nym), _pack_rows(gi), sm, _pack_rows(np.stack([gs, gsi]))


def _mask80():
    r = lax.broadcasted_iota(jnp.int32, (80, 80), 0)
    c = lax.broadcasted_iota(jnp.int32, (80, 80), 1)

    def head(i):
        return jnp.where(i < 64, i >> 5, (i - 64) >> 3)

    def pos(i):
        j = i & 31
        return jnp.where(i < 64, jnp.where(j < M, j, j + 8), M + (i & 7))

    same = head(r) == head(c)
    ok = (pos(r) < M) | (pos(c) <= pos(r))
    return jnp.where(same, jnp.where(ok, 1.0, -1e9), -jnp.inf).astype(F32)


def _as_bf(u):
    return pltpu.bitcast(u, BF)


def _as_u32(b):
    return pltpu.bitcast(b, U32)


def _lo_f32(u):
    return pltpu.bitcast(u << 16, F32)


def _hi_f32(u):
    return pltpu.bitcast(u & jnp.uint32(0xFFFF0000), F32)


def _dot(a, b):
    return jnp.dot(a, b, preferred_element_type=F32)


def _dot_nt(a, b):
    return lax.dot_general(a, b, (((1,), (1,)), ((), ())), preferred_element_type=F32)


def _transpose_u32(u):
    return pltpu.bitcast(pltpu.bitcast(u, F32).T, U32)


def _lanes(rows):
    return lax.broadcasted_iota(jnp.int32, (rows, 128), 1)


def _kernel(x_hbm, mem_hbm, wq_hbm, wk_hbm, wv_hbm, wo_hbm, fr_hbm, fi_hbm, gw_hbm,
            gf_hbm, nm_hbm, gi_hbm, sm_hbm, gs_hbm,
            out_hbm,
            x_v, raw_a, raw_b, wqkv, wo, st, sl, fraw, fp, gf, nm, gi, gs, y, v_s, out_v, u_s, cb, z_s, p_s, rs_u, rs_c,
            sto, obuf, ct, a_s, pa_s, bb_s, g_s, stg, pst, ra_s, ts_s, mp, lc, gw_s, mem_ref, mf, sm, xa, nyq, gw_ref, zero_s, sem):
    KH = D // 2
    KQ = KH // NQ
    RB, HB = 128, 16
    raw4 = [r.reshape(3, D, 8, DH) for r in (raw_a, raw_b)]
    w_hbm = (wq_hbm, wk_hbm, wv_hbm)
    f_hbm = (fr_hbm, fi_hbm)

    def w_src(c):
        return w_hbm[c // 2].bitcast(U32).at[:, pl.ds(8 * (c % 2), 8), :]

    def wait(dst, k):
        pltpu.make_async_copy(dst, dst, sem.at[k]).wait()

    def w_half(ref, q, e):
        return ref.at[pl.ds(pl.multiple_of(q * KQ, KQ) + e * KH, KQ)]

    def x_rows(i, a1):
        return pl.ds(pl.multiple_of(i * RB, RB) + QS * a1, RB)

    def f_copies(h):
        return [(f_hbm[a].at[pl.ds(0, D // 2), pl.ds(128 * (4 * h + c), 128)].bitcast(U32),
                 fraw.at[h, a, c], SEM_F + h) for a in range(2) for c in range(4)]

    def w_copy(c):
        return [(w_src(c), raw4[1].at[c - 3], SEM_W + c)]

    copies = [(gf_hbm, gf, SEM_GF)]
    copies += [(x_hbm.at[x_rows(i, a1), :], x_v.at[x_rows(i, a1), :], SEM_X + i)
               for i in range(QS // RB) for a1 in range(4)]
    for n in range(6):
        copies += [(w_half(w_src(n // 2), n % 2, e), w_half(raw4[0].at[n // 2], n % 2, e), SEM_W0 + n)
                   for e in range(2)]
        if n >= 2:
            copies += f_copies(n - 2)
    copies += [(sm_hbm, sm, SEM_SM), (nm_hbm, nm, SEM_NYM)]
    copies += [(f_hbm[a].at[pl.ds(D // 2, 1), :], nyq.at[a], SEM_NYQ) for a in range(2)]
    copies += [(gs_hbm, gs, SEM_GS)]
    for g in range(4):
        copies += w_copy(3 + g) if g < 3 else []
        copies += [(wo_hbm.bitcast(U32).at[:, pl.ds(128 * j, 128)], wo.at[j], SEM_WO + g) for j in (g, g + 4)]
    copies += [(gi_hbm, gi, SEM_GI), (mem_hbm, mem_ref, SEM_MEM), (gw_hbm, gw_ref.at[pl.ds(0, D)], SEM_GW)]
    for src, dst, k in copies:
        pltpu.make_async_copy(src, dst, sem.at[k]).start()

    def prep_rhs(ch, jj, k0):
        a1 = raw_a[ch, pl.ds(k0 * 8 + jj, KQ, stride=8), :]
        a2 = raw_a[ch, pl.ds((KH + k0) * 8 + jj, KQ, stride=8), :]
        b11, b12, b21, b22 = _lo_f32(a1), _hi_f32(a1), _lo_f32(a2), _hi_f32(a2)
        for p, e, b in ((0, 0, b11), (1, 0, b12), (0, 1, b21), (1, 1, b22)):
            row = pl.multiple_of(k0 // 2, KQ // 2) + e * KH // 2
            wqkv[2 * (8 * ch + jj) + p, pl.ds(row, KQ // 2), :] = _as_u32(b.astype(BF))
        return [v.astype(BF) for v in (b11 + b22, b11, b12 - b22, b21 - b11, b22, b11 + b12, b21 + b22)]

    def stage_rhs(item, par, d0, tok):
        raw, jj = raw_b.at[item // 8 - 3], item % 8
        a = [raw[pl.ds((e * KH + d0) * 8 + jj, PB, stride=8), :] for e in range(2)]
        if tok is not None:
            tok = jnp.concatenate([pltpu.bitcast(tok, U32)] * (PB // 8), axis=0)
            a = [anchored(v, tok) for v in a]
        b11, b12, b21, b22 = _lo_f32(a[0]), _hi_f32(a[0]), _lo_f32(a[1]), _hi_f32(a[1])
        for p, e, b in ((0, 0, b11), (1, 0, b12), (0, 1, b21), (1, 1, b22)):
            u = _as_u32(b.astype(BF))
            wqkv[2 * item + p, pl.ds((e * KH + d0) // 2, PB // 2), :] = u
            if p == e:
                rs_u[par, p, d0 // 2:(d0 + PB) // 2, :] = u
        comb = [b11 + b22, b12 - b22, b21 - b11, b11 + b12, b21 + b22]
        rs_c[par, d0:d0 + PB, :] = jnp.concatenate(comb, axis=1).astype(BF)

    def staged_rhs(par):
        c = lambda i: (lambda: rs_c[par, :, 128 * i:128 * i + 128])
        return [c(0), lambda: _as_bf(rs_u[par, 0]), c(1), c(2), lambda: _as_bf(rs_u[par, 1]), c(3), c(4)]

    def strassen(rhs, q, item, init, keep, after_dot):
        def prod(i):
            lhs = sl[q, i] if q is not None else jnp.concatenate([sl[k, i] for k in range(NQ)], axis=1)
            return _dot(_as_bf(lhs), rhs[i]() if callable(rhs[i]) else rhs[i])

        def plus(i, r):
            return r if init is None else init(i) + r

        c12, c21 = (cb.at[5], cb.at[4]) if keep is None else (keep(1), keep(2))
        m = prod(1)
        cb[0] = m
        after_dot(0, m)
        m = prod(4)
        cb[1] = m
        after_dot(1, m)
        m1 = prod(0)
        cb[3] = plus(3, m1 - cb[0])
        cb[2] = plus(0, m1 - cb[1])
        after_dot(2, m1)
        m = prod(3)
        c21[...] = plus(2, cb[0] + m)
        cb[2] = cb[2] + m
        after_dot(3, m)
        m = prod(2)
        c12[...] = plus(1, cb[1] + m)
        cb[3] = cb[3] + m
        after_dot(4, m)
        for k, (i, acc) in enumerate(((6, 2), (5, 3))):
            m = prod(i) + cb[acc]
            if keep is not None:
                keep(3 * k)[...] = m
            store_st(item, k, *((m, c12[...]) if k == 0 else (c21[...], m)))
            after_dot(5 + k, m)

    def store_st(item, e, c1, c2):
        r = jnp.concatenate([c.reshape(NSEG // 2, 8, 128) for c in (c1, c2)], axis=1)
        st[item, 256 * e:256 * e + 256, :] = _as_u32(r.reshape(8 * NSEG, 128).astype(BF))

    def pin(i, c):
        cb[i, 0:8, :] = jnp.zeros((8, 128), F32)
        zero_s[i] = 0
        rs_u[i, 0, 0:8, :] = jnp.zeros((8, 128), U32)
        rs_c[i, 0:16, 0:128] = jnp.zeros((16, 128), BF)
        z_s[i, 0:8, :] = jnp.zeros((8, 128), U32)
        p_s[i, 0:8, :] = jnp.zeros((8, 128), F32)
        u_s[i, 0:8, :] = jnp.zeros((8, 128), U32)
        stg[i, 0, 0:8, :] = jnp.zeros((8, 128), U32)
        obuf[i, 0:8, :] = jnp.zeros((8, 128), U32)
        sto[i, 0:8, :] = jnp.zeros((8, 128), F32)
        lc[i, 0, 0:8, :] = jnp.zeros((8, 128), U32)
        mp[i, 0:8, :] = jnp.zeros((8, 128), F32)
        ts_s[pl.ds(pl.multiple_of(8 * i, 8), 8), 0:128] = jnp.zeros((8, 128), F32)
        ra_s[pl.ds(pl.multiple_of(8 * i, 8), 8), 0:128] = jnp.zeros((8, 128), F32)
        a_s[i, 0:8, 0:128] = jnp.zeros((8, 128), U32)
        pa_s[i, 0:8, :] = jnp.zeros((8, 128), F32)
        bb_s[pl.ds(pl.multiple_of(8 * i, 8), 8), 0:128] = jnp.zeros((8, 128), F32)
        g_s[pl.ds(pl.multiple_of(8 * i, 8), 8), :] = jnp.zeros((8, 128), F32)
        return c

    lax.fori_loop(0, 2, pin, 0)

    mf[0:80, :] = _mask80()
    fraw[4] = jnp.zeros(fraw.shape[1:], U32)

    wait(gf, SEM_GF)

    def f1(i, c):
        for a1 in range(4):
            wait(x_v.at[x_rows(i, a1), :], SEM_X + i)
        base = pl.multiple_of(i * RB, RB)
        alt = (1 - 2 * (_lanes(16) & 1)).astype(F32).astype(BF)

        def rows16(r):
            return jnp.concatenate([x_v[pl.ds(r + d, 16), :].astype(F32)[0:8] for d in (0, SEG)], axis=0)

        for r in (0, 64, QS, QS + 64):
            top, bot = rows16(base + r), rows16(base + (r + 2 * QS))
            a11, a12, a21, a22 = top[:, :KH], top[:, KH:], bot[:, :KH], bot[:, KH:]
            row = pl.multiple_of((base + r) // 8, 8)
            for k, v in enumerate((a11 + a22, a21 + a22, a11, a22, a11 + a12, a21 - a11, a12 - a22)):
                for q in range(NQ):
                    sl[q, k, pl.ds(row, 8), :] = _as_u32(v[:, q * KQ:(q + 1) * KQ].astype(BF))
        for h0 in range(0, RB, HB):
            pieces = []
            for a1 in range(4):
                for r in range(h0, h0 + HB, 16):
                    xs = x_v[pl.ds(base + (QS * a1 + r), 16), :].astype(F32)
                    pieces.append(jnp.concatenate(_bfly8([xs[:, 128 * a:128 * a + 128] for a in range(8)]),
                                                  axis=1))
                    z_s[a1, r // 2:r // 2 + 8, :] = _as_u32(pieces[-1][:, :128].astype(BF))
            ub = jnp.concatenate(pieces, axis=0)
            for g in range(4):
                yy = _dot(ub[:, 256 * g:256 * g + 256].astype(BF), _as_bf(gf[g]))
                v = _fft([(yy[HB * a1:HB * a1 + HB, :128], yy[HB * a1:HB * a1 + HB, 128:])
                          for a1 in range(4)], -1)
                for k1 in range(4):
                    rows = pl.ds(base + (QS * k1 + h0), HB)
                    y[g, 0, rows, :] = v[k1][0]
                    y[g, 1, rows, :] = v[k1][1]
                if h0 + HB == RB and g == 3:
                    for a1 in range(4):
                        xa[pl.ds(4 * a1 + i, 1), :] = _dot_nt(alt, _as_bf(z_s[a1]))[0:1]
        return c

    with jax.named_scope("f1"):
        lax.fori_loop(0, QS // RB, f1, 0)

    def fprep(src, h, c):
        ev, od = [], []
        for r in range(8):
            wr = fraw[src, 0, c, pl.ds(r, 32, stride=8), :]
            wi = fraw[src, 1, c, pl.ds(r, 32, stride=8), :]
            ev.append((wr & jnp.uint32(0xFFFF)) | (wi << 16))
            od.append((wr >> 16) | (wi & jnp.uint32(0xFFFF0000)))
        for g, cls in enumerate(CLASSES):
            t = _transpose_u32(jnp.concatenate([(od if k % 2 else ev)[k // 2] for k in cls], axis=0))
            for q in range(128 // N1):
                row = pl.multiple_of(((4 * h + c) * (128 // N1) + q) * PITCH, 8)
                fp[g, pl.ds(row, N1), :] = t[q * N1:(q + 1) * N1]

    def nyquist():
        twc, tws = sm[0:16], sm[16:32]
        u = _dot(sm[32:64, 0:16].astype(BF), xa[0:16, :].astype(BF))
        ur, ui = u[0:16], u[16:32]
        u = jnp.concatenate([ur * twc + ui * tws, ui * twc - ur * tws], axis=0).astype(BF)
        yield
        xx = _dot(u, _as_bf(nm[...]))
        xr, xi = xx[0:16, :128] + xx[16:32, 128:], xx[16:32, :128] - xx[0:16, 128:]
        w = (pltpu.bitcast(nyq[0].astype(F32), U32) >> 16) | pltpu.bitcast(nyq[1].astype(F32), U32)
        w = jnp.concatenate([w[:, 128 * a:128 * a + 128] for a in range(16)], axis=0)
        wt = _transpose_u32(jnp.concatenate([w] * 8, axis=0))
        blk = _lanes(16) >> 4
        wm = wt[0:16]
        for j in range(1, 8):
            wm = jnp.where(blk == j, wt[16 * j:16 * j + 16], wm)
        wr, wi = _lo_f32(wm), _hi_f32(wm)
        z = jnp.concatenate([xr * wr - xi * wi, xr * wi + xi * wr], axis=0).astype(BF)
        yield
        zc, zs = _dot_nt(z, _as_bf(nm[:, :128])), _dot_nt(z, _as_bf(nm[:, 128:]))
        pr, pi = zc[0:16] - zs[16:32], zs[0:16] + zc[16:32]
        pp = jnp.concatenate([pr * twc - pi * tws, pi * twc + pr * tws], axis=0).astype(BF)
        yield
        cc = _dot(sm[64:80, 0:32].astype(BF), pp) * (1.0 / (S * D))
        ct[...] = jnp.concatenate([cc, jnp.zeros((112, 128), F32)], axis=0).T
        yield

    def s_rows(k1, a0, r):
        return pl.ds(r + (QS * k1 + N2 * a0), 8)

    def anchored(v, tok):
        return jnp.where(zero_s[0] != 0, tok, v)

    def s_prep(g, k1, r, tok):
        v = [(y[g, 0, s_rows(k1, a0, r), :], y[g, 1, s_rows(k1, a0, r), :]) for a0 in range(8)]
        if tok is not None:
            v[0] = (anchored(v[0][0], tok), v[0][1])
        v = _fft([_cmul_const(v[a0], a0 * k1, N1, -1) for a0 in range(8)], -1)
        for k0 in range(8):
            u_s[k1 + 4 * k0, pl.ds(r, 8), :] = _as_u32(jnp.concatenate(v[k0], axis=0).astype(BF))

    def s_fwd(g, ka, tok):
        xx = _dot(_as_bf(gs[0, ka]), _as_bf(u_s[ka]))
        w32 = fp[g, pl.ds(ka, N2, stride=PITCH), :]
        wr, wi = _lo_f32(w32), _hi_f32(w32)
        xr, xi = xx[:N2], xx[N2:]
        z_s[ka] = _as_u32(jnp.concatenate([xr * wr - xi * wi, xr * wi + xi * wr], axis=0).astype(BF))

    def s_inv(ka, tok):
        p_s[ka] = _dot(_as_bf(gs[1, ka]), _as_bf(z_s[ka]))

    def s_post(g, k1, r, tok):
        v = [(p_s[k1 + 4 * k0, r:r + 8, :], p_s[k1 + 4 * k0, N2 + r:N2 + r + 8, :]) for k0 in range(8)]
        v[0] = (anchored(v[0][0], tok), anchored(v[0][1], tok))
        v = _fft(v, 1)
        for a0 in range(8):
            vr, vi = _cmul_const(v[a0], a0 * k1, N1, 1)
            v_s[g, 0, s_rows(k1, a0, r), :] = vr
            v_s[g, 1, s_rows(k1, a0, r), :] = vi

    def wc_block(c, jc):
        return raw_a.at[c // 2, pl.ds(pl.multiple_of(4096 * (c % 2) + 1024 * jc, 1024), 1024), :]

    def wo_comb(jc, p, r, tok):
        nr = 64 // WSP
        u = [wo[jc + 4 * f, 128 * p + 64 * e + r:128 * p + 64 * e + r + nr, :] for e in range(2) for f in range(2)]
        tok = jnp.concatenate([pltpu.bitcast(tok, U32)] * (nr // 8), axis=0)
        u[0], u[3] = anchored(u[0], tok), anchored(u[3], tok)
        b11, b12, b21, b22 = [_as_bf(v).astype(F32) for v in u]
        for c, v in enumerate((b11 + b22, b12 - b22, b21 - b11, b11 + b12, b21 + b22)):
            wc_block(c, jc)[64 * p + r:64 * p + r + nr, :] = _as_u32(v.astype(BF))

    def bulk(where, n, events, q=None):
        for i in range(n):
            ch, jj = where(i)

            def hook(k, m):
                pieces = events.get(7 * i + k, ())
                vec = [pc for pc in pieces if isinstance(pc, P) and pc.func in (s_prep, s_post, wo_comb, stage_rhs)]
                for piece in pieces:
                    r = 8 * ((32 * vec.index(piece)) // len(vec)) if piece in vec else 0
                    piece(m[r:r + 8])

            def keep(k):
                return v_s.at[jj // 4, (jj // 2) % 2, pl.ds(1024 * (jj % 2) + 256 * k, 256), :]

            def init(k):
                return jnp.where(q > 0, keep(k)[...], 0.0)

            rhs = staged_rhs(i % 2) if q is None else prep_rhs(ch, jj, pl.multiple_of(q * KQ, KQ))
            strassen(rhs, q, 8 * ch + jj,
                     None if q is None else init, None if q is None else keep, hook)

    def spread(events, pieces, q0, q1):
        for i, piece in enumerate(pieces):
            events.setdefault(q0 + ((q1 - q0) * i) // len(pieces), []).append(piece)

    P = functools.partial

    def loop_a(n, c):
        for e in range(2):
            wait(w_half(raw4[0].at[n // 2], n % 2, e), SEM_W0 + n)
        h = jnp.maximum(n - 2, 0)

        @pl.when(n >= 2)
        def _():
            wait(fraw.at[h], SEM_F + h)

        src = jnp.where(n >= 2, h, 4)
        events = {}
        spread(events, [lambda tok, c=c: fprep(src, h, c) for c in range(4)], 0, 48)
        bulk(lambda i: (n // 2, i), 8, events, n % 2)
        return c

    def loop_b(g, c):
        @pl.when((g >= 1) & (g < 3))
        def _():
            wait(raw4[1].at[g], SEM_W + 3 + g)

        for e in range(2):
            wait(wo.at[g + 4 * e], SEM_WO + g)
        gn = jnp.minimum(g + 1, 3)
        events = {}
        for k1 in range(4):
            q = BD * k1
            spread(events, [P(s_fwd, g, k1 + 4 * k0) for k0 in range(8)], q, q + BW)
            spread(events, [P(s_prep, gn, k1, r) for r in range(0, N2, 8)], q + BW, q + BW + BV)
            q += BL
            spread(events, [P(s_inv, k1 + 4 * k0) for k0 in range(8)], q, q + BW)
            spread(events, [P(s_post, g, k1, r) for r in range(0, N2, 8)], q + BW, q + BW + BV)
        spread(events, [P(wo_comb, g, p, r) for p in range(NP) for r in range(0, 64, 64 // WSP)], W0, W1)
        for i in range(6):
            nxt = jnp.minimum(24 + 6 * g + i + 1, 3 * NP - 1)
            spread(events, [P(stage_rhs, nxt, (i + 1) % 2, d0) for d0 in range(0, KH, PB)], 7 * i, 7 * i + SE)
        ny = nyquist()
        spread(events, [lambda tok: next(ny)] * 4, NY0, NY1)
        assert max(events) < 41
        bulk(lambda i: ((24 + 6 * g + i) // 8, (24 + 6 * g + i) % 8), 6, events)
        return c

    def prep0(i, c):
        for k1 in range(4):
            s_prep(0, k1, pl.multiple_of(i * 8, 8), None)
        return c

    lax.fori_loop(0, N2 // 8, prep0, 0)
    with jax.named_scope("loop_a"):
        lax.fori_loop(0, 6, loop_a, 0)
    wait(sm, SEM_SM)
    wait(nm, SEM_NYM)
    wait(nyq, SEM_NYQ)
    wait(gs, SEM_GS)
    with jax.named_scope("loop_b"):
        wait(raw4[1].at[0], SEM_W + 3)
        for d0 in range(0, KH, PB):
            stage_rhs(24, 0, d0, None)
        lax.fori_loop(0, 4, loop_b, 0)
    wait(gi, SEM_GI)
    wait(mem_ref, SEM_MEM)
    wait(gw_ref.at[pl.ds(0, D)], SEM_GW)

    scale = DH ** -0.5

    gw_s[...] = jnp.broadcast_to(gw_ref[pl.ds(0, D)].astype(F32).reshape(1, D), (8, D))

    def softmax(s):
        fill = mf[0:80, :]
        s = jnp.where(fill > 0.0, s * scale, fill)
        m = jnp.max(s, axis=-1, keepdims=True)
        e = jnp.exp(s - m)
        l = jnp.sum(e, axis=-1, keepdims=True)
        r = pl.reciprocal(l, approx=True)
        return (e * (r * (2.0 - l * r))).astype(BF)

    def lhs_rows(mem, seg):
        xs = x_v[pl.ds(pl.multiple_of(seg * SEG, SEG), SEG), :].astype(F32)
        return jnp.concatenate([mem, xs[8:SEG]], axis=0).astype(BF)

    def proj2(a, m, j):
        return jnp.concatenate([_dot(_as_bf(a[...]), _as_bf(wqkv[H * m + 2 * j + p])).astype(BF)
                                for p in range(2)], axis=0)

    def proj_lo(a):
        for i in range(6):
            pa_s[i] = _dot(_as_bf(a[:, :KH]), _as_bf(wqkv[H * (i // 2) + i % 2, 0:KH // 2, :]))

    def proj_hi(a):
        full = [(_dot(_as_bf(a[:, KH:]), _as_bf(wqkv[H * (i // 2) + i % 2, KH // 2:KH, :]))
                 + pa_s[i]).astype(BF) for i in range(6)]
        for m in range(3):
            stg[m, 0] = _as_u32(jnp.concatenate(full[2 * m:2 * m + 2], axis=0))

    def step(a, seg, k, hooks, late):
        srow = pl.multiple_of(seg * 8, 8)
        a = a[...]

        def get(m, j):
            return _as_bf(jnp.concatenate([stg[m, j % 8], st[NP * m + j, pl.ds(srow, 8), :]], axis=0))

        def proj(j, m):
            if j > 0:
                stg[m, j % 8] = _as_u32(proj2(a, m, j))
            elif m == 0:
                if k > 0:
                    proj_lo(a)
                proj_hi(a)

        def scores(j):
            pst[j % 8] = _as_u32(softmax(_dot_nt(get(0, j), get(1, j))))

        def pv(j):
            o = _dot(_as_bf(pst[j % 8]), get(2, j))
            if k < 3:
                for i in range(2):
                    sto[2 * j + i, 8 * k:8 * k + 8, :] = o[64 + 8 * i:72 + 8 * i]
                    obuf[2 * j + i] = _as_u32(o[32 * i:32 * i + 32].astype(BF))
            else:
                a11, a12 = o[0:32], o[32:64]
                a21, a22 = [jnp.concatenate([sto[2 * j + i, 0:24, :], o[64 + 8 * i:72 + 8 * i]], axis=0)
                            for i in range(2)]
                for i, v in enumerate((a11 + a22, a21 + a22, a11, a22, a11 + a12, a21 - a11, a12 - a22)):
                    lc[i, j] = _as_u32(v.astype(BF))

        def wo_part(j, h0, h1):
            og = jnp.concatenate([_as_bf(obuf[h]) for h in range(h0, h1)], axis=1)
            return _dot(og, _as_bf(wo[j, h0 * 64:h1 * 64, :]))

        def prod(i, jc, p0, p1):
            lhs = jnp.concatenate([_as_bf(lc[i, p]) for p in range(p0, p1)], axis=1)
            if i in (1, 4):
                e = i // 4
                rhs = jnp.concatenate([wo[jc + 4 * e, 128 * p + 64 * e:128 * p + 64 * e + 64, :]
                                       for p in range(p0, p1)], axis=0)
            else:
                rhs = wc_block((0, None, 1, 2, None, 3, 4)[i], jc)[64 * p0:64 * p1, :]
            return _dot(lhs, _as_bf(rhs))

        early = [(i, jc) for i in (0, 3, 4, 6) for jc in range(4)]
        parts = []
        for i in range(NP + 4):
            for ch in ORDER:
                if ch in "qkv":
                    m = "qkv".index(ch)
                    if i < NP:
                        proj(i, m)
                    elif m < 2:
                        for n in range(1 if k < 3 else 2):
                            r = wo_part(len(parts), 0, SPLIT) if k < 3 else prod(*early[len(parts)], 0, SP3)
                            mp[len(parts)] = r
                            parts.append(r[0:8])
                elif ch == "s" and 0 <= i - LAG1 < NP:
                    scores(i - LAG1)
                elif ch == "p" and 0 <= i - LAG2 < NP:
                    pv(i - LAG2)
            if i == HOOK_AT:
                for hook in hooks[k]:
                    hook()
        if k < 3:
            return jnp.concatenate([wo_part(j, SPLIT, H) + mp[j] for j in range(8)], axis=1)
        toks, c11, c12 = parts[T0:], [], []
        for jc in range(4):
            m1, m4, m5 = [prod(i, jc, SP3, NP) + mp[4 * n + jc] for n, i in enumerate((0, 3, 4))]
            c11.append(prod(6, jc, SP3, NP) + (mp[12 + jc] + (m1 + m4 - m5)))
            mp[jc], mp[4 + jc], mp[8 + jc] = m1, m4, m5
            toks += [m1[0:8]] * (jc % 2)
        for jc in range(4):
            m3 = prod(2, jc, 0, NP)
            c12.append(m3 + mp[8 + jc])
            mp[jc] = mp[jc] + m3
            toks.append(m3[0:8])
        for n, piece in enumerate(late):
            piece(toks[(n * len(toks)) // len(late)])
        c21 = []
        for jc in range(4):
            m2 = prod(1, jc, 0, NP)
            c21.append(m2 + mp[4 + jc])
            mp[jc] = mp[jc] - m2
        c22 = [prod(5, jc, 0, NP) + mp[jc] for jc in range(4)]
        return jnp.concatenate(c11 + c12, axis=1), jnp.concatenate(c21 + c22, axis=1)

    def start_quad(mem, u):
        a_s[0] = _as_u32(lhs_rows(mem, 4 * u))
        proj_lo(a_s.at[0])

    def quad(u, c):
        base = pl.multiple_of(u * 128, 128)
        roll = lambda v: pltpu.roll(v, 64, 1)
        a1 = u // 4
        s2 = (1 - 2 * (a1 & 1)).astype(F32)
        sg = (1 - (a1 & 2)).astype(F32)
        cc, ss = sg * (1 - (a1 & 1)).astype(F32), sg * (a1 & 1).astype(F32)

        def irfft_dots(r0):
            off = pl.multiple_of((u % 4) * 128, 128) + r0
            for g in range(4):
                q = [[v_s[g, e, pl.ds(off + QS * k1, SEG), :] for e in range(2)] for k1 in range(4)]
                br, bi = q[1][0] + s2 * q[3][0], q[1][1] + s2 * q[3][1]
                vr = q[0][0] + s2 * q[2][0] + (cc * br - ss * bi)
                vi = q[0][1] + s2 * q[2][1] + (cc * bi + ss * br)
                tin = _half_pre(vr, vi, _lanes(SEG) < 64, roll, jnp.where)
                for e in range(2):
                    ts_s[r0:r0 + SEG, 128 * (2 * g + e):128 * (2 * g + e + 1)] = _dot(
                        tin[e].astype(BF), _as_bf(gi[2 * g + e]))

        def mix(r0, tok):
            lane = _lanes(8)
            t = [anchored(ts_s[r0:r0 + 8, 128 * i:128 * i + 128], tok) for i in range(8)]
            nyc = jnp.sum(jnp.where(lane == u, anchored(ct[r0:r0 + 8, :], tok), 0.0), axis=-1, keepdims=True)
            t[0] = t[0] + nyc * (1 - 2 * (lane & 1)).astype(F32)
            t = sum([list(_half_post(g, t[2 * g], t[2 * g + 1], lane < 64, roll, jnp.where))
                     for g in range(4)], [])
            b = jnp.concatenate(_bfly8_t(t), axis=1).astype(BF).astype(F32)
            xg = x_v[pl.ds(base + r0, 8), :].astype(F32) * gw_s[...]
            xg = functools.reduce(jnp.add, [xg[:, 128 * i:128 * i + 128] for i in range(8)])
            gate = jax.nn.sigmoid(jnp.sum(anchored(xg, tok), axis=-1, keepdims=True))
            bb = (1.0 - gate) * b
            if r0 % SEG and r0 < 96:
                out_v[pl.ds(base + r0, 8), :] = (bb + gate * ra_s[r0:r0 + 8, :]).astype(BF)
            else:
                bb_s[r0:r0 + 8, :] = bb
                g_s[r0:r0 + 8, :] = jnp.broadcast_to(gate, (8, 128))

        hooks = [[P(irfft_dots, SEG * n) for n in range(4) if HMAP[n] == str(k)] for k in range(4)]
        late = [P(mix, r0) for r0 in range(0, 128, 8)]
        for k in range(3):
            res = step(a_s.at[k % 2], 4 * u + k, k, hooks, late)
            ra_s[32 * k + 8:32 * k + 32, :] = res[8:32]
            a_s[(k + 1) % 2] = _as_u32(lhs_rows(res[0:8], 4 * u + k + 1))
        res, first8 = step(a_s.at[1], 4 * u + 3, 3, hooks, late)

        def emit(r0, n, att):
            out_v[pl.ds(base + r0, n), :] = (
                bb_s[r0:r0 + n, :] + jnp.concatenate([g_s[r0:r0 + n, :]] * 8, axis=1) * att).astype(BF)

        emit(104, 24, res[8:32])
        for k in range(4):
            emit(32 * k, 8, first8[8 * k:8 * k + 8])
        pltpu.make_async_copy(out_v.at[pl.ds(base, 128), :], out_hbm.at[pl.ds(base, 128), :],
                              sem.at[SEM_OUT]).start()
        start_quad(res[0:8], jnp.minimum(u + 1, S // 128 - 1))
        return c

    with jax.named_scope("chain"):
        start_quad(mem_ref[...].astype(F32), 0)
        lax.fori_loop(0, S // 128, quad, 0)
    pltpu.make_async_copy(out_v, out_hbm, sem.at[SEM_OUT]).wait()


@jax.jit
def pallas_gated_mix__memory_aug_recurrent_mem_tr__spectral_gfnet__prompt_kernel(
    A_x, A_mem0, A_Wq, A_Wk, A_Wv, A_Wo, A_seg_len, B_x, B_w_r, B_w_i, gate_w,
):
    assert A_x.shape == (1, S, D) and A_mem0.shape == (1, M, D) and A_Wq.shape == (D, H, DH)
    consts = [jnp.asarray(c) for c in _constants()]
    any_spec = pl.BlockSpec(memory_space=pl.ANY)
    out = pl.pallas_call(
        _kernel,
        out_shape=jax.ShapeDtypeStruct((S, D), BF),
        in_specs=[any_spec] * 14,
        out_specs=any_spec,
        scratch_shapes=[
            pltpu.VMEM((S, D), BF),
            pltpu.VMEM((3, D * 8, DH), U32),
            pltpu.VMEM((3, D * 8, DH), U32),
            pltpu.VMEM((3 * H, D // 2, DH), U32),
            pltpu.VMEM((8, H * DH // 2, 128), U32),
            pltpu.VMEM((3 * NP, 8 * NSEG, 128), U32),
            pltpu.VMEM((NQ, 7, 2 * NSEG, D // 2 // NQ), U32),
            pltpu.VMEM((5, 2, 4, 256, 128), U32),
            pltpu.VMEM((4, N2 * PITCH, 128), U32),
            pltpu.VMEM((4, 128, 256), U32),
            pltpu.VMEM((64, 256), U32),
            pltpu.VMEM((8, 64, 128), U32),
            pltpu.VMEM((2, N1, N2, 2 * N2), U32),
            pltpu.VMEM((4, 2, S, 128), F32),
            pltpu.VMEM((4, 2, S, 128), F32),
            pltpu.VMEM((S, D), BF),
            pltpu.VMEM((N1, N2, 128), U32),
            pltpu.VMEM((6, 256, 128), F32),
            pltpu.VMEM((N1, N2, 128), U32),
            pltpu.VMEM((N1, 2 * N2, 128), F32),
            pltpu.VMEM((2, 2, D // 4, 128), U32),
            pltpu.VMEM((2, D // 2, 5 * 128), BF),
            pltpu.VMEM((H, 32, 128), F32),
            pltpu.VMEM((H, 16, 128), U32),
            pltpu.VMEM((128, 128), F32),
            pltpu.VMEM((2, 16, D), U32),
            pltpu.VMEM((6, 32, 128), F32),
            pltpu.VMEM((128, D), F32),
            pltpu.VMEM((128, 128), F32),
            pltpu.VMEM((3, 8, 32, 128), U32),
            pltpu.VMEM((8, 40, 80), U32),
            pltpu.VMEM((128, D), F32),
            pltpu.VMEM((128, D), F32),
            pltpu.VMEM((16, 32, 128), F32),
            pltpu.VMEM((7, NP, 16, 128), U32),
            pltpu.VMEM((8, D), F32),
            pltpu.VMEM((M, D), BF),
            pltpu.VMEM((96, 80), F32),
            pltpu.VMEM((96, 128), F32),
            pltpu.VMEM((32, 128), F32),
            pltpu.VMEM((2, 1, S), BF),
            pltpu.VMEM((8 * D,), BF),
            pltpu.SMEM((2,), jnp.int32),
            pltpu.SemaphoreType.DMA((NSEM,)),
        ],
        compiler_params=pltpu.CompilerParams(vmem_limit_bytes=120 * 1024 * 1024,
                                             disable_bounds_checks=True,
                                             disable_semaphore_checks=True),
    )(
        A_x.reshape(S, D), A_mem0.reshape(M, D), A_Wq, A_Wk, A_Wv,
        A_Wo.reshape(H * DH, D), B_w_r.T, B_w_i.T, gate_w, *consts,
    )
    return out.reshape(1, S, D)
```

```python
import functools
import math

import numpy as np
import jax
import jax.numpy as jnp
from jax import lax
import jax.experimental.pallas as pl
import jax.experimental.pallas.tpu as pltpu

BF, F32, U32 = jnp.bfloat16, jnp.float32, jnp.uint32

S, D, H, DH, M, SEG = 2048, 1024, 32, 128, 8, 32
NSEG = S // SEG
NP = H // 2
N1, N2 = 32, 64
QS = S // 4
PITCH = N1 + 8
CLASSES = ((0, 8, 4, 12), (1, 15, 9, 7), (2, 14, 10, 6), (3, 13, 11, 5))
LAG1, LAG2, SPLIT, HOOK_AT = 1, 2, 27, 18
ORDER = "qksvp"
PB, SE = 16, 6
WSP, W0, W1 = 8, 0, 40
T0 = 6
HMAP = "0123"
SP3 = 13
NY0, NY1 = 32, 40
BD, BW, BV, BL = 7, 8, 8, 3
NQ = 2
(SEM_W, SEM_GF, SEM_GI, SEM_SM, SEM_GS, SEM_NYQ, SEM_NYM, SEM_MEM, SEM_GW, SEM_OUT, SEM_F, SEM_X,
 SEM_W0) = 0, 6, 7, 8, 9, 10, 11, 12, 13, 14, 15, 19, 23
SEM_WO = SEM_W0 + 6
NSEM = SEM_WO + 4
RSQ2 = float(np.float32(math.sqrt(0.5)))


def _bfly8(x):
    s = [x[i] + x[i + 4] for i in range(4)]
    d = [x[i] - x[i + 4] for i in range(4)]
    e, f = s[0] + s[2], s[1] + s[3]
    t1, t2 = (d[1] - d[3]) * RSQ2, (d[1] + d[3]) * RSQ2
    return [e + f, e - f, d[0] + t1, t2 + d[2], s[0] - s[2], s[1] - s[3], d[0] - t1, t2 - d[2]]


def _bfly8_t(t):
    e, f = t[0] + t[1], t[0] - t[1]
    s = [e + t[4], f + t[5], e - t[4], f - t[5]]
    t1, t2 = t[2] - t[6], t[3] + t[7]
    d = [t[2] + t[6], (t1 + t2) * RSQ2, t[3] - t[7], (t2 - t1) * RSQ2]
    return [s[i] + d[i] for i in range(4)] + [s[i] - d[i] for i in range(4)]


def _half_pre(vr, vi, lo, roll, where):
    ri = roll(vi)
    return where(lo, vr, ri), where(lo, ri, vr)


def _half_post(g, tp, tm, lo, roll, where):
    if g == 0:
        return tp, tm
    c = float(np.float32(math.cos(math.pi * g / 8)))
    s = float(np.float32(math.sin(math.pi * g / 8)))
    p, r = tp + tm, tp - tm
    rm = roll(where(lo, r, p))
    return where(lo, p, c * rm + s * r), where(lo, rm, c * r - s * rm)


def _cmul_const(v, k, n, sign):
    re, im = v
    k %= n
    if k == 0:
        return re, im
    if 4 * k == n:
        return (-im, re) if sign > 0 else (im, -re)
    if 8 * k == n:
        return (((re - im) * RSQ2, (re + im) * RSQ2) if sign > 0
                else ((re + im) * RSQ2, (im - re) * RSQ2))
    if 8 * k == 3 * n:
        return (((re + im) * -RSQ2, (re - im) * RSQ2) if sign > 0
                else ((im - re) * RSQ2, (re + im) * -RSQ2))
    c, s = math.cos(2 * math.pi * k / n), sign * math.sin(2 * math.pi * k / n)
    return re * c - im * s, re * s + im * c


def _fft(v, sign):
    n = len(v)
    if n == 1:
        return v
    ev, od = _fft(v[0::2], sign), _fft(v[1::2], sign)
    lo, hi = [], []
    for k in range(n // 2):
        er, ei = ev[k]
        if 4 * k == n:
            xr, xi = od[k]
            if sign > 0:
                lo.append((er - xi, ei + xr)); hi.append((er + xi, ei - xr))
            else:
                lo.append((er + xi, ei - xr)); hi.append((er - xi, ei + xr))
            continue
        tr, ti = _cmul_const(od[k], k, n, sign)
        lo.append((er + tr, ei + ti))
        hi.append((er - tr, ei - ti))
    return lo + hi


def _pack_rows(a):
    u = np.ascontiguousarray(a, dtype=np.float32).view(np.uint32)
    b = ((u + 0x7FFF + ((u >> 16) & 1)) >> 16).astype(np.uint32)
    return (b[..., 0::2, :] | (b[..., 1::2, :] << 16)).astype(np.uint32)


def _diag_blocks(full, n, tol):
    k = full.shape[0] // n
    blk = np.kron(np.eye(k), np.ones((n, n)))
    assert np.abs(full * (1 - blk)).max() < tol
    return np.stack([full[n * g:n * g + n, n * g:n * g + n] for g in range(k)])


@functools.lru_cache(maxsize=None)
def _constants():
    k2 = np.stack([np.concatenate([c + 16 * np.arange(32) for c in cls]) for cls in CLASSES])
    n2 = np.arange(D)
    ang = 2 * np.pi * ((k2[:, :, None] * n2[None, None, :]) % D) / D
    rows = np.stack([np.cos(ang), -np.sin(ang)], axis=1)
    wgt = np.where(k2 == 0, 1.0, 2.0)[:, None, :, None]
    fwd = rows.reshape(D, D).T
    inv = (rows * wgt).reshape(D, D) / (S * D)
    bf = np.stack(_bfly8(list(np.eye(8))))
    binv = np.kron(np.linalg.inv(bf), np.eye(128))
    gd = _diag_blocks(binv.T @ fwd, 256, 1e-6)
    gdi = _diag_blocks(inv @ binv, 256, 1e-12)
    eye, lo = np.eye(256), np.arange(128) < 64
    roll = lambda v: np.roll(v, 64, axis=1)
    pre = np.concatenate(_half_pre(eye[:, :128], eye[:, 128:], lo, roll, np.where), axis=1)
    gi = []
    for g in range(4):
        post = np.concatenate(_half_post(g, eye[:, :128], eye[:, 128:], lo, roll, np.where), axis=1)
        gi.append(_diag_blocks(np.linalg.inv(pre) @ gdi[g] @ np.linalg.inv(post), 128, 1e-12))
    gi = np.concatenate(gi)

    b = np.arange(N2)
    k1 = np.arange(N1)[:, None] + N1 * np.arange(N2)[None, :]
    th = 2 * np.pi * ((k1[:, :, None] * b[None, None, :]) % S) / S
    gr, gim = np.cos(th), -np.sin(th)
    gs = np.block([[gr, -gim], [gim, gr]])
    hr, hi = np.swapaxes(gr, 1, 2), -np.swapaxes(gim, 1, 2)
    gsi = np.block([[hr, -hi], [hi, hr]])

    lane = np.arange(128)
    kb = 8 * (lane % 16) + lane // 16
    t128 = 2 * np.pi * ((lane[:, None] * kb[None, :]) % 128) / 128
    nym = np.concatenate([np.cos(t128), np.sin(t128)], axis=1)
    i16 = np.arange(16)
    t16 = 2 * np.pi * ((i16[:, None] * i16[None, :]) % 16) / 16
    tw = 2 * np.pi * (i16[:, None] * lane[None, :]) / S
    sm = np.zeros((96, 128), np.float32)
    sm[0:16], sm[16:32] = np.cos(tw), np.sin(tw)
    sm[32:48, :16], sm[48:64, :16] = np.cos(t16), -np.sin(t16)
    sm[64:80, :16], sm[64:80, 16:32] = np.cos(t16), -np.sin(t16)

    return _pack_rows(gd), _pack_rows(nym), _pack_rows(gi), sm, _pack_rows(np.stack([gs, gsi]))


def _mask80():
    r = lax.broadcasted_iota(jnp.int32, (80, 80), 0)
    c = lax.broadcasted_iota(jnp.int32, (80, 80), 1)

    def head(i):
        return jnp.where(i < 64, i >> 5, (i - 64) >> 3)

    def pos(i):
        j = i & 31
        return jnp.where(i < 64, jnp.where(j < M, j, j + 8), M + (i & 7))

    same = head(r) == head(c)
    ok = (pos(r) < M) | (pos(c) <= pos(r))
    return jnp.where(same, jnp.where(ok, 1.0, -1e9), -jnp.inf).astype(F32)


def _as_bf(u):
    return pltpu.bitcast(u, BF)


def _as_u32(b):
    return pltpu.bitcast(b, U32)


def _lo_f32(u):
    return pltpu.bitcast(u << 16, F32)


def _hi_f32(u):
    return pltpu.bitcast(u & jnp.uint32(0xFFFF0000), F32)


def _dot(a, b):
    return jnp.dot(a, b, preferred_element_type=F32)


def _dot_nt(a, b):
    return lax.dot_general(a, b, (((1,), (1,)), ((), ())), preferred_element_type=F32)


def _transpose_u32(u):
    return pltpu.bitcast(pltpu.bitcast(u, F32).T, U32)


def _lanes(rows):
    return lax.broadcasted_iota(jnp.int32, (rows, 128), 1)


def _kernel(x_hbm, mem_hbm, wq_hbm, wk_hbm, wv_hbm, wo_hbm, fr_hbm, fi_hbm, gw_hbm,
            gf_hbm, nm_hbm, gi_hbm, sm_hbm, gs_hbm,
            out_hbm,
            x_v, raw_a, raw_b, wqkv, wo, st, sl, fraw, fp, gf, nm, gi, gs, y, v_s, out_v, cb, z_s, p_s, rs_u, rs_c, u_b, z_b,
            sto, obuf, ct, a_s, pa_s, bb_s, g_s, stg, pst, ra_s, ts_s, mp, lc, gw_s, mem_ref, mf, sm, xa, nyq, gw_ref, zero_s, sem):
    KH = D // 2
    KQ = KH // NQ
    RB, HB = 128, 16
    raw4 = [r.reshape(3, D, 8, DH) for r in (raw_a, raw_b)]
    w_hbm = (wq_hbm, wk_hbm, wv_hbm)
    f_hbm = (fr_hbm, fi_hbm)

    def w_src(c):
        return w_hbm[c // 2].bitcast(U32).at[:, pl.ds(8 * (c % 2), 8), :]

    def wait(dst, k):
        pltpu.make_async_copy(dst, dst, sem.at[k]).wait()

    def w_half(ref, q, e):
        return ref.at[pl.ds(pl.multiple_of(q * KQ, KQ) + e * KH, KQ)]

    def x_rows(i, a1):
        return pl.ds(pl.multiple_of(i * RB, RB) + QS * a1, RB)

    def f_copies(h):
        return [(f_hbm[a].at[pl.ds(0, D // 2), pl.ds(128 * (4 * h + c), 128)].bitcast(U32),
                 fraw.at[h, a, c], SEM_F + h) for a in range(2) for c in range(4)]

    def w_copy(c):
        return [(w_src(c), raw4[1].at[c - 3], SEM_W + c)]

    copies = [(gf_hbm, gf, SEM_GF)]
    copies += [(x_hbm.at[x_rows(i, a1), :], x_v.at[x_rows(i, a1), :], SEM_X + i)
               for i in range(QS // RB) for a1 in range(4)]
    for n in range(6):
        copies += [(w_half(w_src(n // 2), n % 2, e), w_half(raw4[0].at[n // 2], n % 2, e), SEM_W0 + n)
                   for e in range(2)]
        if n >= 2:
            copies += f_copies(n - 2)
    copies += [(sm_hbm, sm, SEM_SM), (nm_hbm, nm, SEM_NYM)]
    copies += [(f_hbm[a].at[pl.ds(D // 2, 1), :], nyq.at[a], SEM_NYQ) for a in range(2)]
    copies += [(gs_hbm, gs, SEM_GS)]
    for g in range(4):
        copies += w_copy(3 + g) if g < 3 else []
        copies += [(wo_hbm.bitcast(U32).at[:, pl.ds(128 * j, 128)], wo.at[j], SEM_WO + g) for j in (g, g + 4)]
    copies += [(gi_hbm, gi, SEM_GI), (mem_hbm, mem_ref, SEM_MEM), (gw_hbm, gw_ref.at[pl.ds(0, D)], SEM_GW)]
    for src, dst, k in copies:
        pltpu.make_async_copy(src, dst, sem.at[k]).start()

    def prep_rhs(ch, jj, k0):
        a1 = raw_a[ch, pl.ds(k0 * 8 + jj, KQ, stride=8), :]
        a2 = raw_a[ch, pl.ds((KH + k0) * 8 + jj, KQ, stride=8), :]
        b11, b12, b21, b22 = _lo_f32(a1), _hi_f32(a1), _lo_f32(a2), _hi_f32(a2)
        for p, e, b in ((0, 0, b11), (1, 0, b12), (0, 1, b21), (1, 1, b22)):
            row = pl.multiple_of(k0 // 2, KQ // 2) + e * KH // 2
            wqkv[2 * (8 * ch + jj) + p, pl.ds(row, KQ // 2), :] = _as_u32(b.astype(BF))
        return [v.astype(BF) for v in (b11 + b22, b11, b12 - b22, b21 - b11, b22, b11 + b12, b21 + b22)]

    def stage_rhs(item, par, d0, tok):
        raw, jj = raw_b.at[item // 8 - 3], item % 8
        a = [raw[pl.ds((e * KH + d0) * 8 + jj, PB, stride=8), :] for e in range(2)]
        if tok is not None:
            tok = jnp.concatenate([pltpu.bitcast(tok, U32)] * (PB // 8), axis=0)
            a = [anchored(v, tok) for v in a]
        b11, b12, b21, b22 = _lo_f32(a[0]), _hi_f32(a[0]), _lo_f32(a[1]), _hi_f32(a[1])
        for p, e, b in ((0, 0, b11), (1, 0, b12), (0, 1, b21), (1, 1, b22)):
            u = _as_u32(b.astype(BF))
            wqkv[2 * item + p, pl.ds((e * KH + d0) // 2, PB // 2), :] = u
            if p == e:
                rs_u[par, p, d0 // 2:(d0 + PB) // 2, :] = u
        comb = [b11 + b22, b12 - b22, b21 - b11, b11 + b12, b21 + b22]
        rs_c[par, d0:d0 + PB, :] = jnp.concatenate(comb, axis=1).astype(BF)

    def staged_rhs(par):
        c = lambda i: (lambda: rs_c[par, :, 128 * i:128 * i + 128])
        return [c(0), lambda: _as_bf(rs_u[par, 0]), c(1), c(2), lambda: _as_bf(rs_u[par, 1]), c(3), c(4)]

    def strassen(rhs, q, item, init, keep, after_dot):
        def prod(i):
            lhs = sl[q, i] if q is not None else jnp.concatenate([sl[k, i] for k in range(NQ)], axis=1)
            return _dot(_as_bf(lhs), rhs[i]() if callable(rhs[i]) else rhs[i])

        def plus(i, r):
            return r if init is None else init(i) + r

        c12, c21 = (cb.at[5], cb.at[4]) if keep is None else (keep(1), keep(2))
        m = prod(1)
        cb[0] = m
        after_dot(0, m)
        m = prod(4)
        cb[1] = m
        after_dot(1, m)
        m1 = prod(0)
        cb[3] = plus(3, m1 - cb[0])
        cb[2] = plus(0, m1 - cb[1])
        after_dot(2, m1)
        m = prod(3)
        c21[...] = plus(2, cb[0] + m)
        cb[2] = cb[2] + m
        after_dot(3, m)
        m = prod(2)
        c12[...] = plus(1, cb[1] + m)
        cb[3] = cb[3] + m
        after_dot(4, m)
        for k, (i, acc) in enumerate(((6, 2), (5, 3))):
            m = prod(i) + cb[acc]
            if keep is not None:
                keep(3 * k)[...] = m
            store_st(item, k, *((m, c12[...]) if k == 0 else (c21[...], m)))
            after_dot(5 + k, m)

    def store_st(item, e, c1, c2):
        r = jnp.concatenate([c.reshape(NSEG // 2, 8, 128) for c in (c1, c2)], axis=1)
        st[item, 256 * e:256 * e + 256, :] = _as_u32(r.reshape(8 * NSEG, 128).astype(BF))

    def pin(i, c):
        cb[i, 0:8, :] = jnp.zeros((8, 128), F32)
        zero_s[i] = 0
        z_b[i, 0:16, 0:128] = jnp.zeros((16, 128), BF)
        rs_u[i, 0, 0:8, :] = jnp.zeros((8, 128), U32)
        rs_c[i, 0:16, 0:128] = jnp.zeros((16, 128), BF)
        z_s[i, 0:8, :] = jnp.zeros((8, 128), U32)
        p_s[i, 0:8, :] = jnp.zeros((8, 128), F32)
        stg[i, 0, 0:8, :] = jnp.zeros((8, 128), U32)
        obuf[i, 0:8, :] = jnp.zeros((8, 128), U32)
        sto[i, 0:8, :] = jnp.zeros((8, 128), F32)
        lc[i, 0, 0:8, :] = jnp.zeros((8, 128), U32)
        mp[i, 0:8, :] = jnp.zeros((8, 128), F32)
        ts_s[pl.ds(pl.multiple_of(8 * i, 8), 8), 0:128] = jnp.zeros((8, 128), F32)
        ra_s[pl.ds(pl.multiple_of(8 * i, 8), 8), 0:128] = jnp.zeros((8, 128), F32)
        a_s[i, 0:8, 0:128] = jnp.zeros((8, 128), U32)
        pa_s[i, 0:8, :] = jnp.zeros((8, 128), F32)
        bb_s[pl.ds(pl.multiple_of(8 * i, 8), 8), 0:128] = jnp.zeros((8, 128), F32)
        g_s[pl.ds(pl.multiple_of(8 * i, 8), 8), :] = jnp.zeros((8, 128), F32)
        return c

    lax.fori_loop(0, 2, pin, 0)

    mf[0:80, :] = _mask80()
    fraw[4] = jnp.zeros(fraw.shape[1:], U32)

    wait(gf, SEM_GF)

    def f1(i, c):
        for a1 in range(4):
            wait(x_v.at[x_rows(i, a1), :], SEM_X + i)
        base = pl.multiple_of(i * RB, RB)
        alt = (1 - 2 * (_lanes(16) & 1)).astype(F32).astype(BF)

        def rows16(r):
            return jnp.concatenate([x_v[pl.ds(r + d, 16), :].astype(F32)[0:8] for d in (0, SEG)], axis=0)

        for r in (0, 64, QS, QS + 64):
            top, bot = rows16(base + r), rows16(base + (r + 2 * QS))
            a11, a12, a21, a22 = top[:, :KH], top[:, KH:], bot[:, :KH], bot[:, KH:]
            row = pl.multiple_of((base + r) // 8, 8)
            for k, v in enumerate((a11 + a22, a21 + a22, a11, a22, a11 + a12, a21 - a11, a12 - a22)):
                for q in range(NQ):
                    sl[q, k, pl.ds(row, 8), :] = _as_u32(v[:, q * KQ:(q + 1) * KQ].astype(BF))
        for h0 in range(0, RB, HB):
            pieces = []
            for a1 in range(4):
                for r in range(h0, h0 + HB, 16):
                    xs = x_v[pl.ds(base + (QS * a1 + r), 16), :].astype(F32)
                    pieces.append(jnp.concatenate(_bfly8([xs[:, 128 * a:128 * a + 128] for a in range(8)]),
                                                  axis=1))
                    z_s[a1, r // 2:r // 2 + 8, :] = _as_u32(pieces[-1][:, :128].astype(BF))
            ub = jnp.concatenate(pieces, axis=0)
            for g in range(4):
                yy = _dot(ub[:, 256 * g:256 * g + 256].astype(BF), _as_bf(gf[g]))
                v = _fft([(yy[HB * a1:HB * a1 + HB, :128], yy[HB * a1:HB * a1 + HB, 128:])
                          for a1 in range(4)], -1)
                for k1 in range(4):
                    rows = pl.ds(base + (QS * k1 + h0), HB)
                    y[g, 0, rows, :] = v[k1][0]
                    y[g, 1, rows, :] = v[k1][1]
                if h0 + HB == RB and g == 3:
                    for a1 in range(4):
                        xa[pl.ds(4 * a1 + i, 1), :] = _dot_nt(alt, _as_bf(z_s[a1]))[0:1]
        return c

    with jax.named_scope("f1"):
        lax.fori_loop(0, QS // RB, f1, 0)

    def fprep(src, h, c):
        ev, od = [], []
        for r in range(8):
            wr = fraw[src, 0, c, pl.ds(r, 32, stride=8), :]
            wi = fraw[src, 1, c, pl.ds(r, 32, stride=8), :]
            ev.append((wr & jnp.uint32(0xFFFF)) | (wi << 16))
            od.append((wr >> 16) | (wi & jnp.uint32(0xFFFF0000)))
        for g, cls in enumerate(CLASSES):
            t = _transpose_u32(jnp.concatenate([(od if k % 2 else ev)[k // 2] for k in cls], axis=0))
            for q in range(128 // N1):
                row = pl.multiple_of(((4 * h + c) * (128 // N1) + q) * PITCH, 8)
                fp[g, pl.ds(row, N1), :] = t[q * N1:(q + 1) * N1]

    def nyquist():
        twc, tws = sm[0:16], sm[16:32]
        u = _dot(sm[32:64, 0:16].astype(BF), xa[0:16, :].astype(BF))
        ur, ui = u[0:16], u[16:32]
        u = jnp.concatenate([ur * twc + ui * tws, ui * twc - ur * tws], axis=0).astype(BF)
        yield
        xx = _dot(u, _as_bf(nm[...]))
        xr, xi = xx[0:16, :128] + xx[16:32, 128:], xx[16:32, :128] - xx[0:16, 128:]
        w = (pltpu.bitcast(nyq[0].astype(F32), U32) >> 16) | pltpu.bitcast(nyq[1].astype(F32), U32)
        w = jnp.concatenate([w[:, 128 * a:128 * a + 128] for a in range(16)], axis=0)
        wt = _transpose_u32(jnp.concatenate([w] * 8, axis=0))
        blk = _lanes(16) >> 4
        wm = wt[0:16]
        for j in range(1, 8):
            wm = jnp.where(blk == j, wt[16 * j:16 * j + 16], wm)
        wr, wi = _lo_f32(wm), _hi_f32(wm)
        z = jnp.concatenate([xr * wr - xi * wi, xr * wi + xi * wr], axis=0).astype(BF)
        yield
        zc, zs = _dot_nt(z, _as_bf(nm[:, :128])), _dot_nt(z, _as_bf(nm[:, 128:]))
        pr, pi = zc[0:16] - zs[16:32], zs[0:16] + zc[16:32]
        pp = jnp.concatenate([pr * twc - pi * tws, pi * twc + pr * tws], axis=0).astype(BF)
        yield
        cc = _dot(sm[64:80, 0:32].astype(BF), pp) * (1.0 / (S * D))
        ct[...] = jnp.concatenate([cc, jnp.zeros((112, 128), F32)], axis=0).T
        yield

    def s_rows(k1, a0, r):
        return pl.ds(r + (QS * k1 + N2 * a0), 8)

    def anchored(v, tok):
        return jnp.where(zero_s[0] != 0, tok, v)

    def s_prep(g, k1, r, tok):
        v = [(y[g, 0, s_rows(k1, a0, r), :], y[g, 1, s_rows(k1, a0, r), :]) for a0 in range(8)]
        if tok is not None:
            v[0] = (anchored(v[0][0], tok), v[0][1])
        v = _fft([_cmul_const(v[a0], a0 * k1, N1, -1) for a0 in range(8)], -1)
        for k0 in range(8):
            u_b[k1 + 4 * k0, pl.ds(r, 8), :] = jnp.concatenate(v[k0], axis=1).astype(BF)

    def stacked(ref, ka):
        return jnp.concatenate([ref[ka, :, :128], ref[ka, :, 128:]], axis=0)

    def s_fwd(g, ka, tok):
        xx = _dot(_as_bf(gs[0, ka]), stacked(u_b, ka))
        w32 = fp[g, pl.ds(ka, N2, stride=PITCH), :]
        wr, wi = _lo_f32(w32), _hi_f32(w32)
        xr, xi = xx[:N2], xx[N2:]
        z_b[ka] = jnp.concatenate([xr * wr - xi * wi, xr * wi + xi * wr], axis=1).astype(BF)

    def s_inv(ka, tok):
        p_s[ka] = _dot(_as_bf(gs[1, ka]), stacked(z_b, ka))

    def s_post(g, k1, r, tok):
        v = [(p_s[k1 + 4 * k0, r:r + 8, :], p_s[k1 + 4 * k0, N2 + r:N2 + r + 8, :]) for k0 in range(8)]
        v[0] = (anchored(v[0][0], tok), anchored(v[0][1], tok))
        v = _fft(v, 1)
        for a0 in range(8):
            vr, vi = _cmul_const(v[a0], a0 * k1, N1, 1)
            v_s[g, 0, s_rows(k1, a0, r), :] = vr
            v_s[g, 1, s_rows(k1, a0, r), :] = vi

    def wc_block(c, jc):
        return raw_a.at[c // 2, pl.ds(pl.multiple_of(4096 * (c % 2) + 1024 * jc, 1024), 1024), :]

    def wo_comb(jc, p, r, tok):
        nr = 64 // WSP
        u = [wo[jc + 4 * f, 128 * p + 64 * e + r:128 * p + 64 * e + r + nr, :] for e in range(2) for f in range(2)]
        tok = jnp.concatenate([pltpu.bitcast(tok, U32)] * (nr // 8), axis=0)
        u[0], u[3] = anchored(u[0], tok), anchored(u[3], tok)
        b11, b12, b21, b22 = [_as_bf(v).astype(F32) for v in u]
        for c, v in enumerate((b11 + b22, b12 - b22, b21 - b11, b11 + b12, b21 + b22)):
            wc_block(c, jc)[64 * p + r:64 * p + r + nr, :] = _as_u32(v.astype(BF))

    def bulk(where, n, events, q=None):
        for i in range(n):
            ch, jj = where(i)

            def hook(k, m):
                pieces = events.get(7 * i + k, ())
                vec = [pc for pc in pieces if isinstance(pc, P) and pc.func in (s_prep, s_post, wo_comb, stage_rhs)]
                for piece in pieces:
                    r = 8 * ((32 * vec.index(piece)) // len(vec)) if piece in vec else 0
                    piece(m[r:r + 8])

            def keep(k):
                return v_s.at[jj // 4, (jj // 2) % 2, pl.ds(1024 * (jj % 2) + 256 * k, 256), :]

            def init(k):
                return jnp.where(q > 0, keep(k)[...], 0.0)

            rhs = staged_rhs(i % 2) if q is None else prep_rhs(ch, jj, pl.multiple_of(q * KQ, KQ))
            strassen(rhs, q, 8 * ch + jj,
                     None if q is None else init, None if q is None else keep, hook)

    def spread(events, pieces, q0, q1):
        for i, piece in enumerate(pieces):
            events.setdefault(q0 + ((q1 - q0) * i) // len(pieces), []).append(piece)

    P = functools.partial

    def loop_a(n, c):
        for e in range(2):
            wait(w_half(raw4[0].at[n // 2], n % 2, e), SEM_W0 + n)
        h = jnp.maximum(n - 2, 0)

        @pl.when(n >= 2)
        def _():
            wait(fraw.at[h], SEM_F + h)

        src = jnp.where(n >= 2, h, 4)
        events = {}
        spread(events, [lambda tok, c=c: fprep(src, h, c) for c in range(4)], 0, 48)
        bulk(lambda i: (n // 2, i), 8, events, n % 2)
        return c

    def loop_b(g, c):
        @pl.when((g >= 1) & (g < 3))
        def _():
            wait(raw4[1].at[g], SEM_W + 3 + g)

        for e in range(2):
            wait(wo.at[g + 4 * e], SEM_WO + g)
        gn = jnp.minimum(g + 1, 3)
        events = {}
        for k1 in range(4):
            q = BD * k1
            spread(events, [P(s_fwd, g, k1 + 4 * k0) for k0 in range(8)], q, q + BW)
            spread(events, [P(s_prep, gn, k1, r) for r in range(0, N2, 8)], q + BW, q + BW + BV)
            q += BL
            spread(events, [P(s_inv, k1 + 4 * k0) for k0 in range(8)], q, q + BW)
            spread(events, [P(s_post, g, k1, r) for r in range(0, N2, 8)], q + BW, q + BW + BV)
        spread(events, [P(wo_comb, g, p, r) for p in range(NP) for r in range(0, 64, 64 // WSP)], W0, W1)
        for i in range(6):
            nxt = jnp.minimum(24 + 6 * g + i + 1, 3 * NP - 1)
            spread(events, [P(stage_rhs, nxt, (i + 1) % 2, d0) for d0 in range(0, KH, PB)], 7 * i, 7 * i + SE)
        ny = nyquist()
        spread(events, [lambda tok: next(ny)] * 4, NY0, NY1)
        assert max(events) < 41
        bulk(lambda i: ((24 + 6 * g + i) // 8, (24 + 6 * g + i) % 8), 6, events)
        return c

    def prep0(i, c):
        for k1 in range(4):
            s_prep(0, k1, pl.multiple_of(i * 8, 8), None)
        return c

    lax.fori_loop(0, N2 // 8, prep0, 0)
    with jax.named_scope("loop_a"):
        lax.fori_loop(0, 6, loop_a, 0)
    wait(sm, SEM_SM)
    wait(nm, SEM_NYM)
    wait(nyq, SEM_NYQ)
    wait(gs, SEM_GS)
    with jax.named_scope("loop_b"):
        wait(raw4[1].at[0], SEM_W + 3)
        for d0 in range(0, KH, PB):
            stage_rhs(24, 0, d0, None)
        lax.fori_loop(0, 4, loop_b, 0)
    wait(gi, SEM_GI)
    wait(mem_ref, SEM_MEM)
    wait(gw_ref.at[pl.ds(0, D)], SEM_GW)

    scale = DH ** -0.5

    gw_s[...] = jnp.broadcast_to(gw_ref[pl.ds(0, D)].astype(F32).reshape(1, D), (8, D))

    def softmax(s):
        fill = mf[0:80, :]
        s = jnp.where(fill > 0.0, s * scale, fill)
        m = jnp.max(s, axis=-1, keepdims=True)
        e = jnp.exp(s - m)
        l = jnp.sum(e, axis=-1, keepdims=True)
        r = pl.reciprocal(l, approx=True)
        return (e * (r * (2.0 - l * r))).astype(BF)

    def lhs_rows(mem, seg):
        xs = x_v[pl.ds(pl.multiple_of(seg * SEG, SEG), SEG), :].astype(F32)
        return jnp.concatenate([mem, xs[8:SEG]], axis=0).astype(BF)

    def proj2(a, m, j):
        return jnp.concatenate([_dot(_as_bf(a[...]), _as_bf(wqkv[H * m + 2 * j + p])).astype(BF)
                                for p in range(2)], axis=0)

    def proj_lo(a):
        for i in range(6):
            pa_s[i] = _dot(_as_bf(a[:, :KH]), _as_bf(wqkv[H * (i // 2) + i % 2, 0:KH // 2, :]))

    def proj_hi(a):
        full = [(_dot(_as_bf(a[:, KH:]), _as_bf(wqkv[H * (i // 2) + i % 2, KH // 2:KH, :]))
                 + pa_s[i]).astype(BF) for i in range(6)]
        for m in range(3):
            stg[m, 0] = _as_u32(jnp.concatenate(full[2 * m:2 * m + 2], axis=0))

    def step(a, seg, k, hooks, late):
        srow = pl.multiple_of(seg * 8, 8)
        a = a[...]

        def get(m, j):
            return _as_bf(jnp.concatenate([stg[m, j % 8], st[NP * m + j, pl.ds(srow, 8), :]], axis=0))

        def proj(j, m):
            if j > 0:
                stg[m, j % 8] = _as_u32(proj2(a, m, j))
            elif m == 0:
                if k > 0:
                    proj_lo(a)
                proj_hi(a)

        def scores(j):
            pst[j % 8] = _as_u32(softmax(_dot_nt(get(0, j), get(1, j))))

        def pv(j):
            o = _dot(_as_bf(pst[j % 8]), get(2, j))
            if k < 3:
                for i in range(2):
                    sto[2 * j + i, 8 * k:8 * k + 8, :] = o[64 + 8 * i:72 + 8 * i]
                    obuf[2 * j + i] = _as_u32(o[32 * i:32 * i + 32].astype(BF))
            else:
                a11, a12 = o[0:32], o[32:64]
                a21, a22 = [jnp.concatenate([sto[2 * j + i, 0:24, :], o[64 + 8 * i:72 + 8 * i]], axis=0)
                            for i in range(2)]
                for i, v in enumerate((a11 + a22, a21 + a22, a11, a22, a11 + a12, a21 - a11, a12 - a22)):
                    lc[i, j] = _as_u32(v.astype(BF))

        def wo_part(j, h0, h1):
            og = jnp.concatenate([_as_bf(obuf[h]) for h in range(h0, h1)], axis=1)
            return _dot(og, _as_bf(wo[j, h0 * 64:h1 * 64, :]))

        def prod(i, jc, p0, p1):
            lhs = jnp.concatenate([_as_bf(lc[i, p]) for p in range(p0, p1)], axis=1)
            if i in (1, 4):
                e = i // 4
                rhs = jnp.concatenate([wo[jc + 4 * e, 128 * p + 64 * e:128 * p + 64 * e + 64, :]
                                       for p in range(p0, p1)], axis=0)
            else:
                rhs = wc_block((0, None, 1, 2, None, 3, 4)[i], jc)[64 * p0:64 * p1, :]
            return _dot(lhs, _as_bf(rhs))

        early = [(i, jc) for i in (0, 3, 4, 6) for jc in range(4)]
        parts = []
        for i in range(NP + 4):
            for ch in ORDER:
                if ch in "qkv":
                    m = "qkv".index(ch)
                    if i < NP:
                        proj(i, m)
                    elif m < 2:
                        for n in range(1 if k < 3 else 2):
                            r = wo_part(len(parts), 0, SPLIT) if k < 3 else prod(*early[len(parts)], 0, SP3)
                            mp[len(parts)] = r
                            parts.append(r[0:8])
                elif ch == "s" and 0 <= i - LAG1 < NP:
                    scores(i - LAG1)
                elif ch == "p" and 0 <= i - LAG2 < NP:
                    pv(i - LAG2)
            if i == HOOK_AT:
                for hook in hooks[k]:
                    hook()
        if k < 3:
            return jnp.concatenate([wo_part(j, SPLIT, H) + mp[j] for j in range(8)], axis=1)
        toks, c11, c12 = parts[T0:], [], []
        for jc in range(4):
            m1, m4, m5 = [prod(i, jc, SP3, NP) + mp[4 * n + jc] for n, i in enumerate((0, 3, 4))]
            c11.append(prod(6, jc, SP3, NP) + (mp[12 + jc] + (m1 + m4 - m5)))
            mp[jc], mp[4 + jc], mp[8 + jc] = m1, m4, m5
            toks += [m1[0:8]] * (jc % 2)
        for jc in range(4):
            m3 = prod(2, jc, 0, NP)
            c12.append(m3 + mp[8 + jc])
            mp[jc] = mp[jc] + m3
            toks.append(m3[0:8])
        for n, piece in enumerate(late):
            piece(toks[(n * len(toks)) // len(late)])
        c21 = []
        for jc in range(4):
            m2 = prod(1, jc, 0, NP)
            c21.append(m2 + mp[4 + jc])
            mp[jc] = mp[jc] - m2
        c22 = [prod(5, jc, 0, NP) + mp[jc] for jc in range(4)]
        return jnp.concatenate(c11 + c12, axis=1), jnp.concatenate(c21 + c22, axis=1)

    def start_quad(mem, u):
        a_s[0] = _as_u32(lhs_rows(mem, 4 * u))
        proj_lo(a_s.at[0])

    def quad(u, c):
        base = pl.multiple_of(u * 128, 128)
        roll = lambda v: pltpu.roll(v, 64, 1)
        a1 = u // 4
        s2 = (1 - 2 * (a1 & 1)).astype(F32)
        sg = (1 - (a1 & 2)).astype(F32)
        cc, ss = sg * (1 - (a1 & 1)).astype(F32), sg * (a1 & 1).astype(F32)

        def irfft_dots(r0):
            off = pl.multiple_of((u % 4) * 128, 128) + r0
            for g in range(4):
                q = [[v_s[g, e, pl.ds(off + QS * k1, SEG), :] for e in range(2)] for k1 in range(4)]
                br, bi = q[1][0] + s2 * q[3][0], q[1][1] + s2 * q[3][1]
                vr = q[0][0] + s2 * q[2][0] + (cc * br - ss * bi)
                vi = q[0][1] + s2 * q[2][1] + (cc * bi + ss * br)
                tin = _half_pre(vr, vi, _lanes(SEG) < 64, roll, jnp.where)
                for e in range(2):
                    ts_s[r0:r0 + SEG, 128 * (2 * g + e):128 * (2 * g + e + 1)] = _dot(
                        tin[e].astype(BF), _as_bf(gi[2 * g + e]))

        def mix(r0, tok):
            lane = _lanes(8)
            t = [anchored(ts_s[r0:r0 + 8, 128 * i:128 * i + 128], tok) for i in range(8)]
            nyc = jnp.sum(jnp.where(lane == u, anchored(ct[r0:r0 + 8, :], tok), 0.0), axis=-1, keepdims=True)
            t[0] = t[0] + nyc * (1 - 2 * (lane & 1)).astype(F32)
            t = sum([list(_half_post(g, t[2 * g], t[2 * g + 1], lane < 64, roll, jnp.where))
                     for g in range(4)], [])
            b = jnp.concatenate(_bfly8_t(t), axis=1).astype(BF).astype(F32)
            xg = x_v[pl.ds(base + r0, 8), :].astype(F32) * gw_s[...]
            xg = functools.reduce(jnp.add, [xg[:, 128 * i:128 * i + 128] for i in range(8)])
            gate = jax.nn.sigmoid(jnp.sum(anchored(xg, tok), axis=-1, keepdims=True))
            bb = (1.0 - gate) * b
            if r0 % SEG and r0 < 96:
                out_v[pl.ds(base + r0, 8), :] = (bb + gate * ra_s[r0:r0 + 8, :]).astype(BF)
            else:
                bb_s[r0:r0 + 8, :] = bb
                g_s[r0:r0 + 8, :] = jnp.broadcast_to(gate, (8, 128))

        hooks = [[P(irfft_dots, SEG * n) for n in range(4) if HMAP[n] == str(k)] for k in range(4)]
        late = [P(mix, r0) for r0 in range(0, 128, 8)]
        for k in range(3):
            res = step(a_s.at[k % 2], 4 * u + k, k, hooks, late)
            ra_s[32 * k + 8:32 * k + 32, :] = res[8:32]
            a_s[(k + 1) % 2] = _as_u32(lhs_rows(res[0:8], 4 * u + k + 1))
        res, first8 = step(a_s.at[1], 4 * u + 3, 3, hooks, late)

        def emit(r0, n, att):
            out_v[pl.ds(base + r0, n), :] = (
                bb_s[r0:r0 + n, :] + jnp.concatenate([g_s[r0:r0 + n, :]] * 8, axis=1) * att).astype(BF)

        emit(104, 24, res[8:32])
        for k in range(4):
            emit(32 * k, 8, first8[8 * k:8 * k + 8])
        pltpu.make_async_copy(out_v.at[pl.ds(base, 128), :], out_hbm.at[pl.ds(base, 128), :],
                              sem.at[SEM_OUT]).start()
        start_quad(res[0:8], jnp.minimum(u + 1, S // 128 - 1))
        return c

    with jax.named_scope("chain"):
        start_quad(mem_ref[...].astype(F32), 0)
        lax.fori_loop(0, S // 128, quad, 0)
    pltpu.make_async_copy(out_v, out_hbm, sem.at[SEM_OUT]).wait()


@jax.jit
def pallas_gated_mix__memory_aug_recurrent_mem_tr__spectral_gfnet__prompt_kernel(
    A_x, A_mem0, A_Wq, A_Wk, A_Wv, A_Wo, A_seg_len, B_x, B_w_r, B_w_i, gate_w,
):
    assert A_x.shape == (1, S, D) and A_mem0.shape == (1, M, D) and A_Wq.shape == (D, H, DH)
    consts = [jnp.asarray(c) for c in _constants()]
    any_spec = pl.BlockSpec(memory_space=pl.ANY)
    out = pl.pallas_call(
        _kernel,
        out_shape=jax.ShapeDtypeStruct((S, D), BF),
        in_specs=[any_spec] * 14,
        out_specs=any_spec,
        scratch_shapes=[
            pltpu.VMEM((S, D), BF),
            pltpu.VMEM((3, D * 8, DH), U32),
            pltpu.VMEM((3, D * 8, DH), U32),
            pltpu.VMEM((3 * H, D // 2, DH), U32),
            pltpu.VMEM((8, H * DH // 2, 128), U32),
            pltpu.VMEM((3 * NP, 8 * NSEG, 128), U32),
            pltpu.VMEM((NQ, 7, 2 * NSEG, D // 2 // NQ), U32),
            pltpu.VMEM((5, 2, 4, 256, 128), U32),
            pltpu.VMEM((4, N2 * PITCH, 128), U32),
            pltpu.VMEM((4, 128, 256), U32),
            pltpu.VMEM((64, 256), U32),
            pltpu.VMEM((8, 64, 128), U32),
            pltpu.VMEM((2, N1, N2, 2 * N2), U32),
            pltpu.VMEM((4, 2, S, 128), F32),
            pltpu.VMEM((4, 2, S, 128), F32),
            pltpu.VMEM((S, D), BF),
            pltpu.VMEM((6, 256, 128), F32),
            pltpu.VMEM((4, N2, 128), U32),
            pltpu.VMEM((N1, 2 * N2, 128), F32),
            pltpu.VMEM((2, 2, D // 4, 128), U32),
            pltpu.VMEM((2, D // 2, 5 * 128), BF),
            pltpu.VMEM((N1, N2, 256), BF),
            pltpu.VMEM((N1, N2, 256), BF),
            pltpu.VMEM((H, 32, 128), F32),
            pltpu.VMEM((H, 16, 128), U32),
            pltpu.VMEM((128, 128), F32),
            pltpu.VMEM((2, 16, D), U32),
            pltpu.VMEM((6, 32, 128), F32),
            pltpu.VMEM((128, D), F32),
            pltpu.VMEM((128, 128), F32),
            pltpu.VMEM((3, 8, 32, 128), U32),
            pltpu.VMEM((8, 40, 80), U32),
            pltpu.VMEM((128, D), F32),
            pltpu.VMEM((128, D), F32),
            pltpu.VMEM((16, 32, 128), F32),
            pltpu.VMEM((7, NP, 16, 128), U32),
            pltpu.VMEM((8, D), F32),
            pltpu.VMEM((M, D), BF),
            pltpu.VMEM((96, 80), F32),
            pltpu.VMEM((96, 128), F32),
            pltpu.VMEM((32, 128), F32),
            pltpu.VMEM((2, 1, S), BF),
            pltpu.VMEM((8 * D,), BF),
            pltpu.SMEM((2,), jnp.int32),
            pltpu.SemaphoreType.DMA((NSEM,)),
        ],
        compiler_params=pltpu.CompilerParams(vmem_limit_bytes=120 * 1024 * 1024,
                                             disable_bounds_checks=True,
                                             disable_semaphore_checks=True),
    )(
        A_x.reshape(S, D), A_mem0.reshape(M, D), A_Wq, A_Wk, A_Wv,
        A_Wo.reshape(H * DH, D), B_w_r.T, B_w_i.T, gate_w, *consts,
    )
    return out.reshape(1, S, D)
```

```python
import functools
import math

import numpy as np
import jax
import jax.numpy as jnp
from jax import lax
import jax.experimental.pallas as pl
import jax.experimental.pallas.tpu as pltpu

BF, F32, U32 = jnp.bfloat16, jnp.float32, jnp.uint32

S, D, H, DH, M, SEG = 2048, 1024, 32, 128, 8, 32
NSEG = S // SEG
NP = H // 2
N1, N2 = 32, 64
QS = S // 4
PITCH = N1 + 8
CLASSES = ((0, 8, 4, 12), (1, 15, 9, 7), (2, 14, 10, 6), (3, 13, 11, 5))
LAG1, LAG2, SPLIT, HOOK_AT = 1, 2, 27, 18
ORDER = "qksvp"
CP, CW, CS = 120, 45, 55
PB, SE = 16, 6
WSP, W0, W1 = 8, 0, 40
T0 = 6
HMAP = "0123"
SP3 = 13
NY0, NY1 = 32, 40
BD, BW, BV, BL = 7, 8, 8, 3
NQ = 2
(SEM_W, SEM_GF, SEM_GI, SEM_SM, SEM_GS, SEM_NYQ, SEM_NYM, SEM_MEM, SEM_GW, SEM_OUT, SEM_F, SEM_X,
 SEM_W0) = 0, 6, 7, 8, 9, 10, 11, 12, 13, 14, 15, 19, 23
SEM_WO = SEM_W0 + 6
NSEM = SEM_WO + 4
RSQ2 = float(np.float32(math.sqrt(0.5)))


def _bfly8(x):
    s = [x[i] + x[i + 4] for i in range(4)]
    d = [x[i] - x[i + 4] for i in range(4)]
    e, f = s[0] + s[2], s[1] + s[3]
    t1, t2 = (d[1] - d[3]) * RSQ2, (d[1] + d[3]) * RSQ2
    return [e + f, e - f, d[0] + t1, t2 + d[2], s[0] - s[2], s[1] - s[3], d[0] - t1, t2 - d[2]]


def _bfly8_t(t):
    e, f = t[0] + t[1], t[0] - t[1]
    s = [e + t[4], f + t[5], e - t[4], f - t[5]]
    t1, t2 = t[2] - t[6], t[3] + t[7]
    d = [t[2] + t[6], (t1 + t2) * RSQ2, t[3] - t[7], (t2 - t1) * RSQ2]
    return [s[i] + d[i] for i in range(4)] + [s[i] - d[i] for i in range(4)]


def _half_pre(vr, vi, lo, roll, where):
    ri = roll(vi)
    return where(lo, vr, ri), where(lo, ri, vr)


def _half_post(g, tp, tm, lo, roll, where):
    if g == 0:
        return tp, tm
    c = float(np.float32(math.cos(math.pi * g / 8)))
    s = float(np.float32(math.sin(math.pi * g / 8)))
    p, r = tp + tm, tp - tm
    rm = roll(where(lo, r, p))
    return where(lo, p, c * rm + s * r), where(lo, rm, c * r - s * rm)


def _cmul_const(v, k, n, sign):
    re, im = v
    k %= n
    if k == 0:
        return re, im
    if 4 * k == n:
        return (-im, re) if sign > 0 else (im, -re)
    if 8 * k == n:
        return (((re - im) * RSQ2, (re + im) * RSQ2) if sign > 0
                else ((re + im) * RSQ2, (im - re) * RSQ2))
    if 8 * k == 3 * n:
        return (((re + im) * -RSQ2, (re - im) * RSQ2) if sign > 0
                else ((im - re) * RSQ2, (re + im) * -RSQ2))
    c, s = math.cos(2 * math.pi * k / n), sign * math.sin(2 * math.pi * k / n)
    return re * c - im * s, re * s + im * c


def _fft(v, sign):
    n = len(v)
    if n == 1:
        return v
    ev, od = _fft(v[0::2], sign), _fft(v[1::2], sign)
    lo, hi = [], []
    for k in range(n // 2):
        er, ei = ev[k]
        if 4 * k == n:
            xr, xi = od[k]
            if sign > 0:
                lo.append((er - xi, ei + xr)); hi.append((er + xi, ei - xr))
            else:
                lo.append((er + xi, ei - xr)); hi.append((er - xi, ei + xr))
            continue
        tr, ti = _cmul_const(od[k], k, n, sign)
        lo.append((er + tr, ei + ti))
        hi.append((er - tr, ei - ti))
    return lo + hi


def _pack_rows(a):
    u = np.ascontiguousarray(a, dtype=np.float32).view(np.uint32)
    b = ((u + 0x7FFF + ((u >> 16) & 1)) >> 16).astype(np.uint32)
    return (b[..., 0::2, :] | (b[..., 1::2, :] << 16)).astype(np.uint32)


def _diag_blocks(full, n, tol):
    k = full.shape[0] // n
    blk = np.kron(np.eye(k), np.ones((n, n)))
    assert np.abs(full * (1 - blk)).max() < tol
    return np.stack([full[n * g:n * g + n, n * g:n * g + n] for g in range(k)])


@functools.lru_cache(maxsize=None)
def _constants():
    k2 = np.stack([np.concatenate([c + 16 * np.arange(32) for c in cls]) for cls in CLASSES])
    n2 = np.arange(D)
    ang = 2 * np.pi * ((k2[:, :, None] * n2[None, None, :]) % D) / D
    rows = np.stack([np.cos(ang), -np.sin(ang)], axis=1)
    wgt = np.where(k2 == 0, 1.0, 2.0)[:, None, :, None]
    fwd = rows.reshape(D, D).T
    inv = (rows * wgt).reshape(D, D) / (S * D)
    bf = np.stack(_bfly8(list(np.eye(8))))
    binv = np.kron(np.linalg.inv(bf), np.eye(128))
    gd = _diag_blocks(binv.T @ fwd, 256, 1e-6)
    gdi = _diag_blocks(inv @ binv, 256, 1e-12)
    eye, lo = np.eye(256), np.arange(128) < 64
    roll = lambda v: np.roll(v, 64, axis=1)
    pre = np.concatenate(_half_pre(eye[:, :128], eye[:, 128:], lo, roll, np.where), axis=1)
    gi = []
    for g in range(4):
        post = np.concatenate(_half_post(g, eye[:, :128], eye[:, 128:], lo, roll, np.where), axis=1)
        gi.append(_diag_blocks(np.linalg.inv(pre) @ gdi[g] @ np.linalg.inv(post), 128, 1e-12))
    gi = np.concatenate(gi)

    b = np.arange(N2)
    k1 = np.arange(N1)[:, None] + N1 * np.arange(N2)[None, :]
    th = 2 * np.pi * ((k1[:, :, None] * b[None, None, :]) % S) / S
    gr, gim = np.cos(th), -np.sin(th)
    gs = np.concatenate([gr, -gim], axis=2)
    hr, hi = np.swapaxes(gr, 1, 2), -np.swapaxes(gim, 1, 2)
    gsi = np.concatenate([hr, -hi], axis=2)

    lane = np.arange(128)
    kb = 8 * (lane % 16) + lane // 16
    t128 = 2 * np.pi * ((lane[:, None] * kb[None, :]) % 128) / 128
    nym = np.concatenate([np.cos(t128), np.sin(t128)], axis=1)
    i16 = np.arange(16)
    t16 = 2 * np.pi * ((i16[:, None] * i16[None, :]) % 16) / 16
    tw = 2 * np.pi * (i16[:, None] * lane[None, :]) / S
    sm = np.zeros((96, 128), np.float32)
    sm[0:16], sm[16:32] = np.cos(tw), np.sin(tw)
    sm[32:48, :16], sm[48:64, :16] = np.cos(t16), -np.sin(t16)
    sm[64:80, :16], sm[64:80, 16:32] = np.cos(t16), -np.sin(t16)

    return _pack_rows(gd), _pack_rows(nym), _pack_rows(gi), sm, _pack_rows(np.stack([gs, gsi]))


def _mask80():
    r = lax.broadcasted_iota(jnp.int32, (80, 80), 0)
    c = lax.broadcasted_iota(jnp.int32, (80, 80), 1)

    def head(i):
        return jnp.where(i < 64, i >> 5, (i - 64) >> 3)

    def pos(i):
        j = i & 31
        return jnp.where(i < 64, jnp.where(j < M, j, j + 8), M + (i & 7))

    same = head(r) == head(c)
    ok = (pos(r) < M) | (pos(c) <= pos(r))
    return jnp.where(same, jnp.where(ok, 1.0, -1e9), -jnp.inf).astype(F32)


def _as_bf(u):
    return pltpu.bitcast(u, BF)


def _as_u32(b):
    return pltpu.bitcast(b, U32)


def _lo_f32(u):
    return pltpu.bitcast(u << 16, F32)


def _hi_f32(u):
    return pltpu.bitcast(u & jnp.uint32(0xFFFF0000), F32)


def _dot(a, b):
    return jnp.dot(a, b, preferred_element_type=F32)


def _dot_nt(a, b):
    return lax.dot_general(a, b, (((1,), (1,)), ((), ())), preferred_element_type=F32)


def _transpose_u32(u):
    return pltpu.bitcast(pltpu.bitcast(u, F32).T, U32)


def _lanes(rows):
    return lax.broadcasted_iota(jnp.int32, (rows, 128), 1)


def _kernel(x_hbm, mem_hbm, wq_hbm, wk_hbm, wv_hbm, wo_hbm, fr_hbm, fi_hbm, gw_hbm,
            gf_hbm, nm_hbm, gi_hbm, sm_hbm, gs_hbm,
            out_hbm,
            x_v, raw_a, raw_b, wqkv, wo, st, sl, fraw, fp, gf, nm, gi, gs, y, v_s, out_v, cb, z_s, p_s, rs_u, rs_c, u_b, z_b,
            sto, obuf, ct, a_s, pa_s, bb_s, g_s, stg, pst, ra_s, ts_s, mp, lc, gw_s, mem_ref, mf, sm, xa, nyq, gw_ref, zero_s, sem):
    KH = D // 2
    KQ = KH // NQ
    RB, HB = 128, 16
    raw4 = [r.reshape(3, D, 8, DH) for r in (raw_a, raw_b)]
    w_hbm = (wq_hbm, wk_hbm, wv_hbm)
    f_hbm = (fr_hbm, fi_hbm)

    def w_src(c):
        return w_hbm[c // 2].bitcast(U32).at[:, pl.ds(8 * (c % 2), 8), :]

    def wait(dst, k):
        pltpu.make_async_copy(dst, dst, sem.at[k]).wait()

    def w_half(ref, q, e):
        return ref.at[pl.ds(pl.multiple_of(q * KQ, KQ) + e * KH, KQ)]

    def x_rows(i, a1):
        return pl.ds(pl.multiple_of(i * RB, RB) + QS * a1, RB)

    def f_copies(h):
        return [(f_hbm[a].at[pl.ds(0, D // 2), pl.ds(128 * (4 * h + c), 128)].bitcast(U32),
                 fraw.at[h, a, c], SEM_F + h) for a in range(2) for c in range(4)]

    def w_copy(c):
        return [(w_src(c), raw4[1].at[c - 3], SEM_W + c)]

    copies = [(gf_hbm, gf, SEM_GF)]
    copies += [(x_hbm.at[x_rows(i, a1), :], x_v.at[x_rows(i, a1), :], SEM_X + i)
               for i in range(QS // RB) for a1 in range(4)]
    for n in range(6):
        copies += [(w_half(w_src(n // 2), n % 2, e), w_half(raw4[0].at[n // 2], n % 2, e), SEM_W0 + n)
                   for e in range(2)]
        if n >= 2:
            copies += f_copies(n - 2)
    copies += [(sm_hbm, sm, SEM_SM), (nm_hbm, nm, SEM_NYM)]
    copies += [(f_hbm[a].at[pl.ds(D // 2, 1), :], nyq.at[a], SEM_NYQ) for a in range(2)]
    copies += [(gs_hbm, gs, SEM_GS)]
    for g in range(4):
        copies += w_copy(3 + g) if g < 3 else []
        copies += [(wo_hbm.bitcast(U32).at[:, pl.ds(128 * j, 128)], wo.at[j], SEM_WO + g) for j in (g, g + 4)]
    copies += [(gi_hbm, gi, SEM_GI), (mem_hbm, mem_ref, SEM_MEM), (gw_hbm, gw_ref.at[pl.ds(0, D)], SEM_GW)]
    for src, dst, k in copies:
        pltpu.make_async_copy(src, dst, sem.at[k]).start()

    def prep_rhs(ch, jj, k0):
        a1 = raw_a[ch, pl.ds(k0 * 8 + jj, KQ, stride=8), :]
        a2 = raw_a[ch, pl.ds((KH + k0) * 8 + jj, KQ, stride=8), :]
        b11, b12, b21, b22 = _lo_f32(a1), _hi_f32(a1), _lo_f32(a2), _hi_f32(a2)
        for p, e, b in ((0, 0, b11), (1, 0, b12), (0, 1, b21), (1, 1, b22)):
            row = pl.multiple_of(k0 // 2, KQ // 2) + e * KH // 2
            wqkv[2 * (8 * ch + jj) + p, pl.ds(row, KQ // 2), :] = _as_u32(b.astype(BF))
        return [v.astype(BF) for v in (b11 + b22, b11, b12 - b22, b21 - b11, b22, b11 + b12, b21 + b22)]

    def b_item(n, par):
        return 3 + n // 8, (n // 2) % 4

    def stage_rhs(n, par, d0, tok):
        ch, low = b_item(n, par)
        item = 8 * ch + low + 4 * par
        a = [raw_b[ch - 3, pl.ds(low + ((e * KH + d0) * 8 + 4 * par), PB, stride=8), :] for e in range(2)]
        if tok is not None:
            tok = jnp.concatenate([pltpu.bitcast(tok, U32)] * (PB // 8), axis=0)
            a = [anchored(v, tok) for v in a]
        b11, b12, b21, b22 = _lo_f32(a[0]), _hi_f32(a[0]), _lo_f32(a[1]), _hi_f32(a[1])
        for p, e, b in ((0, 0, b11), (1, 0, b12), (0, 1, b21), (1, 1, b22)):
            u = _as_u32(b.astype(BF))
            wqkv[2 * item + p, pl.ds((e * KH + d0) // 2, PB // 2), :] = u
            if p == e:
                rs_u[par, p, d0 // 2:(d0 + PB) // 2, :] = u
        comb = [b11 + b22, b12 - b22, b21 - b11, b11 + b12, b21 + b22]
        rs_c[par, d0:d0 + PB, :] = jnp.concatenate(comb, axis=1).astype(BF)

    def staged_rhs(par):
        c = lambda i: (lambda: rs_c[par, :, 128 * i:128 * i + 128])
        return [c(0), lambda: _as_bf(rs_u[par, 0]), c(1), c(2), lambda: _as_bf(rs_u[par, 1]), c(3), c(4)]

    def strassen(rhs, q, item, init, keep, after_dot):
        def prod(i):
            lhs = sl[q, i] if q is not None else jnp.concatenate([sl[k, i] for k in range(NQ)], axis=1)
            return _dot(_as_bf(lhs), rhs[i]() if callable(rhs[i]) else rhs[i])

        def plus(i, r):
            return r if init is None else init(i) + r

        c12, c21 = (cb.at[5], cb.at[4]) if keep is None else (keep(1), keep(2))
        def done(k, c):
            if keep is not None:
                keep(3 * k)[...] = c
            store_st(item, k, *((c, c12[...]) if k == 0 else (c21[...], c)))

        m = prod(1)
        cb[0] = m
        after_dot(0, m)
        m = prod(5) + plus(3, -cb[0])
        cb[3] = m
        after_dot(1, m)
        m = prod(4)
        cb[1] = m
        after_dot(2, m)
        m = prod(0)
        cb[2] = plus(0, m - cb[1])
        cb[3] = cb[3] + m
        after_dot(3, m)
        m = prod(3)
        c21[...] = plus(2, cb[0] + m)
        cb[2] = cb[2] + m
        after_dot(4, m)
        m = prod(2)
        c12[...] = plus(1, cb[1] + m)
        done(1, cb[3] + m)
        after_dot(5, m)
        m = prod(6) + cb[2]
        done(0, m)
        after_dot(6, m)

    def store_st(item, e, c1, c2):
        r = jnp.concatenate([c.reshape(NSEG // 2, 8, 128) for c in (c1, c2)], axis=1)
        st[item, 256 * e:256 * e + 256, :] = _as_u32(r.reshape(8 * NSEG, 128).astype(BF))

    def pin(i, c):
        cb[i, 0:8, :] = jnp.zeros((8, 128), F32)
        zero_s[i] = 0
        z_b[i, 0:16, 0:128] = jnp.zeros((16, 128), BF)
        rs_u[i, 0, 0:8, :] = jnp.zeros((8, 128), U32)
        rs_c[i, 0:16, 0:128] = jnp.zeros((16, 128), BF)
        z_s[i, 0:8, :] = jnp.zeros((8, 128), U32)
        p_s[i, 0:8, :] = jnp.zeros((8, 128), F32)
        stg[i, 0, 0:8, :] = jnp.zeros((8, 128), U32)
        obuf[i, 0:8, :] = jnp.zeros((8, 128), U32)
        sto[i, 0:8, :] = jnp.zeros((8, 128), F32)
        lc[i, 0, 0:8, :] = jnp.zeros((8, 128), U32)
        mp[i, 0:8, :] = jnp.zeros((8, 128), F32)
        ts_s[pl.ds(pl.multiple_of(8 * i, 8), 8), 0:128] = jnp.zeros((8, 128), F32)
        ra_s[pl.ds(pl.multiple_of(8 * i, 8), 8), 0:128] = jnp.zeros((8, 128), F32)
        a_s[i, 0:8, 0:128] = jnp.zeros((8, 128), U32)
        pa_s[i, 0:8, :] = jnp.zeros((8, 128), F32)
        bb_s[pl.ds(pl.multiple_of(8 * i, 8), 8), 0:128] = jnp.zeros((8, 128), F32)
        g_s[pl.ds(pl.multiple_of(8 * i, 8), 8), :] = jnp.zeros((8, 128), F32)
        return c

    lax.fori_loop(0, 2, pin, 0)

    mf[0:80, :] = _mask80()
    fraw[4] = jnp.zeros(fraw.shape[1:], U32)

    wait(gf, SEM_GF)

    def f1(i, c):
        for a1 in range(4):
            wait(x_v.at[x_rows(i, a1), :], SEM_X + i)
        base = pl.multiple_of(i * RB, RB)
        alt = (1 - 2 * (_lanes(16) & 1)).astype(F32).astype(BF)

        def rows16(r):
            return jnp.concatenate([x_v[pl.ds(r + d, 16), :].astype(F32)[0:8] for d in (0, SEG)], axis=0)

        for r in (0, 64, QS, QS + 64):
            top, bot = rows16(base + r), rows16(base + (r + 2 * QS))
            a11, a12, a21, a22 = top[:, :KH], top[:, KH:], bot[:, :KH], bot[:, KH:]
            row = pl.multiple_of((base + r) // 8, 8)
            for k, v in enumerate((a11 + a22, a21 + a22, a11, a22, a11 + a12, a21 - a11, a12 - a22)):
                for q in range(NQ):
                    sl[q, k, pl.ds(row, 8), :] = _as_u32(v[:, q * KQ:(q + 1) * KQ].astype(BF))
        for h0 in range(0, RB, HB):
            pieces = []
            for a1 in range(4):
                for r in range(h0, h0 + HB, 16):
                    xs = x_v[pl.ds(base + (QS * a1 + r), 16), :].astype(F32)
                    pieces.append(jnp.concatenate(_bfly8([xs[:, 128 * a:128 * a + 128] for a in range(8)]),
                                                  axis=1))
                    z_s[a1, r // 2:r // 2 + 8, :] = _as_u32(pieces[-1][:, :128].astype(BF))
            ub = jnp.concatenate(pieces, axis=0)
            for g in range(4):
                yy = _dot(ub[:, 256 * g:256 * g + 256].astype(BF), _as_bf(gf[g]))
                v = _fft([(yy[HB * a1:HB * a1 + HB, :128], yy[HB * a1:HB * a1 + HB, 128:])
                          for a1 in range(4)], -1)
                for k1 in range(4):
                    rows = pl.ds(base + (QS * k1 + h0), HB)
                    y[g, 0, rows, :] = v[k1][0]
                    y[g, 1, rows, :] = v[k1][1]
                if h0 + HB == RB and g == 3:
                    for a1 in range(4):
                        xa[pl.ds(4 * a1 + i, 1), :] = _dot_nt(alt, _as_bf(z_s[a1]))[0:1]
        return c

    with jax.named_scope("f1"):
        lax.fori_loop(0, QS // RB, f1, 0)

    def fprep(src, h, c):
        ev, od = [], []
        for r in range(8):
            wr = fraw[src, 0, c, pl.ds(r, 32, stride=8), :]
            wi = fraw[src, 1, c, pl.ds(r, 32, stride=8), :]
            ev.append((wr & jnp.uint32(0xFFFF)) | (wi << 16))
            od.append((wr >> 16) | (wi & jnp.uint32(0xFFFF0000)))
        for g, cls in enumerate(CLASSES):
            t = _transpose_u32(jnp.concatenate([(od if k % 2 else ev)[k // 2] for k in cls], axis=0))
            for q in range(128 // N1):
                row = pl.multiple_of(((4 * h + c) * (128 // N1) + q) * PITCH, 8)
                fp[g, pl.ds(row, N1), :] = t[q * N1:(q + 1) * N1]

    def nyquist():
        twc, tws = sm[0:16], sm[16:32]
        u = _dot(sm[32:64, 0:16].astype(BF), xa[0:16, :].astype(BF))
        ur, ui = u[0:16], u[16:32]
        u = jnp.concatenate([ur * twc + ui * tws, ui * twc - ur * tws], axis=0).astype(BF)
        yield
        xx = _dot(u, _as_bf(nm[...]))
        xr, xi = xx[0:16, :128] + xx[16:32, 128:], xx[16:32, :128] - xx[0:16, 128:]
        w = (pltpu.bitcast(nyq[0].astype(F32), U32) >> 16) | pltpu.bitcast(nyq[1].astype(F32), U32)
        w = jnp.concatenate([w[:, 128 * a:128 * a + 128] for a in range(16)], axis=0)
        wt = _transpose_u32(jnp.concatenate([w] * 8, axis=0))
        blk = _lanes(16) >> 4
        wm = wt[0:16]
        for j in range(1, 8):
            wm = jnp.where(blk == j, wt[16 * j:16 * j + 16], wm)
        wr, wi = _lo_f32(wm), _hi_f32(wm)
        z = jnp.concatenate([xr * wr - xi * wi, xr * wi + xi * wr], axis=0).astype(BF)
        yield
        zc, zs = _dot_nt(z, _as_bf(nm[:, :128])), _dot_nt(z, _as_bf(nm[:, 128:]))
        pr, pi = zc[0:16] - zs[16:32], zs[0:16] + zc[16:32]
        pp = jnp.concatenate([pr * twc - pi * tws, pi * twc + pr * tws], axis=0).astype(BF)
        yield
        cc = _dot(sm[64:80, 0:32].astype(BF), pp) * (1.0 / (S * D))
        ct[...] = jnp.concatenate([cc, jnp.zeros((112, 128), F32)], axis=0).T
        yield

    def s_rows(k1, a0, r):
        return pl.ds(r + (QS * k1 + N2 * a0), 8)

    def anchored(v, tok):
        return jnp.where(zero_s[0] != 0, tok, v)

    def s_prep(g, k1, r, tok):
        v = [(y[g, 0, s_rows(k1, a0, r), :], y[g, 1, s_rows(k1, a0, r), :]) for a0 in range(8)]
        if tok is not None:
            v[0] = (anchored(v[0][0], tok), v[0][1])
        v = _fft([_cmul_const(v[a0], a0 * k1, N1, -1) for a0 in range(8)], -1)
        for k0 in range(8):
            u_b[k1 + 4 * k0, pl.ds(r, 8), :] = jnp.concatenate(v[k0], axis=1).astype(BF)

    def cdot(mat, ref, ka):
        vr, vi = ref[ka, :, :128], ref[ka, :, 128:]
        neg = _as_bf(_as_u32(vr) ^ jnp.uint32(0x80008000))
        return [_dot(_as_bf(mat), jnp.concatenate(v, axis=0)) for v in ((vr, vi), (vi, neg))]

    def s_fwd(g, ka, tok):
        xr, xi = cdot(gs[0, ka], u_b, ka)
        w32 = fp[g, pl.ds(ka, N2, stride=PITCH), :]
        wr, wi = _lo_f32(w32), _hi_f32(w32)
        z_b[ka] = jnp.concatenate([xr * wr - xi * wi, xr * wi + xi * wr], axis=1).astype(BF)

    def s_inv(ka, tok):
        p_s[ka] = jnp.concatenate(cdot(gs[1, ka], z_b, ka), axis=0)

    def s_post(g, k1, r, tok):
        v = [(p_s[k1 + 4 * k0, r:r + 8, :], p_s[k1 + 4 * k0, N2 + r:N2 + r + 8, :]) for k0 in range(8)]
        v[0] = (anchored(v[0][0], tok), anchored(v[0][1], tok))
        v = _fft(v, 1)
        for a0 in range(8):
            vr, vi = _cmul_const(v[a0], a0 * k1, N1, 1)
            v_s[g, 0, s_rows(k1, a0, r), :] = vr
            v_s[g, 1, s_rows(k1, a0, r), :] = vi

    def wc_block(c, jc):
        return raw_a.at[c // 2, pl.ds(pl.multiple_of(4096 * (c % 2) + 1024 * jc, 1024), 1024), :]

    def wo_comb(jc, p, r, tok):
        nr = 64 // WSP
        u = [wo[jc + 4 * f, 128 * p + 64 * e + r:128 * p + 64 * e + r + nr, :] for e in range(2) for f in range(2)]
        tok = jnp.concatenate([pltpu.bitcast(tok, U32)] * (nr // 8), axis=0)
        u[0], u[3] = anchored(u[0], tok), anchored(u[3], tok)
        b11, b12, b21, b22 = [_as_bf(v).astype(F32) for v in u]
        for c, v in enumerate((b11 + b22, b12 - b22, b21 - b11, b11 + b12, b21 + b22)):
            wc_block(c, jc)[64 * p + r:64 * p + r + nr, :] = _as_u32(v.astype(BF))

    def cost(piece):
        if not isinstance(piece, P):
            return 0
        return {s_prep: CP, s_post: CP, wo_comb: CW, stage_rhs: CS}.get(piece.func, 0)

    def bulk(where, n, events, q=None):
        for i in range(n):
            ch, jj = where(i)

            def hook(k, m):
                pieces = events.get(7 * i + k, ())
                total, done = sum(cost(pc) for pc in pieces), 0
                for piece in pieces:
                    r = 8 * ((32 * done) // total) if cost(piece) else 0
                    done += cost(piece)
                    piece(m[r:r + 8])

            def keep(k):
                return v_s.at[jj // 4, (jj // 2) % 2, pl.ds(1024 * (jj % 2) + 256 * k, 256), :]

            def init(k):
                return jnp.where(q > 0, keep(k)[...], 0.0)

            rhs = staged_rhs(i % 2) if q is None else prep_rhs(ch, jj, pl.multiple_of(q * KQ, KQ))
            strassen(rhs, q, 8 * ch + jj,
                     None if q is None else init, None if q is None else keep, hook)

    def spread(events, pieces, q0, q1):
        for i, piece in enumerate(pieces):
            events.setdefault(q0 + ((q1 - q0) * i) // len(pieces), []).append(piece)

    P = functools.partial

    def loop_a(n, c):
        for e in range(2):
            wait(w_half(raw4[0].at[n // 2], n % 2, e), SEM_W0 + n)
        h = jnp.maximum(n - 2, 0)

        @pl.when(n >= 2)
        def _():
            wait(fraw.at[h], SEM_F + h)

        src = jnp.where(n >= 2, h, 4)
        events = {}
        spread(events, [lambda tok, c=c: fprep(src, h, c) for c in range(4)], 0, 48)
        bulk(lambda i: (n // 2, i), 8, events, n % 2)
        return c

    def loop_b(g, c):
        @pl.when((g >= 1) & (g < 3))
        def _():
            wait(raw4[1].at[g], SEM_W + 3 + g)

        for e in range(2):
            wait(wo.at[g + 4 * e], SEM_WO + g)
        gn = jnp.minimum(g + 1, 3)
        events = {}
        for k1 in range(4):
            q = BD * k1
            spread(events, [P(s_fwd, g, k1 + 4 * k0) for k0 in range(8)], q, q + BW)
            spread(events, [P(s_prep, gn, k1, r) for r in range(0, N2, 8)], q + BW, q + BW + BV)
            q += BL
            spread(events, [P(s_inv, k1 + 4 * k0) for k0 in range(8)], q, q + BW)
            spread(events, [P(s_post, g, k1, r) for r in range(0, N2, 8)], q + BW, q + BW + BV)
        for i in range(6):
            nxt = jnp.minimum(6 * g + i + 1, 23)
            spread(events, [P(stage_rhs, nxt, (i + 1) % 2, d0) for d0 in range(0, KH, PB)], 7 * i, 7 * i + SE)
        combs = [P(wo_comb, g, p, r) for p in range(NP) for r in range(0, 64, 64 // WSP)]
        load = lambda q: sum(cost(pc) for pc in events.get(q, ()))
        for piece in combs:
            events.setdefault(min(range(W0, W1), key=load), []).append(piece)
        ny = nyquist()
        spread(events, [lambda tok: next(ny)] * 4, NY0, NY1)
        assert max(events) < 41
        bulk(lambda i: (b_item(6 * g + i, i % 2)[0], b_item(6 * g + i, i % 2)[1] + 4 * (i % 2)), 6, events)
        return c

    def prep0(i, c):
        for k1 in range(4):
            s_prep(0, k1, pl.multiple_of(i * 8, 8), None)
        return c

    lax.fori_loop(0, N2 // 8, prep0, 0)
    with jax.named_scope("loop_a"):
        lax.fori_loop(0, 6, loop_a, 0)
    wait(sm, SEM_SM)
    wait(nm, SEM_NYM)
    wait(nyq, SEM_NYQ)
    wait(gs, SEM_GS)
    with jax.named_scope("loop_b"):
        wait(raw4[1].at[0], SEM_W + 3)
        for d0 in range(0, KH, PB):
            stage_rhs(0, 0, d0, None)
        lax.fori_loop(0, 4, loop_b, 0)
    wait(gi, SEM_GI)
    wait(mem_ref, SEM_MEM)
    wait(gw_ref.at[pl.ds(0, D)], SEM_GW)

    scale = DH ** -0.5

    gw_s[...] = jnp.broadcast_to(gw_ref[pl.ds(0, D)].astype(F32).reshape(1, D), (8, D))

    def softmax(s):
        fill = mf[0:80, :]
        s = jnp.where(fill > 0.0, s * scale, fill)
        m = jnp.max(s, axis=-1, keepdims=True)
        e = jnp.exp(s - m)
        l = jnp.sum(e, axis=-1, keepdims=True)
        r = pl.reciprocal(l, approx=True)
        return (e * (r * (2.0 - l * r))).astype(BF)

    def lhs_rows(mem, seg):
        xs = x_v[pl.ds(pl.multiple_of(seg * SEG, SEG), SEG), :].astype(F32)
        return jnp.concatenate([mem, xs[8:SEG]], axis=0).astype(BF)

    def proj2(a, m, j):
        return jnp.concatenate([_dot(_as_bf(a[...]), _as_bf(wqkv[H * m + 2 * j + p])).astype(BF)
                                for p in range(2)], axis=0)

    def proj_lo(a):
        for i in range(6):
            pa_s[i] = _dot(_as_bf(a[:, :KH]), _as_bf(wqkv[H * (i // 2) + i % 2, 0:KH // 2, :]))

    def proj_hi(a):
        full = [(_dot(_as_bf(a[:, KH:]), _as_bf(wqkv[H * (i // 2) + i % 2, KH // 2:KH, :]))
                 + pa_s[i]).astype(BF) for i in range(6)]
        for m in range(3):
            stg[m, 0] = _as_u32(jnp.concatenate(full[2 * m:2 * m + 2], axis=0))

    def step(a, seg, k, hooks, late):
        srow = pl.multiple_of(seg * 8, 8)
        a = a[...]

        def get(m, j):
            return _as_bf(jnp.concatenate([stg[m, j % 8], st[NP * m + j, pl.ds(srow, 8), :]], axis=0))

        def proj(j, m):
            if j > 0:
                stg[m, j % 8] = _as_u32(proj2(a, m, j))
            elif m == 0:
                if k > 0:
                    proj_lo(a)
                proj_hi(a)

        def scores(j):
            pst[j % 8] = _as_u32(softmax(_dot_nt(get(0, j), get(1, j))))

        def pv(j):
            o = _dot(_as_bf(pst[j % 8]), get(2, j))
            if k < 3:
                for i in range(2):
                    sto[2 * j + i, 8 * k:8 * k + 8, :] = o[64 + 8 * i:72 + 8 * i]
                    obuf[2 * j + i] = _as_u32(o[32 * i:32 * i + 32].astype(BF))
            else:
                a11, a12 = o[0:32], o[32:64]
                a21, a22 = [jnp.concatenate([sto[2 * j + i, 0:24, :], o[64 + 8 * i:72 + 8 * i]], axis=0)
                            for i in range(2)]
                for i, v in enumerate((a11 + a22, a21 + a22, a11, a22, a11 + a12, a21 - a11, a12 - a22)):
                    lc[i, j] = _as_u32(v.astype(BF))

        def wo_part(j, h0, h1):
            og = jnp.concatenate([_as_bf(obuf[h]) for h in range(h0, h1)], axis=1)
            return _dot(og, _as_bf(wo[j, h0 * 64:h1 * 64, :]))

        def prod(i, jc, p0, p1):
            lhs = jnp.concatenate([_as_bf(lc[i, p]) for p in range(p0, p1)], axis=1)
            if i in (1, 4):
                e = i // 4
                rhs = jnp.concatenate([wo[jc + 4 * e, 128 * p + 64 * e:128 * p + 64 * e + 64, :]
                                       for p in range(p0, p1)], axis=0)
            else:
                rhs = wc_block((0, None, 1, 2, None, 3, 4)[i], jc)[64 * p0:64 * p1, :]
            return _dot(lhs, _as_bf(rhs))

        early = [(i, jc) for i in (0, 3, 4, 6) for jc in range(4)]
        parts = []
        for i in range(NP + 4):
            for ch in ORDER:
                if ch in "qkv":
                    m = "qkv".index(ch)
                    if i < NP:
                        proj(i, m)
                    elif m < 2:
                        for n in range(1 if k < 3 else 2):
                            r = wo_part(len(parts), 0, SPLIT) if k < 3 else prod(*early[len(parts)], 0, SP3)
                            mp[len(parts)] = r
                            parts.append(r[0:8])
                elif ch == "s" and 0 <= i - LAG1 < NP:
                    scores(i - LAG1)
                elif ch == "p" and 0 <= i - LAG2 < NP:
                    pv(i - LAG2)
            if i == HOOK_AT:
                for hook in hooks[k]:
                    hook()
        if k < 3:
            return jnp.concatenate([wo_part(j, SPLIT, H) + mp[j] for j in range(8)], axis=1)
        toks, c11, c12 = parts[T0:], [], []
        for jc in range(4):
            m1, m4, m5 = [prod(i, jc, SP3, NP) + mp[4 * n + jc] for n, i in enumerate((0, 3, 4))]
            c11.append(prod(6, jc, SP3, NP) + (mp[12 + jc] + (m1 + m4 - m5)))
            mp[jc], mp[4 + jc], mp[8 + jc] = m1, m4, m5
            toks += [m1[0:8]] * (jc % 2)
        for jc in range(4):
            m3 = prod(2, jc, 0, NP)
            c12.append(m3 + mp[8 + jc])
            mp[jc] = mp[jc] + m3
            toks.append(m3[0:8])
        for n, piece in enumerate(late):
            piece(toks[(n * len(toks)) // len(late)])
        c21 = []
        for jc in range(4):
            m2 = prod(1, jc, 0, NP)
            c21.append(m2 + mp[4 + jc])
            mp[jc] = mp[jc] - m2
        c22 = [prod(5, jc, 0, NP) + mp[jc] for jc in range(4)]
        return jnp.concatenate(c11 + c12, axis=1), jnp.concatenate(c21 + c22, axis=1)

    def start_quad(mem, u):
        a_s[0] = _as_u32(lhs_rows(mem, 4 * u))
        proj_lo(a_s.at[0])

    def quad(u, c):
        base = pl.multiple_of(u * 128, 128)
        roll = lambda v: pltpu.roll(v, 64, 1)
        a1 = u // 4
        s2 = (1 - 2 * (a1 & 1)).astype(F32)
        sg = (1 - (a1 & 2)).astype(F32)
        cc, ss = sg * (1 - (a1 & 1)).astype(F32), sg * (a1 & 1).astype(F32)

        def irfft_dots(r0):
            off = pl.multiple_of((u % 4) * 128, 128) + r0
            for g in range(4):
                q = [[v_s[g, e, pl.ds(off + QS * k1, SEG), :] for e in range(2)] for k1 in range(4)]
                br, bi = q[1][0] + s2 * q[3][0], q[1][1] + s2 * q[3][1]
                vr = q[0][0] + s2 * q[2][0] + (cc * br - ss * bi)
                vi = q[0][1] + s2 * q[2][1] + (cc * bi + ss * br)
                tin = _half_pre(vr, vi, _lanes(SEG) < 64, roll, jnp.where)
                for e in range(2):
                    ts_s[r0:r0 + SEG, 128 * (2 * g + e):128 * (2 * g + e + 1)] = _dot(
                        tin[e].astype(BF), _as_bf(gi[2 * g + e]))

        def mix(r0, tok):
            lane = _lanes(8)
            t = [anchored(ts_s[r0:r0 + 8, 128 * i:128 * i + 128], tok) for i in range(8)]
            nyc = jnp.sum(jnp.where(lane == u, anchored(ct[r0:r0 + 8, :], tok), 0.0), axis=-1, keepdims=True)
            t[0] = t[0] + nyc * (1 - 2 * (lane & 1)).astype(F32)
            t = sum([list(_half_post(g, t[2 * g], t[2 * g + 1], lane < 64, roll, jnp.where))
                     for g in range(4)], [])
            b = jnp.concatenate(_bfly8_t(t), axis=1).astype(BF).astype(F32)
            xg = x_v[pl.ds(base + r0, 8), :].astype(F32) * gw_s[...]
            xg = functools.reduce(jnp.add, [xg[:, 128 * i:128 * i + 128] for i in range(8)])
            gate = jax.nn.sigmoid(jnp.sum(anchored(xg, tok), axis=-1, keepdims=True))
            bb = (1.0 - gate) * b
            if r0 % SEG and r0 < 96:
                out_v[pl.ds(base + r0, 8), :] = (bb + gate * ra_s[r0:r0 + 8, :]).astype(BF)
            else:
                bb_s[r0:r0 + 8, :] = bb
                g_s[r0:r0 + 8, :] = jnp.broadcast_to(gate, (8, 128))

        hooks = [[P(irfft_dots, SEG * n) for n in range(4) if HMAP[n] == str(k)] for k in range(4)]
        late = [P(mix, r0) for r0 in range(0, 128, 8)]
        for k in range(3):
            res = step(a_s.at[k % 2], 4 * u + k, k, hooks, late)
            ra_s[32 * k + 8:32 * k + 32, :] = res[8:32]
            a_s[(k + 1) % 2] = _as_u32(lhs_rows(res[0:8], 4 * u + k + 1))
        res, first8 = step(a_s.at[1], 4 * u + 3, 3, hooks, late)

        def emit(r0, n, att):
            out_v[pl.ds(base + r0, n), :] = (
                bb_s[r0:r0 + n, :] + jnp.concatenate([g_s[r0:r0 + n, :]] * 8, axis=1) * att).astype(BF)

        emit(104, 24, res[8:32])
        for k in range(4):
            emit(32 * k, 8, first8[8 * k:8 * k + 8])
        pltpu.make_async_copy(out_v.at[pl.ds(base, 128), :], out_hbm.at[pl.ds(base, 128), :],
                              sem.at[SEM_OUT]).start()
        start_quad(res[0:8], jnp.minimum(u + 1, S // 128 - 1))
        return c

    with jax.named_scope("chain"):
        start_quad(mem_ref[...].astype(F32), 0)
        lax.fori_loop(0, S // 128, quad, 0)
    pltpu.make_async_copy(out_v, out_hbm, sem.at[SEM_OUT]).wait()


@jax.jit
def pallas_gated_mix__memory_aug_recurrent_mem_tr__spectral_gfnet__prompt_kernel(
    A_x, A_mem0, A_Wq, A_Wk, A_Wv, A_Wo, A_seg_len, B_x, B_w_r, B_w_i, gate_w,
):
    assert A_x.shape == (1, S, D) and A_mem0.shape == (1, M, D) and A_Wq.shape == (D, H, DH)
    consts = [jnp.asarray(c) for c in _constants()]
    any_spec = pl.BlockSpec(memory_space=pl.ANY)
    out = pl.pallas_call(
        _kernel,
        out_shape=jax.ShapeDtypeStruct((S, D), BF),
        in_specs=[any_spec] * 14,
        out_specs=any_spec,
        scratch_shapes=[
            pltpu.VMEM((S, D), BF),
            pltpu.VMEM((3, D * 8, DH), U32),
            pltpu.VMEM((3, D * 8, DH), U32),
            pltpu.VMEM((3 * H, D // 2, DH), U32),
            pltpu.VMEM((8, H * DH // 2, 128), U32),
            pltpu.VMEM((3 * NP, 8 * NSEG, 128), U32),
            pltpu.VMEM((NQ, 7, 2 * NSEG, D // 2 // NQ), U32),
            pltpu.VMEM((5, 2, 4, 256, 128), U32),
            pltpu.VMEM((4, N2 * PITCH, 128), U32),
            pltpu.VMEM((4, 128, 256), U32),
            pltpu.VMEM((64, 256), U32),
            pltpu.VMEM((8, 64, 128), U32),
            pltpu.VMEM((2, N1, N2 // 2, 2 * N2), U32),
            pltpu.VMEM((4, 2, S, 128), F32),
            pltpu.VMEM((4, 2, S, 128), F32),
            pltpu.VMEM((S, D), BF),
            pltpu.VMEM((6, 256, 128), F32),
            pltpu.VMEM((4, N2, 128), U32),
            pltpu.VMEM((N1, 2 * N2, 128), F32),
            pltpu.VMEM((2, 2, D // 4, 128), U32),
            pltpu.VMEM((2, D // 2, 5 * 128), BF),
            pltpu.VMEM((N1, N2, 256), BF),
            pltpu.VMEM((N1, N2, 256), BF),
            pltpu.VMEM((H, 32, 128), F32),
            pltpu.VMEM((H, 16, 128), U32),
            pltpu.VMEM((128, 128), F32),
            pltpu.VMEM((2, 16, D), U32),
            pltpu.VMEM((6, 32, 128), F32),
            pltpu.VMEM((128, D), F32),
            pltpu.VMEM((128, 128), F32),
            pltpu.VMEM((3, 8, 32, 128), U32),
            pltpu.VMEM((8, 40, 80), U32),
            pltpu.VMEM((128, D), F32),
            pltpu.VMEM((128, D), F32),
            pltpu.VMEM((16, 32, 128), F32),
            pltpu.VMEM((7, NP, 16, 128), U32),
            pltpu.VMEM((8, D), F32),
            pltpu.VMEM((M, D), BF),
            pltpu.VMEM((96, 80), F32),
            pltpu.VMEM((96, 128), F32),
            pltpu.VMEM((32, 128), F32),
            pltpu.VMEM((2, 1, S), BF),
            pltpu.VMEM((8 * D,), BF),
            pltpu.SMEM((2,), jnp.int32),
            pltpu.SemaphoreType.DMA((NSEM,)),
        ],
        compiler_params=pltpu.CompilerParams(vmem_limit_bytes=120 * 1024 * 1024,
                                             disable_bounds_checks=True,
                                             disable_semaphore_checks=True),
    )(
        A_x.reshape(S, D), A_mem0.reshape(M, D), A_Wq, A_Wk, A_Wv,
        A_Wo.reshape(H * DH, D), B_w_r.T, B_w_i.T, gate_w, *consts,
    )
    return out.reshape(1, S, D)
```

```python
import functools
import math

import numpy as np
import jax
import jax.numpy as jnp
from jax import lax
import jax.experimental.pallas as pl
import jax.experimental.pallas.tpu as pltpu

BF, F32, U32 = jnp.bfloat16, jnp.float32, jnp.uint32

S, D, H, DH, M, SEG = 2048, 1024, 32, 128, 8, 32
NSEG = S // SEG
NP = H // 2
N1, N2 = 32, 64
QS = S // 4
PITCH = N1 + 8
CLASSES = ((0, 8, 4, 12), (1, 15, 9, 7), (2, 14, 10, 6), (3, 13, 11, 5))
LAG1, LAG2, SPLIT, HOOK_AT = 1, 2, 27, 18
ORDER = "qksvp"
CP, CW, CS = 100, 45, 45
PB, SE = 16, 5
WSP, W0, W1 = 8, 0, 41
T0 = 6
HMAP = "0123"
SP3 = 13
NY0, NY1 = 30, 38
BD, BW, BV, BL = 7, 8, 8, 4
NQ = 2
(SEM_W, SEM_GF, SEM_GI, SEM_SM, SEM_GS, SEM_NYQ, SEM_NYM, SEM_MEM, SEM_GW, SEM_OUT, SEM_F, SEM_X,
 SEM_W0) = 0, 6, 7, 8, 9, 10, 11, 12, 13, 14, 15, 19, 23
SEM_WO = SEM_W0 + 6
NSEM = SEM_WO + 4
RSQ2 = float(np.float32(math.sqrt(0.5)))


def _bfly8(x):
    s = [x[i] + x[i + 4] for i in range(4)]
    d = [x[i] - x[i + 4] for i in range(4)]
    e, f = s[0] + s[2], s[1] + s[3]
    t1, t2 = (d[1] - d[3]) * RSQ2, (d[1] + d[3]) * RSQ2
    return [e + f, e - f, d[0] + t1, t2 + d[2], s[0] - s[2], s[1] - s[3], d[0] - t1, t2 - d[2]]


def _bfly8_t(t):
    e, f = t[0] + t[1], t[0] - t[1]
    s = [e + t[4], f + t[5], e - t[4], f - t[5]]
    t1, t2 = t[2] - t[6], t[3] + t[7]
    d = [t[2] + t[6], (t1 + t2) * RSQ2, t[3] - t[7], (t2 - t1) * RSQ2]
    return [s[i] + d[i] for i in range(4)] + [s[i] - d[i] for i in range(4)]


def _half_pre(vr, vi, lo, roll, where):
    ri = roll(vi)
    return where(lo, vr, ri), where(lo, ri, vr)


def _half_post(g, tp, tm, lo, roll, where):
    if g == 0:
        return tp, tm
    c = float(np.float32(math.cos(math.pi * g / 8)))
    s = float(np.float32(math.sin(math.pi * g / 8)))
    p, r = tp + tm, tp - tm
    rm = roll(where(lo, r, p))
    return where(lo, p, c * rm + s * r), where(lo, rm, c * r - s * rm)


def _cmul_const(v, k, n, sign):
    re, im = v
    k %= n
    if k == 0:
        return re, im
    if 4 * k == n:
        return (-im, re) if sign > 0 else (im, -re)
    if 8 * k == n:
        return (((re - im) * RSQ2, (re + im) * RSQ2) if sign > 0
                else ((re + im) * RSQ2, (im - re) * RSQ2))
    if 8 * k == 3 * n:
        return (((re + im) * -RSQ2, (re - im) * RSQ2) if sign > 0
                else ((im - re) * RSQ2, (re + im) * -RSQ2))
    c, s = math.cos(2 * math.pi * k / n), sign * math.sin(2 * math.pi * k / n)
    return re * c - im * s, re * s + im * c


def _fft(v, sign):
    n = len(v)
    if n == 1:
        return v
    ev, od = _fft(v[0::2], sign), _fft(v[1::2], sign)
    lo, hi = [], []
    for k in range(n // 2):
        er, ei = ev[k]
        if 4 * k == n:
            xr, xi = od[k]
            if sign > 0:
                lo.append((er - xi, ei + xr)); hi.append((er + xi, ei - xr))
            else:
                lo.append((er + xi, ei - xr)); hi.append((er - xi, ei + xr))
            continue
        tr, ti = _cmul_const(od[k], k, n, sign)
        lo.append((er + tr, ei + ti))
        hi.append((er - tr, ei - ti))
    return lo + hi


def _pack_rows(a):
    u = np.ascontiguousarray(a, dtype=np.float32).view(np.uint32)
    b = ((u + 0x7FFF + ((u >> 16) & 1)) >> 16).astype(np.uint32)
    return (b[..., 0::2, :] | (b[..., 1::2, :] << 16)).astype(np.uint32)


def _diag_blocks(full, n, tol):
    k = full.shape[0] // n
    blk = np.kron(np.eye(k), np.ones((n, n)))
    assert np.abs(full * (1 - blk)).max() < tol
    return np.stack([full[n * g:n * g + n, n * g:n * g + n] for g in range(k)])


@functools.lru_cache(maxsize=None)
def _constants():
    k2 = np.stack([np.concatenate([c + 16 * np.arange(32) for c in cls]) for cls in CLASSES])
    n2 = np.arange(D)
    ang = 2 * np.pi * ((k2[:, :, None] * n2[None, None, :]) % D) / D
    rows = np.stack([np.cos(ang), -np.sin(ang)], axis=1)
    wgt = np.where(k2 == 0, 1.0, 2.0)[:, None, :, None]
    fwd = rows.reshape(D, D).T
    inv = (rows * wgt).reshape(D, D) / (S * D)
    bf = np.stack(_bfly8(list(np.eye(8))))
    binv = np.kron(np.linalg.inv(bf), np.eye(128))
    gd = _diag_blocks(binv.T @ fwd, 256, 1e-6)
    gdi = _diag_blocks(inv @ binv, 256, 1e-12)
    eye, lo = np.eye(256), np.arange(128) < 64
    roll = lambda v: np.roll(v, 64, axis=1)
    pre = np.concatenate(_half_pre(eye[:, :128], eye[:, 128:], lo, roll, np.where), axis=1)
    gi = []
    for g in range(4):
        post = np.concatenate(_half_post(g, eye[:, :128], eye[:, 128:], lo, roll, np.where), axis=1)
        gi.append(_diag_blocks(np.linalg.inv(pre) @ gdi[g] @ np.linalg.inv(post), 128, 1e-12))
    gi = np.concatenate(gi)

    b = np.arange(N2)
    k1 = np.arange(N1)[:, None] + N1 * np.arange(N2)[None, :]
    th = 2 * np.pi * ((k1[:, :, None] * b[None, None, :]) % S) / S
    gr, gim = np.cos(th), -np.sin(th)
    gs = np.concatenate([gr, -gim], axis=2)
    hr, hi = np.swapaxes(gr, 1, 2), -np.swapaxes(gim, 1, 2)
    gsi = np.concatenate([hr, -hi], axis=2)

    lane = np.arange(128)
    kb = 8 * (lane % 16) + lane // 16
    t128 = 2 * np.pi * ((lane[:, None] * kb[None, :]) % 128) / 128
    nym = np.concatenate([np.cos(t128), np.sin(t128)], axis=1)
    i16 = np.arange(16)
    t16 = 2 * np.pi * ((i16[:, None] * i16[None, :]) % 16) / 16
    tw = 2 * np.pi * (i16[:, None] * lane[None, :]) / S
    sm = np.zeros((96, 128), np.float32)
    sm[0:16], sm[16:32] = np.cos(tw), np.sin(tw)
    sm[32:48, :16], sm[48:64, :16] = np.cos(t16), -np.sin(t16)
    sm[64:80, :16], sm[64:80, 16:32] = np.cos(t16), -np.sin(t16)

    return _pack_rows(gd), _pack_rows(nym), _pack_rows(gi), sm, _pack_rows(np.stack([gs, gsi]))


def _mask80():
    r = lax.broadcasted_iota(jnp.int32, (80, 80), 0)
    c = lax.broadcasted_iota(jnp.int32, (80, 80), 1)

    def head(i):
        return jnp.where(i < 64, i >> 5, (i - 64) >> 3)

    def pos(i):
        j = i & 31
        return jnp.where(i < 64, jnp.where(j < M, j, j + 8), M + (i & 7))

    same = head(r) == head(c)
    ok = (pos(r) < M) | (pos(c) <= pos(r))
    return jnp.where(same, jnp.where(ok, 1.0, -1e9), -jnp.inf).astype(F32)


def _as_bf(u):
    return pltpu.bitcast(u, BF)


def _as_u32(b):
    return pltpu.bitcast(b, U32)


def _lo_f32(u):
    return pltpu.bitcast(u << 16, F32)


def _hi_f32(u):
    return pltpu.bitcast(u & jnp.uint32(0xFFFF0000), F32)


def _dot(a, b):
    return jnp.dot(a, b, preferred_element_type=F32)


def _dot_nt(a, b):
    return lax.dot_general(a, b, (((1,), (1,)), ((), ())), preferred_element_type=F32)


def _transpose_u32(u):
    return pltpu.bitcast(pltpu.bitcast(u, F32).T, U32)


def _lanes(rows):
    return lax.broadcasted_iota(jnp.int32, (rows, 128), 1)


def _kernel(x_hbm, mem_hbm, wq_hbm, wk_hbm, wv_hbm, wo_hbm, fr_hbm, fi_hbm, gw_hbm,
            gf_hbm, nm_hbm, gi_hbm, sm_hbm, gs_hbm,
            out_hbm,
            x_v, raw_a, raw_b, wqkv, wo, st, sl, fraw, fp, gf, nm, gi, gs, y, v_s, out_v, cb, z_s, p_s,
            rs_u, rs_c, u_b, z_b, sto, obuf, ct, a_s, pa_s, bb_s, g_s, stg, pst, ra_s, ts_s, mp, lc, gw_s,
            mem_ref, mf, sm, xa, nyq, gw_ref, zero_s, sem):
    KH = D // 2
    KQ = KH // NQ
    RB, HB = 128, 16
    raw4 = [r.reshape(3, D, 8, DH) for r in (raw_a, raw_b)]
    w_hbm = (wq_hbm, wk_hbm, wv_hbm)
    f_hbm = (fr_hbm, fi_hbm)

    def w_src(c):
        return w_hbm[c // 2].bitcast(U32).at[:, pl.ds(8 * (c % 2), 8), :]

    def wait(dst, k):
        pltpu.make_async_copy(dst, dst, sem.at[k]).wait()

    def w_half(ref, q, e):
        return ref.at[pl.ds(pl.multiple_of(q * KQ, KQ) + e * KH, KQ)]

    def x_rows(i, a1):
        return pl.ds(pl.multiple_of(i * RB, RB) + QS * a1, RB)

    def f_copies(h):
        return [(f_hbm[a].at[pl.ds(0, D // 2), pl.ds(128 * (4 * h + c), 128)].bitcast(U32),
                 fraw.at[h, a, c], SEM_F + h) for a in range(2) for c in range(4)]

    def w_copy(c):
        return [(w_src(c), raw4[1].at[c - 3], SEM_W + c)]

    copies = [(gf_hbm, gf, SEM_GF)]
    copies += [(x_hbm.at[x_rows(i, a1), :], x_v.at[x_rows(i, a1), :], SEM_X + i)
               for i in range(QS // RB) for a1 in range(4)]
    for n in range(6):
        copies += [(w_half(w_src(n // 2), n % 2, e), w_half(raw4[0].at[n // 2], n % 2, e), SEM_W0 + n)
                   for e in range(2)]
        if n >= 2:
            copies += f_copies(n - 2)
    copies += [(sm_hbm, sm, SEM_SM), (nm_hbm, nm, SEM_NYM)]
    copies += [(f_hbm[a].at[pl.ds(D // 2, 1), :], nyq.at[a], SEM_NYQ) for a in range(2)]
    copies += [(gs_hbm, gs, SEM_GS)]
    for g in range(4):
        copies += w_copy(3 + g) if g < 3 else []
        copies += [(wo_hbm.bitcast(U32).at[:, pl.ds(128 * j, 128)], wo.at[j], SEM_WO + g) for j in (g, g + 4)]
    copies += [(gi_hbm, gi, SEM_GI), (mem_hbm, mem_ref, SEM_MEM), (gw_hbm, gw_ref.at[pl.ds(0, D)], SEM_GW)]
    for src, dst, k in copies:
        pltpu.make_async_copy(src, dst, sem.at[k]).start()

    def prep_rhs(ch, jj, k0):
        a1 = raw_a[ch, pl.ds(k0 * 8 + jj, KQ, stride=8), :]
        a2 = raw_a[ch, pl.ds((KH + k0) * 8 + jj, KQ, stride=8), :]
        b11, b12, b21, b22 = _lo_f32(a1), _hi_f32(a1), _lo_f32(a2), _hi_f32(a2)
        for p, e, b in ((0, 0, b11), (1, 0, b12), (0, 1, b21), (1, 1, b22)):
            row = pl.multiple_of(k0 // 2, KQ // 2) + e * KH // 2
            wqkv[2 * (8 * ch + jj) + p, pl.ds(row, KQ // 2), :] = _as_u32(b.astype(BF))
        return [v.astype(BF) for v in (b11 + b22, b11, b12 - b22, b21 - b11, b22, b11 + b12, b21 + b22)]

    def b_item(n, par):
        return 3 + n // 8, (n // 2) % 4

    def stage_rhs(n, par, d0, tok):
        ch, low = b_item(n, par)
        item = 8 * ch + low + 4 * par
        a = [raw_b[ch - 3, pl.ds(low + ((e * KH + d0) * 8 + 4 * par), PB, stride=8), :] for e in range(2)]
        if tok is not None:
            tok = jnp.concatenate([pltpu.bitcast(tok, U32)] * (PB // 8), axis=0)
            a = [anchored(v, tok) for v in a]
        b11, b12, b21, b22 = _lo_f32(a[0]), _hi_f32(a[0]), _lo_f32(a[1]), _hi_f32(a[1])
        for p, e, b in ((0, 0, b11), (1, 0, b12), (0, 1, b21), (1, 1, b22)):
            u = _as_u32(b.astype(BF))
            wqkv[2 * item + p, pl.ds((e * KH + d0) // 2, PB // 2), :] = u
            if p == e:
                rs_u[par, p, d0 // 2:(d0 + PB) // 2, :] = u
        comb = [b11 + b22, b12 - b22, b21 - b11, b11 + b12, b21 + b22]
        rs_c[par, d0:d0 + PB, :] = jnp.concatenate(comb, axis=1).astype(BF)

    def staged_rhs(par):
        c = lambda i: (lambda: rs_c[par, :, 128 * i:128 * i + 128])
        return [c(0), lambda: _as_bf(rs_u[par, 0]), c(1), c(2), lambda: _as_bf(rs_u[par, 1]), c(3), c(4)]

    def strassen(rhs, q, item, init, keep, after_dot):
        def prod(i):
            lhs = sl[q, i] if q is not None else jnp.concatenate([sl[k, i] for k in range(NQ)], axis=1)
            return _dot(_as_bf(lhs), rhs[i]() if callable(rhs[i]) else rhs[i])

        def plus(i, r):
            return r if init is None else init(i) + r

        c12, c21 = (cb.at[5], cb.at[4]) if keep is None else (keep(1), keep(2))

        def done(k, c):
            if keep is not None:
                keep(3 * k)[...] = c
            store_st(item, k, *((c, c12[...]) if k == 0 else (c21[...], c)))

        m = prod(1)
        cb[0] = m
        after_dot(0, m)
        m = prod(5) + plus(3, -cb[0])
        cb[3] = m
        after_dot(1, m)
        m = prod(4)
        cb[1] = m
        after_dot(2, m)
        m = prod(0)
        cb[2] = plus(0, m - cb[1])
        cb[3] = cb[3] + m
        after_dot(3, m)
        m = prod(3)
        c21[...] = plus(2, cb[0] + m)
        cb[2] = cb[2] + m
        after_dot(4, m)
        m = prod(2)
        c12[...] = plus(1, cb[1] + m)
        done(1, cb[3] + m)
        after_dot(5, m)
        m = prod(6) + cb[2]
        done(0, m)
        after_dot(6, m)

    def store_st(item, e, c1, c2):
        r = jnp.concatenate([c.reshape(NSEG // 2, 8, 128) for c in (c1, c2)], axis=1)
        st[item, 256 * e:256 * e + 256, :] = _as_u32(r.reshape(8 * NSEG, 128).astype(BF))

    def pin(i, c):
        cb[i, 0:8, :] = jnp.zeros((8, 128), F32)
        zero_s[i] = 0
        z_b[i, 0:16, 0:128] = jnp.zeros((16, 128), BF)
        rs_u[i, 0, 0:8, :] = jnp.zeros((8, 128), U32)
        rs_c[i, 0:16, 0:128] = jnp.zeros((16, 128), BF)
        z_s[i, 0:8, :] = jnp.zeros((8, 128), U32)
        p_s[i, 0:8, :] = jnp.zeros((8, 128), F32)
        stg[i, 0, 0:8, :] = jnp.zeros((8, 128), U32)
        obuf[i, 0:8, :] = jnp.zeros((8, 128), U32)
        sto[i, 0:8, :] = jnp.zeros((8, 128), F32)
        lc[i, 0, 0:8, :] = jnp.zeros((8, 128), U32)
        mp[i, 0:8, :] = jnp.zeros((8, 128), F32)
        ts_s[pl.ds(pl.multiple_of(8 * i, 8), 8), 0:128] = jnp.zeros((8, 128), F32)
        ra_s[pl.ds(pl.multiple_of(8 * i, 8), 8), 0:128] = jnp.zeros((8, 128), F32)
        a_s[i, 0:8, 0:128] = jnp.zeros((8, 128), U32)
        pa_s[i, 0:8, :] = jnp.zeros((8, 128), F32)
        bb_s[pl.ds(pl.multiple_of(8 * i, 8), 8), 0:128] = jnp.zeros((8, 128), F32)
        g_s[pl.ds(pl.multiple_of(8 * i, 8), 8), :] = jnp.zeros((8, 128), F32)
        return c

    lax.fori_loop(0, 2, pin, 0)

    mf[0:80, :] = _mask80()
    fraw[4] = jnp.zeros(fraw.shape[1:], U32)

    wait(gf, SEM_GF)

    def f1(i, c):
        for a1 in range(4):
            wait(x_v.at[x_rows(i, a1), :], SEM_X + i)
        base = pl.multiple_of(i * RB, RB)
        alt = (1 - 2 * (_lanes(16) & 1)).astype(F32).astype(BF)

        def rows16(r):
            return jnp.concatenate([x_v[pl.ds(r + d, 16), :].astype(F32)[0:8] for d in (0, SEG)], axis=0)

        for r in (0, 64, QS, QS + 64):
            top, bot = rows16(base + r), rows16(base + (r + 2 * QS))
            a11, a12, a21, a22 = top[:, :KH], top[:, KH:], bot[:, :KH], bot[:, KH:]
            row = pl.multiple_of((base + r) // 8, 8)
            for k, v in enumerate((a11 + a22, a21 + a22, a11, a22, a11 + a12, a21 - a11, a12 - a22)):
                for q in range(NQ):
                    sl[q, k, pl.ds(row, 8), :] = _as_u32(v[:, q * KQ:(q + 1) * KQ].astype(BF))
        for h0 in range(0, RB, HB):
            pieces = []
            for a1 in range(4):
                for r in range(h0, h0 + HB, 16):
                    xs = x_v[pl.ds(base + (QS * a1 + r), 16), :].astype(F32)
                    pieces.append(jnp.concatenate(_bfly8([xs[:, 128 * a:128 * a + 128] for a in range(8)]),
                                                  axis=1))
                    z_s[a1, r // 2:r // 2 + 8, :] = _as_u32(pieces[-1][:, :128].astype(BF))
            ub = jnp.concatenate(pieces, axis=0)
            for g in range(4):
                yy = _dot(ub[:, 256 * g:256 * g + 256].astype(BF), _as_bf(gf[g]))
                v = _fft([(yy[HB * a1:HB * a1 + HB, :128], yy[HB * a1:HB * a1 + HB, 128:])
                          for a1 in range(4)], -1)
                for k1 in range(4):
                    rows = pl.ds(base + (QS * k1 + h0), HB)
                    y[g, 0, rows, :] = v[k1][0]
                    y[g, 1, rows, :] = v[k1][1]
                if h0 + HB == RB and g == 3:
                    for a1 in range(4):
                        xa[pl.ds(4 * a1 + i, 1), :] = _dot_nt(alt, _as_bf(z_s[a1]))[0:1]
        return c

    with jax.named_scope("f1"):
        lax.fori_loop(0, QS // RB, f1, 0)

    def fprep(src, h, c):
        ev, od = [], []
        for r in range(8):
            wr = fraw[src, 0, c, pl.ds(r, 32, stride=8), :]
            wi = fraw[src, 1, c, pl.ds(r, 32, stride=8), :]
            ev.append((wr & jnp.uint32(0xFFFF)) | (wi << 16))
            od.append((wr >> 16) | (wi & jnp.uint32(0xFFFF0000)))
        for g, cls in enumerate(CLASSES):
            t = _transpose_u32(jnp.concatenate([(od if k % 2 else ev)[k // 2] for k in cls], axis=0))
            for q in range(128 // N1):
                row = pl.multiple_of(((4 * h + c) * (128 // N1) + q) * PITCH, 8)
                fp[g, pl.ds(row, N1), :] = t[q * N1:(q + 1) * N1]

    def nyquist():
        twc, tws = sm[0:16], sm[16:32]
        u = _dot(sm[32:64, 0:16].astype(BF), xa[0:16, :].astype(BF))
        ur, ui = u[0:16], u[16:32]
        u = jnp.concatenate([ur * twc + ui * tws, ui * twc - ur * tws], axis=0).astype(BF)
        yield
        xx = _dot(u, _as_bf(nm[...]))
        xr, xi = xx[0:16, :128] + xx[16:32, 128:], xx[16:32, :128] - xx[0:16, 128:]
        w = (pltpu.bitcast(nyq[0].astype(F32), U32) >> 16) | pltpu.bitcast(nyq[1].astype(F32), U32)
        w = jnp.concatenate([w[:, 128 * a:128 * a + 128] for a in range(16)], axis=0)
        wt = _transpose_u32(jnp.concatenate([w] * 8, axis=0))
        blk = _lanes(16) >> 4
        wm = wt[0:16]
        for j in range(1, 8):
            wm = jnp.where(blk == j, wt[16 * j:16 * j + 16], wm)
        wr, wi = _lo_f32(wm), _hi_f32(wm)
        z = jnp.concatenate([xr * wr - xi * wi, xr * wi + xi * wr], axis=0).astype(BF)
        yield
        zc, zs = _dot_nt(z, _as_bf(nm[:, :128])), _dot_nt(z, _as_bf(nm[:, 128:]))
        pr, pi = zc[0:16] - zs[16:32], zs[0:16] + zc[16:32]
        pp = jnp.concatenate([pr * twc - pi * tws, pi * twc + pr * tws], axis=0).astype(BF)
        yield
        cc = _dot(sm[64:80, 0:32].astype(BF), pp) * (1.0 / (S * D))
        ct[...] = jnp.concatenate([cc, jnp.zeros((112, 128), F32)], axis=0).T
        yield

    def s_rows(k1, a0, r):
        return pl.ds(r + (QS * k1 + N2 * a0), 8)

    def anchored(v, tok):
        return jnp.where(zero_s[0] != 0, tok, v)

    def s_prep(g, k1, r, tok):
        v = [(y[g, 0, s_rows(k1, a0, r), :], y[g, 1, s_rows(k1, a0, r), :]) for a0 in range(8)]
        if tok is not None:
            v[0] = (anchored(v[0][0], tok), v[0][1])
        v = _fft([_cmul_const(v[a0], a0 * k1, N1, -1) for a0 in range(8)], -1)
        for k0 in range(8):
            u_b[k1 + 4 * k0, pl.ds(r, 8), :] = jnp.concatenate(v[k0], axis=1).astype(BF)

    def cdot(mat, ref, ka):
        vr, vi = ref[ka, :, :128], ref[ka, :, 128:]
        neg = _as_bf(_as_u32(vr) ^ jnp.uint32(0x80008000))
        return [_dot(_as_bf(mat), jnp.concatenate(v, axis=0)) for v in ((vr, vi), (vi, neg))]

    def s_fwd(g, ka, tok):
        xr, xi = cdot(gs[0, ka], u_b, ka)
        w32 = fp[g, pl.ds(ka, N2, stride=PITCH), :]
        wr, wi = _lo_f32(w32), _hi_f32(w32)
        z_b[ka] = jnp.concatenate([xr * wr - xi * wi, xr * wi + xi * wr], axis=1).astype(BF)

    def s_inv(ka, tok):
        p_s[ka] = jnp.concatenate(cdot(gs[1, ka], z_b, ka), axis=0)

    def s_post(g, k1, r, tok):
        v = [(p_s[k1 + 4 * k0, r:r + 8, :], p_s[k1 + 4 * k0, N2 + r:N2 + r + 8, :]) for k0 in range(8)]
        v[0] = (anchored(v[0][0], tok), anchored(v[0][1], tok))
        v = _fft(v, 1)
        for a0 in range(8):
            vr, vi = _cmul_const(v[a0], a0 * k1, N1, 1)
            v_s[g, 0, s_rows(k1, a0, r), :] = vr
            v_s[g, 1, s_rows(k1, a0, r), :] = vi

    def wc_block(c, jc):
        return raw_a.at[c // 2, pl.ds(pl.multiple_of(4096 * (c % 2) + 1024 * jc, 1024), 1024), :]

    def wo_comb(jc, p, r, tok):
        nr = 64 // WSP
        u = [wo[jc + 4 * f, 128 * p + 64 * e + r:128 * p + 64 * e + r + nr, :] for e in range(2) for f in range(2)]
        tok = jnp.concatenate([pltpu.bitcast(tok, U32)] * (nr // 8), axis=0)
        u[0], u[3] = anchored(u[0], tok), anchored(u[3], tok)
        b11, b12, b21, b22 = [_as_bf(v).astype(F32) for v in u]
        for c, v in enumerate((b11 + b22, b12 - b22, b21 - b11, b11 + b12, b21 + b22)):
            wc_block(c, jc)[64 * p + r:64 * p + r + nr, :] = _as_u32(v.astype(BF))

    def cost(piece):
        if not isinstance(piece, P):
            return 0
        return {s_prep: CP, s_post: CP, wo_comb: CW, stage_rhs: CS}.get(piece.func, 0)

    def bulk(where, n, events, q=None):
        for i in range(n):
            ch, jj = where(i)

            def hook(k, m):
                pieces = events.get(7 * i + k, ())
                total, done = sum(cost(pc) for pc in pieces), 0
                for piece in pieces:
                    r = 8 * ((32 * done) // total) if cost(piece) else 0
                    done += cost(piece)
                    piece(m[r:r + 8])

            def keep(k):
                return v_s.at[jj // 4, (jj // 2) % 2, pl.ds(1024 * (jj % 2) + 256 * k, 256), :]

            def init(k):
                return jnp.where(q > 0, keep(k)[...], 0.0)

            rhs = staged_rhs(i % 2) if q is None else prep_rhs(ch, jj, pl.multiple_of(q * KQ, KQ))
            strassen(rhs, q, 8 * ch + jj,
                     None if q is None else init, None if q is None else keep, hook)

    def spread(events, pieces, q0, q1):
        for i, piece in enumerate(pieces):
            events.setdefault(q0 + ((q1 - q0) * i) // len(pieces), []).append(piece)

    P = functools.partial

    def loop_a(n, c):
        for e in range(2):
            wait(w_half(raw4[0].at[n // 2], n % 2, e), SEM_W0 + n)
        h = jnp.maximum(n - 2, 0)

        @pl.when(n >= 2)
        def _():
            wait(fraw.at[h], SEM_F + h)

        src = jnp.where(n >= 2, h, 4)
        events = {}
        spread(events, [lambda tok, c=c: fprep(src, h, c) for c in range(4)], 0, 48)
        bulk(lambda i: (n // 2, i), 8, events, n % 2)
        return c

    def loop_b(g, c):
        @pl.when((g >= 1) & (g < 3))
        def _():
            wait(raw4[1].at[g], SEM_W + 3 + g)

        for e in range(2):
            wait(wo.at[g + 4 * e], SEM_WO + g)
        gn = jnp.minimum(g + 1, 3)
        events = {}
        for k1 in range(4):
            q = BD * k1
            spread(events, [P(s_fwd, g, k1 + 4 * k0) for k0 in range(8)], q, q + BW)
            spread(events, [P(s_prep, gn, k1, r) for r in range(0, N2, 8)], q + BW, q + BW + BV)
            q += BL
            spread(events, [P(s_inv, k1 + 4 * k0) for k0 in range(8)], q, q + BW)
            spread(events, [P(s_post, g, k1, r) for r in range(0, N2, 8)], q + BW, q + BW + BV)
        for i in range(6):
            nxt = jnp.minimum(6 * g + i + 1, 23)
            spread(events, [P(stage_rhs, nxt, (i + 1) % 2, d0) for d0 in range(0, KH, PB)], 7 * i, 7 * i + SE)
        combs = [P(wo_comb, g, p, r) for p in range(NP) for r in range(0, 64, 64 // WSP)]
        load = lambda q: sum(cost(pc) for pc in events.get(q, ()))
        for piece in combs:
            events.setdefault(min(range(W0, W1), key=load), []).append(piece)
        ny = nyquist()
        spread(events, [lambda tok: next(ny)] * 4, NY0, NY1)
        assert max(events) < 41
        bulk(lambda i: (b_item(6 * g + i, i % 2)[0], b_item(6 * g + i, i % 2)[1] + 4 * (i % 2)), 6, events)
        return c

    def prep0(i, c):
        for k1 in range(4):
            s_prep(0, k1, pl.multiple_of(i * 8, 8), None)
        return c

    lax.fori_loop(0, N2 // 8, prep0, 0)
    with jax.named_scope("loop_a"):
        lax.fori_loop(0, 6, loop_a, 0)
    wait(sm, SEM_SM)
    wait(nm, SEM_NYM)
    wait(nyq, SEM_NYQ)
    wait(gs, SEM_GS)
    with jax.named_scope("loop_b"):
        wait(raw4[1].at[0], SEM_W + 3)
        for d0 in range(0, KH, PB):
            stage_rhs(0, 0, d0, None)
        lax.fori_loop(0, 4, loop_b, 0)
    wait(gi, SEM_GI)
    wait(mem_ref, SEM_MEM)
    wait(gw_ref.at[pl.ds(0, D)], SEM_GW)

    scale = DH ** -0.5

    gw_s[...] = jnp.broadcast_to(gw_ref[pl.ds(0, D)].astype(F32).reshape(1, D), (8, D))

    def softmax(s):
        fill = mf[0:80, :]
        s = jnp.where(fill > 0.0, s * scale, fill)
        m = jnp.max(s, axis=-1, keepdims=True)
        e = jnp.exp(s - m)
        l = jnp.sum(e, axis=-1, keepdims=True)
        r = pl.reciprocal(l, approx=True)
        return (e * (r * (2.0 - l * r))).astype(BF)

    def lhs_rows(mem, seg):
        xs = x_v[pl.ds(pl.multiple_of(seg * SEG, SEG), SEG), :].astype(F32)
        return jnp.concatenate([mem, xs[8:SEG]], axis=0).astype(BF)

    def proj2(a, m, j):
        return jnp.concatenate([_dot(_as_bf(a[...]), _as_bf(wqkv[H * m + 2 * j + p])).astype(BF)
                                for p in range(2)], axis=0)

    def proj_lo(a):
        for i in range(6):
            pa_s[i] = _dot(_as_bf(a[:, :KH]), _as_bf(wqkv[H * (i // 2) + i % 2, 0:KH // 2, :]))

    def proj_hi(a):
        full = [(_dot(_as_bf(a[:, KH:]), _as_bf(wqkv[H * (i // 2) + i % 2, KH // 2:KH, :]))
                 + pa_s[i]).astype(BF) for i in range(6)]
        for m in range(3):
            stg[m, 0] = _as_u32(jnp.concatenate(full[2 * m:2 * m + 2], axis=0))

    def step(a, seg, k, hooks, late):
        srow = pl.multiple_of(seg * 8, 8)
        a = a[...]

        def get(m, j):
            return _as_bf(jnp.concatenate([stg[m, j % 8], st[NP * m + j, pl.ds(srow, 8), :]], axis=0))

        def proj(j, m):
            if j > 0:
                stg[m, j % 8] = _as_u32(proj2(a, m, j))
            elif m == 0:
                if k > 0:
                    proj_lo(a)
                proj_hi(a)

        def scores(j):
            pst[j % 8] = _as_u32(softmax(_dot_nt(get(0, j), get(1, j))))

        def pv(j):
            o = _dot(_as_bf(pst[j % 8]), get(2, j))
            if k < 3:
                for i in range(2):
                    sto[2 * j + i, 8 * k:8 * k + 8, :] = o[64 + 8 * i:72 + 8 * i]
                    obuf[2 * j + i] = _as_u32(o[32 * i:32 * i + 32].astype(BF))
            else:
                a11, a12 = o[0:32], o[32:64]
                a21, a22 = [jnp.concatenate([sto[2 * j + i, 0:24, :], o[64 + 8 * i:72 + 8 * i]], axis=0)
                            for i in range(2)]
                for i, v in enumerate((a11 + a22, a21 + a22, a11, a22, a11 + a12, a21 - a11, a12 - a22)):
                    lc[i, j] = _as_u32(v.astype(BF))

        def wo_part(j, h0, h1):
            og = jnp.concatenate([_as_bf(obuf[h]) for h in range(h0, h1)], axis=1)
            return _dot(og, _as_bf(wo[j, h0 * 64:h1 * 64, :]))

        def prod(i, jc, p0, p1):
            lhs = jnp.concatenate([_as_bf(lc[i, p]) for p in range(p0, p1)], axis=1)
            if i in (1, 4):
                e = i // 4
                rhs = jnp.concatenate([wo[jc + 4 * e, 128 * p + 64 * e:128 * p + 64 * e + 64, :]
                                       for p in range(p0, p1)], axis=0)
            else:
                rhs = wc_block((0, None, 1, 2, None, 3, 4)[i], jc)[64 * p0:64 * p1, :]
            return _dot(lhs, _as_bf(rhs))

        early = [(i, jc) for i in (0, 3, 4, 6) for jc in range(4)]
        parts = []
        for i in range(NP + 4):
            for ch in ORDER:
                if ch in "qkv":
                    m = "qkv".index(ch)
                    if i < NP:
                        proj(i, m)
                    elif m < 2:
                        for n in range(1 if k < 3 else 2):
                            r = wo_part(len(parts), 0, SPLIT) if k < 3 else prod(*early[len(parts)], 0, SP3)
                            mp[len(parts)] = r
                            parts.append(r[0:8])
                elif ch == "s" and 0 <= i - LAG1 < NP:
                    scores(i - LAG1)
                elif ch == "p" and 0 <= i - LAG2 < NP:
                    pv(i - LAG2)
            if i == HOOK_AT:
                for hook in hooks[k]:
                    hook()
        if k < 3:
            return jnp.concatenate([wo_part(j, SPLIT, H) + mp[j] for j in range(8)], axis=1)
        toks, c11, c12 = parts[T0:], [], []
        for jc in range(4):
            m1, m4, m5 = [prod(i, jc, SP3, NP) + mp[4 * n + jc] for n, i in enumerate((0, 3, 4))]
            c11.append(prod(6, jc, SP3, NP) + (mp[12 + jc] + (m1 + m4 - m5)))
            mp[jc], mp[4 + jc], mp[8 + jc] = m1, m4, m5
            toks += [m1[0:8]] * (jc % 2)
        for jc in range(4):
            m3 = prod(2, jc, 0, NP)
            c12.append(m3 + mp[8 + jc])
            mp[jc] = mp[jc] + m3
            toks.append(m3[0:8])
        for n, piece in enumerate(late):
            piece(toks[(n * len(toks)) // len(late)])
        c21 = []
        for jc in range(4):
            m2 = prod(1, jc, 0, NP)
            c21.append(m2 + mp[4 + jc])
            mp[jc] = mp[jc] - m2
        c22 = [prod(5, jc, 0, NP) + mp[jc] for jc in range(4)]
        return jnp.concatenate(c11 + c12, axis=1), jnp.concatenate(c21 + c22, axis=1)

    def start_quad(mem, u):
        a_s[0] = _as_u32(lhs_rows(mem, 4 * u))
        proj_lo(a_s.at[0])

    def quad(u, c):
        base = pl.multiple_of(u * 128, 128)
        roll = lambda v: pltpu.roll(v, 64, 1)
        a1 = u // 4
        s2 = (1 - 2 * (a1 & 1)).astype(F32)
        sg = (1 - (a1 & 2)).astype(F32)
        cc, ss = sg * (1 - (a1 & 1)).astype(F32), sg * (a1 & 1).astype(F32)

        def irfft_dots(r0):
            off = pl.multiple_of((u % 4) * 128, 128) + r0
            for g in range(4):
                q = [[v_s[g, e, pl.ds(off + QS * k1, SEG), :] for e in range(2)] for k1 in range(4)]
                br, bi = q[1][0] + s2 * q[3][0], q[1][1] + s2 * q[3][1]
                vr = q[0][0] + s2 * q[2][0] + (cc * br - ss * bi)
                vi = q[0][1] + s2 * q[2][1] + (cc * bi + ss * br)
                tin = _half_pre(vr, vi, _lanes(SEG) < 64, roll, jnp.where)
                for e in range(2):
                    ts_s[r0:r0 + SEG, 128 * (2 * g + e):128 * (2 * g + e + 1)] = _dot(
                        tin[e].astype(BF), _as_bf(gi[2 * g + e]))

        def mix(r0, tok):
            lane = _lanes(8)
            t = [anchored(ts_s[r0:r0 + 8, 128 * i:128 * i + 128], tok) for i in range(8)]
            nyc = jnp.sum(jnp.where(lane == u, anchored(ct[r0:r0 + 8, :], tok), 0.0), axis=-1, keepdims=True)
            t[0] = t[0] + nyc * (1 - 2 * (lane & 1)).astype(F32)
            t = sum([list(_half_post(g, t[2 * g], t[2 * g + 1], lane < 64, roll, jnp.where))
                     for g in range(4)], [])
            b = jnp.concatenate(_bfly8_t(t), axis=1).astype(BF).astype(F32)
            xg = x_v[pl.ds(base + r0, 8), :].astype(F32) * gw_s[...]
            xg = functools.reduce(jnp.add, [xg[:, 128 * i:128 * i + 128] for i in range(8)])
            gate = jax.nn.sigmoid(jnp.sum(anchored(xg, tok), axis=-1, keepdims=True))
            bb = (1.0 - gate) * b
            if r0 % SEG and r0 < 96:
                out_v[pl.ds(base + r0, 8), :] = (bb + gate * ra_s[r0:r0 + 8, :]).astype(BF)
            else:
                bb_s[r0:r0 + 8, :] = bb
                g_s[r0:r0 + 8, :] = jnp.broadcast_to(gate, (8, 128))

        hooks = [[P(irfft_dots, SEG * n) for n in range(4) if HMAP[n] == str(k)] for k in range(4)]
        late = [P(mix, r0) for r0 in range(0, 128, 8)]
        for k in range(3):
            res = step(a_s.at[k % 2], 4 * u + k, k, hooks, late)
            ra_s[32 * k + 8:32 * k + 32, :] = res[8:32]
            a_s[(k + 1) % 2] = _as_u32(lhs_rows(res[0:8], 4 * u + k + 1))
        res, first8 = step(a_s.at[1], 4 * u + 3, 3, hooks, late)

        def emit(r0, n, att):
            out_v[pl.ds(base + r0, n), :] = (
                bb_s[r0:r0 + n, :] + jnp.concatenate([g_s[r0:r0 + n, :]] * 8, axis=1) * att).astype(BF)

        emit(104, 24, res[8:32])
        for k in range(4):
            emit(32 * k, 8, first8[8 * k:8 * k + 8])
        pltpu.make_async_copy(out_v.at[pl.ds(base, 128), :], out_hbm.at[pl.ds(base, 128), :],
                              sem.at[SEM_OUT]).start()
        start_quad(res[0:8], jnp.minimum(u + 1, S // 128 - 1))
        return c

    with jax.named_scope("chain"):
        start_quad(mem_ref[...].astype(F32), 0)
        lax.fori_loop(0, S // 128, quad, 0)
    pltpu.make_async_copy(out_v, out_hbm, sem.at[SEM_OUT]).wait()


@jax.jit
def pallas_gated_mix__memory_aug_recurrent_mem_tr__spectral_gfnet__prompt_kernel(
    A_x, A_mem0, A_Wq, A_Wk, A_Wv, A_Wo, A_seg_len, B_x, B_w_r, B_w_i, gate_w,
):
    assert A_x.shape == (1, S, D) and A_mem0.shape == (1, M, D) and A_Wq.shape == (D, H, DH)
    consts = [jnp.asarray(c) for c in _constants()]
    any_spec = pl.BlockSpec(memory_space=pl.ANY)
    out = pl.pallas_call(
        _kernel,
        out_shape=jax.ShapeDtypeStruct((S, D), BF),
        in_specs=[any_spec] * 14,
        out_specs=any_spec,
        scratch_shapes=[
            pltpu.VMEM((S, D), BF),
            pltpu.VMEM((3, D * 8, DH), U32),
            pltpu.VMEM((3, D * 8, DH), U32),
            pltpu.VMEM((3 * H, D // 2, DH), U32),
            pltpu.VMEM((8, H * DH // 2, 128), U32),
            pltpu.VMEM((3 * NP, 8 * NSEG, 128), U32),
            pltpu.VMEM((NQ, 7, 2 * NSEG, D // 2 // NQ), U32),
            pltpu.VMEM((5, 2, 4, 256, 128), U32),
            pltpu.VMEM((4, N2 * PITCH, 128), U32),
            pltpu.VMEM((4, 128, 256), U32),
            pltpu.VMEM((64, 256), U32),
            pltpu.VMEM((8, 64, 128), U32),
            pltpu.VMEM((2, N1, N2 // 2, 2 * N2), U32),
            pltpu.VMEM((4, 2, S, 128), F32),
            pltpu.VMEM((4, 2, S, 128), F32),
            pltpu.VMEM((S, D), BF),
            pltpu.VMEM((6, 256, 128), F32),
            pltpu.VMEM((4, N2, 128), U32),
            pltpu.VMEM((N1, 2 * N2, 128), F32),
            pltpu.VMEM((2, 2, D // 4, 128), U32),
            pltpu.VMEM((2, D // 2, 5 * 128), BF),
            pltpu.VMEM((N1, N2, 256), BF),
            pltpu.VMEM((N1, N2, 256), BF),
            pltpu.VMEM((H, 32, 128), F32),
            pltpu.VMEM((H, 16, 128), U32),
            pltpu.VMEM((128, 128), F32),
            pltpu.VMEM((2, 16, D), U32),
            pltpu.VMEM((6, 32, 128), F32),
            pltpu.VMEM((128, D), F32),
            pltpu.VMEM((128, 128), F32),
            pltpu.VMEM((3, 8, 32, 128), U32),
            pltpu.VMEM((8, 40, 80), U32),
            pltpu.VMEM((128, D), F32),
            pltpu.VMEM((128, D), F32),
            pltpu.VMEM((16, 32, 128), F32),
            pltpu.VMEM((7, NP, 16, 128), U32),
            pltpu.VMEM((8, D), F32),
            pltpu.VMEM((M, D), BF),
            pltpu.VMEM((96, 80), F32),
            pltpu.VMEM((96, 128), F32),
            pltpu.VMEM((32, 128), F32),
            pltpu.VMEM((2, 1, S), BF),
            pltpu.VMEM((8 * D,), BF),
            pltpu.SMEM((2,), jnp.int32),
            pltpu.SemaphoreType.DMA((NSEM,)),
        ],
        compiler_params=pltpu.CompilerParams(vmem_limit_bytes=120 * 1024 * 1024,
                                             disable_bounds_checks=True,
                                             disable_semaphore_checks=True),
    )(
        A_x.reshape(S, D), A_mem0.reshape(M, D), A_Wq, A_Wk, A_Wv,
        A_Wo.reshape(H * DH, D), B_w_r.T, B_w_i.T, gate_w, *consts,
    )
    return out.reshape(1, S, D)
```
